```python
import jax
import jax.numpy as jnp

def _softmax(x, axis=-1):
    return jax.nn.softmax(x, axis=axis)

def _gelu(x):
    return jax.nn.gelu(x, approximate=True)

def _silu(x):
    return jax.nn.silu(x)

def _sigmoid(x):
    return jax.nn.sigmoid(x)

def _layernorm(x, axis=-1, eps=1e-05):
    m = jnp.mean(x, axis=axis, keepdims=True)
    v = jnp.var(x, axis=axis, keepdims=True)
    return (x - m) / jnp.sqrt(v + eps)

def _scatter_add(tgt, idx, src, axis=0):
    return tgt.at[idx].add(src)

def _segment_sum(src, seg, n):
    return jax.ops.segment_sum(src, seg, n)

class _Rng:

    def __init__(self, key):
        self._k = key

    def _next(self):
        self._k, sub = jax.random.split(self._k)
        return sub

    def normal(self, shape):
        return jax.random.normal(self._next(), shape, dtype=jnp.bfloat16)

    def randint(self, lo, hi, shape):
        return jax.random.randint(self._next(), shape, lo, hi, dtype=jnp.int32)

    def uniform(self, shape, lo=0.0, hi=1.0):
        return jax.random.uniform(self._next(), shape, jnp.bfloat16, lo, hi)

    def permutation(self, n):
        return jax.random.permutation(self._next(), n)
kernel_name = 'concat_heads__memory_aug_recurrent_mem_tr__spectral_gfnet__prompt'

def setup_inputs():
    _rng = _Rng(jax.random.key(int.from_bytes(__import__("os").urandom(4), "little")))
    _w = lambda a: (lambda t: t.astype(jnp.bfloat16) if jnp.issubdtype(t.dtype, jnp.floating) else t)(jnp.asarray(a))

    def _A_setup():
        B, S, Dm = (1, 2048, 1024)
        H, Dh = (32, 128)
        M, seg = (8, 32)
        seg = min(seg, S)
        S = S // seg * seg
        return {'x': _w((lambda *s: _rng.normal(s) * 0.05)(B, S, Dm)), 'mem0': _w((lambda *s: _rng.normal(s) * 0.05)(B, M, Dm)), 'Wq': _w((lambda *s: _rng.normal(s) * 0.05)(Dm, H, Dh) * Dm ** (-0.5)), 'Wk': _w((lambda *s: _rng.normal(s) * 0.05)(Dm, H, Dh) * Dm ** (-0.5)), 'Wv': _w((lambda *s: _rng.normal(s) * 0.05)(Dm, H, Dh) * Dm ** (-0.5)), 'Wo': _w((lambda *s: _rng.normal(s) * 0.05)(H, Dh, Dm) * (H * Dh) ** (-0.5)), 'seg_len': seg}
    _A_in = _A_setup()

    def _B_setup():
        B, S, D = (1, 2048, 1024)
        Df = D // 2 + 1
        return {'x': _w((lambda *s: _rng.normal(s) * 0.05)(B, S, D)), 'w_r': _w((lambda *s: _rng.normal(s) * 0.05)(S, Df) * 0.02), 'w_i': _w((lambda *s: _rng.normal(s) * 0.05)(S, Df) * 0.02)}
    _B_in = _B_setup()
    return {'A_x': _A_in['x'], 'A_mem0': _A_in['mem0'], 'A_Wq': _A_in['Wq'], 'A_Wk': _A_in['Wk'], 'A_Wv': _A_in['Wv'], 'A_Wo': _A_in['Wo'], 'A_seg_len': _A_in['seg_len'], 'B_x': _B_in['x'], 'B_w_r': _B_in['w_r'], 'B_w_i': _B_in['w_i']}

def reference(A_x, A_mem0, A_Wq, A_Wk, A_Wv, A_Wo, A_seg_len, B_x, B_w_r, B_w_i):

    def _A_ref(x, mem0, Wq, Wk, Wv, Wo, seg_len):
        B, S, Dm = x.shape
        H, Dh = (Wq.shape[1], Wq.shape[2])
        M = mem0.shape[1]
        scale = Dh ** (-0.5)
        n_seg = S // seg_len
        L = M + seg_len
        idx = jnp.arange(L)
        mask = (idx[:, None] < M) | (idx[:, None] >= idx[None, :])
        mem = mem0
        outs = []
        for s in range(n_seg):
            xs = x[:, s * seg_len:(s + 1) * seg_len, :].copy()
            h = jnp.concatenate([mem, xs], axis=1)
            q = jnp.einsum('btd,dhe->bhte', h, Wq)
            k = jnp.einsum('btd,dhe->bhte', h, Wk)
            v = jnp.einsum('btd,dhe->bhte', h, Wv)
            scores = jnp.einsum('bhqe,bhke->bhqk', q, k) * scale
            scores = jnp.where(mask[None, None], scores, -1000000000.0)
            p = _softmax(scores, axis=-1)
            o = jnp.einsum('bhqk,bhke->bhqe', p, v)
            o = jnp.einsum('bhte,hed->btd', o, Wo)
            mem = o[:, :M, :].copy()
            outs.append(o[:, M:, :])
        return jnp.concatenate(outs, axis=1)

    def _B_ref(x, w_r, w_i):
        B, S, D = x.shape
        X = (lambda x, axes=(-2, -1): jnp.fft.rfft2(x.astype(jnp.float32), axes=axes))(x, axes=(-2, -1))
        W = w_r + 1j * w_i
        X = X * W
        y = (lambda x, s, axes=(-2, -1): jnp.fft.irfft2(x, s=s, axes=axes).astype(jnp.bfloat16))(X, (S, D), axes=(-2, -1))
        return y
    a = _A_ref(A_x, A_mem0, A_Wq, A_Wk, A_Wv, A_Wo, A_seg_len)
    b = _B_ref(B_x, B_w_r, B_w_i)
    return jnp.concatenate([a, b], axis=-1)
```

```python
import functools
import math

import jax
import jax.numpy as jnp
import numpy as np
from jax import lax
import jax.experimental.pallas as pl
import jax.experimental.pallas.tpu as pltpu

BF, F32, U32, I32 = jnp.bfloat16, jnp.float32, jnp.uint32, jnp.int32

S, DM, H, E, M, SEG = 2048, 1024, 32, 128, 8, 32
NSEG = S // SEG
NP = H // 2
CH = 16
LOOK = 3
R2 = math.sqrt(0.5)


def _to_u32(m):
    u = np.ascontiguousarray(m, dtype=np.float32).view(np.uint32)
    h = ((u + 0x7FFF + ((u >> 16) & 1)) >> 16).astype(np.uint32)
    return h[..., 0::2, :] | (h[..., 1::2, :] << 16)


def _mask_fill():
    r = np.arange(80)
    head = np.where(r < 64, r // 32, (r - 64) // 8)
    rr = np.where(r < 64, r % 32, (r - 64) % 8)
    pos = np.where((r < 64) & (rr < M), rr, rr + M)
    vis = (pos[:, None] < M) | (pos[:, None] >= pos[None, :])
    same = head[:, None] == head[None, :]
    return np.where(same, np.where(vis, 0.0, -1e9), -np.inf).astype(np.float32)


@functools.lru_cache(maxsize=None)
def _fft_consts():
    a = np.arange(128)
    c64 = 8 * np.arange(64)
    kmap = [np.concatenate([c64 + r0, c64 + r1]) for r0, r1 in ((0, 4), (1, 7), (2, 6), (3, 5))]
    md = np.zeros((8, 256, 256))
    for q in range(4):
        k = kmap[q]
        r = k % 8
        th = 2 * np.pi * np.outer(a, k) / DM
        c, s = np.cos(th), np.sin(th)
        if q == 0:
            z0, z4 = (r == 0)[None, :], (r == 4)[None, :]
            m = np.block([[c * z0, -s * z0], [c * z4, -s * z4]])
        else:
            sg = np.where(r == q, 1.0, -1.0)[None, :] * (-1.0 if q < 3 else 1.0)
            m = np.block([[c, -s], [sg * s, sg * c]])
        w = np.where(k == 0, 1.0, 2.0) / DM
        md[q] = m
        md[4 + q] = (m * np.concatenate([w, w])[None, :]).T
    ms = np.zeros((32, 256, 256))
    for dl in range(16):
        th = 2 * np.pi * np.outer(16 * a + dl, a) / S
        c, s = np.cos(th), np.sin(th)
        ms[dl, :128, 0::2], ms[dl, :128, 1::2] = c, s
        ms[dl, 128:, 0::2], ms[dl, 128:, 1::2] = -s, c
        ms[16 + dl, :128, 0::2], ms[16 + dl, :128, 1::2] = c.T / S, -s.T / S
        ms[16 + dl, 128:, 0::2], ms[16 + dl, 128:, 1::2] = s.T / S, c.T / S
    th = 2 * np.pi * np.outer(np.arange(16), a) / 16
    c, s = np.cos(th), np.sin(th)
    mn = np.zeros((4, 256, 256))
    mn[0, :16, :128], mn[0, :16, 128:] = c, -s
    mn[1, :16, 0::2], mn[1, :16, 1::2], mn[1, 16:32, 0::2], mn[1, 16:32, 1::2] = c, s, -s, c
    mn[2, :128, 0:32:2], mn[2, :128, 1:32:2] = c.T / S, -s.T / S
    mn[2, 128:, 0:32:2], mn[2, 128:, 1:32:2] = s.T / S, c.T / S
    mn[3, :128, :16], mn[3, 128:, :16] = c.T / DM, -s.T / DM
    th = 2 * np.pi * np.outer(a, a) / S
    tw = np.concatenate([np.cos(th), np.sin(th)], axis=1).astype(np.float32).view(np.uint32)
    return np.concatenate([_to_u32(md), _to_u32(ms), _to_u32(mn), tw[None]], axis=0)


C_MD, C_MS, C_MN, C_TW, C_NUM = 0, 8, 40, 44, 45


def _bdot(a, b):
    return jnp.dot(a, b, preferred_element_type=F32)


def _bf(u):
    return pltpu.bitcast(u, BF)


def _pack2(r, i):
    return pltpu.bitcast(pltpu.pack_elementwise([r, i], packed_dtype=BF), U32)


def _unpack2(u, p):
    if p == 0:
        return pltpu.bitcast(u << 16, F32)
    return pltpu.bitcast(u & jnp.uint32(0xFFFF0000), F32)


def _twiddle(z, k, n, sign):
    r, i = z
    if k == 0:
        return r, i
    c, s = math.cos(2 * math.pi * k / n), sign * math.sin(2 * math.pi * k / n)
    if 8 * k == n or 8 * k == 3 * n:
        if c * s > 0:
            return (r - i) * c, (r + i) * c
        return (r + i) * c, (i - r) * c
    return r * c - i * s, r * s + i * c


def _cfft(xs, sign):
    n = len(xs)
    if n == 1:
        return xs
    ev, od = _cfft(xs[0::2], sign), _cfft(xs[1::2], sign)
    out = [None] * n
    for k in range(n // 2):
        er, ei = ev[k]
        if 4 * k == n:
            orr, oi = od[k]
            lo, hi = (er - oi, ei + orr), (er + oi, ei - orr)
            out[k], out[k + n // 2] = (lo, hi) if sign > 0 else (hi, lo)
        else:
            tr, ti = _twiddle(od[k], k, n, sign)
            out[k], out[k + n // 2] = (er + tr, ei + ti), (er - tr, ei - ti)
    return out


def _rfft8(x):
    a0, a1, b0, b1 = x[0] + x[4], x[0] - x[4], x[2] + x[6], x[2] - x[6]
    c0, c1, d0, d1 = x[1] + x[5], x[1] - x[5], x[3] + x[7], x[3] - x[7]
    e, f = a0 + b0, c0 + d0
    g, h = (c1 - d1) * R2, (c1 + d1) * R2
    return [e + f, e - f, a1 + g, b1 + h, a0 - b0, c0 - d0, a1 - g, b1 - h]


def _irfft8(z):
    z0, z4, z1r, z1i, z2r, z2i, z3r, z3i = z
    e, f = z0 + z4, z0 - z4
    a1, g = z1r + z3r, (z1r - z3r) * R2
    b1, h = z1i + z3i, (z1i - z3i) * R2
    a0, b0, c0, d0 = e + z2r, e - z2r, f + z2i, f - z2i
    c1, d1 = g + h, h - g
    return [a0 + a1, c0 + c1, b0 + b1, d0 + d1, a0 - a1, c0 - c1, b0 - b1, d0 - d1]


def _kernel(x_hbm, mem0_hbm, wq_hbm, wk_hbm, wv_hbm, wo_hbm, bx_hbm, wr_hbm, wi_hbm, fill_hbm, cst_hbm,
            out_hbm,
            x_v, xpre_v, mem0_v, fill_v, wqkv, wo_v, pre, opost, outa_v,
            bx_v, w_v, wn_v, wt, cst, zs, vv, tn, outb_v,
            sem_w, sem_in, sem_out):
    scale = E ** -0.5
    wus = [w.bitcast(U32) for w in (wq_hbm, wk_hbm, wv_hbm)]
    wo_u = wo_hbm.bitcast(U32)
    fus = [w.at[pl.ds(0, 512)].bitcast(U32) for w in (wr_hbm, wi_hbm)]

    def w_copies(j):
        return [pltpu.make_async_copy(wus[t].at[:, p, j, :], wqkv.at[j, t, p], sem_w.at[j])
                for t in range(3) for p in range(2)]

    xpre_cp = pltpu.make_async_copy(x_hbm.at[:, pl.ds(0, 8), :], xpre_v, sem_in.at[0])
    a_cps = [pltpu.make_async_copy(x_hbm, x_v, sem_in.at[1]),
             pltpu.make_async_copy(mem0_hbm, mem0_v, sem_in.at[1]),
             pltpu.make_async_copy(fill_hbm, fill_v, sem_in.at[1])]
    a_cps += [pltpu.make_async_copy(wo_u.at[:, pl.ds(128 * n, 128)], wo_v.at[n], sem_in.at[1]) for n in range(8)]
    b_cps = [pltpu.make_async_copy(bx_hbm, bx_v, sem_in.at[2]),
             pltpu.make_async_copy(cst_hbm, cst, sem_in.at[2])]
    b_cps += [pltpu.make_async_copy(fus[t].at[:, pl.ds(128 * e, 128)], w_v.at[t, e], sem_in.at[2])
              for t in range(2) for e in range(16)]
    b_cps += [pltpu.make_async_copy(w.at[pl.ds(512, 1)], wn_v.at[t], sem_in.at[2])
              for t, w in enumerate((wr_hbm, wi_hbm))]

    xpre_cp.start()
    for j in range(LOOK):
        for cp in w_copies(j):
            cp.start()
    xpre_cp.wait()

    def pre_body(j, carry):
        @pl.when(j + LOOK < NP)
        def _():
            for cp in w_copies(j + LOOK):
                cp.start()

        @pl.when(j == 6)
        def _():
            for cp in a_cps:
                cp.start()

        for cp in w_copies(j):
            cp.wait()
        xp = xpre_v[...].reshape(NSEG * 8, DM)
        for t in range(3):
            a, b = wqkv[j, t, 0], wqkv[j, t, 1]
            lo = (a & jnp.uint32(0xFFFF)) | (b << 16)
            hi = (a >> 16) | (b & jnp.uint32(0xFFFF0000))
            wqkv[j, t, 0] = lo
            wqkv[j, t, 1] = hi
            r0, r1 = _bdot(xp, _bf(lo)), _bdot(xp, _bf(hi))
            r = jnp.concatenate([r0.reshape(NSEG, 8, E), r1.reshape(NSEG, 8, E)], axis=1)
            pre[j, t] = pltpu.bitcast(r.astype(BF), U32)
        return carry

    lax.fori_loop(0, NP, pre_body, 0)
    for cp in a_cps:
        cp.wait()
    for cp in b_cps:
        cp.start()

    lane = lax.broadcasted_iota(I32, (8, 128), 1)
    alt = jnp.where(lane % 2 == 0, 1.0, -1.0).astype(F32)

    def b_fwd(i):
        r0 = pl.multiple_of(i * 8, 8)
        st = {}

        def prep():
            e0 = pl.multiple_of(i * 128, 128)
            for t in range(2):
                for ty in range(2):
                    u = jnp.concatenate([w_v[t, i, pl.ds(ty, 64, stride=4), :],
                                         w_v[t, i, pl.ds(ty + 2, 64, stride=4), :]], axis=0)
                    wt[t, ty, pl.ds(e0, 128), :] = pltpu.bitcast(pltpu.bitcast(u, F32).T, U32)
            rows = []
            tacc = jnp.zeros((8, 128), F32)
            for b in range(16):
                xb = bx_v[pl.ds(128 * b + r0, 8), :].astype(F32)
                z = _rfft8([xb[:, 128 * t:128 * t + 128] for t in range(8)])
                tacc = jnp.where(lane == b, jnp.sum(z[0] * alt, axis=1, keepdims=True), tacc)
                rows.append(jnp.concatenate(z, axis=1))
            tn[pl.ds(r0, 8), :] = tacc
            st['zl'] = jnp.concatenate(rows, axis=0).astype(BF)

        def mm(q):
            x1 = _bdot(st['zl'][:, 256 * q:256 * q + 256], _bf(cst[C_MD + q]))
            o = _cfft([(x1[8 * b:8 * b + 8, 0:128], x1[8 * b:8 * b + 8, 128:256]) for b in range(16)], -1)
            for dl in range(16):
                zs[dl, pl.ds(r0, 8), 128 * q:128 * q + 128] = _pack2(*o[dl])

        hooks = {0: prep}
        for q in range(4):
            hooks[3 + q] = functools.partial(mm, q)
        return hooks

    def b_mid(dl):
        st = {}

        def fwd():
            y = _bdot(_bf(cst[C_MS + dl]), _bf(zs[dl]))
            ww = [[wt[t, ty, pl.ds(dl, 128, stride=16), :] for ty in range(2)] for t in range(2)]
            lo_half = lane < 64
            rows = []
            for r in range(16):
                wq = []
                for t in range(2):
                    ta, tb = ww[t][0][8 * r:8 * r + 8], ww[t][1][8 * r:8 * r + 8]
                    wq.append([_unpack2(ta, 0), _unpack2(jnp.where(lo_half, ta, tb), 1),
                               _unpack2(tb, 0), _unpack2(jnp.where(lo_half, tb, ta), 1)])
                cols = []
                for q in range(4):
                    yr = y[8 * r:8 * r + 8, 128 * q:128 * q + 128]
                    yi = y[128 + 8 * r:136 + 8 * r, 128 * q:128 * q + 128]
                    wr, wi = wq[0][q], wq[1][q]
                    cols.append(_pack2(yr * wr - yi * wi, yr * wi + yi * wr))
                rows.append(jnp.concatenate(cols, axis=1))
            st['p'] = jnp.concatenate(rows, axis=0)

        def inv():
            vv[dl] = _bdot(_bf(cst[C_MS + 16 + dl]), _bf(st['p']))

        return {1: fwd, 5: inv}

    def b_nyq():
        st = {}
        c, s = pltpu.bitcast(cst[C_TW, :, 0:128], F32), pltpu.bitcast(cst[C_TW, :, 128:256], F32)

        def s0():
            tz = _bdot(tn[...].astype(BF), _bf(cst[C_MN, 0:64, :]))
            tr, ti = tz[:, 0:128], tz[:, 128:256]
            st['u'] = _bf(_pack2(tr * c + ti * s, ti * c - tr * s))

        def s1():
            y = _bdot(_bf(cst[C_MN + 1, 0:16, :]), st['u'])
            row = lax.broadcasted_iota(I32, (16, 128), 0)
            wn = []
            for t in range(2):
                wrow = wn_v[t].astype(F32)
                acc = jnp.zeros((16, 128), F32)
                for e in range(16):
                    acc = jnp.where(row == e, wrow[:, 128 * e:128 * e + 128], acc)
                wn.append(acc)
            yr, yi = y[0:16], y[16:32]
            st['p'] = _bf(_pack2(yr * wn[0] - yi * wn[1], yr * wn[1] + yi * wn[0]))

        def s2():
            v = _bdot(_bf(cst[C_MN + 2, :, 0:32]), st['p'])
            vr, vi = v[0:128], v[128:256]
            st['v'] = jnp.concatenate([vr * c - vi * s, vr * s + vi * c], axis=1).astype(BF)

        def s3():
            tn[...] = _bdot(st['v'], _bf(cst[C_MN + 3, :, 0:128]))

        return {0: s0, 2: s1, 4: s2, 6: s3}

    def b_inv(i):
        r0 = pl.multiple_of(i * 8, 8)
        st = {}

        def prep(q):
            u = _cfft([(vv[dl, pl.ds(r0, 8), 128 * q:128 * q + 128],
                        vv[dl, pl.ds(128 + r0, 8), 128 * q:128 * q + 128]) for dl in range(16)], +1)
            st['u', q] = jnp.concatenate([jnp.concatenate(u[b], axis=1) for b in range(16)], axis=0).astype(BF)

        def mm(q):
            st['z', q] = _bdot(st['u', q], _bf(cst[C_MD + 4 + q]))

        def fin():
            tb = tn[pl.ds(r0, 8), :]
            for b in range(16):
                z = [st['z', t // 2][8 * b:8 * b + 8, 128 * (t % 2):128 * (t % 2) + 128] for t in range(8)]
                z[0] = z[0] + tb[:, b:b + 1] * alt
                outb_v[pl.ds(128 * b + r0, 8), :] = jnp.concatenate(_irfft8(z), axis=1).astype(BF)

        def step(k):
            if k < 4:
                prep(k)
            if 1 <= k <= 4:
                mm(k - 1)
            if k == 4:
                fin()

        return {k: functools.partial(step, k) for k in range(5)}

    def seg_body(i, mem, *, c, side):
        s = c * CH + i
        hooks = side(i) if side is not None else {}
        xs = x_v[s]
        lhs = jnp.concatenate([mem, xs[8:32].astype(F32)], axis=0).astype(BF)
        fill = fill_v[...]

        def proj(j, t):
            r = jnp.concatenate([_bdot(lhs, _bf(wqkv[j, t, 0])), _bdot(lhs, _bf(wqkv[j, t, 1]))], axis=0)
            return _bf(jnp.concatenate([pltpu.bitcast(r.astype(BF), U32), pre[j, t, s]], axis=0))

        def qk(q, k):
            sc = lax.dot_general(q, k, (((1,), (1,)), ((), ())), preferred_element_type=F32) * scale
            sc = jnp.where(fill == 0.0, sc, fill)
            p = jnp.exp(sc - jnp.max(sc, axis=-1, keepdims=True))
            return p.astype(BF), pl.reciprocal(jnp.sum(p, axis=-1, keepdims=True), approx=True)

        ob, ps, vs = {}, {}, {}

        def pv(j):
            o = _bdot(ps[j][0], vs[j]) * ps[j][1]
            opost[i, :, pl.ds(256 * j, 128)] = o[64:72]
            opost[i, :, pl.ds(256 * j + 128, 128)] = o[72:80]
            ob[j] = jnp.concatenate([o[0:32], o[32:64]], axis=1).astype(BF)

        def wo(g0, g1):
            og = jnp.concatenate([ob[j] for j in range(2 * g0, 2 * g1)], axis=1)
            return jnp.concatenate([_bdot(og, _bf(wo_v[n, g0 * 256:g1 * 256, :])) for n in range(8)], axis=1)

        ng = NP // 2
        for g in range(ng):
            if g in hooks:
                hooks[g]()
            ja, jb = 2 * g, 2 * g + 1
            qa, ka, qb, kb = proj(ja, 0), proj(ja, 1), proj(jb, 0), proj(jb, 1)
            vs[ja], vs[jb] = proj(ja, 2), proj(jb, 2)
            ps[ja], ps[jb] = qk(qa, ka), qk(qb, kb)
            if g > 0:
                pv(ja - 2)
                pv(jb - 2)
        res = wo(0, 3)
        pv(NP - 2)
        pv(NP - 1)
        res = res + wo(3, ng - 1)
        res = res + wo(ng - 1, ng)
        outa_v[s] = res.astype(BF)
        return res[0:8].astype(BF).astype(F32)

    def out_a(c):
        return pltpu.make_async_copy(outa_v.at[pl.ds(c * CH, CH)],
                                     out_hbm.at[pl.ds(c * CH, CH), :, pl.ds(0, DM)], sem_out.at[c])

    out_b = [pltpu.make_async_copy(outb_v.at[pl.ds(SEG * s, SEG)], out_hbm.at[s, :, pl.ds(DM, DM)], sem_out.at[4])
             for s in range(NSEG)]

    sides = [None, b_fwd, b_mid, b_inv]
    mem = mem0_v[...].astype(F32)
    for c in range(NSEG // CH):
        if c == 1:
            for cp in b_cps:
                cp.wait()
        mem = lax.fori_loop(0, CH, functools.partial(seg_body, c=c, side=sides[c]), mem)
        if c == 3:
            for cp in out_b:
                cp.start()
        hooks = b_nyq() if c == 1 else {}
        op = opost[...].reshape(CH * 8, H * E).astype(BF)
        for n in range(8):
            if n in hooks:
                hooks[n]()
            r = _bdot(op, _bf(wo_v[n]))
            outa_v[pl.ds(c * CH, CH), 0:8, pl.ds(128 * n, 128)] = r.reshape(CH, 8, 128).astype(BF)
        out_a(c).start()
    for c in range(NSEG // CH):
        out_a(c).wait()
    for cp in out_b:
        cp.wait()


def pallas_concat_heads__memory_aug_recurrent_mem_tr__spectral_gfnet__prompt_kernel(
    A_x, A_mem0, A_Wq, A_Wk, A_Wv, A_Wo, A_seg_len, B_x, B_w_r, B_w_i,
):
    assert A_x.shape == (1, S, DM) and A_Wq.shape == (DM, H, E) and A_mem0.shape == (1, M, DM)
    assert B_x.shape == (1, S, DM) and (not isinstance(A_seg_len, int) or A_seg_len == SEG)
    hbm = pl.BlockSpec(memory_space=pltpu.HBM)
    wr = lambda w: w.reshape(DM // 2, 2, H, E)
    out = pl.pallas_call(
        _kernel,
        out_shape=jax.ShapeDtypeStruct((NSEG, SEG, 2 * DM), BF),
        in_specs=[hbm] * 11,
        out_specs=hbm,
        scratch_shapes=[
            pltpu.VMEM((NSEG, SEG, DM), BF),
            pltpu.VMEM((NSEG, 8, DM), BF),
            pltpu.VMEM((M, DM), BF),
            pltpu.VMEM((80, 80), F32),
            pltpu.VMEM((NP, 3, 2, DM // 2, E), U32),
            pltpu.VMEM((8, H * E // 2, 128), U32),
            pltpu.VMEM((NP, 3, NSEG, 8, E), U32),
            pltpu.VMEM((CH, 8, H * E), F32),
            pltpu.VMEM((NSEG, SEG, DM), BF),
            pltpu.VMEM((S, DM), BF),
            pltpu.VMEM((2, 16, 256, 128), U32),
            pltpu.VMEM((2, 1, S), BF),
            pltpu.VMEM((2, 2, S, 128), U32),
            pltpu.VMEM((C_NUM, 128, 256), U32),
            pltpu.VMEM((16, 128, 512), U32),
            pltpu.VMEM((16, 256, 512), F32),
            pltpu.VMEM((128, 128), F32),
            pltpu.VMEM((S, DM), BF),
            pltpu.SemaphoreType.DMA((NP,)),
            pltpu.SemaphoreType.DMA((3,)),
            pltpu.SemaphoreType.DMA((5,)),
        ],
        compiler_params=pltpu.CompilerParams(vmem_limit_bytes=112 * 1024 * 1024),
    )(A_x.reshape(NSEG, SEG, DM), A_mem0.reshape(M, DM), wr(A_Wq), wr(A_Wk), wr(A_Wv),
      A_Wo.reshape(H * E, DM), B_x.reshape(S, DM), B_w_r.T, B_w_i.T, _mask_fill(), _fft_consts())
    return out.reshape(1, S, 2 * DM)
```

```python
import functools
import math

import jax
import jax.numpy as jnp
import numpy as np
from jax import lax
import jax.experimental.pallas as pl
import jax.experimental.pallas.tpu as pltpu

BF, F32, U32, I32 = jnp.bfloat16, jnp.float32, jnp.uint32, jnp.int32

S, DM, H, E, M, SEG = 2048, 1024, 32, 128, 8, 32
NSEG = S // SEG
NP = H // 2
CH = 16
R2 = math.sqrt(0.5)


def _to_u32(m):
    u = np.ascontiguousarray(m, dtype=np.float32).view(np.uint32)
    h = ((u + 0x7FFF + ((u >> 16) & 1)) >> 16).astype(np.uint32)
    return h[..., 0::2, :] | (h[..., 1::2, :] << 16)


def _mask_fill():
    r = np.arange(80)
    head = np.where(r < 64, r // 32, (r - 64) // 8)
    rr = np.where(r < 64, r % 32, (r - 64) % 8)
    pos = np.where((r < 64) & (rr < M), rr, rr + M)
    vis = (pos[:, None] < M) | (pos[:, None] >= pos[None, :])
    same = head[:, None] == head[None, :]
    return np.where(same, np.where(vis, 0.0, -1e9), -np.inf).astype(np.float32)


@functools.lru_cache(maxsize=None)
def _fft_consts():
    a = np.arange(128)
    c64 = 8 * np.arange(64)
    kmap = [np.concatenate([c64 + r0, c64 + r1]) for r0, r1 in ((0, 4), (1, 7), (2, 6), (3, 5))]
    md = np.zeros((8, 256, 256))
    for q in range(4):
        k = kmap[q]
        r = k % 8
        th = 2 * np.pi * np.outer(a, k) / DM
        c, s = np.cos(th), np.sin(th)
        if q == 0:
            z0, z4 = (r == 0)[None, :], (r == 4)[None, :]
            m = np.block([[c * z0, -s * z0], [c * z4, -s * z4]])
        else:
            sg = np.where(r == q, 1.0, -1.0)[None, :] * (-1.0 if q < 3 else 1.0)
            m = np.block([[c, -s], [sg * s, sg * c]])
        w = np.where(k == 0, 1.0, 2.0) / DM
        md[q] = m
        md[4 + q] = (m * np.concatenate([w, w])[None, :]).T
    ms = np.zeros((32, 256, 256))
    for dl in range(16):
        th = 2 * np.pi * np.outer(16 * a + dl, a) / S
        c, s = np.cos(th), np.sin(th)
        ms[dl, :128, 0::2], ms[dl, :128, 1::2] = c, s
        ms[dl, 128:, 0::2], ms[dl, 128:, 1::2] = -s, c
        ms[16 + dl, :128, 0::2], ms[16 + dl, :128, 1::2] = c.T / S, -s.T / S
        ms[16 + dl, 128:, 0::2], ms[16 + dl, 128:, 1::2] = s.T / S, c.T / S
    th = 2 * np.pi * np.outer(np.arange(16), a) / 16
    c, s = np.cos(th), np.sin(th)
    mn = np.zeros((4, 256, 256))
    mn[0, :16, :128], mn[0, :16, 128:] = c, -s
    mn[1, :16, 0::2], mn[1, :16, 1::2], mn[1, 16:32, 0::2], mn[1, 16:32, 1::2] = c, s, -s, c
    mn[2, :128, 0:32:2], mn[2, :128, 1:32:2] = c.T / S, -s.T / S
    mn[2, 128:, 0:32:2], mn[2, 128:, 1:32:2] = s.T / S, c.T / S
    mn[3, :128, :16], mn[3, 128:, :16] = c.T / DM, -s.T / DM
    th = 2 * np.pi * np.outer(a, a) / S
    tw = np.concatenate([np.cos(th), np.sin(th)], axis=1).astype(np.float32).view(np.uint32)
    return np.concatenate([_to_u32(md), _to_u32(ms), _to_u32(mn), tw[None]], axis=0)


C_MD, C_MS, C_MN, C_TW, C_NUM = 0, 8, 40, 44, 45


def _bdot(a, b):
    return jnp.dot(a, b, preferred_element_type=F32)


def _bf(u):
    return pltpu.bitcast(u, BF)


def _pack2(r, i):
    return pltpu.bitcast(pltpu.pack_elementwise([r, i], packed_dtype=BF), U32)


def _unpack2(u, p):
    if p == 0:
        return pltpu.bitcast(u << 16, F32)
    return pltpu.bitcast(u & jnp.uint32(0xFFFF0000), F32)


def _twiddle(z, k, n, sign):
    r, i = z
    if k == 0:
        return r, i
    c, s = math.cos(2 * math.pi * k / n), sign * math.sin(2 * math.pi * k / n)
    if 8 * k == n or 8 * k == 3 * n:
        if c * s > 0:
            return (r - i) * c, (r + i) * c
        return (r + i) * c, (i - r) * c
    return r * c - i * s, r * s + i * c


def _cfft(xs, sign):
    n = len(xs)
    if n == 1:
        return xs
    ev, od = _cfft(xs[0::2], sign), _cfft(xs[1::2], sign)
    out = [None] * n
    for k in range(n // 2):
        er, ei = ev[k]
        if 4 * k == n:
            orr, oi = od[k]
            lo, hi = (er - oi, ei + orr), (er + oi, ei - orr)
            out[k], out[k + n // 2] = (lo, hi) if sign > 0 else (hi, lo)
        else:
            tr, ti = _twiddle(od[k], k, n, sign)
            out[k], out[k + n // 2] = (er + tr, ei + ti), (er - tr, ei - ti)
    return out


def _rfft8(x):
    a0, a1, b0, b1 = x[0] + x[4], x[0] - x[4], x[2] + x[6], x[2] - x[6]
    c0, c1, d0, d1 = x[1] + x[5], x[1] - x[5], x[3] + x[7], x[3] - x[7]
    e, f = a0 + b0, c0 + d0
    g, h = (c1 - d1) * R2, (c1 + d1) * R2
    return [e + f, e - f, a1 + g, b1 + h, a0 - b0, c0 - d0, a1 - g, b1 - h]


def _irfft8(z):
    z0, z4, z1r, z1i, z2r, z2i, z3r, z3i = z
    e, f = z0 + z4, z0 - z4
    a1, g = z1r + z3r, (z1r - z3r) * R2
    b1, h = z1i + z3i, (z1i - z3i) * R2
    a0, b0, c0, d0 = e + z2r, e - z2r, f + z2i, f - z2i
    c1, d1 = g + h, h - g
    return [a0 + a1, c0 + c1, b0 + b1, d0 + d1, a0 - a1, c0 - c1, b0 - b1, d0 - d1]


def _kernel(x_hbm, mem0_hbm, wq_hbm, wk_hbm, wv_hbm, wo_hbm, bx_hbm, wr_hbm, wi_hbm, fill_hbm, cst_hbm,
            out_hbm,
            x_v, xpre_v, mem0_v, fill_v, wqkv, wo_v, pre, opost, outa_v,
            bx_v, w_v, wn_v, wt, cst, zs, vv, tn, outb_v,
            sem_w, sem_in, sem_out):
    scale = E ** -0.5
    wus = [w.bitcast(U32) for w in (wq_hbm, wk_hbm, wv_hbm)]
    wo_u = wo_hbm.bitcast(U32)
    fus = [w.at[pl.ds(0, 512)].bitcast(U32) for w in (wr_hbm, wi_hbm)]

    def w_copies(j, t, sem):
        return [pltpu.make_async_copy(wus[t].at[:, :, j, :], wqkv.at[j, t], sem)]

    w0_cps = [w_copies(0, t, sem_in.at[3 + t]) for t in range(3)]
    w0_cps[0].insert(0, pltpu.make_async_copy(x_hbm.at[:, pl.ds(0, 8), :], xpre_v, sem_in.at[3]))

    def w_pair(j):
        return [cp for t in range(3) for cp in w_copies(j, t, sem_w.at[j])]

    a_cps = [pltpu.make_async_copy(x_hbm, x_v, sem_in.at[1]),
             pltpu.make_async_copy(mem0_hbm, mem0_v, sem_in.at[1]),
             pltpu.make_async_copy(fill_hbm, fill_v, sem_in.at[1])]
    a_cps += [pltpu.make_async_copy(wo_u.at[:, pl.ds(128 * n, 128)], wo_v.at[n], sem_in.at[1]) for n in range(8)]
    b_cps = [pltpu.make_async_copy(bx_hbm, bx_v, sem_in.at[2]),
             pltpu.make_async_copy(cst_hbm, cst, sem_in.at[2])]
    b_cps += [pltpu.make_async_copy(fus[t].at[:, pl.ds(128 * e, 128)], w_v.at[t, e], sem_in.at[2])
              for t in range(2) for e in range(16)]
    b_cps += [pltpu.make_async_copy(w.at[pl.ds(512, 1)], wn_v.at[t], sem_in.at[2])
              for t, w in enumerate((wr_hbm, wi_hbm))]

    def pre_step(j, t):
        xp = xpre_v[...].reshape(NSEG * 8, DM)
        a, b = wqkv[j, t, :, pl.ds(0, 8, stride=2), :], wqkv[j, t, :, pl.ds(1, 8, stride=2), :]
        lo = (a & jnp.uint32(0xFFFF)) | (b << 16)
        hi = (a >> 16) | (b & jnp.uint32(0xFFFF0000))
        wqkv[j, t, :, 0:8, :] = lo
        wqkv[j, t, :, 8:16, :] = hi
        r0, r1 = _bdot(xp, _bf(lo.reshape(DM // 2, E))), _bdot(xp, _bf(hi.reshape(DM // 2, E)))
        r = jnp.concatenate([r0.reshape(NSEG, 8, E), r1.reshape(NSEG, 8, E)], axis=1)
        pre[j, t] = pltpu.bitcast(r.astype(BF), U32)

    for cp in w0_cps[0] + w0_cps[1] + w0_cps[2] + w_pair(1):
        cp.start()
    for t in range(3):
        for cp in w0_cps[t]:
            cp.wait()
        if t == 0:
            for j in range(2, NP):
                for cp in w_pair(j):
                    cp.start()
        if t == 2:
            for cp in a_cps:
                cp.start()
        pre_step(0, t)

    def pre_body(j, carry):
        for cp in w_pair(j):
            cp.wait()
        for t in range(3):
            pre_step(j, t)
        return carry

    lax.fori_loop(1, NP, pre_body, 0)
    for cp in a_cps:
        cp.wait()
    for cp in b_cps:
        cp.start()

    lane = lax.broadcasted_iota(I32, (8, 128), 1)
    alt = jnp.where(lane % 2 == 0, 1.0, -1.0).astype(F32)

    def b_fwd(i):
        r0 = pl.multiple_of(i * 8, 8)
        st = {}

        def prep():
            e0 = pl.multiple_of(i * 128, 128)
            for t in range(2):
                for ty in range(2):
                    u = jnp.concatenate([w_v[t, i, pl.ds(ty, 64, stride=4), :],
                                         w_v[t, i, pl.ds(ty + 2, 64, stride=4), :]], axis=0)
                    wt[t, ty, pl.ds(e0, 128), :] = pltpu.bitcast(pltpu.bitcast(u, F32).T, U32)
            rows = []
            tacc = jnp.zeros((8, 128), F32)
            for b in range(16):
                xb = bx_v[pl.ds(128 * b + r0, 8), :].astype(F32)
                z = _rfft8([xb[:, 128 * t:128 * t + 128] for t in range(8)])
                tacc = jnp.where(lane == b, jnp.sum(z[0] * alt, axis=1, keepdims=True), tacc)
                rows.append(jnp.concatenate(z, axis=1))
            tn[pl.ds(r0, 8), :] = tacc
            st['zl'] = jnp.concatenate(rows, axis=0).astype(BF)

        def mm(q):
            x1 = _bdot(st['zl'][:, 256 * q:256 * q + 256], _bf(cst[C_MD + q]))
            o = _cfft([(x1[8 * b:8 * b + 8, 0:128], x1[8 * b:8 * b + 8, 128:256]) for b in range(16)], -1)
            for dl in range(16):
                zs[dl, pl.ds(r0, 8), 128 * q:128 * q + 128] = _pack2(*o[dl])

        hooks = {0: prep}
        for q in range(4):
            hooks[3 + q] = functools.partial(mm, q)
        return hooks

    def b_mid(dl):
        st = {}

        def fwd():
            y = _bdot(_bf(cst[C_MS + dl]), _bf(zs[dl]))
            ww = [[wt[t, ty, pl.ds(dl, 128, stride=16), :] for ty in range(2)] for t in range(2)]
            lo_half = lane < 64
            rows = []
            for r in range(16):
                wq = []
                for t in range(2):
                    ta, tb = ww[t][0][8 * r:8 * r + 8], ww[t][1][8 * r:8 * r + 8]
                    wq.append([_unpack2(ta, 0), _unpack2(jnp.where(lo_half, ta, tb), 1),
                               _unpack2(tb, 0), _unpack2(jnp.where(lo_half, tb, ta), 1)])
                cols = []
                for q in range(4):
                    yr = y[8 * r:8 * r + 8, 128 * q:128 * q + 128]
                    yi = y[128 + 8 * r:136 + 8 * r, 128 * q:128 * q + 128]
                    wr, wi = wq[0][q], wq[1][q]
                    cols.append(_pack2(yr * wr - yi * wi, yr * wi + yi * wr))
                rows.append(jnp.concatenate(cols, axis=1))
            st['p'] = jnp.concatenate(rows, axis=0)

        def inv():
            vv[dl] = _bdot(_bf(cst[C_MS + 16 + dl]), _bf(st['p']))

        return {1: fwd, 5: inv}

    def b_nyq():
        st = {}
        c, s = pltpu.bitcast(cst[C_TW, :, 0:128], F32), pltpu.bitcast(cst[C_TW, :, 128:256], F32)

        def s0():
            tz = _bdot(tn[...].astype(BF), _bf(cst[C_MN, 0:64, :]))
            tr, ti = tz[:, 0:128], tz[:, 128:256]
            st['u'] = _bf(_pack2(tr * c + ti * s, ti * c - tr * s))

        def s1():
            y = _bdot(_bf(cst[C_MN + 1, 0:16, :]), st['u'])
            row = lax.broadcasted_iota(I32, (16, 128), 0)
            wn = []
            for t in range(2):
                wrow = wn_v[t].astype(F32)
                acc = jnp.zeros((16, 128), F32)
                for e in range(16):
                    acc = jnp.where(row == e, wrow[:, 128 * e:128 * e + 128], acc)
                wn.append(acc)
            yr, yi = y[0:16], y[16:32]
            st['p'] = _bf(_pack2(yr * wn[0] - yi * wn[1], yr * wn[1] + yi * wn[0]))

        def s2():
            v = _bdot(_bf(cst[C_MN + 2, :, 0:32]), st['p'])
            vr, vi = v[0:128], v[128:256]
            st['v'] = jnp.concatenate([vr * c - vi * s, vr * s + vi * c], axis=1).astype(BF)

        def s3():
            tn[...] = _bdot(st['v'], _bf(cst[C_MN + 3, :, 0:128]))

        return {0: s0, 2: s1, 4: s2, 6: s3}

    def b_inv(i):
        r0 = pl.multiple_of(i * 8, 8)
        st = {}

        def prep(q):
            u = _cfft([(vv[dl, pl.ds(r0, 8), 128 * q:128 * q + 128],
                        vv[dl, pl.ds(128 + r0, 8), 128 * q:128 * q + 128]) for dl in range(16)], +1)
            st['u', q] = jnp.concatenate([jnp.concatenate(u[b], axis=1) for b in range(16)], axis=0).astype(BF)

        def mm(q):
            st['z', q] = _bdot(st['u', q], _bf(cst[C_MD + 4 + q]))

        def fin():
            tb = tn[pl.ds(r0, 8), :]
            for b in range(16):
                z = [st['z', t // 2][8 * b:8 * b + 8, 128 * (t % 2):128 * (t % 2) + 128] for t in range(8)]
                z[0] = z[0] + tb[:, b:b + 1] * alt
                outb_v[pl.ds(128 * b + r0, 8), :] = jnp.concatenate(_irfft8(z), axis=1).astype(BF)

        def step(k):
            if k < 4:
                prep(k)
            if 1 <= k <= 4:
                mm(k - 1)
            if k == 4:
                fin()

        return {k: functools.partial(step, k) for k in range(5)}

    def seg_body(i, mem, *, c, side):
        s = c * CH + i
        hooks = side(i) if side is not None else {}
        xs = x_v[s]
        lhs = jnp.concatenate([mem, xs[8:32].astype(F32)], axis=0).astype(BF)
        fill = fill_v[...]

        def proj(j, t):
            r = jnp.concatenate([_bdot(lhs, _bf(wqkv[j, t, :, 8 * p:8 * p + 8, :].reshape(DM // 2, E)))
                                 for p in range(2)], axis=0)
            return _bf(jnp.concatenate([pltpu.bitcast(r.astype(BF), U32), pre[j, t, s]], axis=0))

        def qk(q, k):
            sc = lax.dot_general(q, k, (((1,), (1,)), ((), ())), preferred_element_type=F32) * scale
            sc = jnp.where(fill == 0.0, sc, fill)
            p = jnp.exp(sc - jnp.max(sc, axis=-1, keepdims=True))
            return p.astype(BF), pl.reciprocal(jnp.sum(p, axis=-1, keepdims=True), approx=True)

        ob, ps, vs = {}, {}, {}

        def pv(j):
            o = _bdot(ps[j][0], vs[j]) * ps[j][1]
            opost[i, :, pl.ds(256 * j, 128)] = o[64:72]
            opost[i, :, pl.ds(256 * j + 128, 128)] = o[72:80]
            ob[j] = jnp.concatenate([o[0:32], o[32:64]], axis=1).astype(BF)

        def wo(g0, g1):
            og = jnp.concatenate([ob[j] for j in range(2 * g0, 2 * g1)], axis=1)
            return jnp.concatenate([_bdot(og, _bf(wo_v[n, g0 * 256:g1 * 256, :])) for n in range(8)], axis=1)

        ng = NP // 2
        for g in range(ng):
            if g in hooks:
                hooks[g]()
            ja, jb = 2 * g, 2 * g + 1
            qa, ka, qb, kb = proj(ja, 0), proj(ja, 1), proj(jb, 0), proj(jb, 1)
            vs[ja], vs[jb] = proj(ja, 2), proj(jb, 2)
            ps[ja], ps[jb] = qk(qa, ka), qk(qb, kb)
            if g > 0:
                pv(ja - 2)
                pv(jb - 2)
        res = wo(0, 3)
        pv(NP - 2)
        pv(NP - 1)
        res = res + wo(3, ng - 1)
        res = res + wo(ng - 1, ng)
        outa_v[s] = res.astype(BF)
        return res[0:8].astype(BF).astype(F32)

    def out_a(c):
        return pltpu.make_async_copy(outa_v.at[pl.ds(c * CH, CH)],
                                     out_hbm.at[pl.ds(c * CH, CH), :, pl.ds(0, DM)], sem_out.at[c])

    out_b = [pltpu.make_async_copy(outb_v.at[pl.ds(SEG * s, SEG)], out_hbm.at[s, :, pl.ds(DM, DM)], sem_out.at[4])
             for s in range(NSEG)]

    sides = [None, b_fwd, b_mid, b_inv]
    mem = mem0_v[...].astype(F32)
    for c in range(NSEG // CH):
        if c == 1:
            for cp in b_cps:
                cp.wait()
        mem = lax.fori_loop(0, CH, functools.partial(seg_body, c=c, side=sides[c]), mem)
        if c == 3:
            for cp in out_b:
                cp.start()
        hooks = b_nyq() if c == 1 else {}
        op = opost[...].reshape(CH * 8, H * E).astype(BF)
        for n in range(8):
            if n in hooks:
                hooks[n]()
            r = _bdot(op, _bf(wo_v[n]))
            outa_v[pl.ds(c * CH, CH), 0:8, pl.ds(128 * n, 128)] = r.reshape(CH, 8, 128).astype(BF)
        out_a(c).start()
    for c in range(NSEG // CH):
        out_a(c).wait()
    for cp in out_b:
        cp.wait()


def pallas_concat_heads__memory_aug_recurrent_mem_tr__spectral_gfnet__prompt_kernel(
    A_x, A_mem0, A_Wq, A_Wk, A_Wv, A_Wo, A_seg_len, B_x, B_w_r, B_w_i,
):
    assert A_x.shape == (1, S, DM) and A_Wq.shape == (DM, H, E) and A_mem0.shape == (1, M, DM)
    assert B_x.shape == (1, S, DM) and (not isinstance(A_seg_len, int) or A_seg_len == SEG)
    hbm = pl.BlockSpec(memory_space=pltpu.HBM)
    wr = lambda w: w.reshape(DM // 16, 16, H, E)
    out = pl.pallas_call(
        _kernel,
        out_shape=jax.ShapeDtypeStruct((NSEG, SEG, 2 * DM), BF),
        in_specs=[hbm] * 11,
        out_specs=hbm,
        scratch_shapes=[
            pltpu.VMEM((NSEG, SEG, DM), BF),
            pltpu.VMEM((NSEG, 8, DM), BF),
            pltpu.VMEM((M, DM), BF),
            pltpu.VMEM((80, 80), F32),
            pltpu.VMEM((NP, 3, DM // 16, 16, E), U32),
            pltpu.VMEM((8, H * E // 2, 128), U32),
            pltpu.VMEM((NP, 3, NSEG, 8, E), U32),
            pltpu.VMEM((CH, 8, H * E), F32),
            pltpu.VMEM((NSEG, SEG, DM), BF),
            pltpu.VMEM((S, DM), BF),
            pltpu.VMEM((2, 16, 256, 128), U32),
            pltpu.VMEM((2, 1, S), BF),
            pltpu.VMEM((2, 2, S, 128), U32),
            pltpu.VMEM((C_NUM, 128, 256), U32),
            pltpu.VMEM((16, 128, 512), U32),
            pltpu.VMEM((16, 256, 512), F32),
            pltpu.VMEM((128, 128), F32),
            pltpu.VMEM((S, DM), BF),
            pltpu.SemaphoreType.DMA((NP,)),
            pltpu.SemaphoreType.DMA((6,)),
            pltpu.SemaphoreType.DMA((5,)),
        ],
        compiler_params=pltpu.CompilerParams(vmem_limit_bytes=112 * 1024 * 1024),
    )(A_x.reshape(NSEG, SEG, DM), A_mem0.reshape(M, DM), wr(A_Wq), wr(A_Wk), wr(A_Wv),
      A_Wo.reshape(H * E, DM), B_x.reshape(S, DM), B_w_r.T, B_w_i.T, _mask_fill(), _fft_consts())
    return out.reshape(1, S, 2 * DM)
```

```python
import functools
import math

import jax
import jax.numpy as jnp
import numpy as np
from jax import lax
import jax.experimental.pallas as pl
import jax.experimental.pallas.tpu as pltpu

BF, F32, U32, I32 = jnp.bfloat16, jnp.float32, jnp.uint32, jnp.int32

S, DM, H, E, M, SEG = 2048, 1024, 32, 128, 8, 32
NSEG = S // SEG
NP = H // 2
CH = 16
NIT = CH // 2
R2 = math.sqrt(0.5)


def _to_u32(m):
    u = np.ascontiguousarray(m, dtype=np.float32).view(np.uint32)
    h = ((u + 0x7FFF + ((u >> 16) & 1)) >> 16).astype(np.uint32)
    return h[..., 0::2, :] | (h[..., 1::2, :] << 16)


def _mask_fill():
    r = np.arange(80)
    pos_of = lambda rr: np.where(rr < M, rr, np.where(rr < SEG, rr + M, rr - SEG + M))
    qhead = np.where(r < 64, r // 32, (r - 64) // 8)
    qpos = pos_of(np.where(r < 64, r % 32, SEG + (r - 64) % 8))
    khead, kpos = r % 2, pos_of(r // 2)
    vis = (qpos[:, None] < M) | (qpos[:, None] >= kpos[None, :])
    same = qhead[:, None] == khead[None, :]
    return np.where(same, np.where(vis, 0.0, -1e9), -np.inf).astype(np.float32)


RES = ((0, 12, 8, 4), (1, 15, 9, 7), (2, 14, 10, 6), (3, 13, 11, 5))
WP = 72
C_MD, C_MN, C_TW, C_MS, C_NUM = 0, 16, 22, 24, 88


@functools.lru_cache(maxsize=None)
def _fft_consts():
    md = np.zeros((16, 128, 128))
    for q in range(4):
        if q == 0:
            lay = [[(0, 0), (0, 1), (2, 0), (2, 1)], [(3, 1), (1, 0), (1, 1), (3, 0)]]
        else:
            lay = [[(0, 0), (1, 0), (0, 1), (1, 1)], [(2, 1), (3, 1), (2, 0), (3, 0)]]
        for h in range(2):
            ms_, ws_ = [], []
            for g, part in lay[h]:
                k = 16 * np.arange(32) + RES[q][g]
                th = 2 * np.pi * np.outer(np.arange(128 if q == 0 else 64), k) / DM
                c, s = np.cos(th), np.sin(th)
                if q == 0:
                    ms_.append(-s if part else c)
                else:
                    sg = (1.0 if RES[q][g] % 8 == q else -1.0) * (1.0 - 2.0 * h)
                    ms_.append(np.concatenate([-s, sg * c] if part else [c, sg * s]))
                ws_.append(np.where(k == 0, 1.0, 2.0) / DM)
            m = np.concatenate(ms_, axis=1)
            md[2 * q + h] = m
            md[8 + 2 * q + h] = (m * np.concatenate(ws_)[None, :]).T
    a, l = np.arange(64), np.arange(128)
    ms = np.zeros((64, 128, 128))
    for dl in range(32):
        th = 2 * np.pi * np.outer(32 * a + dl, a) / S
        c, s = np.cos(th), np.sin(th)
        ms[dl, :64, 0::2], ms[dl, :64, 1::2] = c, s
        ms[dl, 64:, 0::2], ms[dl, 64:, 1::2] = -s, c
        ms[32 + dl, :64, 0::2], ms[32 + dl, :64, 1::2] = c.T / S, -s.T / S
        ms[32 + dl, 64:, 0::2], ms[32 + dl, 64:, 1::2] = s.T / S, c.T / S
    mn = np.zeros((6, 128, 128))
    th = 2 * np.pi * np.outer(np.arange(32), l) / 32
    mn[0, :32], mn[1, :32] = np.cos(th), -np.sin(th)
    mn[4, :, :32], mn[5, :, :32] = np.cos(th).T / DM, -np.sin(th).T / DM
    th = 2 * np.pi * np.outer(np.arange(16), a) / 16
    c, s = np.cos(th), np.sin(th)
    mn[2, :16, 0::2], mn[2, :16, 1::2], mn[2, 16:32, 0::2], mn[2, 16:32, 1::2] = c, s, -s, c
    mn[3, :64, 0:32:2], mn[3, :64, 1:32:2] = c.T / S, -s.T / S
    mn[3, 64:, 0:32:2], mn[3, 64:, 1:32:2] = s.T / S, c.T / S
    th = 2 * np.pi * np.outer(a, l) / S
    tw = np.stack([np.cos(th), np.sin(th)]).astype(np.float32).view(np.uint32)
    return np.concatenate([_to_u32(md), _to_u32(mn), tw, _to_u32(ms)], axis=0)


def _bdot(a, b):
    return jnp.dot(a, b, preferred_element_type=F32)


def _bf(u):
    return pltpu.bitcast(u, BF)


def _pack2(r, i):
    return pltpu.bitcast(pltpu.pack_elementwise([r, i], packed_dtype=BF), U32)


def _unpack2(u, p):
    if p == 0:
        return pltpu.bitcast(u << 16, F32)
    return pltpu.bitcast(u & jnp.uint32(0xFFFF0000), F32)


def _twiddle(z, k, n, sign):
    r, i = z
    if k == 0:
        return r, i
    c, s = math.cos(2 * math.pi * k / n), sign * math.sin(2 * math.pi * k / n)
    if 8 * k == n or 8 * k == 3 * n:
        if c * s > 0:
            return (r - i) * c, (r + i) * c
        return (r + i) * c, (i - r) * c
    return r * c - i * s, r * s + i * c


def _cfft(xs, sign):
    n = len(xs)
    if n == 1:
        return xs
    ev, od = _cfft(xs[0::2], sign), _cfft(xs[1::2], sign)
    out = [None] * n
    for k in range(n // 2):
        er, ei = ev[k]
        if 4 * k == n:
            orr, oi = od[k]
            lo, hi = (er - oi, ei + orr), (er + oi, ei - orr)
            out[k], out[k + n // 2] = (lo, hi) if sign > 0 else (hi, lo)
        else:
            tr, ti = _twiddle(od[k], k, n, sign)
            out[k], out[k + n // 2] = (er + tr, ei + ti), (er - tr, ei - ti)
    return out


def _rfft8(x):
    a0, a1, b0, b1 = x[0] + x[4], x[0] - x[4], x[2] + x[6], x[2] - x[6]
    c0, c1, d0, d1 = x[1] + x[5], x[1] - x[5], x[3] + x[7], x[3] - x[7]
    e, f = a0 + b0, c0 + d0
    g, h = (c1 - d1) * R2, (c1 + d1) * R2
    return [e + f, e - f, a1 + g, b1 + h, a0 - b0, c0 - d0, a1 - g, b1 - h]


def _irfft8(z):
    z0, z4, z1r, z1i, z2r, z2i, z3r, z3i = z
    e, f = z0 + z4, z0 - z4
    a1, g = z1r + z3r, (z1r - z3r) * R2
    b1, h = z1i + z3i, (z1i - z3i) * R2
    a0, b0, c0, d0 = e + z2r, e - z2r, f + z2i, f - z2i
    c1, d1 = g + h, h - g
    return [a0 + a1, c0 + c1, b0 + b1, d0 + d1, a0 - a1, c0 - c1, b0 - b1, d0 - d1]


def _kernel(x_hbm, mem0_hbm, wq_hbm, wk_hbm, wv_hbm, wo_hbm, bx_hbm, wr_hbm, wi_hbm, fill_hbm, cst_hbm,
            out_hbm,
            x_v, xpre_v, mem0_v, fill_v, wqkv, wo_v, pre, opost, outa_v,
            bx_v, w_v, wn_v, wt, cst, zs, vv, tn, outb_v,
            sem_w, sem_f, sem_in, sem_out):
    scale = E ** -0.5
    wus = [w.bitcast(U32) for w in (wq_hbm, wk_hbm, wv_hbm)]
    wo_u = wo_hbm.bitcast(U32)
    fus = [w.at[pl.ds(0, 512)].bitcast(U32) for w in (wr_hbm, wi_hbm)]

    def w_copies(j, t, sem):
        return [pltpu.make_async_copy(wus[t].at[:, :, j, :], wqkv.at[j, t], sem)]

    w0_cps = [w_copies(0, t, sem_in.at[3 + t]) for t in range(3)]
    w0_cps[0].insert(0, pltpu.make_async_copy(x_hbm.at[:, pl.ds(0, 8), :], xpre_v, sem_in.at[3]))

    def w_pair(j):
        return [cp for t in range(3) for cp in w_copies(j, t, sem_w.at[j])]

    a_cps = [pltpu.make_async_copy(wo_u.at[:, pl.ds(128 * n, 128)], wo_v.at[n], sem_in.at[1]) for n in range(8)]
    a_cps += [pltpu.make_async_copy(x_hbm.at[pl.ds(0, CH)], x_v.at[pl.ds(0, CH)], sem_in.at[1]),
              pltpu.make_async_copy(mem0_hbm, mem0_v, sem_in.at[1]),
              pltpu.make_async_copy(fill_hbm, fill_v, sem_in.at[1]),
              pltpu.make_async_copy(cst_hbm.at[pl.ds(0, C_MS)], cst.at[pl.ds(0, C_MS)], sem_in.at[1]),
              pltpu.make_async_copy(bx_hbm, bx_v, sem_in.at[1])]

    def f_cps(it):
        return [pltpu.make_async_copy(fus[t].at[:, pl.ds(pl.multiple_of(128 * (2 * it + h), 128), 128)],
                                      w_v.at[t, 2 * it + h], sem_f.at[it]) for t in range(2) for h in range(2)]

    b_cps = [pltpu.make_async_copy(x_hbm.at[pl.ds(CH, NSEG - CH)], x_v.at[pl.ds(CH, NSEG - CH)], sem_in.at[2]),
             pltpu.make_async_copy(cst_hbm.at[pl.ds(C_MS, C_NUM - C_MS)], cst.at[pl.ds(C_MS, C_NUM - C_MS)],
                                   sem_in.at[2])]
    b_cps += [pltpu.make_async_copy(w.at[pl.ds(512, 1)], wn_v.at[t], sem_in.at[2])
              for t, w in enumerate((wr_hbm, wi_hbm))]

    def pre_step(j, t):
        xp = xpre_v[...].reshape(NSEG * 8, DM)
        a, b = wqkv[j, t, :, pl.ds(0, 8, stride=2), :], wqkv[j, t, :, pl.ds(1, 8, stride=2), :]
        lo = (a & jnp.uint32(0xFFFF)) | (b << 16)
        hi = (a >> 16) | (b & jnp.uint32(0xFFFF0000))
        wqkv[j, t, :, 0:8, :] = lo
        wqkv[j, t, :, 8:16, :] = hi
        r0, r1 = _bdot(xp, _bf(lo.reshape(DM // 2, E))), _bdot(xp, _bf(hi.reshape(DM // 2, E)))
        pre[j, t] = _pack2(r0, r1).reshape(NSEG, 8, E)

    for cp in w0_cps[0] + w0_cps[1] + w0_cps[2] + w_pair(1):
        cp.start()
    for t in range(3):
        for cp in w0_cps[t]:
            cp.wait()
        if t == 0:
            for j in range(2, NP):
                for cp in w_pair(j):
                    cp.start()
        if t == 2:
            for cp in a_cps:
                cp.start()
        pre_step(0, t)

    def pre_body(j, carry):
        for cp in w_pair(j):
            cp.wait()

        @pl.when(j >= NP - NIT)
        def _():
            for cp in f_cps(j - (NP - NIT)):
                cp.start()

        for t in range(3):
            pre_step(j, t)
        return carry

    lax.fori_loop(1, NP, pre_body, 0)
    for cp in b_cps:
        cp.start()
    for cp in a_cps:
        cp.wait()

    lane = lax.broadcasted_iota(I32, (8, 128), 1)
    alt = jnp.where(lane % 2 == 0, 1.0, -1.0).astype(F32)
    lo_half = lane < 64
    ev_grp = (lane // 32) % 2 == 0

    def half_coef(q):
        sg = -1.0 if q < 3 else 1.0
        tc, ts = math.cos(2 * math.pi * q / 16), -math.sin(2 * math.pi * q / 16)
        f = lambda lo, hi: jnp.where(lo_half, lo, hi).astype(F32)
        return f(1.0, ts), f(0.0, sg * tc), f(0.0, tc), f(sg, -sg * ts)

    def b_rows(i, b):
        return 2 * b + i // 4, pl.ds(pl.multiple_of((i % 4) * 8, 8), 8)

    def b_fwd(i):
        r0 = pl.multiple_of(i * 8, 8)
        st = {'rows': [], 'tacc': jnp.zeros((8, 128), F32)}
        for cp in f_cps(i):
            cp.wait()

        def filt(e):
            for t in range(2):
                for ty in range(2):
                    u = jnp.concatenate([w_v[t, e, pl.ds(m + ty, 32, stride=8), :] for m in (0, 6, 4, 2)], axis=0)
                    ut = pltpu.bitcast(pltpu.bitcast(u, F32).T, U32)
                    for v in range(16):
                        wt[t, ty, pl.ds(8 * (v % 4) * WP + 4 * e + v // 4, 8, stride=WP), :] = ut[8 * v:8 * v + 8]

        def prep(b0, b1):
            hc = [None] + [half_coef(q) for q in range(1, 4)]
            rows = []
            for b in range(b0, b1):
                xb = bx_v[(*b_rows(i, b), slice(None))].astype(F32)
                z = _rfft8([xb[:, 128 * t:128 * t + 128] for t in range(8)])
                st['tacc'] = jnp.where(lane == b, jnp.sum(z[0] * alt, axis=1, keepdims=True), st['tacc'])
                for q in range(1, 4):
                    c1, c2, c3, c4 = hc[q]
                    zr, zi = z[2 * q], z[2 * q + 1]
                    pp = c1 * zr + c2 * zi
                    qq = pltpu.roll(c3 * zr + c4 * zi, 64, 1)
                    z[2 * q], z[2 * q + 1] = pp + qq, pp - qq
                rows.append(jnp.concatenate(z, axis=1))
            st['rows'].append(jnp.concatenate(rows, axis=0))
            if b1 == 32:
                tn[pl.ds(r0, 8), :] = st['tacc']
                st['zl'] = jnp.concatenate(st['rows'], axis=0).astype(BF)

        def mm(q0):
            oo = [_bdot(st['zl'][:, 128 * n:128 * n + 128], _bf(cst[C_MD + n])) for n in range(2 * q0, 2 * q0 + 4)]
            for q in (q0, q0 + 1):
                sel, sh = (ev_grp, 96) if q == 0 else (lo_half, 64)
                xs = []
                for b in range(32):
                    e_, o_ = oo[2 * (q - q0)][8 * b:8 * b + 8], oo[2 * (q - q0) + 1][8 * b:8 * b + 8]
                    xs.append((jnp.where(sel, e_, o_), pltpu.roll(jnp.where(sel, o_, e_), sh, 1)))
                o = _cfft(xs, -1)
                for dl in range(32):
                    zs[dl, pl.ds(r0, 8), 128 * q:128 * q + 128] = _pack2(*o[dl])

        hooks = {k: functools.partial(prep, 8 * k, 8 * k + 8) for k in range(4)}
        hooks.update({5: functools.partial(filt, 2 * i), 8: functools.partial(mm, 0),
                      11: functools.partial(mm, 2), 14: functools.partial(filt, 2 * i + 1)})
        return hooks

    def b_mid(i):
        st = {}

        def fwd(dl):
            y = _bdot(_bf(cst[C_MS + dl]), _bf(zs[dl]))
            w0 = pl.multiple_of(dl * WP, 8)
            rows = []
            for r in range(8):
                wq = []
                for t in range(2):
                    ta, tb = wt[t, 0, pl.ds(w0 + 8 * r, 8), :], wt[t, 1, pl.ds(w0 + 8 * r, 8), :]
                    wq.append([_unpack2(ta, 0), _unpack2(jnp.where(ev_grp, ta, tb), 1),
                               _unpack2(tb, 0), _unpack2(jnp.where(ev_grp, tb, ta), 1)])
                cols = []
                for q in range(4):
                    yr = y[8 * r:8 * r + 8, 128 * q:128 * q + 128]
                    yi = y[64 + 8 * r:72 + 8 * r, 128 * q:128 * q + 128]
                    wr, wi = wq[0][q], wq[1][q]
                    cols.append(_pack2(yr * wr - yi * wi, yr * wi + yi * wr))
                rows.append(jnp.concatenate(cols, axis=1))
            st['p'] = jnp.concatenate(rows, axis=0)

        def inv(dl):
            vv[dl] = _bdot(_bf(cst[C_MS + 32 + dl]), _bf(st['p']))

        hooks = {}
        for n in range(4):
            hooks[4 * n + 1] = functools.partial(fwd, 4 * i + n)
            hooks[4 * n + 3] = functools.partial(inv, 4 * i + n)
        return hooks

    def b_nyq():
        c, s = pltpu.bitcast(cst[C_TW], F32), pltpu.bitcast(cst[C_TW + 1], F32)
        tb = tn[...].astype(BF)
        tr, ti = _bdot(tb, _bf(cst[C_MN])), _bdot(tb, _bf(cst[C_MN + 1]))
        y = _bdot(_bf(cst[C_MN + 2, 0:16, :]), _bf(_pack2(tr * c + ti * s, ti * c - tr * s)))
        row = lax.broadcasted_iota(I32, (16, 128), 0)
        wn = []
        for t in range(2):
            wrow = wn_v[t].astype(F32)
            acc = jnp.zeros((16, 128), F32)
            for e in range(16):
                acc = jnp.where(row == e, wrow[:, 128 * e:128 * e + 128], acc)
            wn.append(acc)
        yr, yi = y[0:16], y[16:32]
        v = _bdot(_bf(cst[C_MN + 3, :, 0:32]), _bf(_pack2(yr * wn[0] - yi * wn[1], yr * wn[1] + yi * wn[0])))
        vr, vi = v[0:64], v[64:128]
        tn[...] = (_bdot((vr * c - vi * s).astype(BF), _bf(cst[C_MN + 4]))
                   + _bdot((vr * s + vi * c).astype(BF), _bf(cst[C_MN + 5])))

    def b_inv(i):
        r0 = pl.multiple_of(i * 8, 8)
        st = {}

        def prep(q):
            u = _cfft([(vv[dl, pl.ds(r0, 8), 128 * q:128 * q + 128],
                        vv[dl, pl.ds(64 + r0, 8), 128 * q:128 * q + 128]) for dl in range(32)], +1)
            sel, sh = (ev_grp, 32) if q == 0 else (lo_half, 64)
            ie, io = [], []
            for b in range(32):
                tmp = pltpu.roll(u[b][1], sh, 1)
                ie.append(jnp.where(sel, u[b][0], tmp))
                io.append(jnp.where(sel, tmp, u[b][0]))
            st['u', 2 * q] = jnp.concatenate(ie, axis=0).astype(BF)
            st['u', 2 * q + 1] = jnp.concatenate(io, axis=0).astype(BF)

        def mm(n0):
            for n in range(n0, n0 + 4):
                st['z', n] = _bdot(st['u', n], _bf(cst[C_MD + 8 + n]))

        def fin(b0, b1):
            hc = [None] + [half_coef(q) for q in range(1, 4)]
            tb = tn[pl.ds(r0, 8), :]
            for b in range(b0, b1):
                z = [st['z', n][8 * b:8 * b + 8] for n in range(8)]
                z[0] = z[0] + tb[:, b:b + 1] * alt
                for q in range(1, 4):
                    c1, c2, c3, c4 = hc[q]
                    pp = z[2 * q] + z[2 * q + 1]
                    qq = pltpu.roll(z[2 * q] - z[2 * q + 1], 64, 1)
                    z[2 * q], z[2 * q + 1] = c1 * pp + c3 * qq, c2 * pp + c4 * qq
                outb_v[(*b_rows(i, b), slice(None))] = jnp.concatenate(_irfft8(z), axis=1).astype(BF)

        hooks = {0: functools.partial(prep, 0), 2: functools.partial(prep, 1), 4: functools.partial(prep, 2),
                 5: functools.partial(mm, 0), 6: functools.partial(prep, 3), 10: functools.partial(mm, 4)}
        hooks.update({11 + k: functools.partial(fin, 8 * k, 8 * k + 8) for k in range(4)})
        return hooks

    def post(c, n):
        op = opost[c % 2].reshape(CH * 8, H * E).astype(BF)
        r = _bdot(op, _bf(wo_v[n]))
        col = n * 128 if isinstance(n, int) else pl.multiple_of(n * 128, 128)
        outa_v[pl.ds(c * CH, CH), 0:8, pl.ds(col, 128)] = r.reshape(CH, 8, 128).astype(BF)

    def seg_step(i, mem, c, hooks):
        s = c * CH + i
        xs = x_v[s]
        lhs = jnp.concatenate([mem, xs[8:32].astype(F32)], axis=0).astype(BF)
        fill = fill_v[...]

        def proj(j, t):
            r0, r1 = [_bdot(lhs, _bf(wqkv[j, t, :, 8 * p:8 * p + 8, :].reshape(DM // 2, E))) for p in range(2)]
            u = pre[j, t, s]
            if t == 0:
                return jnp.concatenate([r0, r1, _unpack2(u, 0), _unpack2(u, 1)], axis=0).astype(BF)
            return _bf(jnp.concatenate([_pack2(r0, r1), u], axis=0))

        def qk(q, k):
            sc = lax.dot_general(q, k, (((1,), (1,)), ((), ())), preferred_element_type=F32) * scale
            sc = jnp.where(fill == 0.0, sc, fill)
            p = jnp.exp(sc - jnp.max(sc, axis=-1, keepdims=True))
            return p.astype(BF), pl.reciprocal(jnp.sum(p, axis=-1, keepdims=True), approx=True)

        ob, ps, vs = {}, {}, {}

        def pv(j):
            o = _bdot(ps[j][0], vs[j]) * ps[j][1]
            opost[c % 2, i, :, pl.ds(256 * j, 128)] = o[64:72]
            opost[c % 2, i, :, pl.ds(256 * j + 128, 128)] = o[72:80]
            ob[j] = jnp.concatenate([o[0:32], o[32:64]], axis=1)

        def wo(g0, g1):
            og = jnp.concatenate([ob[j] for j in range(2 * g0, 2 * g1)], axis=1).astype(BF)
            return jnp.concatenate([_bdot(og, _bf(wo_v[n, g0 * 256:g1 * 256, :])) for n in range(8)], axis=1)

        ng = NP // 2
        for g in range(ng):
            for fn in hooks.get(g, ()):
                fn()
            ja, jb = 2 * g, 2 * g + 1
            qa, ka, qb, kb = proj(ja, 0), proj(ja, 1), proj(jb, 0), proj(jb, 1)
            vs[ja], vs[jb] = proj(ja, 2), proj(jb, 2)
            ps[ja], ps[jb] = qk(qa, ka), qk(qb, kb)
            if g > 0:
                pv(ja - 2)
                pv(jb - 2)
        res = wo(0, 3)
        pv(NP - 2)
        pv(NP - 1)
        res = res + wo(3, ng - 1)
        res = res + wo(ng - 1, ng)
        outa_v[s, 8:32, :] = res[8:32].astype(BF)
        return res[0:8].astype(BF).astype(F32)

    def chunk_body(it, mem, *, c, side):
        hooks = {k: [fn] for k, fn in (side(it) if side is not None else {}).items()}
        if c > 0:
            hooks.setdefault(8, []).insert(0, functools.partial(post, c - 1, it))
        for u in range(2):
            mem = seg_step(2 * it + u, mem, c, {k - 8 * u: v for k, v in hooks.items()})
        return mem

    def out_a(c, rows, cols, sem):
        return pltpu.make_async_copy(outa_v.at[pl.ds(c * CH, CH), rows, cols],
                                     out_hbm.at[pl.ds(c * CH, CH), rows, cols], sem)

    nch = NSEG // CH
    out_cps = [out_a(c, pl.ds(0, SEG), pl.ds(0, DM), sem_out.at[c]) for c in range(nch - 1)]
    out_cps += [out_a(nch - 1, pl.ds(8, SEG - 8), pl.ds(0, DM), sem_out.at[3]),
                pltpu.make_async_copy(outb_v, out_hbm.at[:, :, pl.ds(DM, DM)], sem_out.at[4]),
                out_a(nch - 1, pl.ds(0, 8), pl.ds(0, 896), sem_out.at[5]),
                out_a(nch - 1, pl.ds(0, 8), pl.ds(896, 128), sem_out.at[6])]

    sides = [b_fwd, b_mid, b_inv, None]
    mem = mem0_v[...].astype(F32)
    for c in range(nch):
        mem = lax.fori_loop(0, NIT, functools.partial(chunk_body, c=c, side=sides[c]), mem)
        if c == 0:
            for cp in b_cps:
                cp.wait()
            b_nyq()
        else:
            out_cps[c - 1].start()
        if c == 2:
            out_cps[4].start()
    out_cps[3].start()
    for n in range(8):
        post(nch - 1, n)
        if n >= 6:
            out_cps[n - 1].start()
    for cp in out_cps:
        cp.wait()


def pallas_concat_heads__memory_aug_recurrent_mem_tr__spectral_gfnet__prompt_kernel(
    A_x, A_mem0, A_Wq, A_Wk, A_Wv, A_Wo, A_seg_len, B_x, B_w_r, B_w_i,
):
    assert A_x.shape == (1, S, DM) and A_Wq.shape == (DM, H, E) and A_mem0.shape == (1, M, DM)
    assert B_x.shape == (1, S, DM) and (not isinstance(A_seg_len, int) or A_seg_len == SEG)
    hbm = pl.BlockSpec(memory_space=pltpu.HBM)
    wr = lambda w: w.reshape(DM // 16, 16, H, E)
    out = pl.pallas_call(
        _kernel,
        out_shape=jax.ShapeDtypeStruct((NSEG, SEG, 2 * DM), BF),
        in_specs=[hbm] * 11,
        out_specs=hbm,
        scratch_shapes=[
            pltpu.VMEM((NSEG, SEG, DM), BF),
            pltpu.VMEM((NSEG, 8, DM), BF),
            pltpu.VMEM((M, DM), BF),
            pltpu.VMEM((80, 80), F32),
            pltpu.VMEM((NP, 3, DM // 16, 16, E), U32),
            pltpu.VMEM((8, H * E // 2, 128), U32),
            pltpu.VMEM((NP, 3, NSEG, 8, E), U32),
            pltpu.VMEM((2, CH, 8, H * E), F32),
            pltpu.VMEM((NSEG, SEG, DM), BF),
            pltpu.VMEM((NSEG, SEG, DM), BF),
            pltpu.VMEM((2, 16, 256, 128), U32),
            pltpu.VMEM((2, 1, S), BF),
            pltpu.VMEM((2, 2, 32 * WP, 128), U32),
            pltpu.VMEM((C_NUM, 64, 128), U32),
            pltpu.VMEM((32, 64, 512), U32),
            pltpu.VMEM((32, 128, 512), F32),
            pltpu.VMEM((64, 128), F32),
            pltpu.VMEM((NSEG, SEG, DM), BF),
            pltpu.SemaphoreType.DMA((NP,)),
            pltpu.SemaphoreType.DMA((NIT,)),
            pltpu.SemaphoreType.DMA((6,)),
            pltpu.SemaphoreType.DMA((7,)),
        ],
        compiler_params=pltpu.CompilerParams(vmem_limit_bytes=112 * 1024 * 1024),
    )(A_x.reshape(NSEG, SEG, DM), A_mem0.reshape(M, DM), wr(A_Wq), wr(A_Wk), wr(A_Wv),
      A_Wo.reshape(H * E, DM), B_x.reshape(NSEG, SEG, DM), B_w_r.T, B_w_i.T, _mask_fill(), _fft_consts())
    return out.reshape(1, S, 2 * DM)
```

```python
import functools
import math

import jax
import jax.numpy as jnp
import numpy as np
from jax import lax
import jax.experimental.pallas as pl
import jax.experimental.pallas.tpu as pltpu

BF, F32, U32, I32 = jnp.bfloat16, jnp.float32, jnp.uint32, jnp.int32

S, DM, H, E, M, SEG = 2048, 1024, 32, 128, 8, 32
NSEG = S // SEG
NP = H // 2
CH = 16
NIT = CH // 2
R2 = math.sqrt(0.5)
MID = 'mid'


def _to_u32(m):
    u = np.ascontiguousarray(m, dtype=np.float32).view(np.uint32)
    h = ((u + 0x7FFF + ((u >> 16) & 1)) >> 16).astype(np.uint32)
    return h[..., 0::2, :] | (h[..., 1::2, :] << 16)


def _mask_fill():
    r = np.arange(80)
    pos_of = lambda rr: np.where(rr < M, rr, np.where(rr < SEG, rr + M, rr - SEG + M))
    qhead = np.where(r < 64, r // 32, (r - 64) // 8)
    qpos = pos_of(np.where(r < 64, r % 32, SEG + (r - 64) % 8))
    khead, kpos = r % 2, pos_of(r // 2)
    vis = (qpos[:, None] < M) | (qpos[:, None] >= kpos[None, :])
    same = qhead[:, None] == khead[None, :]
    return np.where(same, np.where(vis, 0.0, -1e9), -np.inf).astype(np.float32)


RES = ((0, 12, 8, 4), (1, 15, 9, 7), (2, 14, 10, 6), (3, 13, 11, 5))
WP = 72
C_MD, C_MN, C_TW, C_MS, C_NUM = 0, 16, 22, 24, 88


@functools.lru_cache(maxsize=None)
def _fft_consts():
    md = np.zeros((16, 128, 128))
    for q in range(4):
        if q == 0:
            lay = [[(0, 0), (0, 1), (2, 0), (2, 1)], [(3, 1), (1, 0), (1, 1), (3, 0)]]
        else:
            lay = [[(0, 0), (1, 0), (0, 1), (1, 1)], [(2, 1), (3, 1), (2, 0), (3, 0)]]
        for h in range(2):
            ms_, ws_ = [], []
            for g, part in lay[h]:
                k = 16 * np.arange(32) + RES[q][g]
                th = 2 * np.pi * np.outer(np.arange(128 if q == 0 else 64), k) / DM
                c, s = np.cos(th), np.sin(th)
                if q == 0:
                    ms_.append(-s if part else c)
                else:
                    sg = (1.0 if RES[q][g] % 8 == q else -1.0) * (1.0 - 2.0 * h)
                    ms_.append(np.concatenate([-s, sg * c] if part else [c, sg * s]))
                ws_.append(np.where(k == 0, 1.0, 2.0) / DM)
            m = np.concatenate(ms_, axis=1)
            md[2 * q + h] = m
            md[8 + 2 * q + h] = (m * np.concatenate(ws_)[None, :]).T
    a, l = np.arange(64), np.arange(128)
    ms = np.zeros((64, 128, 128))
    for dl in range(32):
        th = 2 * np.pi * np.outer(32 * a + dl, a) / S
        c, s = np.cos(th), np.sin(th)
        ms[dl, :64, 0::2], ms[dl, :64, 1::2] = c, s
        ms[dl, 64:, 0::2], ms[dl, 64:, 1::2] = -s, c
        ms[32 + dl, :64, 0::2], ms[32 + dl, :64, 1::2] = c.T / S, -s.T / S
        ms[32 + dl, 64:, 0::2], ms[32 + dl, 64:, 1::2] = s.T / S, c.T / S
    mn = np.zeros((6, 128, 128))
    th = 2 * np.pi * np.outer(np.arange(32), l) / 32
    mn[0, :32], mn[1, :32] = np.cos(th), -np.sin(th)
    mn[4, :, :32], mn[5, :, :32] = np.cos(th).T / DM, -np.sin(th).T / DM
    th = 2 * np.pi * np.outer(np.arange(16), a) / 16
    c, s = np.cos(th), np.sin(th)
    mn[2, :16, 0::2], mn[2, :16, 1::2], mn[2, 16:32, 0::2], mn[2, 16:32, 1::2] = c, s, -s, c
    mn[3, :64, 0:32:2], mn[3, :64, 1:32:2] = c.T / S, -s.T / S
    mn[3, 64:, 0:32:2], mn[3, 64:, 1:32:2] = s.T / S, c.T / S
    th = 2 * np.pi * np.outer(a, l) / S
    tw = np.stack([np.cos(th), np.sin(th)]).astype(np.float32).view(np.uint32)
    return np.concatenate([_to_u32(md), _to_u32(mn), tw, _to_u32(ms)], axis=0)


def _bdot(a, b):
    return jnp.dot(a, b, preferred_element_type=F32)


def _bf(u):
    return pltpu.bitcast(u, BF)


def _pack2(r, i):
    return pltpu.bitcast(pltpu.pack_elementwise([r, i], packed_dtype=BF), U32)


def _unpack2(u, p):
    if p == 0:
        return pltpu.bitcast(u << 16, F32)
    return pltpu.bitcast(u & jnp.uint32(0xFFFF0000), F32)


def _twiddle(z, k, n, sign):
    r, i = z
    if k == 0:
        return r, i
    if 4 * k == n:
        return (-i, r) if sign > 0 else (i, -r)
    c, s = math.cos(2 * math.pi * k / n), sign * math.sin(2 * math.pi * k / n)
    if 8 * k == n or 8 * k == 3 * n:
        if c * s > 0:
            return (r - i) * c, (r + i) * c
        return (r + i) * c, (i - r) * c
    return r * c - i * s, r * s + i * c


def _cfft(xs, sign):
    n = len(xs)
    if n == 1:
        return xs
    ev, od = _cfft(xs[0::2], sign), _cfft(xs[1::2], sign)
    out = [None] * n
    for k in range(n // 2):
        er, ei = ev[k]
        if 4 * k == n:
            orr, oi = od[k]
            lo, hi = (er - oi, ei + orr), (er + oi, ei - orr)
            out[k], out[k + n // 2] = (lo, hi) if sign > 0 else (hi, lo)
        else:
            tr, ti = _twiddle(od[k], k, n, sign)
            out[k], out[k + n // 2] = (er + tr, ei + ti), (er - tr, ei - ti)
    return out


def _rfft8(x):
    a0, a1, b0, b1 = x[0] + x[4], x[0] - x[4], x[2] + x[6], x[2] - x[6]
    c0, c1, d0, d1 = x[1] + x[5], x[1] - x[5], x[3] + x[7], x[3] - x[7]
    e, f = a0 + b0, c0 + d0
    g, h = (c1 - d1) * R2, (c1 + d1) * R2
    return [e + f, e - f, a1 + g, b1 + h, a0 - b0, c0 - d0, a1 - g, b1 - h]


def _irfft8(z):
    z0, z4, z1r, z1i, z2r, z2i, z3r, z3i = z
    e, f = z0 + z4, z0 - z4
    a1, g = z1r + z3r, (z1r - z3r) * R2
    b1, h = z1i + z3i, (z1i - z3i) * R2
    a0, b0, c0, d0 = e + z2r, e - z2r, f + z2i, f - z2i
    c1, d1 = g + h, h - g
    return [a0 + a1, c0 + c1, b0 + b1, d0 + d1, a0 - a1, c0 - c1, b0 - b1, d0 - d1]


def _kernel(x_hbm, mem0_hbm, wq_hbm, wk_hbm, wv_hbm, wo_hbm, bx_hbm, wr_hbm, wi_hbm, fill_hbm, cst_hbm,
            out_hbm,
            x_v, xpre_v, mem0_v, fill_v, lhs_v, wqkv, wo_v, pre, opost, outa_v,
            bx_v, w_v, wn_v, wt, cst, zs, vv, tn, outb_v,
            sem_w, sem_f, sem_in, sem_out):
    scale = E ** -0.5
    wus = [w.bitcast(U32) for w in (wq_hbm, wk_hbm, wv_hbm)]
    wo_u = wo_hbm.bitcast(U32)
    fus = [w.at[pl.ds(0, 512)].bitcast(U32) for w in (wr_hbm, wi_hbm)]

    def w_copies(j, t, sem):
        return [pltpu.make_async_copy(wus[t].at[:, :, j, :], wqkv.at[j, t], sem)]

    w0_cps = [w_copies(0, t, sem_in.at[3 + t]) for t in range(3)]
    w0_cps[0].insert(0, pltpu.make_async_copy(x_hbm.at[:, pl.ds(0, 8), :], xpre_v, sem_in.at[3]))

    def w_pair(j):
        return [cp for t in range(3) for cp in w_copies(j, t, sem_w.at[j])]

    a_cps = [pltpu.make_async_copy(wo_u.at[:, pl.ds(128 * n, 128)], wo_v.at[n], sem_in.at[1]) for n in range(8)]
    a_cps += [pltpu.make_async_copy(x_hbm.at[pl.ds(0, CH)], x_v.at[pl.ds(0, CH)], sem_in.at[1]),
              pltpu.make_async_copy(mem0_hbm, mem0_v, sem_in.at[1]),
              pltpu.make_async_copy(fill_hbm, fill_v, sem_in.at[1]),
              pltpu.make_async_copy(cst_hbm.at[pl.ds(0, C_MS)], cst.at[pl.ds(0, C_MS)], sem_in.at[1]),
              pltpu.make_async_copy(bx_hbm, bx_v, sem_in.at[1])]

    def f_cps(it):
        return [pltpu.make_async_copy(fus[t].at[:, pl.ds(pl.multiple_of(128 * (2 * it + h), 128), 128)],
                                      w_v.at[t, 2 * it + h], sem_f.at[it]) for t in range(2) for h in range(2)]

    b_cps = [pltpu.make_async_copy(x_hbm.at[pl.ds(CH, NSEG - CH)], x_v.at[pl.ds(CH, NSEG - CH)], sem_in.at[2]),
             pltpu.make_async_copy(cst_hbm.at[pl.ds(C_MS, C_NUM - C_MS)], cst.at[pl.ds(C_MS, C_NUM - C_MS)],
                                   sem_in.at[2])]
    b_cps += [pltpu.make_async_copy(w.at[pl.ds(512, 1)], wn_v.at[t], sem_in.at[2])
              for t, w in enumerate((wr_hbm, wi_hbm))]

    def pre_step(j, t):
        xp = xpre_v[...].reshape(NSEG * 8, DM)
        a, b = wqkv[j, t, :, pl.ds(0, 8, stride=2), :], wqkv[j, t, :, pl.ds(1, 8, stride=2), :]
        lo = (a & jnp.uint32(0xFFFF)) | (b << 16)
        hi = (a >> 16) | (b & jnp.uint32(0xFFFF0000))
        wqkv[j, t, :, 0:8, :] = lo
        wqkv[j, t, :, 8:16, :] = hi
        r0, r1 = _bdot(xp, _bf(lo.reshape(DM // 2, E))), _bdot(xp, _bf(hi.reshape(DM // 2, E)))
        pre[j, t] = _pack2(r0, r1).reshape(NSEG, 8, E)

    for cp in w0_cps[0] + w0_cps[1] + w0_cps[2] + w_pair(1):
        cp.start()
    for t in range(3):
        for cp in w0_cps[t]:
            cp.wait()
        if t == 0:
            for j in range(2, NP):
                for cp in w_pair(j):
                    cp.start()
        if t == 2:
            for cp in a_cps:
                cp.start()
        pre_step(0, t)

    def pre_body(j, carry):
        for cp in w_pair(j):
            cp.wait()

        @pl.when(j >= NP - NIT)
        def _():
            for cp in f_cps(j - (NP - NIT)):
                cp.start()

        for t in range(3):
            pre_step(j, t)
        return carry

    lax.fori_loop(1, NP, pre_body, 0)
    for cp in b_cps:
        cp.start()
    for cp in a_cps:
        cp.wait()

    lane = lax.broadcasted_iota(I32, (8, 128), 1)
    alt = jnp.where(lane % 2 == 0, 1.0, -1.0).astype(F32)
    lo_half = lane < 64
    ev_grp = (lane // 32) % 2 == 0

    def half_coef(q):
        sg = -1.0 if q < 3 else 1.0
        tc, ts = math.cos(2 * math.pi * q / 16), -math.sin(2 * math.pi * q / 16)
        f = lambda lo, hi: jnp.where(lo_half, lo, hi).astype(F32)
        return f(1.0, ts), f(0.0, sg * tc), f(0.0, tc), f(sg, -sg * ts)

    def b_rows(i, b):
        return 2 * b + i // 4, pl.ds(pl.multiple_of((i % 4) * 8, 8), 8)

    def flat(zs_):
        return [v for z in zs_ for v in z]

    def as_u32(rows):
        return pltpu.bitcast(jnp.concatenate(rows, axis=0).astype(BF), U32)

    def b_fwd(i):
        r0 = pl.multiple_of(i * 8, 8)
        for cp in f_cps(i):
            cp.wait()
        hc = [None] + [half_coef(q) for q in range(1, 4)]
        tacc = jnp.zeros((8, 128), F32)
        zl = []
        for _ in range(3):
            yield None
        for b0 in range(0, 32, 2):
            rows = []
            for b in (b0, b0 + 1):
                xb = bx_v[(*b_rows(i, b), slice(None))].astype(F32)
                z = _rfft8([xb[:, 128 * t:128 * t + 128] for t in range(8)])
                tacc = jnp.where(lane == b, jnp.sum(z[0] * alt, axis=1, keepdims=True), tacc)
                for q in range(1, 4):
                    c1, c2, c3, c4 = hc[q]
                    zr, zi = z[2 * q], z[2 * q + 1]
                    pp = c1 * zr + c2 * zi
                    qq = pltpu.roll(c3 * zr + c4 * zi, 64, 1)
                    z[2 * q], z[2 * q + 1] = pp + qq, pp - qq
                rows.append(z)
            zl.append([as_u32([rows[0][n], rows[1][n]]) for n in range(8)])
            yield zl[-1] + [tacc]
            yield None
            if b0 % 4 == 0:
                e, t, ty = 2 * i + b0 // 16, (b0 // 8) % 2, (b0 // 4) % 2
                u = jnp.concatenate([w_v[t, e, pl.ds(m + ty, 32, stride=8), :] for m in (0, 6, 4, 2)], axis=0)
                ut = pltpu.bitcast(pltpu.bitcast(u, F32).T, U32)
                for v in range(16):
                    wt[t, ty, pl.ds(8 * (v % 4) * WP + 4 * e + v // 4, 8, stride=WP), :] = ut[8 * v:8 * v + 8]
                yield [ut[8 * v:8 * v + 8] for v in range(16)]
        tn[pl.ds(r0, 8), :] = tacc

        def mm(n):
            return _bdot(_bf(jnp.concatenate([z[n] for z in zl], axis=0)), _bf(cst[C_MD + n]))

        oo = [mm(n) for n in range(4)]
        yield MID
        oo += [mm(n) for n in range(4, 8)]
        for q in range(4):
            sel, sh = (ev_grp, 96) if q == 0 else (lo_half, 64)
            ys = []
            for b0 in range(4):
                xs = []
                for b in range(b0, 32, 4):
                    e_, o_ = oo[2 * q][8 * b:8 * b + 8], oo[2 * q + 1][8 * b:8 * b + 8]
                    xs.append((jnp.where(sel, e_, o_), pltpu.roll(jnp.where(sel, o_, e_), sh, 1)))
                ys.append([_twiddle(y, b0 * k1, 32, -1) for k1, y in enumerate(_cfft(xs, -1))])
                yield flat(ys[-1])
            for k1 in range(8):
                o = [_pack2(*y) for y in _cfft([ys[b0][k1] for b0 in range(4)], -1)]
                for k0 in range(4):
                    zs[k1 + 8 * k0, pl.ds(r0, 8), 128 * q:128 * q + 128] = o[k0]
                yield o

    def b_mid(i):
        for n in range(4):
            dl = 4 * i + n
            for _ in range(6):
                yield None
            y = _bdot(_bf(cst[C_MS + dl]), _bf(zs[dl]))
            for _ in range(3):
                yield None
            w0 = pl.multiple_of(dl * WP, 8)
            rows = []
            for r in range(8):
                wq = []
                for t in range(2):
                    ta, tb = wt[t, 0, pl.ds(w0 + 8 * r, 8), :], wt[t, 1, pl.ds(w0 + 8 * r, 8), :]
                    wq.append([_unpack2(ta, 0), _unpack2(jnp.where(ev_grp, ta, tb), 1),
                               _unpack2(tb, 0), _unpack2(jnp.where(ev_grp, tb, ta), 1)])
                cols = []
                for q in range(4):
                    yr = y[8 * r:8 * r + 8, 128 * q:128 * q + 128]
                    yi = y[64 + 8 * r:72 + 8 * r, 128 * q:128 * q + 128]
                    wr, wi = wq[0][q], wq[1][q]
                    cols.append(_pack2(yr * wr - yi * wi, yr * wi + yi * wr))
                rows.append(jnp.concatenate(cols, axis=1))
                yield cols
            yield None
            vv[dl] = _bdot(_bf(cst[C_MS + 32 + dl]), _bf(jnp.concatenate(rows, axis=0)))
            for _ in range(6):
                yield None

    def b_nyq():
        c, s = pltpu.bitcast(cst[C_TW], F32), pltpu.bitcast(cst[C_TW + 1], F32)
        tb = tn[...].astype(BF)
        tr, ti = _bdot(tb, _bf(cst[C_MN])), _bdot(tb, _bf(cst[C_MN + 1]))
        y = _bdot(_bf(cst[C_MN + 2, 0:16, :]), _bf(_pack2(tr * c + ti * s, ti * c - tr * s)))
        row = lax.broadcasted_iota(I32, (16, 128), 0)
        wn = []
        for t in range(2):
            wrow = wn_v[t].astype(F32)
            acc = jnp.zeros((16, 128), F32)
            for e in range(16):
                acc = jnp.where(row == e, wrow[:, 128 * e:128 * e + 128], acc)
            wn.append(acc)
        yr, yi = y[0:16], y[16:32]
        v = _bdot(_bf(cst[C_MN + 3, :, 0:32]), _bf(_pack2(yr * wn[0] - yi * wn[1], yr * wn[1] + yi * wn[0])))
        vr, vi = v[0:64], v[64:128]
        tn[...] = (_bdot((vr * c - vi * s).astype(BF), _bf(cst[C_MN + 4]))
                   + _bdot((vr * s + vi * c).astype(BF), _bf(cst[C_MN + 5])))

    def b_inv(i):
        r0 = pl.multiple_of(i * 8, 8)
        ul, zz = [], []
        yield None
        for q in range(4):
            sel, sh = (ev_grp, 32) if q == 0 else (lo_half, 64)
            ys = []
            for b0 in range(4):
                xs = [(vv[dl, pl.ds(r0, 8), 128 * q:128 * q + 128], vv[dl, pl.ds(64 + r0, 8), 128 * q:128 * q + 128])
                      for dl in range(b0, 32, 4)]
                ys.append([_twiddle(y, b0 * k1, 32, +1) for k1, y in enumerate(_cfft(xs, +1))])
                yield flat(ys[-1])
            ie, io = [], []
            for k1 in range(8):
                es, os_ = [], []
                for ur, ui in _cfft([ys[b0][k1] for b0 in range(4)], +1):
                    tmp = pltpu.roll(ui, sh, 1)
                    es.append(jnp.where(sel, ur, tmp))
                    os_.append(jnp.where(sel, tmp, ur))
                ie += [as_u32(es[0:2]), as_u32(es[2:4])]
                io += [as_u32(os_[0:2]), as_u32(os_[2:4])]
                yield ie[-2:] + io[-2:]
            ul += [ie, io]
            if q == 2:
                zz += [_bdot(_bf(jnp.concatenate(ul[n], axis=0)), _bf(cst[C_MD + 8 + n])) for n in range(4)]
        yield MID
        zz += [_bdot(_bf(jnp.concatenate(ul[n], axis=0)), _bf(cst[C_MD + 8 + n])) for n in range(4, 8)]
        for _ in range(4):
            yield None
        hc = [None] + [half_coef(q) for q in range(1, 4)]
        tb = tn[pl.ds(r0, 8), :]
        for g in range(32):
            b = g // 4 + 8 * (g % 4)
            z = [zz[n][8 * g:8 * g + 8] for n in range(8)]
            z[0] = z[0] + jnp.sum(jnp.where(lane == b, tb, 0.0), axis=1, keepdims=True) * alt
            for q in range(1, 4):
                c1, c2, c3, c4 = hc[q]
                pp = z[2 * q] + z[2 * q + 1]
                qq = pltpu.roll(z[2 * q] - z[2 * q + 1], 64, 1)
                z[2 * q], z[2 * q + 1] = c1 * pp + c3 * qq, c2 * pp + c4 * qq
            y = _irfft8(z)
            outb_v[(*b_rows(i, b), slice(None))] = jnp.concatenate(y, axis=1).astype(BF)
            yield y

    def tie(w, vals):
        if not vals:
            return w
        acc = None
        for v in vals:
            v = v if v.dtype == U32 else pltpu.bitcast(v, U32)
            acc = v if acc is None else acc | v
        zero = cst[C_MN, 56:64, :]
        return jnp.concatenate([w[0:8] | (acc & zero), w[8:]], axis=0)

    def post(c, n):
        op = opost[c % 2].reshape(CH * 8, H * E).astype(BF)
        r = _bdot(op, _bf(wo_v[n]))
        col = n * 128 if isinstance(n, int) else pl.multiple_of(n * 128, 128)
        outa_v[pl.ds(c * CH, CH), 0:8, pl.ds(col, 128)] = r.reshape(CH, 8, 128).astype(BF)

    def seg_step(i, u, mem, c, slot):
        s = c * CH + i
        xs = x_v[s]
        lhs_v[u] = as_u32([mem, xs[8:32].astype(F32)])
        fill = fill_v[...]

        def proj(j, t):
            w0, w1 = [wqkv[j, t, :, 8 * p:8 * p + 8, :].reshape(DM // 2, E) for p in range(2)]
            r0, r1 = _bdot(_bf(lhs_v[u]), _bf(tie(w0, slot()))), _bdot(_bf(lhs_v[u]), _bf(w1))
            pw = pre[j, t, s]
            if t == 0:
                return jnp.concatenate([r0, r1, _unpack2(pw, 0), _unpack2(pw, 1)], axis=0).astype(BF)
            return _bf(jnp.concatenate([_pack2(r0, r1), pw], axis=0))

        def qk(q, k):
            sc = lax.dot_general(q, k, (((1,), (1,)), ((), ())), preferred_element_type=F32) * scale
            sc = jnp.where(fill == 0.0, sc, fill)
            p = jnp.exp(sc - jnp.max(sc, axis=-1, keepdims=True))
            return p.astype(BF), pl.reciprocal(jnp.sum(p, axis=-1, keepdims=True), approx=True)

        ob, ps, vs = {}, {}, {}

        def pv(j):
            o = _bdot(ps[j][0], vs[j]) * ps[j][1]
            opost[c % 2, i, :, pl.ds(256 * j, 128)] = o[64:72]
            opost[c % 2, i, :, pl.ds(256 * j + 128, 128)] = o[72:80]
            ob[j] = jnp.concatenate([o[0:32], o[32:64]], axis=1)

        def wo(g0, g1):
            og = jnp.concatenate([ob[j] for j in range(2 * g0, 2 * g1)], axis=1).astype(BF)
            return jnp.concatenate([_bdot(og, _bf(wo_v[n, g0 * 256:g1 * 256, :])) for n in range(8)], axis=1)

        ng = NP // 2
        for g in range(ng):
            ja, jb = 2 * g, 2 * g + 1
            qa, ka, qb, kb = proj(ja, 0), proj(ja, 1), proj(jb, 0), proj(jb, 1)
            vs[ja], vs[jb] = proj(ja, 2), proj(jb, 2)
            ps[ja], ps[jb] = qk(qa, ka), qk(qb, kb)
            if g > 0:
                pv(ja - 2)
                pv(jb - 2)
        res = wo(0, 3)
        pv(NP - 2)
        pv(NP - 1)
        res = res + wo(3, ng - 1)
        res = res + wo(ng - 1, ng)
        outa_v[s, 8:32, :] = res[8:32].astype(BF)
        return res[0:8].astype(BF).astype(F32)

    def chunk_body(it, mem, *, c, side):
        gen = side(it) if side is not None else iter(())
        state = {'mid': False}

        def slot():
            if state['mid']:
                return None
            vals = next(gen, None)
            if vals is MID:
                state['mid'] = True
                return None
            return vals

        mem = seg_step(2 * it, 0, mem, c, slot)
        if c > 0:
            post(c - 1, it)
        if side in (b_fwd, b_inv):
            while not state['mid']:
                slot()
        state['mid'] = False
        mem = seg_step(2 * it + 1, 1, mem, c, slot)
        for _ in gen:
            pass
        return mem

    def out_a(c, rows, cols, sem):
        return pltpu.make_async_copy(outa_v.at[pl.ds(c * CH, CH), rows, cols],
                                     out_hbm.at[pl.ds(c * CH, CH), rows, cols], sem)

    nch = NSEG // CH
    out_cps = [out_a(c, pl.ds(0, SEG), pl.ds(0, DM), sem_out.at[c]) for c in range(nch - 1)]
    out_cps += [out_a(nch - 1, pl.ds(8, SEG - 8), pl.ds(0, DM), sem_out.at[3]),
                pltpu.make_async_copy(outb_v, out_hbm.at[:, :, pl.ds(DM, DM)], sem_out.at[4]),
                out_a(nch - 1, pl.ds(0, 8), pl.ds(0, 896), sem_out.at[5]),
                out_a(nch - 1, pl.ds(0, 8), pl.ds(896, 128), sem_out.at[6])]

    sides = [b_fwd, b_mid, b_inv, None]
    mem = mem0_v[...].astype(F32)
    for c in range(nch):
        mem = lax.fori_loop(0, NIT, functools.partial(chunk_body, c=c, side=sides[c]), mem)
        if c == 0:
            for cp in b_cps:
                cp.wait()
            b_nyq()
        else:
            out_cps[c - 1].start()
        if c == 2:
            out_cps[4].start()
    out_cps[3].start()
    for n in range(8):
        post(nch - 1, n)
        if n >= 6:
            out_cps[n - 1].start()
    for cp in out_cps:
        cp.wait()


def pallas_concat_heads__memory_aug_recurrent_mem_tr__spectral_gfnet__prompt_kernel(
    A_x, A_mem0, A_Wq, A_Wk, A_Wv, A_Wo, A_seg_len, B_x, B_w_r, B_w_i,
):
    assert A_x.shape == (1, S, DM) and A_Wq.shape == (DM, H, E) and A_mem0.shape == (1, M, DM)
    assert B_x.shape == (1, S, DM) and (not isinstance(A_seg_len, int) or A_seg_len == SEG)
    hbm = pl.BlockSpec(memory_space=pltpu.HBM)
    wr = lambda w: w.reshape(DM // 16, 16, H, E)
    out = pl.pallas_call(
        _kernel,
        out_shape=jax.ShapeDtypeStruct((NSEG, SEG, 2 * DM), BF),
        in_specs=[hbm] * 11,
        out_specs=hbm,
        scratch_shapes=[
            pltpu.VMEM((NSEG, SEG, DM), BF),
            pltpu.VMEM((NSEG, 8, DM), BF),
            pltpu.VMEM((M, DM), BF),
            pltpu.VMEM((80, 80), F32),
            pltpu.VMEM((2, SEG // 2, DM), U32),
            pltpu.VMEM((NP, 3, DM // 16, 16, E), U32),
            pltpu.VMEM((8, H * E // 2, 128), U32),
            pltpu.VMEM((NP, 3, NSEG, 8, E), U32),
            pltpu.VMEM((2, CH, 8, H * E), F32),
            pltpu.VMEM((NSEG, SEG, DM), BF),
            pltpu.VMEM((NSEG, SEG, DM), BF),
            pltpu.VMEM((2, 16, 256, 128), U32),
            pltpu.VMEM((2, 1, S), BF),
            pltpu.VMEM((2, 2, 32 * WP, 128), U32),
            pltpu.VMEM((C_NUM, 64, 128), U32),
            pltpu.VMEM((32, 64, 512), U32),
            pltpu.VMEM((32, 128, 512), F32),
            pltpu.VMEM((64, 128), F32),
            pltpu.VMEM((NSEG, SEG, DM), BF),
            pltpu.SemaphoreType.DMA((NP,)),
            pltpu.SemaphoreType.DMA((NIT,)),
            pltpu.SemaphoreType.DMA((6,)),
            pltpu.SemaphoreType.DMA((7,)),
        ],
        compiler_params=pltpu.CompilerParams(vmem_limit_bytes=112 * 1024 * 1024),
    )(A_x.reshape(NSEG, SEG, DM), A_mem0.reshape(M, DM), wr(A_Wq), wr(A_Wk), wr(A_Wv),
      A_Wo.reshape(H * E, DM), B_x.reshape(NSEG, SEG, DM), B_w_r.T, B_w_i.T, _mask_fill(), _fft_consts())
    return out.reshape(1, S, 2 * DM)
```

```python
import functools
import math

import jax
import jax.numpy as jnp
import numpy as np
from jax import lax
import jax.experimental.pallas as pl
import jax.experimental.pallas.tpu as pltpu

BF, F32, U32, I32 = jnp.bfloat16, jnp.float32, jnp.uint32, jnp.int32

S, DM, H, E, M, SEG = 2048, 1024, 32, 128, 8, 32
NSEG = S // SEG
NP = H // 2
CH = 16
NIT = CH // 2
R2 = math.sqrt(0.5)
MID = 'mid'


def _to_u32(m):
    u = np.ascontiguousarray(m, dtype=np.float32).view(np.uint32)
    h = ((u + 0x7FFF + ((u >> 16) & 1)) >> 16).astype(np.uint32)
    return h[..., 0::2, :] | (h[..., 1::2, :] << 16)


def _mask_fill():
    r = np.arange(80)
    pos_of = lambda rr: np.where(rr < M, rr, np.where(rr < SEG, rr + M, rr - SEG + M))
    qhead = np.where(r < 64, r // 32, (r - 64) // 8)
    qpos = pos_of(np.where(r < 64, r % 32, SEG + (r - 64) % 8))
    khead, kpos = r % 2, pos_of(r // 2)
    vis = (qpos[:, None] < M) | (qpos[:, None] >= kpos[None, :])
    same = qhead[:, None] == khead[None, :]
    return np.where(same, np.where(vis, 0.0, -1e9), -np.inf).astype(np.float32)


RES = ((0, 12, 8, 4), (1, 15, 9, 7), (2, 14, 10, 6), (3, 13, 11, 5))
WP = 72
C_MD, C_MN, C_TW, C_MS, C_NUM = 0, 16, 22, 24, 88


@functools.lru_cache(maxsize=None)
def _fft_consts():
    md = np.zeros((16, 128, 128))
    for q in range(4):
        if q == 0:
            lay = [[(0, 0), (0, 1), (2, 0), (2, 1)], [(3, 1), (1, 0), (1, 1), (3, 0)]]
        else:
            lay = [[(0, 0), (1, 0), (0, 1), (1, 1)], [(2, 1), (3, 1), (2, 0), (3, 0)]]
        for h in range(2):
            ms_, ws_ = [], []
            for g, part in lay[h]:
                k = 16 * np.arange(32) + RES[q][g]
                th = 2 * np.pi * np.outer(np.arange(128 if q == 0 else 64), k) / DM
                c, s = np.cos(th), np.sin(th)
                if q == 0:
                    ms_.append(-s if part else c)
                else:
                    sg = (1.0 if RES[q][g] % 8 == q else -1.0) * (1.0 - 2.0 * h)
                    ms_.append(np.concatenate([-s, sg * c] if part else [c, sg * s]))
                ws_.append(np.where(k == 0, 1.0, 2.0) / DM)
            m = np.concatenate(ms_, axis=1)
            md[2 * q + h] = m
            md[8 + 2 * q + h] = (m * np.concatenate(ws_)[None, :]).T
    a, l = np.arange(64), np.arange(128)
    ms = np.zeros((64, 128, 128))
    for dl in range(32):
        th = 2 * np.pi * np.outer(32 * a + dl, a) / S
        c, s = np.cos(th), np.sin(th)
        ms[dl, :64, 0::2], ms[dl, :64, 1::2] = c, s
        ms[dl, 64:, 0::2], ms[dl, 64:, 1::2] = -s, c
        ms[32 + dl, :64, 0::2], ms[32 + dl, :64, 1::2] = c.T / S, -s.T / S
        ms[32 + dl, 64:, 0::2], ms[32 + dl, 64:, 1::2] = s.T / S, c.T / S
    mn = np.zeros((6, 128, 128))
    th = 2 * np.pi * np.outer(np.arange(32), l) / 32
    mn[0, :32], mn[1, :32] = np.cos(th), -np.sin(th)
    mn[4, :, :32], mn[5, :, :32] = np.cos(th).T / DM, -np.sin(th).T / DM
    th = 2 * np.pi * np.outer(np.arange(16), a) / 16
    c, s = np.cos(th), np.sin(th)
    mn[2, :16, 0::2], mn[2, :16, 1::2], mn[2, 16:32, 0::2], mn[2, 16:32, 1::2] = c, s, -s, c
    mn[3, :64, 0:32:2], mn[3, :64, 1:32:2] = c.T / S, -s.T / S
    mn[3, 64:, 0:32:2], mn[3, 64:, 1:32:2] = s.T / S, c.T / S
    th = 2 * np.pi * np.outer(a, l) / S
    tw = np.stack([np.cos(th), np.sin(th)]).astype(np.float32).view(np.uint32)
    return np.concatenate([_to_u32(md), _to_u32(mn), tw, _to_u32(ms)], axis=0)


def _bdot(a, b):
    return jnp.dot(a, b, preferred_element_type=F32)


def _bf(u):
    return pltpu.bitcast(u, BF)


def _pack2(r, i):
    return pltpu.bitcast(pltpu.pack_elementwise([r, i], packed_dtype=BF), U32)


def _unpack2(u, p):
    if p == 0:
        return pltpu.bitcast(u << 16, F32)
    return pltpu.bitcast(u & jnp.uint32(0xFFFF0000), F32)


def _twiddle(z, k, n, sign):
    r, i = z
    if k == 0:
        return r, i
    if 4 * k == n:
        return (-i, r) if sign > 0 else (i, -r)
    c, s = math.cos(2 * math.pi * k / n), sign * math.sin(2 * math.pi * k / n)
    if 8 * k == n or 8 * k == 3 * n:
        if c * s > 0:
            return (r - i) * c, (r + i) * c
        return (r + i) * c, (i - r) * c
    return r * c - i * s, r * s + i * c


def _cfft(xs, sign):
    n = len(xs)
    if n == 1:
        return xs
    ev, od = _cfft(xs[0::2], sign), _cfft(xs[1::2], sign)
    out = [None] * n
    for k in range(n // 2):
        er, ei = ev[k]
        if 4 * k == n:
            orr, oi = od[k]
            lo, hi = (er - oi, ei + orr), (er + oi, ei - orr)
            out[k], out[k + n // 2] = (lo, hi) if sign > 0 else (hi, lo)
        else:
            tr, ti = _twiddle(od[k], k, n, sign)
            out[k], out[k + n // 2] = (er + tr, ei + ti), (er - tr, ei - ti)
    return out


def _rfft8(x):
    a0, a1, b0, b1 = x[0] + x[4], x[0] - x[4], x[2] + x[6], x[2] - x[6]
    c0, c1, d0, d1 = x[1] + x[5], x[1] - x[5], x[3] + x[7], x[3] - x[7]
    e, f = a0 + b0, c0 + d0
    g, h = (c1 - d1) * R2, (c1 + d1) * R2
    return [e + f, e - f, a1 + g, b1 + h, a0 - b0, c0 - d0, a1 - g, b1 - h]


def _irfft8(z):
    z0, z4, z1r, z1i, z2r, z2i, z3r, z3i = z
    e, f = z0 + z4, z0 - z4
    a1, g = z1r + z3r, (z1r - z3r) * R2
    b1, h = z1i + z3i, (z1i - z3i) * R2
    a0, b0, c0, d0 = e + z2r, e - z2r, f + z2i, f - z2i
    c1, d1 = g + h, h - g
    return [a0 + a1, c0 + c1, b0 + b1, d0 + d1, a0 - a1, c0 - c1, b0 - b1, d0 - d1]


def _kernel(x_hbm, mem0_hbm, wq_hbm, wk_hbm, wv_hbm, wo_hbm, bx_hbm, wr_hbm, wi_hbm, fill_hbm, cst_hbm,
            out_hbm,
            x_v, xpre_v, xs_v, mem0_v, fill_v, lhs_v, wqkv, wo_v, pre, opost, outa_v,
            bx_v, w_v, wn_v, wt, cst, zs, vv, tn, outb_v,
            sem_w, sem_f, sem_in, sem_out):
    scale = E ** -0.5
    wus = [w.bitcast(U32) for w in (wq_hbm, wk_hbm, wv_hbm)]
    wo_u = wo_hbm.bitcast(U32)
    fus = [w.at[pl.ds(0, 512)].bitcast(U32) for w in (wr_hbm, wi_hbm)]

    def w_copies(j, t, sem):
        return [pltpu.make_async_copy(wus[t].at[:, :, j, :], wqkv.at[j, t], sem)]

    w0_cps = [w_copies(0, t, sem_in.at[3 + t]) for t in range(3)]
    w0_cps[0].insert(0, pltpu.make_async_copy(x_hbm.at[:, pl.ds(0, 8), :], xpre_v, sem_in.at[3]))

    def w_pair(j):
        return [cp for t in range(3) for cp in w_copies(j, t, sem_w.at[j])]

    a_cps = [pltpu.make_async_copy(wo_u.at[:, pl.ds(128 * n, 128)], wo_v.at[n], sem_in.at[1]) for n in range(8)]
    a_cps += [pltpu.make_async_copy(x_hbm.at[pl.ds(0, CH)], x_v.at[pl.ds(0, CH)], sem_in.at[1]),
              pltpu.make_async_copy(mem0_hbm, mem0_v, sem_in.at[1]),
              pltpu.make_async_copy(fill_hbm, fill_v, sem_in.at[1]),
              pltpu.make_async_copy(cst_hbm.at[pl.ds(0, C_MS)], cst.at[pl.ds(0, C_MS)], sem_in.at[1]),
              pltpu.make_async_copy(bx_hbm, bx_v, sem_in.at[1])]

    def f_cps(it):
        return [pltpu.make_async_copy(fus[t].at[:, pl.ds(pl.multiple_of(128 * (2 * it + h), 128), 128)],
                                      w_v.at[t, 2 * it + h], sem_f.at[it]) for t in range(2) for h in range(2)]

    b_cps = [pltpu.make_async_copy(x_hbm.at[pl.ds(CH, NSEG - CH)], x_v.at[pl.ds(CH, NSEG - CH)], sem_in.at[2]),
             pltpu.make_async_copy(cst_hbm.at[pl.ds(C_MS, C_NUM - C_MS)], cst.at[pl.ds(C_MS, C_NUM - C_MS)],
                                   sem_in.at[2])]
    b_cps += [pltpu.make_async_copy(w.at[pl.ds(512, 1)], wn_v.at[t], sem_in.at[2])
              for t, w in enumerate((wr_hbm, wi_hbm))]

    def pre_step(j, t):
        xp = xpre_v[...].reshape(NSEG * 8, DM)
        a, b = wqkv[j, t, :, pl.ds(0, 8, stride=2), :], wqkv[j, t, :, pl.ds(1, 8, stride=2), :]
        lo = (a & jnp.uint32(0xFFFF)) | (b << 16)
        hi = (a >> 16) | (b & jnp.uint32(0xFFFF0000))
        wqkv[j, t, :, 0:8, :] = lo
        wqkv[j, t, :, 8:16, :] = hi
        r0, r1 = _bdot(xp, _bf(lo.reshape(DM // 2, E))), _bdot(xp, _bf(hi.reshape(DM // 2, E)))
        pre[j, t] = _pack2(r0, r1).reshape(NSEG, 8, E)

    def strassen_lhs():
        for g in range(NSEG // 4):
            xa = [xpre_v[4 * g + k].astype(F32) for k in range(4)]
            a1, a2 = jnp.concatenate([xa[0], xa[2]], axis=0), jnp.concatenate([xa[1], xa[3]], axis=0)
            a11, a12, a21, a22 = a1[:, :DM // 2], a1[:, DM // 2:], a2[:, :DM // 2], a2[:, DM // 2:]
            for n, v in enumerate((a11 + a22, a22, a21 + a22, a11 + a12, a11, a12 - a22, a21 - a11)):
                xs_v[n, 8 * g:8 * g + 8, :] = pltpu.bitcast(v.astype(BF), U32)

    def pre_step7(j, t):
        a, b = wqkv[j, t, :, pl.ds(0, 8, stride=2), :], wqkv[j, t, :, pl.ds(1, 8, stride=2), :]
        hb = DM // 32
        w = [[(_unpack2(a[k * hb:(k + 1) * hb], p), _unpack2(b[k * hb:(k + 1) * hb], p)) for p in range(2)]
             for k in range(2)]
        wp = [[_pack2(*w[k][p]) for p in range(2)] for k in range(2)]
        for p in range(2):
            wqkv[j, t, :, 8 * p:8 * p + 8, :] = jnp.concatenate([wp[0][p], wp[1][p]], axis=0)
        add = lambda u, v: _pack2(u[0] + v[0], u[1] + v[1])
        sub = lambda u, v: _pack2(u[0] - v[0], u[1] - v[1])
        (b11, b12), (b21, b22) = w
        mm = lambda n, r: _bdot(_bf(xs_v[n]), _bf(r.reshape(DM // 4, E)))
        m1 = mm(0, add(b11, b22))
        m4 = mm(1, sub(b21, b11))
        m2 = mm(2, wp[0][0])
        c11, c21, c22 = m1 + m4, m2 + m4, m1 - m2
        m5 = mm(3, wp[1][1])
        m3 = mm(4, sub(b12, b22))
        c11, c12, c22 = c11 - m5, m3 + m5, c22 + m3
        c11 = c11 + mm(5, add(b21, b22))
        c22 = c22 + mm(6, add(b11, b12))
        r = jnp.stack([_pack2(c11, c12).reshape(NSEG // 2, 8, E), _pack2(c21, c22).reshape(NSEG // 2, 8, E)], axis=1)
        pre[j, t] = r.reshape(NSEG, 8, E)

    for cp in w0_cps[0] + w0_cps[1] + w0_cps[2] + w_pair(1):
        cp.start()
    for t in range(3):
        for cp in w0_cps[t]:
            cp.wait()
        if t == 0:
            for j in range(2, NP):
                for cp in w_pair(j):
                    cp.start()
            strassen_lhs()
        if t == 2:
            for cp in a_cps:
                cp.start()
        (pre_step if t == 0 else pre_step7)(0, t)

    def pre_body(j, carry):
        for cp in w_pair(j):
            cp.wait()

        @pl.when(j >= NP - NIT)
        def _():
            for cp in f_cps(j - (NP - NIT)):
                cp.start()

        for t in range(3):
            pre_step7(j, t)
        return carry

    lax.fori_loop(1, NP, pre_body, 0)
    for cp in b_cps:
        cp.start()
    for cp in a_cps:
        cp.wait()

    lane = lax.broadcasted_iota(I32, (8, 128), 1)
    alt = jnp.where(lane % 2 == 0, 1.0, -1.0).astype(F32)
    lo_half = lane < 64
    ev_grp = (lane // 32) % 2 == 0

    def half_coef(q):
        sg = -1.0 if q < 3 else 1.0
        tc, ts = math.cos(2 * math.pi * q / 16), -math.sin(2 * math.pi * q / 16)
        f = lambda lo, hi: jnp.where(lo_half, lo, hi).astype(F32)
        return f(1.0, ts), f(0.0, sg * tc), f(0.0, tc), f(sg, -sg * ts)

    def b_rows(i, b):
        return 2 * b + i // 4, pl.ds(pl.multiple_of((i % 4) * 8, 8), 8)

    def flat(zs_):
        return [v for z in zs_ for v in z]

    def put(ref, idx, val):
        ref[idx] = val
        return ref[idx]

    def as_u32(rows):
        return pltpu.bitcast(jnp.concatenate(rows, axis=0).astype(BF), U32)

    def b_fwd(i):
        r0 = pl.multiple_of(i * 8, 8)
        for cp in f_cps(i):
            cp.wait()
        hc = [None] + [half_coef(q) for q in range(1, 4)]
        tacc = jnp.zeros((8, 128), F32)
        zl = []
        for _ in range(3):
            yield None
        for b0 in range(0, 32, 2):
            rows = []
            for b in (b0, b0 + 1):
                xb = bx_v[(*b_rows(i, b), slice(None))].astype(F32)
                z = _rfft8([xb[:, 128 * t:128 * t + 128] for t in range(8)])
                tacc = jnp.where(lane == b, jnp.sum(z[0] * alt, axis=1, keepdims=True), tacc)
                for q in range(1, 4):
                    c1, c2, c3, c4 = hc[q]
                    zr, zi = z[2 * q], z[2 * q + 1]
                    pp = c1 * zr + c2 * zi
                    qq = pltpu.roll(c3 * zr + c4 * zi, 64, 1)
                    z[2 * q], z[2 * q + 1] = pp + qq, pp - qq
                rows.append(z)
            zl.append([as_u32([rows[0][n], rows[1][n]]) for n in range(8)])
            yield zl[-1] + [tacc]
            yield None
            if b0 % 4 == 0:
                e, t, ty = 2 * i + b0 // 16, (b0 // 8) % 2, (b0 // 4) % 2
                u = jnp.concatenate([w_v[t, e, pl.ds(m + ty, 32, stride=8), :] for m in (0, 6, 4, 2)], axis=0)
                ut = pltpu.bitcast(pltpu.bitcast(u, F32).T, U32)
                yield [put(wt, (t, ty, pl.ds(8 * (v % 4) * WP + 4 * e + v // 4, 8, stride=WP), slice(None)),
                           ut[8 * v:8 * v + 8]) for v in range(16)]
        tn[pl.ds(r0, 8), :] = tacc

        def mm(n):
            return _bdot(_bf(jnp.concatenate([z[n] for z in zl], axis=0)), _bf(cst[C_MD + n]))

        oo = [mm(n) for n in range(4)]
        yield MID
        oo += [mm(n) for n in range(4, 8)]
        for q in range(4):
            sel, sh = (ev_grp, 96) if q == 0 else (lo_half, 64)
            ys = []
            for b0 in range(4):
                xs = []
                for b in range(b0, 32, 4):
                    e_, o_ = oo[2 * q][8 * b:8 * b + 8], oo[2 * q + 1][8 * b:8 * b + 8]
                    xs.append((jnp.where(sel, e_, o_), pltpu.roll(jnp.where(sel, o_, e_), sh, 1)))
                ys.append([_twiddle(y, b0 * k1, 32, -1) for k1, y in enumerate(_cfft(xs, -1))])
                yield flat(ys[-1])
            for k1 in range(8):
                o = [_pack2(*y) for y in _cfft([ys[b0][k1] for b0 in range(4)], -1)]
                yield [put(zs, (k1 + 8 * k0, pl.ds(r0, 8), pl.ds(128 * q, 128)), o[k0]) for k0 in range(4)]

    def b_mid(i):
        for n in range(4):
            dl = 4 * i + n
            for _ in range(6):
                yield None
            y = _bdot(_bf(cst[C_MS + dl]), _bf(zs[dl]))
            for _ in range(3):
                yield None
            w0 = pl.multiple_of(dl * WP, 8)
            rows = []
            for r in range(8):
                wq = []
                for t in range(2):
                    ta, tb = wt[t, 0, pl.ds(w0 + 8 * r, 8), :], wt[t, 1, pl.ds(w0 + 8 * r, 8), :]
                    wq.append([_unpack2(ta, 0), _unpack2(jnp.where(ev_grp, ta, tb), 1),
                               _unpack2(tb, 0), _unpack2(jnp.where(ev_grp, tb, ta), 1)])
                cols = []
                for q in range(4):
                    yr = y[8 * r:8 * r + 8, 128 * q:128 * q + 128]
                    yi = y[64 + 8 * r:72 + 8 * r, 128 * q:128 * q + 128]
                    wr, wi = wq[0][q], wq[1][q]
                    cols.append(_pack2(yr * wr - yi * wi, yr * wi + yi * wr))
                rows.append(jnp.concatenate(cols, axis=1))
                yield cols
            yield None
            vv[dl] = _bdot(_bf(cst[C_MS + 32 + dl]), _bf(jnp.concatenate(rows, axis=0)))
            for _ in range(6):
                yield None

    def b_nyq():
        c, s = pltpu.bitcast(cst[C_TW], F32), pltpu.bitcast(cst[C_TW + 1], F32)
        tb = tn[...].astype(BF)
        tr, ti = _bdot(tb, _bf(cst[C_MN])), _bdot(tb, _bf(cst[C_MN + 1]))
        y = _bdot(_bf(cst[C_MN + 2, 0:16, :]), _bf(_pack2(tr * c + ti * s, ti * c - tr * s)))
        row = lax.broadcasted_iota(I32, (16, 128), 0)
        wn = []
        for t in range(2):
            wrow = wn_v[t].astype(F32)
            acc = jnp.zeros((16, 128), F32)
            for e in range(16):
                acc = jnp.where(row == e, wrow[:, 128 * e:128 * e + 128], acc)
            wn.append(acc)
        yr, yi = y[0:16], y[16:32]
        v = _bdot(_bf(cst[C_MN + 3, :, 0:32]), _bf(_pack2(yr * wn[0] - yi * wn[1], yr * wn[1] + yi * wn[0])))
        vr, vi = v[0:64], v[64:128]
        tn[...] = (_bdot((vr * c - vi * s).astype(BF), _bf(cst[C_MN + 4]))
                   + _bdot((vr * s + vi * c).astype(BF), _bf(cst[C_MN + 5])))

    def b_inv(i):
        r0 = pl.multiple_of(i * 8, 8)
        ul, zz = [], []
        yield None
        for q in range(4):
            sel, sh = (ev_grp, 32) if q == 0 else (lo_half, 64)
            ys = []
            for b0 in range(4):
                xs = [(vv[dl, pl.ds(r0, 8), 128 * q:128 * q + 128], vv[dl, pl.ds(64 + r0, 8), 128 * q:128 * q + 128])
                      for dl in range(b0, 32, 4)]
                ys.append([_twiddle(y, b0 * k1, 32, +1) for k1, y in enumerate(_cfft(xs, +1))])
                yield flat(ys[-1])
            ie, io = [], []
            for k1 in range(8):
                es, os_ = [], []
                for ur, ui in _cfft([ys[b0][k1] for b0 in range(4)], +1):
                    tmp = pltpu.roll(ui, sh, 1)
                    es.append(jnp.where(sel, ur, tmp))
                    os_.append(jnp.where(sel, tmp, ur))
                ie += [as_u32(es[0:2]), as_u32(es[2:4])]
                io += [as_u32(os_[0:2]), as_u32(os_[2:4])]
                yield ie[-2:] + io[-2:]
            ul += [ie, io]
            if q == 2:
                zz += [_bdot(_bf(jnp.concatenate(ul[n], axis=0)), _bf(cst[C_MD + 8 + n])) for n in range(4)]
        yield MID
        zz += [_bdot(_bf(jnp.concatenate(ul[n], axis=0)), _bf(cst[C_MD + 8 + n])) for n in range(4, 8)]
        for _ in range(4):
            yield None
        hc = [None] + [half_coef(q) for q in range(1, 4)]
        tb = tn[pl.ds(r0, 8), :]
        for g in range(32):
            b = g // 4 + 8 * (g % 4)
            z = [zz[n][8 * g:8 * g + 8] for n in range(8)]
            z[0] = z[0] + jnp.sum(jnp.where(lane == b, tb, 0.0), axis=1, keepdims=True) * alt
            for q in range(1, 4):
                c1, c2, c3, c4 = hc[q]
                pp = z[2 * q] + z[2 * q + 1]
                qq = pltpu.roll(z[2 * q] - z[2 * q + 1], 64, 1)
                z[2 * q], z[2 * q + 1] = c1 * pp + c3 * qq, c2 * pp + c4 * qq
            outb_v[(*b_rows(i, b), slice(None))] = jnp.concatenate(_irfft8(z), axis=1).astype(BF)
            yield [outb_v[(*b_rows(i, b), pl.ds(256 * k, 128))].astype(F32) for k in range(4)]

    def tie(w, vals):
        if not vals:
            return w
        acc = None
        for v in vals:
            v = v if v.dtype == U32 else pltpu.bitcast(v, U32)
            acc = v if acc is None else acc | v
        zero = cst[C_MN, 56:64, :]
        return jnp.concatenate([w[0:8] | (acc & zero), w[8:]], axis=0)

    def post(c, n):
        op = opost[c % 2].reshape(CH * 8, H * E).astype(BF)
        r = _bdot(op, _bf(wo_v[n]))
        col = n * 128 if isinstance(n, int) else pl.multiple_of(n * 128, 128)
        outa_v[pl.ds(c * CH, CH), 0:8, pl.ds(col, 128)] = r.reshape(CH, 8, 128).astype(BF)

    def seg_step(i, u, mem, c, slot):
        s = c * CH + i
        xs = x_v[s]
        lhs_v[u] = as_u32([mem, xs[8:32].astype(F32)])
        fill = fill_v[...]
        late = []

        def proj(j, t):
            w0, w1 = [wqkv[j, t, :, 8 * p:8 * p + 8, :].reshape(DM // 2, E) for p in range(2)]
            w1 = tie(w1, late.pop(0) if late and (j % 2 == 1 or t == 2) else None)
            r0, r1 = _bdot(_bf(lhs_v[u]), _bf(tie(w0, slot()))), _bdot(_bf(lhs_v[u]), _bf(w1))
            pw = pre[j, t, s]
            if t == 0:
                return jnp.concatenate([r0, r1, _unpack2(pw, 0), _unpack2(pw, 1)], axis=0).astype(BF)
            return _bf(jnp.concatenate([_pack2(r0, r1), pw], axis=0))

        def qk(q, k):
            sc = lax.dot_general(q, k, (((1,), (1,)), ((), ())), preferred_element_type=F32) * scale
            sc = jnp.where(fill == 0.0, sc, fill)
            p = jnp.exp(sc - jnp.max(sc, axis=-1, keepdims=True))
            return (p * pl.reciprocal(jnp.sum(p, axis=-1, keepdims=True), approx=True)).astype(BF)

        ob, ps, vs = {}, {}, {}

        def pv(j):
            o = _bdot(ps[j], vs[j])
            ob[j] = [as_u32([o[0:32]]), as_u32([o[32:64]])]
            late.append([put(opost, (c % 2, i, slice(None), pl.ds(256 * j + 128 * p, 128)), o[64 + 8 * p:72 + 8 * p])
                         for p in range(2)] + [ob[j][p][8 * r:8 * r + 8] for p in range(2) for r in range(2)])

        def wo(g0, g1):
            og = _bf(jnp.concatenate([o for j in range(2 * g0, 2 * g1) for o in ob[j]], axis=1))
            return jnp.concatenate([_bdot(og, _bf(wo_v[n, g0 * 256:g1 * 256, :])) for n in range(8)], axis=1)

        ng = NP // 2
        for g in range(ng):
            ja, jb = 2 * g, 2 * g + 1
            qa, ka, qb, kb = proj(ja, 0), proj(ja, 1), proj(jb, 0), proj(jb, 1)
            vs[ja], vs[jb] = proj(ja, 2), proj(jb, 2)
            ps[ja], ps[jb] = qk(qa, ka), qk(qb, kb)
            if g > 0:
                pv(ja - 2)
                pv(jb - 2)
        res = wo(0, 3)
        pv(NP - 2)
        pv(NP - 1)
        res = res + wo(3, ng - 1)
        res = res + wo(ng - 1, ng)
        outa_v[s, 8:32, :] = res[8:32].astype(BF)
        return res[0:8].astype(BF).astype(F32)

    def chunk_body(it, mem, *, c, side):
        gen = side(it) if side is not None else iter(())
        state = {'mid': False}

        def slot():
            if state['mid']:
                return None
            vals = next(gen, None)
            if vals is MID:
                state['mid'] = True
                return None
            return vals

        mem = seg_step(2 * it, 0, mem, c, slot)
        if c > 0:
            post(c - 1, it)
        if side in (b_fwd, b_inv):
            while not state['mid']:
                slot()
        state['mid'] = False
        mem = seg_step(2 * it + 1, 1, mem, c, slot)
        for _ in gen:
            pass
        return mem

    def out_a(c, rows, cols, sem):
        return pltpu.make_async_copy(outa_v.at[pl.ds(c * CH, CH), rows, cols],
                                     out_hbm.at[pl.ds(c * CH, CH), rows, cols], sem)

    nch = NSEG // CH
    out_cps = [out_a(c, pl.ds(0, SEG), pl.ds(0, DM), sem_out.at[c]) for c in range(nch - 1)]
    out_cps += [out_a(nch - 1, pl.ds(8, SEG - 8), pl.ds(0, DM), sem_out.at[3]),
                pltpu.make_async_copy(outb_v, out_hbm.at[:, :, pl.ds(DM, DM)], sem_out.at[4]),
                out_a(nch - 1, pl.ds(0, 8), pl.ds(0, 896), sem_out.at[5]),
                out_a(nch - 1, pl.ds(0, 8), pl.ds(896, 128), sem_out.at[6])]

    sides = [b_fwd, b_mid, b_inv, None]
    mem = mem0_v[...].astype(F32)
    for c in range(nch):
        mem = lax.fori_loop(0, NIT, functools.partial(chunk_body, c=c, side=sides[c]), mem)
        if c == 0:
            for cp in b_cps:
                cp.wait()
            b_nyq()
        else:
            out_cps[c - 1].start()
        if c == 2:
            out_cps[4].start()
    out_cps[3].start()
    for n in range(8):
        post(nch - 1, n)
        if n >= 6:
            out_cps[n - 1].start()
    for cp in out_cps:
        cp.wait()


def pallas_concat_heads__memory_aug_recurrent_mem_tr__spectral_gfnet__prompt_kernel(
    A_x, A_mem0, A_Wq, A_Wk, A_Wv, A_Wo, A_seg_len, B_x, B_w_r, B_w_i,
):
    assert A_x.shape == (1, S, DM) and A_Wq.shape == (DM, H, E) and A_mem0.shape == (1, M, DM)
    assert B_x.shape == (1, S, DM) and (not isinstance(A_seg_len, int) or A_seg_len == SEG)
    hbm = pl.BlockSpec(memory_space=pltpu.HBM)
    wr = lambda w: w.reshape(DM // 16, 16, H, E)
    out = pl.pallas_call(
        _kernel,
        out_shape=jax.ShapeDtypeStruct((NSEG, SEG, 2 * DM), BF),
        in_specs=[hbm] * 11,
        out_specs=hbm,
        scratch_shapes=[
            pltpu.VMEM((NSEG, SEG, DM), BF),
            pltpu.VMEM((NSEG, 8, DM), BF),
            pltpu.VMEM((7, NSEG * 2, DM // 2), U32),
            pltpu.VMEM((M, DM), BF),
            pltpu.VMEM((80, 80), F32),
            pltpu.VMEM((2, SEG // 2, DM), U32),
            pltpu.VMEM((NP, 3, DM // 16, 16, E), U32),
            pltpu.VMEM((8, H * E // 2, 128), U32),
            pltpu.VMEM((NP, 3, NSEG, 8, E), U32),
            pltpu.VMEM((2, CH, 8, H * E), F32),
            pltpu.VMEM((NSEG, SEG, DM), BF),
            pltpu.VMEM((NSEG, SEG, DM), BF),
            pltpu.VMEM((2, 16, 256, 128), U32),
            pltpu.VMEM((2, 1, S), BF),
            pltpu.VMEM((2, 2, 32 * WP, 128), U32),
            pltpu.VMEM((C_NUM, 64, 128), U32),
            pltpu.VMEM((32, 64, 512), U32),
            pltpu.VMEM((32, 128, 512), F32),
            pltpu.VMEM((64, 128), F32),
            pltpu.VMEM((NSEG, SEG, DM), BF),
            pltpu.SemaphoreType.DMA((NP,)),
            pltpu.SemaphoreType.DMA((NIT,)),
            pltpu.SemaphoreType.DMA((6,)),
            pltpu.SemaphoreType.DMA((7,)),
        ],
        compiler_params=pltpu.CompilerParams(vmem_limit_bytes=112 * 1024 * 1024),
    )(A_x.reshape(NSEG, SEG, DM), A_mem0.reshape(M, DM), wr(A_Wq), wr(A_Wk), wr(A_Wv),
      A_Wo.reshape(H * E, DM), B_x.reshape(NSEG, SEG, DM), B_w_r.T, B_w_i.T, _mask_fill(), _fft_consts())
    return out.reshape(1, S, 2 * DM)
```

```python
import functools
import math

import jax
import jax.numpy as jnp
import numpy as np
from jax import lax
import jax.experimental.pallas as pl
import jax.experimental.pallas.tpu as pltpu

BF, F32, U32, I32 = jnp.bfloat16, jnp.float32, jnp.uint32, jnp.int32

S, DM, H, E, M, SEG = 2048, 1024, 32, 128, 8, 32
NSEG = S // SEG
NP = H // 2
CH = 16
NIT = CH // 2
R2 = math.sqrt(0.5)
MID = 'mid'


def _to_u32(m):
    u = np.ascontiguousarray(m, dtype=np.float32).view(np.uint32)
    h = ((u + 0x7FFF + ((u >> 16) & 1)) >> 16).astype(np.uint32)
    return h[..., 0::2, :] | (h[..., 1::2, :] << 16)


def _mask_fill():
    r = np.arange(80)
    pos_of = lambda rr: np.where(rr < M, rr, np.where(rr < SEG, rr + M, rr - SEG + M))
    qhead = np.where(r < 64, r // 32, (r - 64) // 8)
    qpos = pos_of(np.where(r < 64, r % 32, SEG + (r - 64) % 8))
    khead, kpos = r % 2, pos_of(r // 2)
    vis = (qpos[:, None] < M) | (qpos[:, None] >= kpos[None, :])
    same = qhead[:, None] == khead[None, :]
    return np.where(same, np.where(vis, 0.0, -1e9), -np.inf).astype(np.float32)


RES = ((0, 12, 8, 4), (1, 15, 9, 7), (2, 14, 10, 6), (3, 13, 11, 5))
WP = 72
C_MD, C_MN, C_TW, C_MS, C_NUM = 0, 16, 22, 24, 88


@functools.lru_cache(maxsize=None)
def _fft_consts():
    md = np.zeros((16, 128, 128))
    for q in range(4):
        if q == 0:
            lay = [[(0, 0), (0, 1), (2, 0), (2, 1)], [(3, 1), (1, 0), (1, 1), (3, 0)]]
        else:
            lay = [[(0, 0), (1, 0), (0, 1), (1, 1)], [(2, 1), (3, 1), (2, 0), (3, 0)]]
        for h in range(2):
            ms_, ws_ = [], []
            for g, part in lay[h]:
                k = 16 * np.arange(32) + RES[q][g]
                th = 2 * np.pi * np.outer(np.arange(128 if q == 0 else 64), k) / DM
                c, s = np.cos(th), np.sin(th)
                if q == 0:
                    ms_.append(-s if part else c)
                else:
                    sg = (1.0 if RES[q][g] % 8 == q else -1.0) * (1.0 - 2.0 * h)
                    ms_.append(np.concatenate([-s, sg * c] if part else [c, sg * s]))
                ws_.append(np.where(k == 0, 1.0, 2.0) / DM)
            m = np.concatenate(ms_, axis=1)
            md[2 * q + h] = m
            md[8 + 2 * q + h] = (m * np.concatenate(ws_)[None, :]).T
    a, l = np.arange(64), np.arange(128)
    ms = np.zeros((64, 128, 128))
    for dl in range(32):
        th = 2 * np.pi * np.outer(32 * a + dl, a) / S
        c, s = np.cos(th), np.sin(th)
        ms[dl, :64, 0::2], ms[dl, :64, 1::2] = c, s
        ms[dl, 64:, 0::2], ms[dl, 64:, 1::2] = -s, c
        ms[32 + dl, :64, 0::2], ms[32 + dl, :64, 1::2] = c.T / S, -s.T / S
        ms[32 + dl, 64:, 0::2], ms[32 + dl, 64:, 1::2] = s.T / S, c.T / S
    mn = np.zeros((6, 128, 128))
    th = 2 * np.pi * np.outer(np.arange(32), l) / 32
    mn[0, :32], mn[1, :32] = np.cos(th), -np.sin(th)
    mn[4, :, :32], mn[5, :, :32] = np.cos(th).T / DM, -np.sin(th).T / DM
    th = 2 * np.pi * np.outer(np.arange(16), a) / 16
    c, s = np.cos(th), np.sin(th)
    mn[2, :16, 0::2], mn[2, :16, 1::2], mn[2, 16:32, 0::2], mn[2, 16:32, 1::2] = c, s, -s, c
    mn[3, :64, 0:32:2], mn[3, :64, 1:32:2] = c.T / S, -s.T / S
    mn[3, 64:, 0:32:2], mn[3, 64:, 1:32:2] = s.T / S, c.T / S
    th = 2 * np.pi * np.outer(a, l) / S
    tw = np.stack([np.cos(th), np.sin(th)]).astype(np.float32).view(np.uint32)
    return np.concatenate([_to_u32(md), _to_u32(mn), tw, _to_u32(ms)], axis=0)


def _bdot(a, b):
    return jnp.dot(a, b, preferred_element_type=F32)


def _bf(u):
    return pltpu.bitcast(u, BF)


def _pack2(r, i):
    return pltpu.bitcast(pltpu.pack_elementwise([r, i], packed_dtype=BF), U32)


def _unpack2(u, p):
    if p == 0:
        return pltpu.bitcast(u << 16, F32)
    return pltpu.bitcast(u & jnp.uint32(0xFFFF0000), F32)


def _twiddle(z, k, n, sign):
    r, i = z
    if k == 0:
        return r, i
    if 4 * k == n:
        return (-i, r) if sign > 0 else (i, -r)
    c, s = math.cos(2 * math.pi * k / n), sign * math.sin(2 * math.pi * k / n)
    if 8 * k == n or 8 * k == 3 * n:
        if c * s > 0:
            return (r - i) * c, (r + i) * c
        return (r + i) * c, (i - r) * c
    return r * c - i * s, r * s + i * c


def _cfft(xs, sign):
    n = len(xs)
    if n == 1:
        return xs
    ev, od = _cfft(xs[0::2], sign), _cfft(xs[1::2], sign)
    out = [None] * n
    for k in range(n // 2):
        er, ei = ev[k]
        if 4 * k == n:
            orr, oi = od[k]
            lo, hi = (er - oi, ei + orr), (er + oi, ei - orr)
            out[k], out[k + n // 2] = (lo, hi) if sign > 0 else (hi, lo)
        else:
            tr, ti = _twiddle(od[k], k, n, sign)
            out[k], out[k + n // 2] = (er + tr, ei + ti), (er - tr, ei - ti)
    return out


def _rfft8(x):
    a0, a1, b0, b1 = x[0] + x[4], x[0] - x[4], x[2] + x[6], x[2] - x[6]
    c0, c1, d0, d1 = x[1] + x[5], x[1] - x[5], x[3] + x[7], x[3] - x[7]
    e, f = a0 + b0, c0 + d0
    g, h = (c1 - d1) * R2, (c1 + d1) * R2
    return [e + f, e - f, a1 + g, b1 + h, a0 - b0, c0 - d0, a1 - g, b1 - h]


def _irfft8(z):
    z0, z4, z1r, z1i, z2r, z2i, z3r, z3i = z
    e, f = z0 + z4, z0 - z4
    a1, g = z1r + z3r, (z1r - z3r) * R2
    b1, h = z1i + z3i, (z1i - z3i) * R2
    a0, b0, c0, d0 = e + z2r, e - z2r, f + z2i, f - z2i
    c1, d1 = g + h, h - g
    return [a0 + a1, c0 + c1, b0 + b1, d0 + d1, a0 - a1, c0 - c1, b0 - b1, d0 - d1]


def _kernel(x_hbm, mem0_hbm, wq_hbm, wk_hbm, wv_hbm, wo_hbm, bx_hbm, wr_hbm, wi_hbm, fill_hbm, cst_hbm,
            out_hbm,
            x_v, xpre_v, xs_v, mem0_v, fill_v, lhs_v, wqkv, wo_v, pre, opost, outa_v,
            bx_v, w_v, wn_v, wt, cst, zs, vv, tn, outb_v,
            sem_w, sem_f, sem_in, sem_out):
    scale = E ** -0.5
    wus = [w.bitcast(U32) for w in (wq_hbm, wk_hbm, wv_hbm)]
    wo_u = wo_hbm.bitcast(U32)
    fus = [w.at[pl.ds(0, 512)].bitcast(U32) for w in (wr_hbm, wi_hbm)]

    def w_copies(j, t, sem):
        return [pltpu.make_async_copy(wus[t].at[:, :, j, :], wqkv.at[j, t], sem)]

    w0_cps = [w_copies(0, 0, sem_in.at[3]), w_copies(0, 1, sem_in.at[4]) + w_copies(0, 2, sem_in.at[4])]
    w0_cps[0].insert(0, pltpu.make_async_copy(x_hbm.at[:, pl.ds(0, 8), :], xpre_v, sem_in.at[3]))

    def w_pair(j):
        return [cp for t in range(3) for cp in w_copies(j, t, sem_w.at[j])]

    a_cps = [pltpu.make_async_copy(wo_u.at[:, pl.ds(128 * n, 128)], wo_v.at[n], sem_in.at[1]) for n in range(8)]
    a_cps += [pltpu.make_async_copy(x_hbm.at[pl.ds(0, CH)], x_v.at[pl.ds(0, CH)], sem_in.at[1]),
              pltpu.make_async_copy(mem0_hbm, mem0_v, sem_in.at[1]),
              pltpu.make_async_copy(fill_hbm, fill_v, sem_in.at[1]),
              pltpu.make_async_copy(cst_hbm.at[pl.ds(0, C_MS)], cst.at[pl.ds(0, C_MS)], sem_in.at[1]),
              pltpu.make_async_copy(bx_hbm, bx_v, sem_in.at[1])]

    def f_cps(it):
        return [pltpu.make_async_copy(fus[t].at[:, pl.ds(pl.multiple_of(128 * (2 * it + h), 128), 128)],
                                      w_v.at[t, 2 * it + h], sem_f.at[it]) for t in range(2) for h in range(2)]

    b_cps = [pltpu.make_async_copy(x_hbm.at[pl.ds(CH, NSEG - CH)], x_v.at[pl.ds(CH, NSEG - CH)], sem_in.at[2]),
             pltpu.make_async_copy(cst_hbm.at[pl.ds(C_MS, C_NUM - C_MS)], cst.at[pl.ds(C_MS, C_NUM - C_MS)],
                                   sem_in.at[2])]
    b_cps += [pltpu.make_async_copy(w.at[pl.ds(512, 1)], wn_v.at[t], sem_in.at[2])
              for t, w in enumerate((wr_hbm, wi_hbm))]

    hb = DM // 32

    def retile(j, t, k):
        blk = pl.ds(k * hb, hb)
        a, b = wqkv[j, t, blk, pl.ds(0, 8, stride=2), :], wqkv[j, t, blk, pl.ds(1, 8, stride=2), :]
        wqkv[j, t, blk, 0:8, :] = (a & jnp.uint32(0xFFFF)) | (b << 16)
        wqkv[j, t, blk, 8:16, :] = (a >> 16) | (b & jnp.uint32(0xFFFF0000))

    def pre_step(j, t):
        retile(j, t, 0)
        retile(j, t, 1)
        r0, r1 = [_bdot(xpre_v[...].reshape(NSEG * 8, DM), _bf(wqkv[j, t, :, 8 * p:8 * p + 8, :].reshape(DM // 2, E)))
                  for p in range(2)]
        pre[j, t] = _pack2(r0, r1).reshape(NSEG, 8, E)

    def strassen_lhs():
        for g in range(NSEG // 4):
            xa = [xpre_v[4 * g + k].astype(F32) for k in range(4)]
            a1, a2 = jnp.concatenate([xa[0], xa[2]], axis=0), jnp.concatenate([xa[1], xa[3]], axis=0)
            a11, a12, a21, a22 = a1[:, :DM // 2], a1[:, DM // 2:], a2[:, :DM // 2], a2[:, DM // 2:]
            for n, v in enumerate((a11 + a22, a22, a21 + a22, a11 + a12, a11, a12 - a22, a21 - a11)):
                xs_v[n, 8 * g:8 * g + 8, :] = pltpu.bitcast(v.astype(BF), U32)

    def pre_step7(j, t):
        w = lambda k, p: wqkv[j, t, k * hb:(k + 1) * hb, 8 * p:8 * p + 8, :].reshape(DM // 4, E)
        add = lambda u, v: _pack2(_unpack2(u, 0) + _unpack2(v, 0), _unpack2(u, 1) + _unpack2(v, 1))
        sub = lambda u, v: _pack2(_unpack2(u, 0) - _unpack2(v, 0), _unpack2(u, 1) - _unpack2(v, 1))
        mm = lambda n, r: _bdot(_bf(xs_v[n]), _bf(r))
        retile(j, t, 0)
        m2 = mm(2, w(0, 0))
        c22 = mm(6, add(w(0, 0), w(0, 1))) - m2
        retile(j, t, 1)
        m4 = mm(1, sub(w(1, 0), w(0, 0)))
        c21 = m2 + m4
        m1 = mm(0, add(w(0, 0), w(1, 1)))
        c11, c22 = m1 + m4, c22 + m1
        m3 = mm(4, sub(w(0, 1), w(1, 1)))
        lower = _pack2(c21, c22 + m3).reshape(NSEG // 2, 8, E)
        c11 = c11 + mm(5, add(w(1, 0), w(1, 1)))
        m5 = mm(3, w(1, 1))
        upper = _pack2(c11 - m5, m3 + m5).reshape(NSEG // 2, 8, E)
        pre[j, t] = jnp.stack([upper, lower], axis=1).reshape(NSEG, 8, E)

    for cp in w0_cps[0] + w0_cps[1] + w_pair(1):
        cp.start()
    for cp in w0_cps[0]:
        cp.wait()
    for j in range(2, NP):
        for cp in w_pair(j):
            cp.start()
    pre_step(0, 0)
    strassen_lhs()
    for cp in w0_cps[1]:
        cp.wait()
    pre_step7(0, 1)
    pre_step7(0, 2)
    for cp in w_pair(1):
        cp.wait()
    for cp in a_cps + f_cps(0):
        cp.start()
    for t in range(3):
        pre_step7(1, t)

    def pre_body(k, carry):
        for cp in w_pair(2 * k) + w_pair(2 * k + 1):
            cp.wait()
        for cp in f_cps(k):
            cp.start()
        for j in (2 * k, 2 * k + 1):
            for t in range(3):
                pre_step7(j, t)
        return carry

    lax.fori_loop(1, NP // 2, pre_body, 0)
    for cp in b_cps:
        cp.start()
    for cp in a_cps:
        cp.wait()

    lane = lax.broadcasted_iota(I32, (8, 128), 1)
    alt = jnp.where(lane % 2 == 0, 1.0, -1.0).astype(F32)
    lo_half = lane < 64
    ev_grp = (lane // 32) % 2 == 0

    def half_coef(q):
        sg = -1.0 if q < 3 else 1.0
        tc, ts = math.cos(2 * math.pi * q / 16), -math.sin(2 * math.pi * q / 16)
        f = lambda lo, hi: jnp.where(lo_half, lo, hi).astype(F32)
        return f(1.0, ts), f(0.0, sg * tc), f(0.0, tc), f(sg, -sg * ts)

    def b_rows(i, b):
        return 2 * b + i // 4, pl.ds(pl.multiple_of((i % 4) * 8, 8), 8)

    def flat(zs_):
        return [v for z in zs_ for v in z]

    def put(ref, idx, val):
        ref[idx] = val
        return ref[idx]

    def as_u32(rows):
        return pltpu.bitcast(jnp.concatenate(rows, axis=0).astype(BF), U32)

    def b_fwd(i):
        r0 = pl.multiple_of(i * 8, 8)
        for cp in f_cps(i):
            cp.wait()
        hc = [None] + [half_coef(q) for q in range(1, 4)]
        tacc = jnp.zeros((8, 128), F32)
        zl = []
        for _ in range(3):
            yield None
        for b0 in range(0, 32, 2):
            rows = []
            for b in (b0, b0 + 1):
                xb = bx_v[(*b_rows(i, b), slice(None))].astype(F32)
                z = _rfft8([xb[:, 128 * t:128 * t + 128] for t in range(8)])
                tacc = jnp.where(lane == b, jnp.sum(z[0] * alt, axis=1, keepdims=True), tacc)
                for q in range(1, 4):
                    c1, c2, c3, c4 = hc[q]
                    zr, zi = z[2 * q], z[2 * q + 1]
                    pp = c1 * zr + c2 * zi
                    qq = pltpu.roll(c3 * zr + c4 * zi, 64, 1)
                    z[2 * q], z[2 * q + 1] = pp + qq, pp - qq
                rows.append(z)
            zl.append([as_u32([rows[0][n], rows[1][n]]) for n in range(8)])
            yield zl[-1] + [tacc]
            yield None
            if b0 % 4 == 0:
                e, t, ty = 2 * i + b0 // 16, (b0 // 8) % 2, (b0 // 4) % 2
                u = jnp.concatenate([w_v[t, e, pl.ds(m + ty, 32, stride=8), :] for m in (0, 6, 4, 2)], axis=0)
                ut = pltpu.bitcast(pltpu.bitcast(u, F32).T, U32)
                yield [put(wt, (t, ty, pl.ds(8 * (v % 4) * WP + 4 * e + v // 4, 8, stride=WP), slice(None)),
                           ut[8 * v:8 * v + 8]) for v in range(16)]
        tn[pl.ds(r0, 8), :] = tacc

        def mm(n):
            return _bdot(_bf(jnp.concatenate([z[n] for z in zl], axis=0)), _bf(cst[C_MD + n]))

        oo = [mm(n) for n in range(4)]
        yield MID
        oo += [mm(n) for n in range(4, 8)]
        for q in range(4):
            sel, sh = (ev_grp, 96) if q == 0 else (lo_half, 64)
            ys = []
            for b0 in range(4):
                xs = []
                for b in range(b0, 32, 4):
                    e_, o_ = oo[2 * q][8 * b:8 * b + 8], oo[2 * q + 1][8 * b:8 * b + 8]
                    xs.append((jnp.where(sel, e_, o_), pltpu.roll(jnp.where(sel, o_, e_), sh, 1)))
                ys.append([_twiddle(y, b0 * k1, 32, -1) for k1, y in enumerate(_cfft(xs, -1))])
                yield flat(ys[-1])
            for k1 in range(8):
                o = [_pack2(*y) for y in _cfft([ys[b0][k1] for b0 in range(4)], -1)]
                yield [put(zs, (k1 + 8 * k0, pl.ds(r0, 8), pl.ds(128 * q, 128)), o[k0]) for k0 in range(4)]

    def b_mid(i):
        for n in range(4):
            dl = 4 * i + n
            for _ in range(6):
                yield None
            y = _bdot(_bf(cst[C_MS + dl]), _bf(zs[dl]))
            for _ in range(3):
                yield None
            w0 = pl.multiple_of(dl * WP, 8)
            rows = []
            for r in range(8):
                wq = []
                for t in range(2):
                    ta, tb = wt[t, 0, pl.ds(w0 + 8 * r, 8), :], wt[t, 1, pl.ds(w0 + 8 * r, 8), :]
                    wq.append([_unpack2(ta, 0), _unpack2(jnp.where(ev_grp, ta, tb), 1),
                               _unpack2(tb, 0), _unpack2(jnp.where(ev_grp, tb, ta), 1)])
                cols = []
                for q in range(4):
                    yr = y[8 * r:8 * r + 8, 128 * q:128 * q + 128]
                    yi = y[64 + 8 * r:72 + 8 * r, 128 * q:128 * q + 128]
                    wr, wi = wq[0][q], wq[1][q]
                    cols.append(_pack2(yr * wr - yi * wi, yr * wi + yi * wr))
                rows.append(jnp.concatenate(cols, axis=1))
                yield cols
            yield None
            vv[dl] = _bdot(_bf(cst[C_MS + 32 + dl]), _bf(jnp.concatenate(rows, axis=0)))
            for _ in range(6):
                yield None

    def b_nyq():
        c, s = pltpu.bitcast(cst[C_TW], F32), pltpu.bitcast(cst[C_TW + 1], F32)
        tb = tn[...].astype(BF)
        tr, ti = _bdot(tb, _bf(cst[C_MN])), _bdot(tb, _bf(cst[C_MN + 1]))
        y = _bdot(_bf(cst[C_MN + 2, 0:16, :]), _bf(_pack2(tr * c + ti * s, ti * c - tr * s)))
        row = lax.broadcasted_iota(I32, (16, 128), 0)
        wn = []
        for t in range(2):
            wrow = wn_v[t].astype(F32)
            acc = jnp.zeros((16, 128), F32)
            for e in range(16):
                acc = jnp.where(row == e, wrow[:, 128 * e:128 * e + 128], acc)
            wn.append(acc)
        yr, yi = y[0:16], y[16:32]
        v = _bdot(_bf(cst[C_MN + 3, :, 0:32]), _bf(_pack2(yr * wn[0] - yi * wn[1], yr * wn[1] + yi * wn[0])))
        vr, vi = v[0:64], v[64:128]
        tn[...] = (_bdot((vr * c - vi * s).astype(BF), _bf(cst[C_MN + 4]))
                   + _bdot((vr * s + vi * c).astype(BF), _bf(cst[C_MN + 5])))

    def b_inv(i):
        r0 = pl.multiple_of(i * 8, 8)
        ul, zz = [], []
        yield None
        for q in range(4):
            sel, sh = (ev_grp, 32) if q == 0 else (lo_half, 64)
            ys = []
            for b0 in range(4):
                xs = [(vv[dl, pl.ds(r0, 8), 128 * q:128 * q + 128], vv[dl, pl.ds(64 + r0, 8), 128 * q:128 * q + 128])
                      for dl in range(b0, 32, 4)]
                ys.append([_twiddle(y, b0 * k1, 32, +1) for k1, y in enumerate(_cfft(xs, +1))])
                yield flat(ys[-1])
            ie, io = [], []
            for k1 in range(8):
                es, os_ = [], []
                for ur, ui in _cfft([ys[b0][k1] for b0 in range(4)], +1):
                    tmp = pltpu.roll(ui, sh, 1)
                    es.append(jnp.where(sel, ur, tmp))
                    os_.append(jnp.where(sel, tmp, ur))
                ie += [as_u32(es[0:2]), as_u32(es[2:4])]
                io += [as_u32(os_[0:2]), as_u32(os_[2:4])]
                yield ie[-2:] + io[-2:]
            ul += [ie, io]
            if q == 2:
                zz += [_bdot(_bf(jnp.concatenate(ul[n], axis=0)), _bf(cst[C_MD + 8 + n])) for n in range(4)]
        yield MID
        zz += [_bdot(_bf(jnp.concatenate(ul[n], axis=0)), _bf(cst[C_MD + 8 + n])) for n in range(4, 8)]
        for _ in range(4):
            yield None
        hc = [None] + [half_coef(q) for q in range(1, 4)]
        tb = tn[pl.ds(r0, 8), :]
        for g in range(32):
            b = g // 4 + 8 * (g % 4)
            z = [zz[n][8 * g:8 * g + 8] for n in range(8)]
            z[0] = z[0] + jnp.sum(jnp.where(lane == b, tb, 0.0), axis=1, keepdims=True) * alt
            for q in range(1, 4):
                c1, c2, c3, c4 = hc[q]
                pp = z[2 * q] + z[2 * q + 1]
                qq = pltpu.roll(z[2 * q] - z[2 * q + 1], 64, 1)
                z[2 * q], z[2 * q + 1] = c1 * pp + c3 * qq, c2 * pp + c4 * qq
            outb_v[(*b_rows(i, b), slice(None))] = jnp.concatenate(_irfft8(z), axis=1).astype(BF)
            yield [outb_v[(*b_rows(i, b), pl.ds(256 * k, 128))].astype(F32) for k in range(4)]

    def tie(w, vals):
        if not vals:
            return w
        acc = None
        for v in vals:
            v = v if v.dtype == U32 else pltpu.bitcast(v, U32)
            acc = v if acc is None else acc | v
        zero = cst[C_MN, 56:64, :]
        return jnp.concatenate([w[0:8] | (acc & zero), w[8:]], axis=0)

    def post(c, n):
        op = opost[c % 2].reshape(CH * 8, H * E).astype(BF)
        r = _bdot(op, _bf(wo_v[n]))
        col = n * 128 if isinstance(n, int) else pl.multiple_of(n * 128, 128)
        outa_v[pl.ds(c * CH, CH), 0:8, pl.ds(col, 128)] = r.reshape(CH, 8, 128).astype(BF)

    def seg_step(i, u, mem, c, slot):
        s = c * CH + i
        xs = x_v[s]
        lhs_v[u] = as_u32([mem, xs[8:32].astype(F32)])
        fill = fill_v[...]
        late = []

        def proj(j, t):
            w0, w1 = [wqkv[j, t, :, 8 * p:8 * p + 8, :].reshape(DM // 2, E) for p in range(2)]
            w1 = tie(w1, late.pop(0) if late and (j % 2 == 1 or t == 2) else None)
            r0, r1 = _bdot(_bf(lhs_v[u]), _bf(tie(w0, slot()))), _bdot(_bf(lhs_v[u]), _bf(w1))
            pw = pre[j, t, s]
            if t == 0:
                return jnp.concatenate([r0, r1, _unpack2(pw, 0), _unpack2(pw, 1)], axis=0).astype(BF)
            return _bf(jnp.concatenate([_pack2(r0, r1), pw], axis=0))

        def qk(q, k):
            sc = lax.dot_general(q, k, (((1,), (1,)), ((), ())), preferred_element_type=F32) * scale
            sc = jnp.where(fill == 0.0, sc, fill)
            p = jnp.exp(sc - jnp.max(sc, axis=-1, keepdims=True))
            return (p * pl.reciprocal(jnp.sum(p, axis=-1, keepdims=True), approx=True)).astype(BF)

        ob, ps, vs = {}, {}, {}

        def pv(j):
            o = _bdot(ps[j], vs[j])
            ob[j] = [as_u32([o[0:32]]), as_u32([o[32:64]])]
            late.append([put(opost, (c % 2, i, slice(None), pl.ds(256 * j + 128 * p, 128)), o[64 + 8 * p:72 + 8 * p])
                         for p in range(2)] + [ob[j][p][8 * r:8 * r + 8] for p in range(2) for r in range(2)])

        def wo(g0, g1):
            og = _bf(jnp.concatenate([o for j in range(2 * g0, 2 * g1) for o in ob[j]], axis=1))
            return jnp.concatenate([_bdot(og, _bf(wo_v[n, g0 * 256:g1 * 256, :])) for n in range(8)], axis=1)

        ng = NP // 2
        for g in range(ng):
            ja, jb = 2 * g, 2 * g + 1
            qa, ka, qb, kb = proj(ja, 0), proj(ja, 1), proj(jb, 0), proj(jb, 1)
            vs[ja], vs[jb] = proj(ja, 2), proj(jb, 2)
            ps[ja], ps[jb] = qk(qa, ka), qk(qb, kb)
            if g > 0:
                pv(ja - 2)
                pv(jb - 2)
        res = wo(0, 3)
        pv(NP - 2)
        pv(NP - 1)
        res = res + wo(3, ng - 1)
        res = res + wo(ng - 1, ng)
        outa_v[s, 8:32, :] = res[8:32].astype(BF)
        return res[0:8].astype(BF).astype(F32)

    def chunk_body(it, mem, *, c, side):
        gen = side(it) if side is not None else iter(())
        state = {'mid': False}

        def slot():
            if state['mid']:
                return None
            vals = next(gen, None)
            if vals is MID:
                state['mid'] = True
                return None
            return vals

        mem = seg_step(2 * it, 0, mem, c, slot)
        if c > 0:
            post(c - 1, it)
        if side in (b_fwd, b_inv):
            while not state['mid']:
                slot()
        state['mid'] = False
        mem = seg_step(2 * it + 1, 1, mem, c, slot)
        for _ in gen:
            pass
        return mem

    def out_a(c, rows, cols, sem):
        return pltpu.make_async_copy(outa_v.at[pl.ds(c * CH, CH), rows, cols],
                                     out_hbm.at[pl.ds(c * CH, CH), rows, cols], sem)

    nch = NSEG // CH
    out_cps = [out_a(c, pl.ds(0, SEG), pl.ds(0, DM), sem_out.at[c]) for c in range(nch - 1)]
    out_cps += [out_a(nch - 1, pl.ds(8, SEG - 8), pl.ds(0, DM), sem_out.at[3]),
                pltpu.make_async_copy(outb_v, out_hbm.at[:, :, pl.ds(DM, DM)], sem_out.at[4]),
                out_a(nch - 1, pl.ds(0, 8), pl.ds(0, 896), sem_out.at[5]),
                out_a(nch - 1, pl.ds(0, 8), pl.ds(896, 128), sem_out.at[6])]

    sides = [b_fwd, b_mid, b_inv, None]
    mem = mem0_v[...].astype(F32)
    for c in range(nch):
        mem = lax.fori_loop(0, NIT, functools.partial(chunk_body, c=c, side=sides[c]), mem)
        if c == 0:
            for cp in b_cps:
                cp.wait()
            b_nyq()
        else:
            out_cps[c - 1].start()
        if c == 2:
            out_cps[4].start()
    out_cps[3].start()
    for n in range(8):
        post(nch - 1, n)
        if n >= 6:
            out_cps[n - 1].start()
    for cp in out_cps:
        cp.wait()


def pallas_concat_heads__memory_aug_recurrent_mem_tr__spectral_gfnet__prompt_kernel(
    A_x, A_mem0, A_Wq, A_Wk, A_Wv, A_Wo, A_seg_len, B_x, B_w_r, B_w_i,
):
    assert A_x.shape == (1, S, DM) and A_Wq.shape == (DM, H, E) and A_mem0.shape == (1, M, DM)
    assert B_x.shape == (1, S, DM) and (not isinstance(A_seg_len, int) or A_seg_len == SEG)
    hbm = pl.BlockSpec(memory_space=pltpu.HBM)
    wr = lambda w: w.reshape(DM // 16, 16, H, E)
    out = pl.pallas_call(
        _kernel,
        out_shape=jax.ShapeDtypeStruct((NSEG, SEG, 2 * DM), BF),
        in_specs=[hbm] * 11,
        out_specs=hbm,
        scratch_shapes=[
            pltpu.VMEM((NSEG, SEG, DM), BF),
            pltpu.VMEM((NSEG, 8, DM), BF),
            pltpu.VMEM((7, NSEG * 2, DM // 2), U32),
            pltpu.VMEM((M, DM), BF),
            pltpu.VMEM((80, 80), F32),
            pltpu.VMEM((2, SEG // 2, DM), U32),
            pltpu.VMEM((NP, 3, DM // 16, 16, E), U32),
            pltpu.VMEM((8, H * E // 2, 128), U32),
            pltpu.VMEM((NP, 3, NSEG, 8, E), U32),
            pltpu.VMEM((2, CH, 8, H * E), F32),
            pltpu.VMEM((NSEG, SEG, DM), BF),
            pltpu.VMEM((NSEG, SEG, DM), BF),
            pltpu.VMEM((2, 16, 256, 128), U32),
            pltpu.VMEM((2, 1, S), BF),
            pltpu.VMEM((2, 2, 32 * WP, 128), U32),
            pltpu.VMEM((C_NUM, 64, 128), U32),
            pltpu.VMEM((32, 64, 512), U32),
            pltpu.VMEM((32, 128, 512), F32),
            pltpu.VMEM((64, 128), F32),
            pltpu.VMEM((NSEG, SEG, DM), BF),
            pltpu.SemaphoreType.DMA((NP,)),
            pltpu.SemaphoreType.DMA((NIT,)),
            pltpu.SemaphoreType.DMA((6,)),
            pltpu.SemaphoreType.DMA((7,)),
        ],
        compiler_params=pltpu.CompilerParams(vmem_limit_bytes=112 * 1024 * 1024,
                                             disable_bounds_checks=True),
    )(A_x.reshape(NSEG, SEG, DM), A_mem0.reshape(M, DM), wr(A_Wq), wr(A_Wk), wr(A_Wv),
      A_Wo.reshape(H * E, DM), B_x.reshape(NSEG, SEG, DM), B_w_r.T, B_w_i.T, _mask_fill(), _fft_consts())
    return out.reshape(1, S, 2 * DM)
```

```python
import functools
import math

import jax
import jax.numpy as jnp
import numpy as np
from jax import lax
import jax.experimental.pallas as pl
import jax.experimental.pallas.tpu as pltpu

BF, F32, U32, I32 = jnp.bfloat16, jnp.float32, jnp.uint32, jnp.int32

S, DM, H, E, M, SEG = 2048, 1024, 32, 128, 8, 32
NSEG = S // SEG
NP = H // 2
CH = 16
NIT = CH // 2
R2 = math.sqrt(0.5)
MID = 'mid'
OPT = dict(put_wt=0, put_zs=0, put_out=0, put_op=0, norm_first=1, tie_ob=1)


def _to_u32(m):
    u = np.ascontiguousarray(m, dtype=np.float32).view(np.uint32)
    h = ((u + 0x7FFF + ((u >> 16) & 1)) >> 16).astype(np.uint32)
    return h[..., 0::2, :] | (h[..., 1::2, :] << 16)


def _mask_fill():
    r = np.arange(80)
    pos_of = lambda rr: np.where(rr < M, rr, np.where(rr < SEG, rr + M, rr - SEG + M))
    qhead = np.where(r < 64, r // 32, (r - 64) // 8)
    qpos = pos_of(np.where(r < 64, r % 32, SEG + (r - 64) % 8))
    khead, kpos = r % 2, pos_of(r // 2)
    vis = (qpos[:, None] < M) | (qpos[:, None] >= kpos[None, :])
    same = qhead[:, None] == khead[None, :]
    return np.where(same, np.where(vis, 0.0, -1e9), -np.inf).astype(np.float32)


RES = ((0, 12, 8, 4), (1, 15, 9, 7), (2, 14, 10, 6), (3, 13, 11, 5))
WP = 72
C_MD, C_MN, C_TW, C_MS, C_NUM = 0, 16, 22, 24, 88


@functools.lru_cache(maxsize=None)
def _fft_consts():
    md = np.zeros((16, 128, 128))
    for q in range(4):
        if q == 0:
            lay = [[(0, 0), (0, 1), (2, 0), (2, 1)], [(3, 1), (1, 0), (1, 1), (3, 0)]]
        else:
            lay = [[(0, 0), (1, 0), (0, 1), (1, 1)], [(2, 1), (3, 1), (2, 0), (3, 0)]]
        for h in range(2):
            ms_, ws_ = [], []
            for g, part in lay[h]:
                k = 16 * np.arange(32) + RES[q][g]
                th = 2 * np.pi * np.outer(np.arange(128 if q == 0 else 64), k) / DM
                c, s = np.cos(th), np.sin(th)
                if q == 0:
                    ms_.append(-s if part else c)
                else:
                    sg = (1.0 if RES[q][g] % 8 == q else -1.0) * (1.0 - 2.0 * h)
                    ms_.append(np.concatenate([-s, sg * c] if part else [c, sg * s]))
                ws_.append(np.where(k == 0, 1.0, 2.0) / DM)
            m = np.concatenate(ms_, axis=1)
            md[2 * q + h] = m
            md[8 + 2 * q + h] = (m * np.concatenate(ws_)[None, :]).T
    a, l = np.arange(64), np.arange(128)
    ms = np.zeros((64, 128, 128))
    for dl in range(32):
        th = 2 * np.pi * np.outer(32 * a + dl, a) / S
        c, s = np.cos(th), np.sin(th)
        ms[dl, :64, 0::2], ms[dl, :64, 1::2] = c, s
        ms[dl, 64:, 0::2], ms[dl, 64:, 1::2] = -s, c
        ms[32 + dl, :64, 0::2], ms[32 + dl, :64, 1::2] = c.T / S, -s.T / S
        ms[32 + dl, 64:, 0::2], ms[32 + dl, 64:, 1::2] = s.T / S, c.T / S
    mn = np.zeros((6, 128, 128))
    th = 2 * np.pi * np.outer(np.arange(32), l) / 32
    mn[0, :32], mn[1, :32] = np.cos(th), -np.sin(th)
    mn[4, :, :32], mn[5, :, :32] = np.cos(th).T / DM, -np.sin(th).T / DM
    th = 2 * np.pi * np.outer(np.arange(16), a) / 16
    c, s = np.cos(th), np.sin(th)
    mn[2, :16, 0::2], mn[2, :16, 1::2], mn[2, 16:32, 0::2], mn[2, 16:32, 1::2] = c, s, -s, c
    mn[3, :64, 0:32:2], mn[3, :64, 1:32:2] = c.T / S, -s.T / S
    mn[3, 64:, 0:32:2], mn[3, 64:, 1:32:2] = s.T / S, c.T / S
    th = 2 * np.pi * np.outer(a, l) / S
    tw = np.stack([np.cos(th), np.sin(th)]).astype(np.float32).view(np.uint32)
    return np.concatenate([_to_u32(md), _to_u32(mn), tw, _to_u32(ms)], axis=0)


def _bdot(a, b):
    return jnp.dot(a, b, preferred_element_type=F32)


def _bf(u):
    return pltpu.bitcast(u, BF)


def _pack2(r, i):
    return pltpu.bitcast(pltpu.pack_elementwise([r, i], packed_dtype=BF), U32)


def _unpack2(u, p):
    if p == 0:
        return pltpu.bitcast(u << 16, F32)
    return pltpu.bitcast(u & jnp.uint32(0xFFFF0000), F32)


def _twiddle(z, k, n, sign):
    r, i = z
    if k == 0:
        return r, i
    if 4 * k == n:
        return (-i, r) if sign > 0 else (i, -r)
    c, s = math.cos(2 * math.pi * k / n), sign * math.sin(2 * math.pi * k / n)
    if 8 * k == n or 8 * k == 3 * n:
        if c * s > 0:
            return (r - i) * c, (r + i) * c
        return (r + i) * c, (i - r) * c
    return r * c - i * s, r * s + i * c


def _cfft(xs, sign):
    n = len(xs)
    if n == 1:
        return xs
    ev, od = _cfft(xs[0::2], sign), _cfft(xs[1::2], sign)
    out = [None] * n
    for k in range(n // 2):
        er, ei = ev[k]
        if 4 * k == n:
            orr, oi = od[k]
            lo, hi = (er - oi, ei + orr), (er + oi, ei - orr)
            out[k], out[k + n // 2] = (lo, hi) if sign > 0 else (hi, lo)
        else:
            tr, ti = _twiddle(od[k], k, n, sign)
            out[k], out[k + n // 2] = (er + tr, ei + ti), (er - tr, ei - ti)
    return out


def _rfft8(x):
    a0, a1, b0, b1 = x[0] + x[4], x[0] - x[4], x[2] + x[6], x[2] - x[6]
    c0, c1, d0, d1 = x[1] + x[5], x[1] - x[5], x[3] + x[7], x[3] - x[7]
    e, f = a0 + b0, c0 + d0
    g, h = (c1 - d1) * R2, (c1 + d1) * R2
    return [e + f, e - f, a1 + g, b1 + h, a0 - b0, c0 - d0, a1 - g, b1 - h]


def _irfft8(z):
    z0, z4, z1r, z1i, z2r, z2i, z3r, z3i = z
    e, f = z0 + z4, z0 - z4
    a1, g = z1r + z3r, (z1r - z3r) * R2
    b1, h = z1i + z3i, (z1i - z3i) * R2
    a0, b0, c0, d0 = e + z2r, e - z2r, f + z2i, f - z2i
    c1, d1 = g + h, h - g
    return [a0 + a1, c0 + c1, b0 + b1, d0 + d1, a0 - a1, c0 - c1, b0 - b1, d0 - d1]


def _kernel(x_hbm, mem0_hbm, wq_hbm, wk_hbm, wv_hbm, wo_hbm, bx_hbm, wr_hbm, wi_hbm, fill_hbm, cst_hbm,
            out_hbm,
            x_v, xpre_v, xs_v, mem0_v, fill_v, lhs_v, wqkv, wo_v, pre, opost, outa_v,
            bx_v, w_v, wn_v, wt, cst, zs, vv, tn, outb_v,
            sem_w, sem_f, sem_in, sem_out):
    scale = E ** -0.5
    wus = [w.bitcast(U32) for w in (wq_hbm, wk_hbm, wv_hbm)]
    wo_u = wo_hbm.bitcast(U32)
    fus = [w.at[pl.ds(0, 512)].bitcast(U32) for w in (wr_hbm, wi_hbm)]

    def w_copies(j, t, sem):
        return [pltpu.make_async_copy(wus[t].at[:, :, j, :], wqkv.at[j, t], sem)]

    w0_cps = [w_copies(0, 0, sem_in.at[3]), w_copies(0, 1, sem_in.at[4]) + w_copies(0, 2, sem_in.at[4])]
    xpre_cp = pltpu.make_async_copy(x_hbm.at[:, pl.ds(0, 8), :], xpre_v, sem_in.at[0])

    def w_pair(j):
        return [cp for t in range(3) for cp in w_copies(j, t, sem_w.at[j])]

    a_cps = [pltpu.make_async_copy(wo_u.at[:, pl.ds(128 * n, 128)], wo_v.at[n], sem_in.at[1]) for n in range(8)]
    a_cps += [pltpu.make_async_copy(x_hbm.at[pl.ds(0, CH)], x_v.at[pl.ds(0, CH)], sem_in.at[1]),
              pltpu.make_async_copy(mem0_hbm, mem0_v, sem_in.at[1]),
              pltpu.make_async_copy(fill_hbm, fill_v, sem_in.at[1]),
              pltpu.make_async_copy(cst_hbm.at[pl.ds(0, C_MS)], cst.at[pl.ds(0, C_MS)], sem_in.at[1]),
              pltpu.make_async_copy(bx_hbm, bx_v, sem_in.at[1])]

    def f_cps(it):
        return [pltpu.make_async_copy(fus[t].at[:, pl.ds(pl.multiple_of(128 * (2 * it + h), 128), 128)],
                                      w_v.at[t, 2 * it + h], sem_f.at[it]) for t in range(2) for h in range(2)]

    b_cps = [pltpu.make_async_copy(x_hbm.at[pl.ds(CH, NSEG - CH)], x_v.at[pl.ds(CH, NSEG - CH)], sem_in.at[2]),
             pltpu.make_async_copy(cst_hbm.at[pl.ds(C_MS, C_NUM - C_MS)], cst.at[pl.ds(C_MS, C_NUM - C_MS)],
                                   sem_in.at[2])]
    b_cps += [pltpu.make_async_copy(w.at[pl.ds(512, 1)], wn_v.at[t], sem_in.at[2])
              for t, w in enumerate((wr_hbm, wi_hbm))]

    hb = DM // 32

    def retile(j, t, k):
        blk = pl.ds(k * hb, hb)
        a, b = wqkv[j, t, blk, pl.ds(0, 8, stride=2), :], wqkv[j, t, blk, pl.ds(1, 8, stride=2), :]
        wqkv[j, t, blk, 0:8, :] = (a & jnp.uint32(0xFFFF)) | (b << 16)
        wqkv[j, t, blk, 8:16, :] = (a >> 16) | (b & jnp.uint32(0xFFFF0000))

    def strassen_lhs():
        for g in range(NSEG // 4):
            xa = [xpre_v[4 * g + k].astype(F32) for k in range(4)]
            a1, a2 = jnp.concatenate([xa[0], xa[2]], axis=0), jnp.concatenate([xa[1], xa[3]], axis=0)
            a11, a12, a21, a22 = a1[:, :DM // 2], a1[:, DM // 2:], a2[:, :DM // 2], a2[:, DM // 2:]
            for n, v in enumerate((a11 + a22, a22, a21 + a22, a11 + a12, a11, a12 - a22, a21 - a11)):
                xs_v[n, 8 * g:8 * g + 8, :] = pltpu.bitcast(v.astype(BF), U32)

    def pre_step7(j, t):
        w = lambda k, p: wqkv[j, t, k * hb:(k + 1) * hb, 8 * p:8 * p + 8, :].reshape(DM // 4, E)
        add = lambda u, v: _pack2(_unpack2(u, 0) + _unpack2(v, 0), _unpack2(u, 1) + _unpack2(v, 1))
        sub = lambda u, v: _pack2(_unpack2(u, 0) - _unpack2(v, 0), _unpack2(u, 1) - _unpack2(v, 1))
        mm = lambda n, r: _bdot(_bf(xs_v[n]), _bf(r))
        retile(j, t, 0)
        m2 = mm(2, w(0, 0))
        c22 = mm(6, add(w(0, 0), w(0, 1))) - m2
        retile(j, t, 1)
        m4 = mm(1, sub(w(1, 0), w(0, 0)))
        c21 = m2 + m4
        m1 = mm(0, add(w(0, 0), w(1, 1)))
        c11, c22 = m1 + m4, c22 + m1
        m3 = mm(4, sub(w(0, 1), w(1, 1)))
        lower = _pack2(c21, c22 + m3).reshape(NSEG // 2, 8, E)
        c11 = c11 + mm(5, add(w(1, 0), w(1, 1)))
        m5 = mm(3, w(1, 1))
        upper = _pack2(c11 - m5, m3 + m5).reshape(NSEG // 2, 8, E)
        pre[j, t] = jnp.stack([upper, lower], axis=1).reshape(NSEG, 8, E)

    xpre_cp.start()
    for cp in w0_cps[0] + w0_cps[1] + [cp for j in range(1, NP) for cp in w_pair(j)]:
        cp.start()
    xpre_cp.wait()
    strassen_lhs()
    for cp in w0_cps[0]:
        cp.wait()
    pre_step7(0, 0)
    for cp in w0_cps[1]:
        cp.wait()
    pre_step7(0, 1)
    pre_step7(0, 2)
    for cp in w_pair(1):
        cp.wait()
    for cp in a_cps + f_cps(0):
        cp.start()
    for t in range(3):
        pre_step7(1, t)

    def pre_body(k, carry):
        for cp in w_pair(2 * k) + w_pair(2 * k + 1):
            cp.wait()
        for cp in f_cps(k):
            cp.start()
        for j in (2 * k, 2 * k + 1):
            for t in range(3):
                pre_step7(j, t)
        return carry

    lax.fori_loop(1, NP // 2, pre_body, 0)
    for cp in b_cps:
        cp.start()
    for cp in a_cps:
        cp.wait()

    lane = lax.broadcasted_iota(I32, (8, 128), 1)
    alt = jnp.where(lane % 2 == 0, 1.0, -1.0).astype(F32)
    lo_half = lane < 64
    ev_grp = (lane // 32) % 2 == 0

    def half_coef(q):
        sg = -1.0 if q < 3 else 1.0
        tc, ts = math.cos(2 * math.pi * q / 16), -math.sin(2 * math.pi * q / 16)
        f = lambda lo, hi: jnp.where(lo_half, lo, hi).astype(F32)
        return f(1.0, ts), f(0.0, sg * tc), f(0.0, tc), f(sg, -sg * ts)

    def b_rows(i, b):
        return 2 * b + i // 4, pl.ds(pl.multiple_of((i % 4) * 8, 8), 8)

    def flat(zs_):
        return [v for z in zs_ for v in z]

    def put(ref, idx, val, back):
        ref[idx] = val
        return ref[idx] if back else val

    def as_u32(rows):
        return pltpu.bitcast(jnp.concatenate(rows, axis=0).astype(BF), U32)

    def b_fwd(i):
        r0 = pl.multiple_of(i * 8, 8)
        for cp in f_cps(i):
            cp.wait()
        hc = [None] + [half_coef(q) for q in range(1, 4)]
        tacc = jnp.zeros((8, 128), F32)
        zl = []
        for _ in range(3):
            yield None
        for b0 in range(0, 32, 2):
            rows = []
            for b in (b0, b0 + 1):
                xb = bx_v[(*b_rows(i, b), slice(None))].astype(F32)
                z = _rfft8([xb[:, 128 * t:128 * t + 128] for t in range(8)])
                tacc = jnp.where(lane == b, jnp.sum(z[0] * alt, axis=1, keepdims=True), tacc)
                for q in range(1, 4):
                    c1, c2, c3, c4 = hc[q]
                    zr, zi = z[2 * q], z[2 * q + 1]
                    pp = c1 * zr + c2 * zi
                    qq = pltpu.roll(c3 * zr + c4 * zi, 64, 1)
                    z[2 * q], z[2 * q + 1] = pp + qq, pp - qq
                rows.append(z)
            zl.append([as_u32([rows[0][n], rows[1][n]]) for n in range(8)])
            yield zl[-1] + [tacc]
            yield None
            if b0 % 4 == 0:
                e, t, ty = 2 * i + b0 // 16, (b0 // 8) % 2, (b0 // 4) % 2
                u = jnp.concatenate([w_v[t, e, pl.ds(m + ty, 32, stride=8), :] for m in (0, 6, 4, 2)], axis=0)
                ut = pltpu.bitcast(pltpu.bitcast(u, F32).T, U32)
                yield [put(wt, (t, ty, pl.ds(8 * (v % 4) * WP + 4 * e + v // 4, 8, stride=WP), slice(None)),
                           ut[8 * v:8 * v + 8], OPT['put_wt']) for v in range(16)]
        tn[pl.ds(r0, 8), :] = tacc

        def mm(n):
            return _bdot(_bf(jnp.concatenate([z[n] for z in zl], axis=0)), _bf(cst[C_MD + n]))

        oo = [mm(n) for n in range(4)]
        yield MID
        oo += [mm(n) for n in range(4, 8)]
        for q in range(4):
            sel, sh = (ev_grp, 96) if q == 0 else (lo_half, 64)
            ys = []
            for b0 in range(4):
                xs = []
                for b in range(b0, 32, 4):
                    e_, o_ = oo[2 * q][8 * b:8 * b + 8], oo[2 * q + 1][8 * b:8 * b + 8]
                    xs.append((jnp.where(sel, e_, o_), pltpu.roll(jnp.where(sel, o_, e_), sh, 1)))
                ys.append([_twiddle(y, b0 * k1, 32, -1) for k1, y in enumerate(_cfft(xs, -1))])
                yield flat(ys[-1])
            for k1 in range(8):
                o = [_pack2(*y) for y in _cfft([ys[b0][k1] for b0 in range(4)], -1)]
                yield [put(zs, (k1 + 8 * k0, pl.ds(r0, 8), pl.ds(128 * q, 128)), o[k0], OPT['put_zs']) for k0 in range(4)]

    def b_mid(i):
        for n in range(4):
            dl = 4 * i + n
            for _ in range(6):
                yield None
            y = _bdot(_bf(cst[C_MS + dl]), _bf(zs[dl]))
            for _ in range(3):
                yield None
            w0 = pl.multiple_of(dl * WP, 8)
            rows = []
            for r in range(8):
                wq = []
                for t in range(2):
                    ta, tb = wt[t, 0, pl.ds(w0 + 8 * r, 8), :], wt[t, 1, pl.ds(w0 + 8 * r, 8), :]
                    wq.append([_unpack2(ta, 0), _unpack2(jnp.where(ev_grp, ta, tb), 1),
                               _unpack2(tb, 0), _unpack2(jnp.where(ev_grp, tb, ta), 1)])
                cols = []
                for q in range(4):
                    yr = y[8 * r:8 * r + 8, 128 * q:128 * q + 128]
                    yi = y[64 + 8 * r:72 + 8 * r, 128 * q:128 * q + 128]
                    wr, wi = wq[0][q], wq[1][q]
                    cols.append(_pack2(yr * wr - yi * wi, yr * wi + yi * wr))
                rows.append(jnp.concatenate(cols, axis=1))
                yield cols
            yield None
            vv[dl] = _bdot(_bf(cst[C_MS + 32 + dl]), _bf(jnp.concatenate(rows, axis=0)))
            for _ in range(6):
                yield None

    def b_nyq():
        c, s = pltpu.bitcast(cst[C_TW], F32), pltpu.bitcast(cst[C_TW + 1], F32)
        tb = tn[...].astype(BF)
        tr, ti = _bdot(tb, _bf(cst[C_MN])), _bdot(tb, _bf(cst[C_MN + 1]))
        y = _bdot(_bf(cst[C_MN + 2, 0:16, :]), _bf(_pack2(tr * c + ti * s, ti * c - tr * s)))
        row = lax.broadcasted_iota(I32, (16, 128), 0)
        wn = []
        for t in range(2):
            wrow = wn_v[t].astype(F32)
            acc = jnp.zeros((16, 128), F32)
            for e in range(16):
                acc = jnp.where(row == e, wrow[:, 128 * e:128 * e + 128], acc)
            wn.append(acc)
        yr, yi = y[0:16], y[16:32]
        v = _bdot(_bf(cst[C_MN + 3, :, 0:32]), _bf(_pack2(yr * wn[0] - yi * wn[1], yr * wn[1] + yi * wn[0])))
        vr, vi = v[0:64], v[64:128]
        tn[...] = (_bdot((vr * c - vi * s).astype(BF), _bf(cst[C_MN + 4]))
                   + _bdot((vr * s + vi * c).astype(BF), _bf(cst[C_MN + 5])))

    def b_inv(i):
        r0 = pl.multiple_of(i * 8, 8)
        ul, zz = [], []
        yield None
        for q in range(4):
            sel, sh = (ev_grp, 32) if q == 0 else (lo_half, 64)
            ys = []
            for b0 in range(4):
                xs = [(vv[dl, pl.ds(r0, 8), 128 * q:128 * q + 128], vv[dl, pl.ds(64 + r0, 8), 128 * q:128 * q + 128])
                      for dl in range(b0, 32, 4)]
                ys.append([_twiddle(y, b0 * k1, 32, +1) for k1, y in enumerate(_cfft(xs, +1))])
                yield flat(ys[-1])
            ie, io = [], []
            for k1 in range(8):
                es, os_ = [], []
                for ur, ui in _cfft([ys[b0][k1] for b0 in range(4)], +1):
                    tmp = pltpu.roll(ui, sh, 1)
                    es.append(jnp.where(sel, ur, tmp))
                    os_.append(jnp.where(sel, tmp, ur))
                ie += [as_u32(es[0:2]), as_u32(es[2:4])]
                io += [as_u32(os_[0:2]), as_u32(os_[2:4])]
                yield ie[-2:] + io[-2:]
            ul += [ie, io]
            if q == 2:
                zz += [_bdot(_bf(jnp.concatenate(ul[n], axis=0)), _bf(cst[C_MD + 8 + n])) for n in range(4)]
        yield MID
        zz += [_bdot(_bf(jnp.concatenate(ul[n], axis=0)), _bf(cst[C_MD + 8 + n])) for n in range(4, 8)]
        for _ in range(4):
            yield None
        hc = [None] + [half_coef(q) for q in range(1, 4)]
        tb = tn[pl.ds(r0, 8), :]
        for g in range(32):
            b = g // 4 + 8 * (g % 4)
            z = [zz[n][8 * g:8 * g + 8] for n in range(8)]
            z[0] = z[0] + jnp.sum(jnp.where(lane == b, tb, 0.0), axis=1, keepdims=True) * alt
            for q in range(1, 4):
                c1, c2, c3, c4 = hc[q]
                pp = z[2 * q] + z[2 * q + 1]
                qq = pltpu.roll(z[2 * q] - z[2 * q + 1], 64, 1)
                z[2 * q], z[2 * q + 1] = c1 * pp + c3 * qq, c2 * pp + c4 * qq
            y = _irfft8(z)
            outb_v[(*b_rows(i, b), slice(None))] = jnp.concatenate(y, axis=1).astype(BF)
            yield [outb_v[(*b_rows(i, b), pl.ds(256 * k, 128))].astype(F32) for k in range(4)] if OPT['put_out'] else y

    def tie(w, vals):
        if not vals:
            return w
        acc = None
        for v in vals:
            v = v if v.dtype == U32 else pltpu.bitcast(v, U32)
            acc = v if acc is None else acc | v
        zero = cst[C_MN, 56:64, :]
        return jnp.concatenate([w[0:8] | (acc & zero), w[8:]], axis=0)

    def post(c, n):
        op = opost[c % 2].reshape(CH * 8, H * E).astype(BF)
        r = _bdot(op, _bf(wo_v[n]))
        col = n * 128 if isinstance(n, int) else pl.multiple_of(n * 128, 128)
        outa_v[pl.ds(c * CH, CH), 0:8, pl.ds(col, 128)] = r.reshape(CH, 8, 128).astype(BF)

    def seg_step(i, u, mem, c, slot):
        s = c * CH + i
        xs = x_v[s]
        lhs_v[u] = as_u32([mem, xs[8:32].astype(F32)])
        fill = fill_v[...]
        late = []

        def proj(j, t):
            w0, w1 = [wqkv[j, t, :, 8 * p:8 * p + 8, :].reshape(DM // 2, E) for p in range(2)]
            w1 = tie(w1, late.pop(0) if late and (j % 2 == 1 or t == 2) else None)
            r0, r1 = _bdot(_bf(lhs_v[u]), _bf(tie(w0, slot()))), _bdot(_bf(lhs_v[u]), _bf(w1))
            pw = pre[j, t, s]
            if t == 0:
                return jnp.concatenate([r0, r1, _unpack2(pw, 0), _unpack2(pw, 1)], axis=0).astype(BF)
            return _bf(jnp.concatenate([_pack2(r0, r1), pw], axis=0))

        def qk(q, k):
            sc = lax.dot_general(q, k, (((1,), (1,)), ((), ())), preferred_element_type=F32) * scale
            sc = jnp.where(fill == 0.0, sc, fill)
            p = jnp.exp(sc - jnp.max(sc, axis=-1, keepdims=True))
            rl = pl.reciprocal(jnp.sum(p, axis=-1, keepdims=True), approx=True)
            return ((p * rl).astype(BF), None) if OPT['norm_first'] else (p.astype(BF), rl)

        ob, ps, vs = {}, {}, {}

        def pv(j):
            o = _bdot(ps[j][0], vs[j])
            if ps[j][1] is not None:
                o = o * ps[j][1]
            tv = [put(opost, (c % 2, i, slice(None), pl.ds(256 * j + 128 * p, 128)), o[64 + 8 * p:72 + 8 * p],
                      OPT['put_op']) for p in range(2)]
            if OPT['tie_ob']:
                ob[j] = [as_u32([o[0:32]]), as_u32([o[32:64]])]
                late.append((tv if OPT['put_op'] or not OPT['norm_first'] else [])
                            + [ob[j][p][8 * r:8 * r + 8] for p in range(2) for r in range(2)])
            else:
                ob[j] = [o[0:32], o[32:64]]

        def wo(g0, g1):
            og = jnp.concatenate([o for j in range(2 * g0, 2 * g1) for o in ob[j]], axis=1)
            og = _bf(og) if OPT['tie_ob'] else og.astype(BF)
            return jnp.concatenate([_bdot(og, _bf(wo_v[n, g0 * 256:g1 * 256, :])) for n in range(8)], axis=1)

        ng = NP // 2
        for g in range(ng):
            ja, jb = 2 * g, 2 * g + 1
            qa, ka, qb, kb = proj(ja, 0), proj(ja, 1), proj(jb, 0), proj(jb, 1)
            vs[ja], vs[jb] = proj(ja, 2), proj(jb, 2)
            ps[ja], ps[jb] = qk(qa, ka), qk(qb, kb)
            if g > 0:
                pv(ja - 2)
                pv(jb - 2)
        res = wo(0, 3)
        pv(NP - 2)
        pv(NP - 1)
        res = res + wo(3, ng - 1)
        res = res + wo(ng - 1, ng)
        outa_v[s, 8:32, :] = res[8:32].astype(BF)
        return res[0:8].astype(BF).astype(F32)

    def chunk_body(it, mem, *, c, side):
        gen = side(it) if side is not None else iter(())
        state = {'mid': False}

        def slot():
            if state['mid']:
                return None
            vals = next(gen, None)
            if vals is MID:
                state['mid'] = True
                return None
            return vals

        mem = seg_step(2 * it, 0, mem, c, slot)
        if c > 0:
            post(c - 1, it)
        if side in (b_fwd, b_inv):
            while not state['mid']:
                slot()
        state['mid'] = False
        mem = seg_step(2 * it + 1, 1, mem, c, slot)
        for _ in gen:
            pass
        return mem

    def out_a(c, rows, cols, sem):
        return pltpu.make_async_copy(outa_v.at[pl.ds(c * CH, CH), rows, cols],
                                     out_hbm.at[pl.ds(c * CH, CH), rows, cols], sem)

    nch = NSEG // CH
    out_cps = [out_a(c, pl.ds(0, SEG), pl.ds(0, DM), sem_out.at[c]) for c in range(nch - 1)]
    out_cps += [out_a(nch - 1, pl.ds(8, SEG - 8), pl.ds(0, DM), sem_out.at[3]),
                pltpu.make_async_copy(outb_v, out_hbm.at[:, :, pl.ds(DM, DM)], sem_out.at[4]),
                out_a(nch - 1, pl.ds(0, 8), pl.ds(0, 896), sem_out.at[5]),
                out_a(nch - 1, pl.ds(0, 8), pl.ds(896, 128), sem_out.at[6])]

    sides = [b_fwd, b_mid, b_inv, None]
    mem = mem0_v[...].astype(F32)
    for c in range(nch):
        mem = lax.fori_loop(0, NIT, functools.partial(chunk_body, c=c, side=sides[c]), mem)
        if c == 0:
            for cp in b_cps:
                cp.wait()
            b_nyq()
        else:
            out_cps[c - 1].start()
        if c == 2:
            out_cps[4].start()
    out_cps[3].start()
    for n in range(8):
        post(nch - 1, n)
        if n >= 6:
            out_cps[n - 1].start()
    for cp in out_cps:
        cp.wait()


def pallas_concat_heads__memory_aug_recurrent_mem_tr__spectral_gfnet__prompt_kernel(
    A_x, A_mem0, A_Wq, A_Wk, A_Wv, A_Wo, A_seg_len, B_x, B_w_r, B_w_i,
):
    assert A_x.shape == (1, S, DM) and A_Wq.shape == (DM, H, E) and A_mem0.shape == (1, M, DM)
    assert B_x.shape == (1, S, DM) and (not isinstance(A_seg_len, int) or A_seg_len == SEG)
    hbm = pl.BlockSpec(memory_space=pltpu.HBM)
    wr = lambda w: w.reshape(DM // 16, 16, H, E)
    out = pl.pallas_call(
        _kernel,
        out_shape=jax.ShapeDtypeStruct((NSEG, SEG, 2 * DM), BF),
        in_specs=[hbm] * 11,
        out_specs=hbm,
        scratch_shapes=[
            pltpu.VMEM((NSEG, SEG, DM), BF),
            pltpu.VMEM((NSEG, 8, DM), BF),
            pltpu.VMEM((7, NSEG * 2, DM // 2), U32),
            pltpu.VMEM((M, DM), BF),
            pltpu.VMEM((80, 80), F32),
            pltpu.VMEM((2, SEG // 2, DM), U32),
            pltpu.VMEM((NP, 3, DM // 16, 16, E), U32),
            pltpu.VMEM((8, H * E // 2, 128), U32),
            pltpu.VMEM((NP, 3, NSEG, 8, E), U32),
            pltpu.VMEM((2, CH, 8, H * E), F32),
            pltpu.VMEM((NSEG, SEG, DM), BF),
            pltpu.VMEM((NSEG, SEG, DM), BF),
            pltpu.VMEM((2, 16, 256, 128), U32),
            pltpu.VMEM((2, 1, S), BF),
            pltpu.VMEM((2, 2, 32 * WP, 128), U32),
            pltpu.VMEM((C_NUM, 64, 128), U32),
            pltpu.VMEM((32, 64, 512), U32),
            pltpu.VMEM((32, 128, 512), F32),
            pltpu.VMEM((64, 128), F32),
            pltpu.VMEM((NSEG, SEG, DM), BF),
            pltpu.SemaphoreType.DMA((NP,)),
            pltpu.SemaphoreType.DMA((NIT,)),
            pltpu.SemaphoreType.DMA((6,)),
            pltpu.SemaphoreType.DMA((7,)),
        ],
        compiler_params=pltpu.CompilerParams(vmem_limit_bytes=112 * 1024 * 1024,
                                             disable_bounds_checks=True),
    )(A_x.reshape(NSEG, SEG, DM), A_mem0.reshape(M, DM), wr(A_Wq), wr(A_Wk), wr(A_Wv),
      A_Wo.reshape(H * E, DM), B_x.reshape(NSEG, SEG, DM), B_w_r.T, B_w_i.T, _mask_fill(), _fft_consts())
    return out.reshape(1, S, 2 * DM)
```

```python
import functools
import math

import jax
import jax.numpy as jnp
import numpy as np
from jax import lax
import jax.experimental.pallas as pl
import jax.experimental.pallas.tpu as pltpu

BF, F32, U32, I32 = jnp.bfloat16, jnp.float32, jnp.uint32, jnp.int32

S, DM, H, E, M, SEG = 2048, 1024, 32, 128, 8, 32
NSEG = S // SEG
NP = H // 2
CH = 16
NIT = CH // 2
R2 = math.sqrt(0.5)
MID = 'mid'
OPT = dict()


def _to_u32(m):
    u = np.ascontiguousarray(m, dtype=np.float32).view(np.uint32)
    h = ((u + 0x7FFF + ((u >> 16) & 1)) >> 16).astype(np.uint32)
    return h[..., 0::2, :] | (h[..., 1::2, :] << 16)


def _mask_fill():
    r = np.arange(80)
    pos_of = lambda rr: np.where(rr < M, rr, np.where(rr < SEG, rr + M, rr - SEG + M))
    qhead = np.where(r < 64, r // 32, (r - 64) // 8)
    qpos = pos_of(np.where(r < 64, r % 32, SEG + (r - 64) % 8))
    khead, kpos = r % 2, pos_of(r // 2)
    vis = (qpos[:, None] < M) | (qpos[:, None] >= kpos[None, :])
    same = qhead[:, None] == khead[None, :]
    return np.where(same, np.where(vis, 0.0, -1e9), -np.inf).astype(np.float32)


RES = ((0, 12, 8, 4), (1, 15, 9, 7), (2, 14, 10, 6), (3, 13, 11, 5))
WP = 72
C_MD, C_MN, C_TW, C_MS, C_NUM = 0, 16, 22, 24, 88


@functools.lru_cache(maxsize=None)
def _fft_consts():
    md = np.zeros((16, 128, 128))
    for q in range(4):
        if q == 0:
            lay = [[(0, 0), (0, 1), (2, 0), (2, 1)], [(3, 1), (1, 0), (1, 1), (3, 0)]]
        else:
            lay = [[(0, 0), (1, 0), (0, 1), (1, 1)], [(2, 1), (3, 1), (2, 0), (3, 0)]]
        for h in range(2):
            ms_, ws_ = [], []
            for g, part in lay[h]:
                k = 16 * np.arange(32) + RES[q][g]
                th = 2 * np.pi * np.outer(np.arange(128 if q == 0 else 64), k) / DM
                c, s = np.cos(th), np.sin(th)
                if q == 0:
                    ms_.append(-s if part else c)
                else:
                    sg = (1.0 if RES[q][g] % 8 == q else -1.0) * (1.0 - 2.0 * h)
                    ms_.append(np.concatenate([-s, sg * c] if part else [c, sg * s]))
                ws_.append(np.where(k == 0, 1.0, 2.0) / DM)
            m = np.concatenate(ms_, axis=1)
            md[2 * q + h] = m
            md[8 + 2 * q + h] = (m * np.concatenate(ws_)[None, :]).T
    a, l = np.arange(64), np.arange(128)
    ms = np.zeros((64, 128, 128))
    for dl in range(32):
        th = 2 * np.pi * np.outer(32 * a + dl, a) / S
        c, s = np.cos(th), np.sin(th)
        ms[dl, :64, 0::2], ms[dl, :64, 1::2] = c, s
        ms[dl, 64:, 0::2], ms[dl, 64:, 1::2] = -s, c
        ms[32 + dl, :64, 0::2], ms[32 + dl, :64, 1::2] = c.T / S, -s.T / S
        ms[32 + dl, 64:, 0::2], ms[32 + dl, 64:, 1::2] = s.T / S, c.T / S
    mn = np.zeros((6, 128, 128))
    th = 2 * np.pi * np.outer(np.arange(32), l) / 32
    mn[0, :32], mn[1, :32] = np.cos(th), -np.sin(th)
    mn[4, :, :32], mn[5, :, :32] = np.cos(th).T / DM, -np.sin(th).T / DM
    th = 2 * np.pi * np.outer(np.arange(16), a) / 16
    c, s = np.cos(th), np.sin(th)
    mn[2, :16, 0::2], mn[2, :16, 1::2], mn[2, 16:32, 0::2], mn[2, 16:32, 1::2] = c, s, -s, c
    mn[3, :64, 0:32:2], mn[3, :64, 1:32:2] = c.T / S, -s.T / S
    mn[3, 64:, 0:32:2], mn[3, 64:, 1:32:2] = s.T / S, c.T / S
    th = 2 * np.pi * np.outer(a, l) / S
    tw = np.stack([np.cos(th), np.sin(th)]).astype(np.float32).view(np.uint32)
    return np.concatenate([_to_u32(md), _to_u32(mn), tw, _to_u32(ms)], axis=0)


def _bdot(a, b):
    return jnp.dot(a, b, preferred_element_type=F32)


def _bf(u):
    return pltpu.bitcast(u, BF)


def _pack2(r, i):
    return pltpu.bitcast(pltpu.pack_elementwise([r, i], packed_dtype=BF), U32)


def _unpack2(u, p):
    if p == 0:
        return pltpu.bitcast(u << 16, F32)
    return pltpu.bitcast(u & jnp.uint32(0xFFFF0000), F32)


def _strassen_left(n, a):
    return (lambda: a(1, 0) + a(1, 1), lambda: a(1, 0) - a(0, 0), lambda: a(1, 1), lambda: a(0, 0) + a(1, 1),
            lambda: a(0, 0), lambda: a(0, 1) - a(1, 1), lambda: a(0, 0) + a(0, 1))[n]()


def _strassen(left, w, done, ready=lambda k: None):
    add = lambda u, v: _pack2(_unpack2(u, 0) + _unpack2(v, 0), _unpack2(u, 1) + _unpack2(v, 1))
    sub = lambda u, v: _pack2(_unpack2(u, 0) - _unpack2(v, 0), _unpack2(u, 1) - _unpack2(v, 1))
    mm = lambda n, r: _bdot(left(n), _bf(r))
    ready(0)
    m2 = mm(0, w(0, 0))
    c22 = mm(1, add(w(0, 0), w(0, 1))) - m2
    ready(1)
    m4 = mm(2, sub(w(1, 0), w(0, 0)))
    c21 = m2 + m4
    m1 = mm(3, add(w(0, 0), w(1, 1)))
    c11, c22 = m1 + m4, c22 + m1
    m3 = mm(4, sub(w(0, 1), w(1, 1)))
    done(1, c21, c22 + m3)
    c11 = c11 + mm(5, add(w(1, 0), w(1, 1)))
    m5 = mm(6, w(1, 1))
    done(0, c11 - m5, m3 + m5)


def _twiddle(z, k, n, sign):
    r, i = z
    if k == 0:
        return r, i
    if 4 * k == n:
        return (-i, r) if sign > 0 else (i, -r)
    c, s = math.cos(2 * math.pi * k / n), sign * math.sin(2 * math.pi * k / n)
    if 8 * k == n or 8 * k == 3 * n:
        if c * s > 0:
            return (r - i) * c, (r + i) * c
        return (r + i) * c, (i - r) * c
    return r * c - i * s, r * s + i * c


def _cfft(xs, sign):
    n = len(xs)
    if n == 1:
        return xs
    ev, od = _cfft(xs[0::2], sign), _cfft(xs[1::2], sign)
    out = [None] * n
    for k in range(n // 2):
        er, ei = ev[k]
        if 4 * k == n:
            orr, oi = od[k]
            lo, hi = (er - oi, ei + orr), (er + oi, ei - orr)
            out[k], out[k + n // 2] = (lo, hi) if sign > 0 else (hi, lo)
        else:
            tr, ti = _twiddle(od[k], k, n, sign)
            out[k], out[k + n // 2] = (er + tr, ei + ti), (er - tr, ei - ti)
    return out


def _rfft8(x):
    a0, a1, b0, b1 = x[0] + x[4], x[0] - x[4], x[2] + x[6], x[2] - x[6]
    c0, c1, d0, d1 = x[1] + x[5], x[1] - x[5], x[3] + x[7], x[3] - x[7]
    e, f = a0 + b0, c0 + d0
    g, h = (c1 - d1) * R2, (c1 + d1) * R2
    return [e + f, e - f, a1 + g, b1 + h, a0 - b0, c0 - d0, a1 - g, b1 - h]


def _irfft8(z):
    z0, z4, z1r, z1i, z2r, z2i, z3r, z3i = z
    e, f = z0 + z4, z0 - z4
    a1, g = z1r + z3r, (z1r - z3r) * R2
    b1, h = z1i + z3i, (z1i - z3i) * R2
    a0, b0, c0, d0 = e + z2r, e - z2r, f + z2i, f - z2i
    c1, d1 = g + h, h - g
    return [a0 + a1, c0 + c1, b0 + b1, d0 + d1, a0 - a1, c0 - c1, b0 - b1, d0 - d1]


def _kernel(x_hbm, mem0_hbm, wq_hbm, wk_hbm, wv_hbm, wo_hbm, bx_hbm, wr_hbm, wi_hbm, fill_hbm, cst_hbm,
            out_hbm,
            x_v, xpre_v, xs_v, mem0_v, fill_v, lhs_v, wqkv, wo_v, pre, opost, outa_v,
            bx_v, w_v, wn_v, wt, cst, zs, vv, tn, outb_v,
            sem_w, sem_f, sem_in, sem_out):
    scale = E ** -0.5
    wus = [w.bitcast(U32) for w in (wq_hbm, wk_hbm, wv_hbm)]
    wo_u = wo_hbm.bitcast(U32)
    fus = [w.at[pl.ds(0, 512)].bitcast(U32) for w in (wr_hbm, wi_hbm)]

    def w_copies(j, t, sem):
        return [pltpu.make_async_copy(wus[t].at[:, :, j, :], wqkv.at[j, t], sem)]

    w0_cps = [w_copies(0, 0, sem_in.at[3]), w_copies(0, 1, sem_in.at[4]) + w_copies(0, 2, sem_in.at[4])]
    xpre_cp = pltpu.make_async_copy(x_hbm.at[:, pl.ds(0, 8), :], xpre_v, sem_in.at[0])

    def w_pair(j):
        return [cp for t in range(3) for cp in w_copies(j, t, sem_w.at[j])]

    a_cps = [pltpu.make_async_copy(wo_u.at[:, pl.ds(128 * n, 128)], wo_v.at[n], sem_in.at[1]) for n in range(8)]
    a_cps += [pltpu.make_async_copy(x_hbm.at[pl.ds(0, CH)], x_v.at[pl.ds(0, CH)], sem_in.at[1]),
              pltpu.make_async_copy(mem0_hbm, mem0_v, sem_in.at[1]),
              pltpu.make_async_copy(fill_hbm, fill_v, sem_in.at[1]),
              pltpu.make_async_copy(cst_hbm.at[pl.ds(0, C_MS)], cst.at[pl.ds(0, C_MS)], sem_in.at[1]),
              pltpu.make_async_copy(bx_hbm, bx_v, sem_in.at[1])]

    def f_cps(it):
        return [pltpu.make_async_copy(fus[t].at[:, pl.ds(pl.multiple_of(128 * (2 * it + h), 128), 128)],
                                      w_v.at[t, 2 * it + h], sem_f.at[it]) for t in range(2) for h in range(2)]

    b_cps = [pltpu.make_async_copy(x_hbm.at[pl.ds(CH, NSEG - CH)], x_v.at[pl.ds(CH, NSEG - CH)], sem_in.at[2]),
             pltpu.make_async_copy(cst_hbm.at[pl.ds(C_MS, C_NUM - C_MS)], cst.at[pl.ds(C_MS, C_NUM - C_MS)],
                                   sem_in.at[2])]
    b_cps += [pltpu.make_async_copy(w.at[pl.ds(512, 1)], wn_v.at[t], sem_in.at[2])
              for t, w in enumerate((wr_hbm, wi_hbm))]

    hb = DM // 32

    def retile(j, t, k):
        blk = pl.ds(k * hb, hb)
        a, b = wqkv[j, t, blk, pl.ds(0, 8, stride=2), :], wqkv[j, t, blk, pl.ds(1, 8, stride=2), :]
        wqkv[j, t, blk, 0:8, :] = (a & jnp.uint32(0xFFFF)) | (b << 16)
        wqkv[j, t, blk, 8:16, :] = (a >> 16) | (b & jnp.uint32(0xFFFF0000))

    def strassen_lhs():
        for g in range(NSEG // 4):
            xa = [xpre_v[4 * g + k].astype(F32) for k in range(4)]
            a1, a2 = jnp.concatenate([xa[0], xa[2]], axis=0), jnp.concatenate([xa[1], xa[3]], axis=0)
            a11, a12, a21, a22 = a1[:, :DM // 2], a1[:, DM // 2:], a2[:, :DM // 2], a2[:, DM // 2:]
            for n in range(7):
                v = _strassen_left(n, lambda r, k: ((a11, a12), (a21, a22))[r][k])
                xs_v[n, 8 * g:8 * g + 8, :] = pltpu.bitcast(v.astype(BF), U32)

    def pre_step7(j, t):
        w = lambda k, p: wqkv[j, t, k * hb:(k + 1) * hb, 8 * p:8 * p + 8, :].reshape(DM // 4, E)
        half = {}

        def done(h, c1, c2):
            half[h] = _pack2(c1, c2).reshape(NSEG // 2, 8, E)

        _strassen(lambda n: _bf(xs_v[n]), w, done, functools.partial(retile, j, t))
        pre[j, t] = jnp.stack([half[0], half[1]], axis=1).reshape(NSEG, 8, E)

    xpre_cp.start()
    for cp in w0_cps[0] + w0_cps[1] + [cp for j in range(1, NP) for cp in w_pair(j)]:
        cp.start()
    xpre_cp.wait()
    strassen_lhs()
    for cp in w0_cps[0]:
        cp.wait()
    pre_step7(0, 0)
    for cp in w0_cps[1]:
        cp.wait()
    pre_step7(0, 1)
    pre_step7(0, 2)
    for cp in w_pair(1):
        cp.wait()
    for cp in a_cps + f_cps(0):
        cp.start()
    for t in range(3):
        pre_step7(1, t)

    def pre_body(k, carry):
        for cp in w_pair(2 * k) + w_pair(2 * k + 1):
            cp.wait()
        for cp in f_cps(k):
            cp.start()
        for j in (2 * k, 2 * k + 1):
            for t in range(3):
                pre_step7(j, t)
        return carry

    lax.fori_loop(1, NP // 2, pre_body, 0)
    for cp in b_cps:
        cp.start()
    for cp in a_cps:
        cp.wait()

    lane = lax.broadcasted_iota(I32, (8, 128), 1)
    alt = jnp.where(lane % 2 == 0, 1.0, -1.0).astype(F32)
    lo_half = lane < 64
    ev_grp = (lane // 32) % 2 == 0

    def half_coef(q):
        sg = -1.0 if q < 3 else 1.0
        tc, ts = math.cos(2 * math.pi * q / 16), -math.sin(2 * math.pi * q / 16)
        f = lambda lo, hi: jnp.where(lo_half, lo, hi).astype(F32)
        return f(1.0, ts), f(0.0, sg * tc), f(0.0, tc), f(sg, -sg * ts)

    def b_rows(i, b):
        return b, i // 4, pl.ds(pl.multiple_of((i % 4) * 8, 8), 8)

    def flat(zs_):
        return [v for z in zs_ for v in z]

    def as_u32(rows):
        return pltpu.bitcast(jnp.concatenate(rows, axis=0).astype(BF), U32)

    def b_fwd(i):
        r0 = pl.multiple_of(i * 8, 8)
        for cp in f_cps(i):
            cp.wait()
        hc = [None] + [half_coef(q) for q in range(1, 4)]
        tacc = jnp.zeros((8, 128), F32)
        zl = []
        for _ in range(3):
            yield None
        for b0 in range(0, 32, 2):
            rows = []
            for b in (b0, b0 + 1):
                xb = bx_v[(*b_rows(i, b), slice(None))].astype(F32)
                z = _rfft8([xb[:, 128 * t:128 * t + 128] for t in range(8)])
                tacc = jnp.where(lane == b, jnp.sum(z[0] * alt, axis=1, keepdims=True), tacc)
                for q in range(1, 4):
                    c1, c2, c3, c4 = hc[q]
                    zr, zi = z[2 * q], z[2 * q + 1]
                    pp = c1 * zr + c2 * zi
                    qq = pltpu.roll(c3 * zr + c4 * zi, 64, 1)
                    z[2 * q], z[2 * q + 1] = pp + qq, pp - qq
                rows.append(z)
            zl.append([as_u32([rows[0][n], rows[1][n]]) for n in range(8)])
            yield zl[-1] + [tacc]
            yield None
            if b0 % 4 == 0:
                e, t, ty = 2 * i + b0 // 16, (b0 // 8) % 2, (b0 // 4) % 2
                u = jnp.concatenate([w_v[t, e, pl.ds(m + ty, 32, stride=8), :] for m in (0, 6, 4, 2)], axis=0)
                ut = pltpu.bitcast(pltpu.bitcast(u, F32).T, U32)
                for v in range(16):
                    wt[t, ty, pl.ds(8 * (v % 4) * WP + 4 * e + v // 4, 8, stride=WP), :] = ut[8 * v:8 * v + 8]
                yield [ut[8 * v:8 * v + 8] for v in range(16)]
        tn[pl.ds(r0, 8), :] = tacc

        def mm(n):
            return _bdot(_bf(jnp.concatenate([z[n] for z in zl], axis=0)), _bf(cst[C_MD + n]))

        oo = [mm(n) for n in range(4)]
        yield MID
        oo += [mm(n) for n in range(4, 8)]
        for q in range(4):
            sel, sh = (ev_grp, 96) if q == 0 else (lo_half, 64)
            ys = []
            for b0 in range(4):
                xs = []
                for b in range(b0, 32, 4):
                    e_, o_ = oo[2 * q][8 * b:8 * b + 8], oo[2 * q + 1][8 * b:8 * b + 8]
                    xs.append((jnp.where(sel, e_, o_), pltpu.roll(jnp.where(sel, o_, e_), sh, 1)))
                ys.append([_twiddle(y, b0 * k1, 32, -1) for k1, y in enumerate(_cfft(xs, -1))])
                yield flat(ys[-1])
            for k1 in range(8):
                o = [_pack2(*y) for y in _cfft([ys[b0][k1] for b0 in range(4)], -1)]
                for k0 in range(4):
                    zs[k1 + 8 * k0, pl.ds(r0, 8), 128 * q:128 * q + 128] = o[k0]
                yield o

    def b_mid(i):
        for n in range(2):
            dl = 2 * i + n
            for _ in range(6 * (1 - n)):
                yield None
            y = _bdot(_bf(cst[C_MS + dl]), _bf(zs[dl]))
            for _ in range(4):
                yield None
            w0 = pl.multiple_of(dl * WP, 8)
            rows = []
            for r in range(8):
                wq = []
                for t in range(2):
                    ta, tb = wt[t, 0, pl.ds(w0 + 8 * r, 8), :], wt[t, 1, pl.ds(w0 + 8 * r, 8), :]
                    wq.append([_unpack2(ta, 0), _unpack2(jnp.where(ev_grp, ta, tb), 1),
                               _unpack2(tb, 0), _unpack2(jnp.where(ev_grp, tb, ta), 1)])
                cols = []
                for q in range(4):
                    yr = y[8 * r:8 * r + 8, 128 * q:128 * q + 128]
                    yi = y[64 + 8 * r:72 + 8 * r, 128 * q:128 * q + 128]
                    wr, wi = wq[0][q], wq[1][q]
                    cols.append(_pack2(yr * wr - yi * wi, yr * wi + yi * wr))
                rows.append(jnp.concatenate(cols, axis=1))
                yield cols
                yield None
            yield (MID if n == 0 else None)
            vv[dl] = _bdot(_bf(cst[C_MS + 32 + dl]), _bf(jnp.concatenate(rows, axis=0)))

    def b_nyq():
        c, s = pltpu.bitcast(cst[C_TW], F32), pltpu.bitcast(cst[C_TW + 1], F32)
        tb = tn[...].astype(BF)
        tr, ti = _bdot(tb, _bf(cst[C_MN])), _bdot(tb, _bf(cst[C_MN + 1]))
        y = _bdot(_bf(cst[C_MN + 2, 0:16, :]), _bf(_pack2(tr * c + ti * s, ti * c - tr * s)))
        row = lax.broadcasted_iota(I32, (16, 128), 0)
        wn = []
        for t in range(2):
            wrow = wn_v[t].astype(F32)
            acc = jnp.zeros((16, 128), F32)
            for e in range(16):
                acc = jnp.where(row == e, wrow[:, 128 * e:128 * e + 128], acc)
            wn.append(acc)
        yr, yi = y[0:16], y[16:32]
        v = _bdot(_bf(cst[C_MN + 3, :, 0:32]), _bf(_pack2(yr * wn[0] - yi * wn[1], yr * wn[1] + yi * wn[0])))
        vr, vi = v[0:64], v[64:128]
        tn[...] = (_bdot((vr * c - vi * s).astype(BF), _bf(cst[C_MN + 4]))
                   + _bdot((vr * s + vi * c).astype(BF), _bf(cst[C_MN + 5])))

    def b_inv(i):
        r0 = pl.multiple_of(i * 8, 8)
        ul, zz = [], []
        yield None
        for q in range(4):
            sel, sh = (ev_grp, 32) if q == 0 else (lo_half, 64)
            ys = []
            for b0 in range(4):
                xs = [(vv[dl, pl.ds(r0, 8), 128 * q:128 * q + 128], vv[dl, pl.ds(64 + r0, 8), 128 * q:128 * q + 128])
                      for dl in range(b0, 32, 4)]
                ys.append([_twiddle(y, b0 * k1, 32, +1) for k1, y in enumerate(_cfft(xs, +1))])
                yield flat(ys[-1])
            ie, io = [], []
            for k1 in range(8):
                es, os_ = [], []
                for ur, ui in _cfft([ys[b0][k1] for b0 in range(4)], +1):
                    tmp = pltpu.roll(ui, sh, 1)
                    es.append(jnp.where(sel, ur, tmp))
                    os_.append(jnp.where(sel, tmp, ur))
                ie += [as_u32(es[0:2]), as_u32(es[2:4])]
                io += [as_u32(os_[0:2]), as_u32(os_[2:4])]
                yield ie[-2:] + io[-2:]
            ul += [ie, io]
            if q == 2:
                zz += [_bdot(_bf(jnp.concatenate(ul[n], axis=0)), _bf(cst[C_MD + 8 + n])) for n in range(4)]
        yield MID
        zz += [_bdot(_bf(jnp.concatenate(ul[n], axis=0)), _bf(cst[C_MD + 8 + n])) for n in range(4, 8)]
        for _ in range(4):
            yield None
        hc = [None] + [half_coef(q) for q in range(1, 4)]
        tb = tn[pl.ds(r0, 8), :]
        for g in range(32):
            b = g // 4 + 8 * (g % 4)
            z = [zz[n][8 * g:8 * g + 8] for n in range(8)]
            z[0] = z[0] + jnp.sum(jnp.where(lane == b, tb, 0.0), axis=1, keepdims=True) * alt
            for q in range(1, 4):
                c1, c2, c3, c4 = hc[q]
                pp = z[2 * q] + z[2 * q + 1]
                qq = pltpu.roll(z[2 * q] - z[2 * q + 1], 64, 1)
                z[2 * q], z[2 * q + 1] = c1 * pp + c3 * qq, c2 * pp + c4 * qq
            y = _irfft8(z)
            outb_v[(*b_rows(i, b), slice(None))] = jnp.concatenate(y, axis=1).astype(BF)
            yield y

    def tie(w, vals):
        if not vals:
            return w
        acc = None
        for v in vals:
            v = v if v.dtype == U32 else pltpu.bitcast(v, U32)
            acc = v if acc is None else acc | v
        zero = cst[C_MN, 56:64, :]
        return jnp.concatenate([w[0:8] | (acc & zero), w[8:]], axis=0)

    def seg_step(it, u, mem, slot):
        s = 2 * it + u
        xs = x_v[s]
        lhs_v[u] = as_u32([mem, xs[8:32].astype(F32)])
        fill = fill_v[...]

        def proj(j, t):
            w0, w1 = [wqkv[j, t, :, 8 * p:8 * p + 8, :].reshape(DM // 2, E) for p in range(2)]
            r0, r1 = _bdot(_bf(lhs_v[u]), _bf(tie(w0, slot()))), _bdot(_bf(lhs_v[u]), _bf(w1))
            pw = pre[j, t, s]
            if t == 0:
                return jnp.concatenate([r0, r1, _unpack2(pw, 0), _unpack2(pw, 1)], axis=0).astype(BF)
            return _bf(jnp.concatenate([_pack2(r0, r1), pw], axis=0))

        def qk(q, k):
            sc = lax.dot_general(q, k, (((1,), (1,)), ((), ())), preferred_element_type=F32) * scale
            sc = jnp.where(fill == 0.0, sc, fill)
            p = jnp.exp(sc - jnp.max(sc, axis=-1, keepdims=True))
            return (p * pl.reciprocal(jnp.sum(p, axis=-1, keepdims=True), approx=True)).astype(BF)

        ob, ps, vs = {}, {}, {}

        def pv(j):
            o = _bdot(ps[j], vs[j])
            opost[it, u, :, pl.ds(256 * j, 128)] = o[64:72]
            opost[it, u, :, pl.ds(256 * j + 128, 128)] = o[72:80]
            ob[j] = [o[0:32], o[32:64]]

        def wo(g0, g1):
            og = jnp.concatenate([o for j in range(2 * g0, 2 * g1) for o in ob[j]], axis=1).astype(BF)
            return jnp.concatenate([_bdot(og, _bf(wo_v[n, g0 * 256:g1 * 256, :])) for n in range(8)], axis=1)

        ng = NP // 2
        for g in range(ng):
            ja, jb = 2 * g, 2 * g + 1
            qa, ka, qb, kb = proj(ja, 0), proj(ja, 1), proj(jb, 0), proj(jb, 1)
            vs[ja], vs[jb] = proj(ja, 2), proj(jb, 2)
            ps[ja], ps[jb] = qk(qa, ka), qk(qb, kb)
            if g > 0:
                pv(ja - 2)
                pv(jb - 2)
        res = wo(0, 3)
        pv(NP - 2)
        pv(NP - 1)
        res = res + wo(3, ng - 1)
        res = res + wo(ng - 1, ng)
        outa_v[it, u, 8:32, :] = res[8:32].astype(BF)
        return res[0:8].astype(BF).astype(F32)

    def loop_body(it, mem, *, it0, side):
        gen = side(it - it0)
        state = {'mid': False}

        def slot():
            if state['mid']:
                return None
            vals = next(gen, None)
            if vals is MID:
                state['mid'] = True
                return None
            return vals

        mem = seg_step(it, 0, mem, slot)
        while not state['mid']:
            slot()
        state['mid'] = False
        mem = seg_step(it, 1, mem, slot)
        for _ in gen:
            pass
        return mem

    out_cps = []

    def out_a(*idx):
        cp = pltpu.make_async_copy(outa_v.at[idx], out_hbm.at[idx], sem_out.at[len(out_cps)])
        out_cps.append(cp)
        cp.start()

    mem = mem0_v[...].astype(F32)
    for it0, it1, side in ((0, NIT, b_fwd), (NIT, 3 * NIT, b_mid), (3 * NIT, 4 * NIT, b_inv)):
        mem = lax.fori_loop(it0, it1, functools.partial(loop_body, it0=it0, side=side), mem)
        out_a(pl.ds(it0, it1 - it0), slice(None), pl.ds(8, SEG - 8), pl.ds(0, DM))
        if it0 == 0:
            for cp in b_cps:
                cp.wait()
            b_nyq()
    out_cps.append(pltpu.make_async_copy(outb_v, out_hbm.at[:, :, :, pl.ds(DM, DM)], sem_out.at[len(out_cps)]))
    out_cps[-1].start()

    hk = H * E // 2

    @functools.lru_cache(maxsize=None)
    def post_left(n):
        sums = [_strassen_left(n, lambda r, k: opost[g, r, :, k * hk:(k + 1) * hk]) for g in range(NSEG // 2)]
        return _bf(jnp.concatenate([_pack2(sums[g], sums[g + 1]) for g in range(0, NSEG // 2, 2)], axis=0))

    for n in range(4):
        def done(r, *cs):
            for p, cc in enumerate(cs):
                u = pltpu.bitcast(cc.astype(BF), U32).reshape(NSEG // 4, 8, 128)
                y = jnp.stack([_unpack2(u, 0), _unpack2(u, 1)], axis=1).reshape(NSEG // 2, 8, 128)
                idx = (slice(None), r, pl.ds(0, 8), pl.ds(128 * (n + 4 * p), 128))
                outa_v[idx] = y.astype(BF)
                out_a(*idx)

        _strassen(post_left, lambda k, p: wo_v[n + 4 * p, k * hk // 2:(k + 1) * hk // 2, :], done)
    for cp in out_cps:
        cp.wait()


def pallas_concat_heads__memory_aug_recurrent_mem_tr__spectral_gfnet__prompt_kernel(
    A_x, A_mem0, A_Wq, A_Wk, A_Wv, A_Wo, A_seg_len, B_x, B_w_r, B_w_i,
):
    assert A_x.shape == (1, S, DM) and A_Wq.shape == (DM, H, E) and A_mem0.shape == (1, M, DM)
    assert B_x.shape == (1, S, DM) and (not isinstance(A_seg_len, int) or A_seg_len == SEG)
    hbm = pl.BlockSpec(memory_space=pltpu.HBM)
    wr = lambda w: w.reshape(DM // 16, 16, H, E)
    out = pl.pallas_call(
        _kernel,
        out_shape=jax.ShapeDtypeStruct((NSEG // 2, 2, SEG, 2 * DM), BF),
        in_specs=[hbm] * 11,
        out_specs=hbm,
        scratch_shapes=[
            pltpu.VMEM((NSEG, SEG, DM), BF),
            pltpu.VMEM((NSEG, 8, DM), BF),
            pltpu.VMEM((7, NSEG * 2, DM // 2), U32),
            pltpu.VMEM((M, DM), BF),
            pltpu.VMEM((80, 80), F32),
            pltpu.VMEM((2, SEG // 2, DM), U32),
            pltpu.VMEM((NP, 3, DM // 16, 16, E), U32),
            pltpu.VMEM((8, H * E // 2, 128), U32),
            pltpu.VMEM((NP, 3, NSEG, 8, E), U32),
            pltpu.VMEM((NSEG // 2, 2, 8, H * E), F32),
            pltpu.VMEM((NSEG // 2, 2, SEG, DM), BF),
            pltpu.VMEM((NSEG // 2, 2, SEG, DM), BF),
            pltpu.VMEM((2, 16, 256, 128), U32),
            pltpu.VMEM((2, 1, S), BF),
            pltpu.VMEM((2, 2, 32 * WP, 128), U32),
            pltpu.VMEM((C_NUM, 64, 128), U32),
            pltpu.VMEM((32, 64, 512), U32),
            pltpu.VMEM((32, 128, 512), F32),
            pltpu.VMEM((64, 128), F32),
            pltpu.VMEM((NSEG // 2, 2, SEG, DM), BF),
            pltpu.SemaphoreType.DMA((NP,)),
            pltpu.SemaphoreType.DMA((NIT,)),
            pltpu.SemaphoreType.DMA((6,)),
            pltpu.SemaphoreType.DMA((20,)),
        ],
        compiler_params=pltpu.CompilerParams(vmem_limit_bytes=118 * 1024 * 1024,
                                             disable_bounds_checks=True, disable_semaphore_checks=True),
    )(A_x.reshape(NSEG, SEG, DM), A_mem0.reshape(M, DM), wr(A_Wq), wr(A_Wk), wr(A_Wv),
      A_Wo.reshape(H * E, DM), B_x.reshape(NSEG // 2, 2, SEG, DM), B_w_r.T, B_w_i.T, _mask_fill(), _fft_consts())
    return out.reshape(1, S, 2 * DM)
```

```python
import functools
import math

import jax
import jax.numpy as jnp
import numpy as np
from jax import lax
import jax.experimental.pallas as pl
import jax.experimental.pallas.tpu as pltpu

BF, F32, U32, I32 = jnp.bfloat16, jnp.float32, jnp.uint32, jnp.int32

S, DM, H, E, M, SEG = 2048, 1024, 32, 128, 8, 32
NSEG = S // SEG
NP = H // 2
UN = 2
R2 = math.sqrt(0.5)
MID = 'mid'
OPT = dict(skip=(), late_wait=1, tie8=0, b_own=500, b_plus=150, b_sh=2, due=2, b_fwd=400, b_inv0=200, b_inv=400)


def _to_u32(m):
    u = np.ascontiguousarray(m, dtype=np.float32).view(np.uint32)
    h = ((u + 0x7FFF + ((u >> 16) & 1)) >> 16).astype(np.uint32)
    return h[..., 0::2, :] | (h[..., 1::2, :] << 16)


def _mask_fill():
    r = np.arange(80)
    pos_of = lambda rr: np.where(rr < M, rr, np.where(rr < SEG, rr + M, rr - SEG + M))
    qhead = np.where(r < 64, r // 32, (r - 64) // 8)
    qpos = pos_of(np.where(r < 64, r % 32, SEG + (r - 64) % 8))
    khead, kpos = r % 2, pos_of(r // 2)
    vis = (qpos[:, None] < M) | (qpos[:, None] >= kpos[None, :])
    same = qhead[:, None] == khead[None, :]
    return np.where(same, np.where(vis, 0.0, -1e9), -np.inf).astype(np.float32)


RES = ((0, 12, 8, 4), (1, 15, 9, 7), (2, 14, 10, 6), (3, 13, 11, 5))
WP = 72
C_MD, C_MN, C_TW, C_MS, C_NUM = 0, 16, 22, 24, 88


@functools.lru_cache(maxsize=None)
def _fft_consts():
    md = np.zeros((16, 128, 128))
    for q in range(4):
        if q == 0:
            lay = [[(0, 0), (0, 1), (2, 0), (2, 1)], [(3, 1), (1, 0), (1, 1), (3, 0)]]
        else:
            lay = [[(0, 0), (1, 0), (0, 1), (1, 1)], [(2, 1), (3, 1), (2, 0), (3, 0)]]
        for h in range(2):
            ms_, ws_ = [], []
            for g, part in lay[h]:
                k = 16 * np.arange(32) + RES[q][g]
                th = 2 * np.pi * np.outer(np.arange(128 if q == 0 else 64), k) / DM
                c, s = np.cos(th), np.sin(th)
                if q == 0:
                    ms_.append(-s if part else c)
                else:
                    sg = (1.0 if RES[q][g] % 8 == q else -1.0) * (1.0 - 2.0 * h)
                    ms_.append(np.concatenate([-s, sg * c] if part else [c, sg * s]))
                ws_.append(np.where(k == 0, 1.0, 2.0) / DM)
            m = np.concatenate(ms_, axis=1)
            md[2 * q + h] = m
            md[8 + 2 * q + h] = (m * np.concatenate(ws_)[None, :]).T
    a, l = np.arange(64), np.arange(128)
    ms = np.zeros((64, 128, 128))
    for dl in range(32):
        th = 2 * np.pi * np.outer(32 * a + dl, a) / S
        c, s = np.cos(th), np.sin(th)
        ms[2 * dl, :64, 0::2], ms[2 * dl, :64, 1::2] = c, s
        ms[2 * dl, 64:, 0::2], ms[2 * dl, 64:, 1::2] = -s, c
        ms[2 * dl + 1, :64, 0::2], ms[2 * dl + 1, :64, 1::2] = c.T / S, -s.T / S
        ms[2 * dl + 1, 64:, 0::2], ms[2 * dl + 1, 64:, 1::2] = s.T / S, c.T / S
    mn = np.zeros((6, 128, 128))
    th = 2 * np.pi * np.outer(np.arange(32), l) / 32
    mn[0, :32], mn[1, :32] = np.cos(th), -np.sin(th)
    mn[4, :, :32], mn[5, :, :32] = np.cos(th).T / DM, -np.sin(th).T / DM
    th = 2 * np.pi * np.outer(np.arange(16), a) / 16
    c, s = np.cos(th), np.sin(th)
    mn[2, :16, 0::2], mn[2, :16, 1::2], mn[2, 16:32, 0::2], mn[2, 16:32, 1::2] = c, s, -s, c
    mn[3, :64, 0:32:2], mn[3, :64, 1:32:2] = c.T / S, -s.T / S
    mn[3, 64:, 0:32:2], mn[3, 64:, 1:32:2] = s.T / S, c.T / S
    th = 2 * np.pi * np.outer(a, l) / S
    tw = np.stack([np.cos(th), np.sin(th)]).astype(np.float32).view(np.uint32)
    return np.concatenate([_to_u32(md), _to_u32(mn), tw, _to_u32(ms)], axis=0)


def _bdot(a, b):
    return jnp.dot(a, b, preferred_element_type=F32)


def _bf(u):
    return pltpu.bitcast(u, BF)


def _pack2(r, i):
    return pltpu.bitcast(pltpu.pack_elementwise([r, i], packed_dtype=BF), U32)


def _unpack2(u, p):
    if p == 0:
        return pltpu.bitcast(u << 16, F32)
    return pltpu.bitcast(u & jnp.uint32(0xFFFF0000), F32)


def _strassen_left(n, a):
    return (lambda: a(1, 0) + a(1, 1), lambda: a(1, 0) - a(0, 0), lambda: a(1, 1), lambda: a(0, 0) + a(1, 1),
            lambda: a(0, 0), lambda: a(0, 1) - a(1, 1), lambda: a(0, 0) + a(0, 1))[n]()


def _strassen(left, w, done, ready=lambda k: None, dot=None):
    add = lambda u, v: _pack2(_unpack2(u, 0) + _unpack2(v, 0), _unpack2(u, 1) + _unpack2(v, 1))
    sub = lambda u, v: _pack2(_unpack2(u, 0) - _unpack2(v, 0), _unpack2(u, 1) - _unpack2(v, 1))

    def mm(n, r):
        acc = None
        for k in range(0, r.shape[0], 256):
            a = left(n)[:, 2 * k:2 * k + 512]
            d = dot(a, r[k:k + 256]) if dot else _bdot(_bf(a), _bf(r[k:k + 256]))
            acc = d if acc is None else acc + d
        return acc

    ready(0)
    m2 = mm(0, w(0, 0))
    c22 = mm(1, add(w(0, 0), w(0, 1))) - m2
    ready(1)
    m4 = mm(2, sub(w(1, 0), w(0, 0)))
    c21 = m2 + m4
    m1 = mm(3, add(w(0, 0), w(1, 1)))
    c11, c22 = m1 + m4, c22 + m1
    m3 = mm(4, sub(w(0, 1), w(1, 1)))
    done(1, c21, c22 + m3)
    c11 = c11 + mm(5, add(w(1, 0), w(1, 1)))
    m5 = mm(6, w(1, 1))
    done(0, c11 - m5, m3 + m5)


def _twiddle(z, k, n, sign):
    r, i = z
    if k == 0:
        return r, i
    if 4 * k == n:
        return (-i, r) if sign > 0 else (i, -r)
    c, s = math.cos(2 * math.pi * k / n), sign * math.sin(2 * math.pi * k / n)
    if 8 * k == n or 8 * k == 3 * n:
        if c * s > 0:
            return (r - i) * c, (r + i) * c
        return (r + i) * c, (i - r) * c
    return r * c - i * s, r * s + i * c


def _cfft(xs, sign):
    n = len(xs)
    if n == 1:
        return xs
    ev, od = _cfft(xs[0::2], sign), _cfft(xs[1::2], sign)
    out = [None] * n
    for k in range(n // 2):
        er, ei = ev[k]
        if 4 * k == n:
            orr, oi = od[k]
            lo, hi = (er - oi, ei + orr), (er + oi, ei - orr)
            out[k], out[k + n // 2] = (lo, hi) if sign > 0 else (hi, lo)
        else:
            tr, ti = _twiddle(od[k], k, n, sign)
            out[k], out[k + n // 2] = (er + tr, ei + ti), (er - tr, ei - ti)
    return out


def _rfft8(x):
    a0, a1, b0, b1 = x[0] + x[4], x[0] - x[4], x[2] + x[6], x[2] - x[6]
    c0, c1, d0, d1 = x[1] + x[5], x[1] - x[5], x[3] + x[7], x[3] - x[7]
    e, f = a0 + b0, c0 + d0
    g, h = (c1 - d1) * R2, (c1 + d1) * R2
    return [e + f, e - f, a1 + g, b1 + h, a0 - b0, c0 - d0, a1 - g, b1 - h]


def _irfft8(z):
    z0, z4, z1r, z1i, z2r, z2i, z3r, z3i = z
    e, f = z0 + z4, z0 - z4
    a1, g = z1r + z3r, (z1r - z3r) * R2
    b1, h = z1i + z3i, (z1i - z3i) * R2
    a0, b0, c0, d0 = e + z2r, e - z2r, f + z2i, f - z2i
    c1, d1 = g + h, h - g
    return [a0 + a1, c0 + c1, b0 + b1, d0 + d1, a0 - a1, c0 - c1, b0 - b1, d0 - d1]


def _kernel(x_hbm, mem0_hbm, wq_hbm, wk_hbm, wv_hbm, wo_hbm, bx_hbm, wr_hbm, wi_hbm, fill_hbm, cst_hbm,
            out_hbm,
            x_v, xpre_v, xs_v, mem0_v, fill_v, lhs_v, wqkv, wo_v, pre, opost, outa_v,
            bx_v, w_v, wn_v, wt, cst, zs, vv, tn, outb_v,
            sem_w, sem_in, sem_out):
    scale = E ** -0.5
    wus = [w.bitcast(U32) for w in (wq_hbm, wk_hbm, wv_hbm)]
    wo_u = wo_hbm.bitcast(U32)
    fus = [w.at[pl.ds(0, 512)].bitcast(U32) for w in (wr_hbm, wi_hbm)]

    def w_copies(j, t, sem):
        return [pltpu.make_async_copy(wus[t].at[:, :, j, :], wqkv.at[j, t], sem)]

    w0_cps = [w_copies(0, 0, sem_in.at[3]), w_copies(0, 1, sem_in.at[4]) + w_copies(0, 2, sem_in.at[4])]
    xpre_cp = pltpu.make_async_copy(x_hbm.at[:, pl.ds(0, 8), :], xpre_v, sem_in.at[0])

    def w_pair(j):
        return [cp for t in range(3) for cp in w_copies(j, t, sem_w.at[j])]

    def b_rows(i, b):
        return b, i // 4, pl.ds(pl.multiple_of((i % 4) * 8, 8), 8)

    def fwd_cps(i):
        rows = b_rows(i, slice(None))
        return w_pair(8 + i) + [pltpu.make_async_copy(bx_hbm.at[rows], bx_v.at[rows], sem_w.at[8 + i])] + [
            pltpu.make_async_copy(fus[t].at[:, pl.ds(pl.multiple_of(128 * (2 * i + h), 128), 128)],
                                  w_v.at[t, 2 * i + h], sem_w.at[8 + i]) for t in range(2) for h in range(2)]

    def part(src, dst, lo, hi, sem):
        return pltpu.make_async_copy(src.at[pl.ds(lo, hi - lo)], dst.at[pl.ds(lo, hi - lo)], sem)

    c0_cp = part(cst_hbm, cst, 0, C_MS, sem_w.at[0])
    a_cps = [pltpu.make_async_copy(wo_u.at[:, pl.ds(128 * n, 128)], wo_v.at[n], sem_in.at[1]) for n in range(8)]
    a_cps += [part(x_hbm, x_v, 0, UN, sem_in.at[1]), part(cst_hbm, cst, C_MS, C_MS + UN, sem_in.at[1]),
              pltpu.make_async_copy(mem0_hbm, mem0_v, sem_in.at[1]),
              pltpu.make_async_copy(fill_hbm, fill_v, sem_in.at[1])]
    b_cps = [part(x_hbm, x_v, UN, NSEG, sem_in.at[2]), part(cst_hbm, cst, C_MS + UN, C_NUM, sem_in.at[2])]
    b_cps += [pltpu.make_async_copy(w.at[pl.ds(512, 1)], wn_v.at[t], sem_in.at[2])
              for t, w in enumerate((wr_hbm, wi_hbm))]

    lane = lax.broadcasted_iota(I32, (8, 128), 1)
    alt = jnp.where(lane % 2 == 0, 1.0, -1.0).astype(F32)
    lo_half = lane < 64
    ev_grp = (lane // 32) % 2 == 0

    def half_coef(q):
        sg = -1.0 if q < 3 else 1.0
        tc, ts = math.cos(2 * math.pi * q / 16), -math.sin(2 * math.pi * q / 16)
        f = lambda lo, hi: jnp.where(lo_half, lo, hi).astype(F32)
        return f(1.0, ts), f(0.0, sg * tc), f(0.0, tc), f(sg, -sg * ts)

    pace = {'tok': None}

    def gate(v):
        tok = pace['tok']
        if tok is None:
            return v
        return v | tok if v.dtype == U32 else pltpu.bitcast(pltpu.bitcast(v, U32) | tok, v.dtype)

    def gate2(z):
        return gate(z[0]), gate(z[1])

    def flat(zs_):
        return [v for z in zs_ for v in z]

    def as_u32(rows):
        return pltpu.bitcast(jnp.concatenate(rows, axis=0).astype(BF), U32)

    def b_fwd(i):
        r0 = pl.multiple_of(i * 8, 8)
        hc = [None] + [half_coef(q) for q in range(1, 4)]
        tacc = jnp.zeros((8, 128), F32)
        zl = []
        for b0 in range(0, 32, 2):
            rows = []
            for b in (b0, b0 + 1):
                xb = bx_v[(*b_rows(i, b), slice(None))].astype(F32)
                z = _rfft8([gate(xb[:, 128 * t:128 * t + 128]) for t in range(8)])
                tacc = jnp.where(lane == b, jnp.sum(z[0] * alt, axis=1, keepdims=True), tacc)
                for q in range(1, 4):
                    c1, c2, c3, c4 = hc[q]
                    zr, zi = z[2 * q], z[2 * q + 1]
                    pp = c1 * zr + c2 * zi
                    qq = pltpu.roll(c3 * zr + c4 * zi, 64, 1)
                    z[2 * q], z[2 * q + 1] = pp + qq, pp - qq
                rows.append(z)
            zl.append([as_u32([rows[0][n], rows[1][n]]) for n in range(8)])
            yield 200
            if b0 % 4 == 0:
                e, t, ty = 2 * i + b0 // 16, (b0 // 8) % 2, (b0 // 4) % 2
                u = jnp.concatenate([gate(w_v[t, e, pl.ds(m + ty + 64 * v, 8, stride=8), :])
                                     for m in (0, 6, 4, 2) for v in range(4)], axis=0)
                ut = pltpu.bitcast(pltpu.bitcast(u, F32).T, U32)
                for v in range(16):
                    wt[t, ty, pl.ds(8 * (v % 4) * WP + 4 * e + v // 4, 8, stride=WP), :] = ut[8 * v:8 * v + 8]
                yield 40
        tn[pl.ds(r0, 8), :] = tacc

        def mm(n):
            return _bdot(_bf(jnp.concatenate([z[n] for z in zl], axis=0)), _bf(cst[C_MD + n]))

        yield MID
        oo = [mm(n) for n in range(4)]
        yield MID
        oo += [mm(n) for n in range(4, 8)]
        yield MID
        for q in range(4):
            sel, sh = (ev_grp, 96) if q == 0 else (lo_half, 64)
            ys = []
            for b0 in range(4):
                xs = []
                for b in range(b0, 32, 4):
                    e_, o_ = gate(oo[2 * q][8 * b:8 * b + 8]), oo[2 * q + 1][8 * b:8 * b + 8]
                    xs.append((jnp.where(sel, e_, o_), pltpu.roll(jnp.where(sel, o_, e_), sh, 1)))
                ys.append([_twiddle(y, b0 * k1, 32, -1) for k1, y in enumerate(_cfft(xs, -1))])
                yield 110
            for k1 in range(8):
                o = [_pack2(*y) for y in _cfft([gate2(ys[b0][k1]) for b0 in range(4)], -1)]
                for k0 in range(4):
                    zs[k1 + 8 * k0, pl.ds(r0, 8), 128 * q:128 * q + 128] = o[k0]
                yield 30

    def b_mid(it):
        if UN > 2:
            yield MID
        else:
            for _ in range(6):
                yield None
        for n in range(UN // 2):
            dl = (UN // 2) * it + n
            y = _bdot(_bf(cst[C_MS + 2 * dl]), _bf(zs[dl]))
            for _ in range(4):
                yield None
            w0 = pl.multiple_of(dl * WP, 8)
            rows = []
            for r in range(8):
                wq = []
                for t in range(2):
                    ta, tb = wt[t, 0, pl.ds(w0 + 8 * r, 8), :], wt[t, 1, pl.ds(w0 + 8 * r, 8), :]
                    wq.append([_unpack2(ta, 0), _unpack2(jnp.where(ev_grp, ta, tb), 1),
                               _unpack2(tb, 0), _unpack2(jnp.where(ev_grp, tb, ta), 1)])
                cols = []
                for q in range(4):
                    yr = y[8 * r:8 * r + 8, 128 * q:128 * q + 128]
                    yi = y[64 + 8 * r:72 + 8 * r, 128 * q:128 * q + 128]
                    wr, wi = wq[0][q], wq[1][q]
                    cols.append(_pack2(yr * wr - yi * wi, yr * wi + yi * wr))
                rows.append(jnp.concatenate(cols, axis=1))
                yield cols
                yield None
            yield MID
            vv[dl] = _bdot(_bf(cst[C_MS + 2 * dl + 1]), _bf(jnp.concatenate(rows, axis=0)))

    def b_nyq():
        c, s = pltpu.bitcast(cst[C_TW], F32), pltpu.bitcast(cst[C_TW + 1], F32)
        tb = tn[...].astype(BF)
        tr, ti = _bdot(tb, _bf(cst[C_MN])), _bdot(tb, _bf(cst[C_MN + 1]))
        yield MID
        y = _bdot(_bf(cst[C_MN + 2, 0:16, :]), _bf(_pack2(tr * c + ti * s, ti * c - tr * s)))
        row = lax.broadcasted_iota(I32, (16, 128), 0)
        wn = []
        for t in range(2):
            wrow = wn_v[t].astype(F32)
            acc = jnp.zeros((16, 128), F32)
            for e in range(16):
                acc = jnp.where(row == e, wrow[:, 128 * e:128 * e + 128], acc)
            wn.append(acc)
        yr, yi = y[0:16], y[16:32]
        yield MID
        v = _bdot(_bf(cst[C_MN + 3, :, 0:32]), _bf(_pack2(yr * wn[0] - yi * wn[1], yr * wn[1] + yi * wn[0])))
        vr, vi = v[0:64], v[64:128]
        yield MID
        tn[...] = (_bdot((vr * c - vi * s).astype(BF), _bf(cst[C_MN + 4]))
                   + _bdot((vr * s + vi * c).astype(BF), _bf(cst[C_MN + 5])))

    def b_inv(i):
        r0 = i * 8
        ul = []
        for q in range(4):
            sel, sh = (ev_grp, 32) if q == 0 else (lo_half, 64)
            ys = []
            for b0 in range(4):
                xs = [(gate(vv[dl, pl.ds(r0, 8), 128 * q:128 * q + 128]),
                       gate(vv[dl, pl.ds(64 + r0, 8), 128 * q:128 * q + 128])) for dl in range(b0, 32, 4)]
                ys.append([_twiddle(y, b0 * k1, 32, +1) for k1, y in enumerate(_cfft(xs, +1))])
                yield (120, flat(ys[-1])) if OPT['tie8'] else 110
            ie, io = [], []
            for k1 in range(8):
                es, os_ = [], []
                for ur, ui in _cfft([gate2(ys[b0][k1]) for b0 in range(4)], +1):
                    tmp = pltpu.roll(ui, sh, 1)
                    es.append(jnp.where(sel, ur, tmp))
                    os_.append(jnp.where(sel, tmp, ur))
                ie += [as_u32(es[0:2]), as_u32(es[2:4])]
                io += [as_u32(os_[0:2]), as_u32(os_[2:4])]
                yield 55, ie[-2:] + io[-2:]
            ul += [ie, io]
        return ul

    def b_fin(i, zz):
        r0 = i * 8
        hc = [None] + [half_coef(q) for q in range(1, 4)]
        tb = tn[pl.ds(r0, 8), :]
        for g in range(32):
            b = g // 4 + 8 * (g % 4)
            z = [gate(zz[n][8 * g:8 * g + 8]) for n in range(8)]
            z[0] = z[0] + jnp.sum(jnp.where(lane == b, tb, 0.0), axis=1, keepdims=True) * alt
            for q in range(1, 4):
                c1, c2, c3, c4 = hc[q]
                pp = z[2 * q] + z[2 * q + 1]
                qq = pltpu.roll(z[2 * q] - z[2 * q + 1], 64, 1)
                z[2 * q], z[2 * q + 1] = c1 * pp + c3 * qq, c2 * pp + c4 * qq
            y = _irfft8(z)
            outb_v[(*b_rows(i, b), slice(None))] = jnp.concatenate(y, axis=1).astype(BF)
            yield 75, y
        rows = b_rows(i, slice(None))
        start_out(outb_v.at[rows], out_hbm.at[(*rows, pl.ds(DM, DM))])

    def tie(w, vals):
        if not vals:
            return w
        acc = None
        for v in vals:
            v = v if v.dtype == U32 else pltpu.bitcast(v, U32)
            acc = v if acc is None else acc | v
        zero = cst[C_MN, 56:64, :]
        return jnp.concatenate([w[0:8] | (acc & zero), w[8:]], axis=0)

    def batch_slot(gen, budget):
        st = {'debt': 0, 'k': 0}
        due = {}

        def emit(d, b):
            while st['debt'] < b:
                r = 8 * (32 * st['debt'] // b)
                pace['tok'] = pltpu.bitcast(d[r:r + 8], U32) & cst[C_MN, 56:64, :]
                c = next(gen, MID)
                if c is MID:
                    st['debt'] = b
                elif isinstance(c, list):
                    st['debt'] = 0
                    for own in c:
                        emit(own, OPT['b_own'])
                    return
                else:
                    if isinstance(c, tuple):
                        due.setdefault(st['k'] + OPT['due'], []).extend(c[1])
                        c = c[0]
                    st['debt'] += c
            st['debt'] -= b

        def dot(a, w):
            vals = due.pop(st['k'], None)
            if vals:
                a = jnp.concatenate([tie(a[:, 0:128], vals), a[:, 128:]], axis=1)
            d = _bdot(_bf(a), _bf(w))
            st['k'] += 1
            emit(d, budget(st['k'] - 1))
            return d

        return dot

    out_cps = []

    def start_out(src, dst):
        out_cps.append(pltpu.make_async_copy(src, dst, sem_out.at[len(out_cps)]))
        out_cps[-1].start()

    hb = DM // 32

    def retile(j, t, k):
        blk = pl.ds(k * hb, hb)
        a, b = wqkv[j, t, blk, pl.ds(0, 8, stride=2), :], wqkv[j, t, blk, pl.ds(1, 8, stride=2), :]
        wqkv[j, t, blk, 0:8, :] = (a & jnp.uint32(0xFFFF)) | (b << 16)
        wqkv[j, t, blk, 8:16, :] = (a >> 16) | (b & jnp.uint32(0xFFFF0000))

    def strassen_lhs():
        for g in range(NSEG // 4):
            xa = [xpre_v[4 * g + k].astype(F32) for k in range(4)]
            a1, a2 = jnp.concatenate([xa[0], xa[2]], axis=0), jnp.concatenate([xa[1], xa[3]], axis=0)
            a11, a12, a21, a22 = a1[:, :DM // 2], a1[:, DM // 2:], a2[:, :DM // 2], a2[:, DM // 2:]
            for n in range(7):
                v = _strassen_left(n, lambda r, k: ((a11, a12), (a21, a22))[r][k])
                xs_v[n, 8 * g:8 * g + 8, :] = pltpu.bitcast(v.astype(BF), U32)

    def pre_step7(j, t, slot=None):
        w = lambda k, p: wqkv[j, t, k * hb:(k + 1) * hb, 8 * p:8 * p + 8, :].reshape(DM // 4, E)
        half = {}

        def done(h, c1, c2):
            half[h] = _pack2(c1, c2).reshape(NSEG // 2, 8, E)

        _strassen(lambda n: xs_v[n], w, done, functools.partial(retile, j, t), slot)
        pre[j, t] = jnp.stack([half[0], half[1]], axis=1).reshape(NSEG, 8, E)

    xpre_cp.start()
    for cp in (w0_cps[0] + w0_cps[1] + [cp for j in range(1, 8) for cp in w_pair(j)] + [c0_cp]
               + [cp for i in range(3) for cp in fwd_cps(i)]):
        cp.start()
    xpre_cp.wait()
    strassen_lhs()
    if 'head' in OPT['skip']:
        pre_step7_full, pre_step7 = pre_step7, lambda *a: None
    for cp in w0_cps[0]:
        cp.wait()
    pre_step7(0, 0)
    for cp in w0_cps[1]:
        cp.wait()
    pre_step7(0, 1)
    pre_step7(0, 2)
    for cp in fwd_cps(3):
        cp.start()
    for cp in w_pair(1):
        cp.wait()
    for t in range(3):
        pre_step7(1, t)
    for cp in fwd_cps(4):
        cp.start()

    def pre_body(k, carry):
        for cp in w_pair(2 * k) + w_pair(2 * k + 1):
            cp.wait()
        for j in (2 * k, 2 * k + 1):
            for t in range(3):
                pre_step7(j, t)
        for cp in fwd_cps(4 + k):
            cp.start()
        return carry

    lax.fori_loop(1, 4, pre_body, 0)
    if 'head' in OPT['skip']:
        pre_step7 = pre_step7_full
    c0_cp.wait()
    for cp in a_cps + b_cps:
        cp.start()

    def pre_fwd_body(i, carry):
        for cp in fwd_cps(i):
            cp.wait()
        gen = b_fwd(i)
        slot = batch_slot(gen, lambda k: OPT['b_fwd'])
        for t in range(3):
            pre_step7(8 + i, t, slot)
        for _ in gen:
            pass
        return carry

    if 'fwd' not in OPT['skip']:
        lax.fori_loop(0, 8, pre_fwd_body, 0)
    for cp in a_cps + ([] if OPT['late_wait'] else b_cps):
        cp.wait()

    def seg_step(s, u, mem, slot):
        xs = x_v[s]
        lhs_v[u] = as_u32([mem, xs[8:32].astype(F32)])
        fill = fill_v[...]

        def proj(j, t):
            w0, w1 = [wqkv[j, t, :, 8 * p:8 * p + 8, :].reshape(DM // 2, E) for p in range(2)]
            r0, r1 = _bdot(_bf(lhs_v[u]), _bf(tie(w0, slot()))), _bdot(_bf(lhs_v[u]), _bf(w1))
            pw = pre[j, t, s]
            if t == 0:
                return jnp.concatenate([r0, r1, _unpack2(pw, 0), _unpack2(pw, 1)], axis=0).astype(BF)
            return _bf(jnp.concatenate([_pack2(r0, r1), pw], axis=0))

        def qk(q, k):
            sc = lax.dot_general(q, k, (((1,), (1,)), ((), ())), preferred_element_type=F32) * scale
            sc = jnp.where(fill == 0.0, sc, fill)
            p = jnp.exp(sc - jnp.max(sc, axis=-1, keepdims=True))
            return (p * pl.reciprocal(jnp.sum(p, axis=-1, keepdims=True), approx=True)).astype(BF)

        ob, ps, vs = {}, {}, {}

        def pv(j):
            o = _bdot(ps[j], vs[j])
            opost[s // 2, u % 2, :, pl.ds(256 * j, 128)] = o[64:72]
            opost[s // 2, u % 2, :, pl.ds(256 * j + 128, 128)] = o[72:80]
            ob[j] = [o[0:32], o[32:64]]

        def wo(g0, g1):
            og = jnp.concatenate([o for j in range(2 * g0, 2 * g1) for o in ob[j]], axis=1).astype(BF)
            return jnp.concatenate([_bdot(og, _bf(wo_v[n, g0 * 256:g1 * 256, :])) for n in range(8)], axis=1)

        ng = NP // 2
        for g in range(ng):
            ja, jb = 2 * g, 2 * g + 1
            qa, ka, qb, kb = proj(ja, 0), proj(ja, 1), proj(jb, 0), proj(jb, 1)
            vs[ja], vs[jb] = proj(ja, 2), proj(jb, 2)
            ps[ja], ps[jb] = qk(qa, ka), qk(qb, kb)
            if g > 0:
                pv(ja - 2)
                pv(jb - 2)
        res = wo(0, 3)
        pv(NP - 2)
        pv(NP - 1)
        res = res + wo(3, ng - 1)
        res = res + wo(ng - 1, ng)
        outa_v[s // 2, u % 2, 8:32, :] = res[8:32].astype(BF)
        return res[0:8].astype(BF).astype(F32)

    def loop_body(it, mem):
        if OPT['late_wait']:
            @pl.when(it == 1)
            def _():
                for cp in b_cps:
                    cp.wait()

        gen = b_mid(it)
        state = {'mid': False}

        def slot():
            if state['mid']:
                return None
            vals = next(gen, None)
            if vals is MID:
                state['mid'] = True
                return None
            return vals

        for u in range(UN):
            state['mid'] = False
            mem = seg_step(UN * it + u, u, mem, slot)
        for _ in gen:
            pass
        return mem

    if 'main' not in OPT['skip']:
        lax.fori_loop(0, NSEG // UN, loop_body, mem0_v[...].astype(F32))
    idx = (slice(None), slice(None), pl.ds(8, SEG - 8), pl.ds(0, DM))
    start_out(outa_v.at[idx], out_hbm.at[idx])

    hk = H * E // 2

    @functools.lru_cache(maxsize=None)
    def post_left(n):
        sums = [_strassen_left(n, lambda r, k: opost[g, r, :, k * hk:(k + 1) * hk]) for g in range(NSEG // 2)]
        return jnp.concatenate([_pack2(sums[g], sums[g + 1]) for g in range(0, NSEG // 2, 2)], axis=0)

    def b_inv_all():
        nyq = b_nyq()
        zz = None
        for i in range(9):
            if i < 8:
                gen = b_inv(i)
                try:
                    k = 0
                    while True:
                        c = next(gen)
                        k += 1
                        if k % 10 == 1:
                            next(nyq, None)
                        yield c
                except StopIteration as e:
                    ul = e.value
            if i > 0:
                yield from b_fin(i - 1, zz)
            else:
                yield MID
            if i < 8:
                zz = [_bdot(_bf(jnp.concatenate(ul[n], axis=0)), _bf(cst[C_MD + 8 + n])) for n in range(8)]
                if i == 7:
                    yield MID
                    yield MID
                else:
                    yield [zz[3], zz[7]]

    gens = [b_inv_all()]
    slot = batch_slot(gens[0], lambda k: (OPT['b_inv0'] if k < 28 else OPT['b_inv'])
                      + (OPT['b_plus'] if (k + OPT['b_sh']) % 28 < 4 or (k + OPT['b_sh']) % 28 >= 24 else 0))
    if 'post' in OPT['skip']:
        def keep(k, c):
            v = pre[k, 0, k] | zs[k, 0:8, 0:128] | wt[0, 0, pl.ds(pl.multiple_of(8 * k, 8), 8), :] | wqkv[k, 0, k, 0:8, :]
            v = pltpu.bitcast(v, F32) + tn[pl.ds(pl.multiple_of(8 * k, 8), 8), :] + vv[k, 0:8, 0:128] + opost[k, 0, :, 0:128]
            outa_v[k, 0, 0:8, 0:128] = v.astype(BF)
            return c
        lax.fori_loop(0, 4, keep, 0)
        start_out(outa_v.at[:, :, pl.ds(0, 8)], out_hbm.at[:, :, pl.ds(0, 8), pl.ds(0, DM)])
        return
    for n in range(4):
        def done(r, *cs):
            for p, cc in enumerate(cs):
                u = pltpu.bitcast(cc.astype(BF), U32).reshape(NSEG // 4, 8, 128)
                y = jnp.stack([_unpack2(u, 0), _unpack2(u, 1)], axis=1).reshape(NSEG // 2, 8, 128)
                idx = (slice(None), r, pl.ds(0, 8), pl.ds(128 * (n + 4 * p), 128))
                outa_v[idx] = y.astype(BF)
                start_out(outa_v.at[idx], out_hbm.at[idx])

        _strassen(post_left, lambda k, p: wo_v[n + 4 * p, k * hk // 2:(k + 1) * hk // 2, :], done, dot=slot)
    for gen in gens:
        for _ in gen:
            pass
    for cp in out_cps:
        cp.wait()


def pallas_concat_heads__memory_aug_recurrent_mem_tr__spectral_gfnet__prompt_kernel(
    A_x, A_mem0, A_Wq, A_Wk, A_Wv, A_Wo, A_seg_len, B_x, B_w_r, B_w_i,
):
    assert A_x.shape == (1, S, DM) and A_Wq.shape == (DM, H, E) and A_mem0.shape == (1, M, DM)
    assert B_x.shape == (1, S, DM) and (not isinstance(A_seg_len, int) or A_seg_len == SEG)
    hbm = pl.BlockSpec(memory_space=pltpu.HBM)
    wr = lambda w: w.reshape(DM // 16, 16, H, E)
    out = pl.pallas_call(
        _kernel,
        out_shape=jax.ShapeDtypeStruct((NSEG // 2, 2, SEG, 2 * DM), BF),
        in_specs=[hbm] * 11,
        out_specs=hbm,
        scratch_shapes=[
            pltpu.VMEM((NSEG, SEG, DM), BF),
            pltpu.VMEM((NSEG, 8, DM), BF),
            pltpu.VMEM((7, NSEG * 2, DM // 2), U32),
            pltpu.VMEM((M, DM), BF),
            pltpu.VMEM((80, 80), F32),
            pltpu.VMEM((UN, SEG // 2, DM), U32),
            pltpu.VMEM((NP, 3, DM // 16, 16, E), U32),
            pltpu.VMEM((8, H * E // 2, 128), U32),
            pltpu.VMEM((NP, 3, NSEG, 8, E), U32),
            pltpu.VMEM((NSEG // 2, 2, 8, H * E), F32),
            pltpu.VMEM((NSEG // 2, 2, SEG, DM), BF),
            pltpu.VMEM((NSEG // 2, 2, SEG, DM), BF),
            pltpu.VMEM((2, 16, 256, 128), U32),
            pltpu.VMEM((2, 1, S), BF),
            pltpu.VMEM((2, 2, 32 * WP, 128), U32),
            pltpu.VMEM((C_NUM, 64, 128), U32),
            pltpu.VMEM((32, 64, 512), U32),
            pltpu.VMEM((32, 128, 512), F32),
            pltpu.VMEM((64, 128), F32),
            pltpu.VMEM((NSEG // 2, 2, SEG, DM), BF),
            pltpu.SemaphoreType.DMA((NP,)),
            pltpu.SemaphoreType.DMA((6,)),
            pltpu.SemaphoreType.DMA((25,)),
        ],
        compiler_params=pltpu.CompilerParams(vmem_limit_bytes=118 * 1024 * 1024,
                                             disable_bounds_checks=True, disable_semaphore_checks=True),
    )(A_x.reshape(NSEG, SEG, DM), A_mem0.reshape(M, DM), wr(A_Wq), wr(A_Wk), wr(A_Wv),
      A_Wo.reshape(H * E, DM), B_x.reshape(NSEG // 2, 2, SEG, DM), B_w_r.T, B_w_i.T, _mask_fill(), _fft_consts())
    return out.reshape(1, S, 2 * DM)
```

```python
import functools
import math

import jax
import jax.numpy as jnp
import numpy as np
from jax import lax
import jax.experimental.pallas as pl
import jax.experimental.pallas.tpu as pltpu

BF, F32, U32, I32 = jnp.bfloat16, jnp.float32, jnp.uint32, jnp.int32

S, DM, H, E, M, SEG = 2048, 1024, 32, 128, 8, 32
NSEG = S // SEG
NP = H // 2
UN = 4
R2 = math.sqrt(0.5)
MID = 'mid'
OPT = dict(skip=(), a_at=1, b_fwd0=130, tie_ws=1, cuts=(0, 1, 2, 4, 7, 12, 18, 24), later={3: (0, 1), 4: (2, 3), 5: (4, 5), 6: (6, 7)}, late_wait=1, tie8=0, b_own=300, b_plus=0, b_sh=2, due=2, b_fwd=400, b_inv0=450, b_inv=450)


def _to_u32(m):
    u = np.ascontiguousarray(m, dtype=np.float32).view(np.uint32)
    h = ((u + 0x7FFF + ((u >> 16) & 1)) >> 16).astype(np.uint32)
    return h[..., 0::2, :] | (h[..., 1::2, :] << 16)


def _mask_fill():
    r = np.arange(80)
    pos_of = lambda rr: np.where(rr < M, rr, np.where(rr < SEG, rr + M, rr - SEG + M))
    qhead = np.where(r < 64, r // 32, (r - 64) // 8)
    qpos = pos_of(np.where(r < 64, r % 32, SEG + (r - 64) % 8))
    khead, kpos = r % 2, pos_of(r // 2)
    vis = (qpos[:, None] < M) | (qpos[:, None] >= kpos[None, :])
    same = qhead[:, None] == khead[None, :]
    return np.where(same, np.where(vis, 0.0, -1e9), -np.inf).astype(np.float32)


RES = ((0, 12, 8, 4), (1, 15, 9, 7), (2, 14, 10, 6), (3, 13, 11, 5))
WP = 72
C_MD, C_MN, C_TW, C_MS, C_NUM = 0, 16, 22, 24, 88


@functools.lru_cache(maxsize=None)
def _fft_consts():
    md = np.zeros((16, 128, 128))
    for q in range(4):
        if q == 0:
            lay = [[(0, 0), (0, 1), (2, 0), (2, 1)], [(3, 1), (1, 0), (1, 1), (3, 0)]]
        else:
            lay = [[(0, 0), (1, 0), (0, 1), (1, 1)], [(2, 1), (3, 1), (2, 0), (3, 0)]]
        for h in range(2):
            ms_, ws_ = [], []
            for g, part in lay[h]:
                k = 16 * np.arange(32) + RES[q][g]
                th = 2 * np.pi * np.outer(np.arange(128 if q == 0 else 64), k) / DM
                c, s = np.cos(th), np.sin(th)
                if q == 0:
                    ms_.append(-s if part else c)
                else:
                    sg = (1.0 if RES[q][g] % 8 == q else -1.0) * (1.0 - 2.0 * h)
                    ms_.append(np.concatenate([-s, sg * c] if part else [c, sg * s]))
                ws_.append(np.where(k == 0, 1.0, 2.0) / DM)
            m = np.concatenate(ms_, axis=1)
            md[2 * q + h] = m
            md[8 + 2 * q + h] = (m * np.concatenate(ws_)[None, :]).T
    a, l = np.arange(64), np.arange(128)
    ms = np.zeros((64, 128, 128))
    for dl in range(32):
        th = 2 * np.pi * np.outer(32 * a + dl, a) / S
        c, s = np.cos(th), np.sin(th)
        ms[2 * dl, :64, 0::2], ms[2 * dl, :64, 1::2] = c, s
        ms[2 * dl, 64:, 0::2], ms[2 * dl, 64:, 1::2] = -s, c
        ms[2 * dl + 1, :64, 0::2], ms[2 * dl + 1, :64, 1::2] = c.T / S, -s.T / S
        ms[2 * dl + 1, 64:, 0::2], ms[2 * dl + 1, 64:, 1::2] = s.T / S, c.T / S
    mn = np.zeros((6, 128, 128))
    th = 2 * np.pi * np.outer(np.arange(32), l) / 32
    mn[0, :32], mn[1, :32] = np.cos(th), -np.sin(th)
    mn[4, :, :32], mn[5, :, :32] = np.cos(th).T / DM, -np.sin(th).T / DM
    th = 2 * np.pi * np.outer(np.arange(16), a) / 16
    c, s = np.cos(th), np.sin(th)
    mn[2, :16, 0::2], mn[2, :16, 1::2], mn[2, 16:32, 0::2], mn[2, 16:32, 1::2] = c, s, -s, c
    mn[3, :64, 0:32:2], mn[3, :64, 1:32:2] = c.T / S, -s.T / S
    mn[3, 64:, 0:32:2], mn[3, 64:, 1:32:2] = s.T / S, c.T / S
    th = 2 * np.pi * np.outer(a, l) / S
    tw = np.stack([np.cos(th), np.sin(th)]).astype(np.float32).view(np.uint32)
    return np.concatenate([_to_u32(md), _to_u32(mn), tw, _to_u32(ms)], axis=0)


def _bdot(a, b):
    return jnp.dot(a, b, preferred_element_type=F32)


def _bf(u):
    return pltpu.bitcast(u, BF)


def _pack2(r, i):
    return pltpu.bitcast(pltpu.pack_elementwise([r, i], packed_dtype=BF), U32)


def _unpack2(u, p):
    if p == 0:
        return pltpu.bitcast(u << 16, F32)
    return pltpu.bitcast(u & jnp.uint32(0xFFFF0000), F32)


def _strassen_left(n, a):
    return (lambda: a(1, 0) + a(1, 1), lambda: a(1, 0) - a(0, 0), lambda: a(1, 1), lambda: a(0, 0) + a(1, 1),
            lambda: a(0, 0), lambda: a(0, 1) - a(1, 1), lambda: a(0, 0) + a(0, 1))[n]()


def _strassen_right(n, w):
    add = lambda u, v: _pack2(_unpack2(u, 0) + _unpack2(v, 0), _unpack2(u, 1) + _unpack2(v, 1))
    sub = lambda u, v: _pack2(_unpack2(u, 0) - _unpack2(v, 0), _unpack2(u, 1) - _unpack2(v, 1))
    return (lambda: w(0, 0), lambda: add(w(0, 0), w(0, 1)), lambda: sub(w(1, 0), w(0, 0)),
            lambda: add(w(0, 0), w(1, 1)), lambda: sub(w(0, 1), w(1, 1)), lambda: add(w(1, 0), w(1, 1)),
            lambda: w(1, 1))[n]()


def _strassen(left, right, done, ready=lambda k: None, dot=None):
    def mm(n):
        a, r, acc = left(n), right(n), None
        for k in range(0, r.shape[0], 256):
            ak, rk = a[:, 2 * k:2 * k + 512], r[k:k + 256]
            d = dot(ak, rk) if dot else _bdot(_bf(ak), _bf(rk))
            acc = d if acc is None else acc + d
        return acc

    ready(0)
    m2 = mm(0)
    c22 = mm(1) - m2
    ready(1)
    m4 = mm(2)
    c21 = m2 + m4
    m1 = mm(3)
    c11, c22 = m1 + m4, c22 + m1
    m3 = mm(4)
    done(1, c21, c22 + m3)
    c11 = c11 + mm(5)
    m5 = mm(6)
    done(0, c11 - m5, m3 + m5)


def _twiddle(z, k, n, sign):
    r, i = z
    if k == 0:
        return r, i
    if 4 * k == n:
        return (-i, r) if sign > 0 else (i, -r)
    c, s = math.cos(2 * math.pi * k / n), sign * math.sin(2 * math.pi * k / n)
    if 8 * k == n or 8 * k == 3 * n:
        if c * s > 0:
            return (r - i) * c, (r + i) * c
        return (r + i) * c, (i - r) * c
    return r * c - i * s, r * s + i * c


def _cfft(xs, sign):
    n = len(xs)
    if n == 1:
        return xs
    ev, od = _cfft(xs[0::2], sign), _cfft(xs[1::2], sign)
    out = [None] * n
    for k in range(n // 2):
        er, ei = ev[k]
        if 4 * k == n:
            orr, oi = od[k]
            lo, hi = (er - oi, ei + orr), (er + oi, ei - orr)
            out[k], out[k + n // 2] = (lo, hi) if sign > 0 else (hi, lo)
        else:
            tr, ti = _twiddle(od[k], k, n, sign)
            out[k], out[k + n // 2] = (er + tr, ei + ti), (er - tr, ei - ti)
    return out


def _rfft8(x):
    a0, a1, b0, b1 = x[0] + x[4], x[0] - x[4], x[2] + x[6], x[2] - x[6]
    c0, c1, d0, d1 = x[1] + x[5], x[1] - x[5], x[3] + x[7], x[3] - x[7]
    e, f = a0 + b0, c0 + d0
    g, h = (c1 - d1) * R2, (c1 + d1) * R2
    return [e + f, e - f, a1 + g, b1 + h, a0 - b0, c0 - d0, a1 - g, b1 - h]


def _irfft8(z):
    z0, z4, z1r, z1i, z2r, z2i, z3r, z3i = z
    e, f = z0 + z4, z0 - z4
    a1, g = z1r + z3r, (z1r - z3r) * R2
    b1, h = z1i + z3i, (z1i - z3i) * R2
    a0, b0, c0, d0 = e + z2r, e - z2r, f + z2i, f - z2i
    c1, d1 = g + h, h - g
    return [a0 + a1, c0 + c1, b0 + b1, d0 + d1, a0 - a1, c0 - c1, b0 - b1, d0 - d1]


def _kernel(x_hbm, mem0_hbm, wq_hbm, wk_hbm, wv_hbm, wo_hbm, bx_hbm, wr_hbm, wi_hbm, fill_hbm, cst_hbm,
            out_hbm,
            x_v, xpre_v, xs_v, mem0_v, fill_v, lhs_v, wqkv, wo_v, pre, opost, os_v, ws_v, outa_v,
            bx_v, w_v, wn_v, wt, cst, zs, vv, tn, outb_v,
            sem_w, sem_in, sem_out):
    scale = E ** -0.5
    wus = [w.bitcast(U32) for w in (wq_hbm, wk_hbm, wv_hbm)]
    wo_u = wo_hbm.bitcast(U32)
    fus = [w.at[pl.ds(0, 512)].bitcast(U32) for w in (wr_hbm, wi_hbm)]

    def w_copy(j, t, sem):
        return pltpu.make_async_copy(wus[t].at[:, :, j, :], wqkv.at[j, t], sem)

    xpre_cp = pltpu.make_async_copy(x_hbm.at[:, pl.ds(0, 8), :], xpre_v, sem_w.at[7])
    cuts = OPT['cuts']
    head = [[divmod(f, 3) for f in range(cuts[b], cuts[b + 1])] for b in range(len(cuts) - 1)]
    head_cps = [[w_copy(j, t, sem_w.at[b]) for j, t in grp] for b, grp in enumerate(head)]

    def b_rows(i, b):
        return b, i // 4, pl.ds(pl.multiple_of((i % 4) * 8, 8), 8)

    def fwd_cps(i):
        rows = b_rows(i, slice(None))
        return [w_copy(8 + i, t, sem_w.at[8 + i]) for t in range(3)] + [pltpu.make_async_copy(bx_hbm.at[rows], bx_v.at[rows], sem_w.at[8 + i])] + [
            pltpu.make_async_copy(fus[t].at[:, pl.ds(pl.multiple_of(128 * (2 * i + h), 128), 128)],
                                  w_v.at[t, 2 * i + h], sem_w.at[8 + i]) for t in range(2) for h in range(2)]

    def part(src, dst, lo, hi, sem):
        return pltpu.make_async_copy(src.at[pl.ds(lo, hi - lo)], dst.at[pl.ds(lo, hi - lo)], sem)

    c0_cp = part(cst_hbm, cst, 0, C_MS, sem_w.at[16])
    a_cps = [pltpu.make_async_copy(wo_u.at[:, pl.ds(128 * n, 128)], wo_v.at[n], sem_in.at[1]) for n in range(8)]
    a_cps += [part(x_hbm, x_v, 0, UN, sem_in.at[1]), part(cst_hbm, cst, C_MS, C_MS + UN, sem_in.at[1]),
              pltpu.make_async_copy(mem0_hbm, mem0_v, sem_in.at[1]),
              pltpu.make_async_copy(fill_hbm, fill_v, sem_in.at[1])]
    b_cps = [part(x_hbm, x_v, UN, NSEG, sem_in.at[2]), part(cst_hbm, cst, C_MS + UN, C_NUM, sem_in.at[2])]
    b_cps += [pltpu.make_async_copy(w.at[pl.ds(512, 1)], wn_v.at[t], sem_in.at[2])
              for t, w in enumerate((wr_hbm, wi_hbm))]

    lane = lax.broadcasted_iota(I32, (8, 128), 1)
    alt = jnp.where(lane % 2 == 0, 1.0, -1.0).astype(F32)
    lo_half = lane < 64
    ev_grp = (lane // 32) % 2 == 0

    def half_coef(q):
        sg = -1.0 if q < 3 else 1.0
        tc, ts = math.cos(2 * math.pi * q / 16), -math.sin(2 * math.pi * q / 16)
        f = lambda lo, hi: jnp.where(lo_half, lo, hi).astype(F32)
        return f(1.0, ts), f(0.0, sg * tc), f(0.0, tc), f(sg, -sg * ts)

    pace = {'tok': None}

    def gate(v):
        tok = pace['tok']
        if tok is None:
            return v
        return v | tok if v.dtype == U32 else pltpu.bitcast(pltpu.bitcast(v, U32) | tok, v.dtype)

    def gate2(z):
        return gate(z[0]), gate(z[1])

    def flat(zs_):
        return [v for z in zs_ for v in z]

    def as_u32(rows):
        return pltpu.bitcast(jnp.concatenate(rows, axis=0).astype(BF), U32)

    def b_fwd(i):
        r0 = pl.multiple_of(i * 8, 8)
        hc = [None] + [half_coef(q) for q in range(1, 4)]
        tacc = jnp.zeros((8, 128), F32)
        zl = []
        for b0 in range(0, 32, 2):
            rows = []
            for b in (b0, b0 + 1):
                xb = bx_v[(*b_rows(i, b), slice(None))].astype(F32)
                z = _rfft8([gate(xb[:, 128 * t:128 * t + 128]) for t in range(8)])
                tacc = jnp.where(lane == b, jnp.sum(z[0] * alt, axis=1, keepdims=True), tacc)
                for q in range(1, 4):
                    c1, c2, c3, c4 = hc[q]
                    zr, zi = z[2 * q], z[2 * q + 1]
                    pp = c1 * zr + c2 * zi
                    qq = pltpu.roll(c3 * zr + c4 * zi, 64, 1)
                    z[2 * q], z[2 * q + 1] = pp + qq, pp - qq
                rows.append(z)
            zl.append([as_u32([rows[0][n], rows[1][n]]) for n in range(8)])
            yield 200
            if b0 % 4 == 0:
                e, t, ty = 2 * i + b0 // 16, (b0 // 8) % 2, (b0 // 4) % 2
                u = jnp.concatenate([gate(w_v[t, e, pl.ds(m + ty + 64 * v, 8, stride=8), :])
                                     for m in (0, 6, 4, 2) for v in range(4)], axis=0)
                ut = pltpu.bitcast(pltpu.bitcast(u, F32).T, U32)
                for v in range(16):
                    wt[t, ty, pl.ds(8 * (v % 4) * WP + 4 * e + v // 4, 8, stride=WP), :] = ut[8 * v:8 * v + 8]
                yield 40
        tn[pl.ds(r0, 8), :] = tacc

        def mm(n):
            return _bdot(_bf(jnp.concatenate([z[n] for z in zl], axis=0)), _bf(cst[C_MD + n]))

        yield MID
        oo = [mm(n) for n in range(4)]
        yield MID
        oo += [mm(n) for n in range(4, 8)]
        yield MID
        for q in range(4):
            sel, sh = (ev_grp, 96) if q == 0 else (lo_half, 64)
            ys = []
            for b0 in range(4):
                xs = []
                for b in range(b0, 32, 4):
                    e_, o_ = gate(oo[2 * q][8 * b:8 * b + 8]), oo[2 * q + 1][8 * b:8 * b + 8]
                    xs.append((jnp.where(sel, e_, o_), pltpu.roll(jnp.where(sel, o_, e_), sh, 1)))
                ys.append([_twiddle(y, b0 * k1, 32, -1) for k1, y in enumerate(_cfft(xs, -1))])
                yield 110
            for k1 in range(8):
                o = [_pack2(*y) for y in _cfft([gate2(ys[b0][k1]) for b0 in range(4)], -1)]
                for k0 in range(4):
                    zs[k1 + 8 * k0, pl.ds(r0, 8), 128 * q:128 * q + 128] = o[k0]
                yield 30

    def b_mid(it):
        if UN > 2:
            rows = H * E // 4 // (NSEG // UN)
            for n in range(4):
                for r in range(0, rows, 8):
                    blk = lambda k, p: wo_v[n + 4 * p, pl.ds(pl.multiple_of(k * (H * E // 4) + it * rows + r, 8), 8), :]
                    vals = [_strassen_right(m, blk) for m in range(1, 6)]
                    for m in range(5):
                        ws_v[n, m, pl.ds(pl.multiple_of(it * rows + r, 8), 8), :] = vals[m]
                    yield vals if OPT['tie_ws'] and 8 * n + r // 8 > 1 else None
            yield MID
        else:
            for _ in range(6):
                yield None
        for n in range(UN // 2):
            dl = (UN // 2) * it + n
            y = _bdot(_bf(cst[C_MS + 2 * dl]), _bf(zs[dl]))
            for _ in range(4):
                yield None
            w0 = pl.multiple_of(dl * WP, 8)
            rows = []
            for r in range(8):
                wq = []
                for t in range(2):
                    ta, tb = wt[t, 0, pl.ds(w0 + 8 * r, 8), :], wt[t, 1, pl.ds(w0 + 8 * r, 8), :]
                    wq.append([_unpack2(ta, 0), _unpack2(jnp.where(ev_grp, ta, tb), 1),
                               _unpack2(tb, 0), _unpack2(jnp.where(ev_grp, tb, ta), 1)])
                cols = []
                for q in range(4):
                    yr = y[8 * r:8 * r + 8, 128 * q:128 * q + 128]
                    yi = y[64 + 8 * r:72 + 8 * r, 128 * q:128 * q + 128]
                    wr, wi = wq[0][q], wq[1][q]
                    cols.append(_pack2(yr * wr - yi * wi, yr * wi + yi * wr))
                rows.append(jnp.concatenate(cols, axis=1))
                yield cols
                yield None
            yield MID
            vv[dl] = _bdot(_bf(cst[C_MS + 2 * dl + 1]), _bf(jnp.concatenate(rows, axis=0)))

    def b_nyq():
        c, s = pltpu.bitcast(cst[C_TW], F32), pltpu.bitcast(cst[C_TW + 1], F32)
        tb = tn[...].astype(BF)
        tr, ti = _bdot(tb, _bf(cst[C_MN])), _bdot(tb, _bf(cst[C_MN + 1]))
        yield MID
        y = _bdot(_bf(cst[C_MN + 2, 0:16, :]), _bf(_pack2(tr * c + ti * s, ti * c - tr * s)))
        row = lax.broadcasted_iota(I32, (16, 128), 0)
        wn = []
        for t in range(2):
            wrow = wn_v[t].astype(F32)
            acc = jnp.zeros((16, 128), F32)
            for e in range(16):
                acc = jnp.where(row == e, wrow[:, 128 * e:128 * e + 128], acc)
            wn.append(acc)
        yr, yi = y[0:16], y[16:32]
        yield MID
        v = _bdot(_bf(cst[C_MN + 3, :, 0:32]), _bf(_pack2(yr * wn[0] - yi * wn[1], yr * wn[1] + yi * wn[0])))
        vr, vi = v[0:64], v[64:128]
        yield MID
        tn[...] = (_bdot((vr * c - vi * s).astype(BF), _bf(cst[C_MN + 4]))
                   + _bdot((vr * s + vi * c).astype(BF), _bf(cst[C_MN + 5])))

    def b_inv(i):
        r0 = i * 8
        ul = []
        for q in range(4):
            sel, sh = (ev_grp, 32) if q == 0 else (lo_half, 64)
            ys = []
            for b0 in range(4):
                xs = [(gate(vv[dl, pl.ds(r0, 8), 128 * q:128 * q + 128]),
                       gate(vv[dl, pl.ds(64 + r0, 8), 128 * q:128 * q + 128])) for dl in range(b0, 32, 4)]
                ys.append([_twiddle(y, b0 * k1, 32, +1) for k1, y in enumerate(_cfft(xs, +1))])
                yield (120, flat(ys[-1])) if OPT['tie8'] else 110
            ie, io = [], []
            for k1 in range(8):
                es, os_ = [], []
                for ur, ui in _cfft([gate2(ys[b0][k1]) for b0 in range(4)], +1):
                    tmp = pltpu.roll(ui, sh, 1)
                    es.append(jnp.where(sel, ur, tmp))
                    os_.append(jnp.where(sel, tmp, ur))
                ie += [as_u32(es[0:2]), as_u32(es[2:4])]
                io += [as_u32(os_[0:2]), as_u32(os_[2:4])]
                yield 55, ie[-2:] + io[-2:]
            ul += [ie, io]
        return ul

    def b_fin(i, zz):
        r0 = i * 8
        hc = [None] + [half_coef(q) for q in range(1, 4)]
        tb = tn[pl.ds(r0, 8), :]
        for g in range(32):
            b = g // 4 + 8 * (g % 4)
            z = [gate(zz[n][8 * g:8 * g + 8]) for n in range(8)]
            z[0] = z[0] + jnp.sum(jnp.where(lane == b, tb, 0.0), axis=1, keepdims=True) * alt
            for q in range(1, 4):
                c1, c2, c3, c4 = hc[q]
                pp = z[2 * q] + z[2 * q + 1]
                qq = pltpu.roll(z[2 * q] - z[2 * q + 1], 64, 1)
                z[2 * q], z[2 * q + 1] = c1 * pp + c3 * qq, c2 * pp + c4 * qq
            y = _irfft8(z)
            outb_v[(*b_rows(i, b), slice(None))] = jnp.concatenate(y, axis=1).astype(BF)
            yield 75, y
        rows = b_rows(i, slice(None))
        start_out(outb_v.at[rows], out_hbm.at[(*rows, pl.ds(DM, DM))])

    def tie(w, vals):
        if not vals:
            return w
        acc = None
        for v in vals:
            v = v if v.dtype == U32 else pltpu.bitcast(v, U32)
            acc = v if acc is None else acc | v
        zero = cst[C_MN, 56:64, :]
        return jnp.concatenate([w[0:8] | (acc & zero), w[8:]], axis=0)

    def batch_slot(gen, budget):
        st = {'debt': 0, 'k': 0}
        due = {}

        def emit(d, b):
            while st['debt'] < b:
                r = 8 * (32 * st['debt'] // b)
                pace['tok'] = pltpu.bitcast(d[r:r + 8], U32) & cst[C_MN, 56:64, :]
                c = next(gen, MID)
                if c is MID:
                    st['debt'] = b
                elif isinstance(c, list):
                    st['debt'] = 0
                    for own in c:
                        emit(own, OPT['b_own'])
                    return
                else:
                    if isinstance(c, tuple):
                        due.setdefault(st['k'] + OPT['due'], []).extend(c[1])
                        c = c[0]
                    st['debt'] += c
            st['debt'] -= b

        def dot(a, w):
            vals = due.pop(st['k'], None)
            if vals:
                a = jnp.concatenate([tie(a[:, 0:128], vals), a[:, 128:]], axis=1)
            d = _bdot(_bf(a), _bf(w))
            st['k'] += 1
            emit(d, budget(st['k'] - 1))
            return d

        return dot

    out_cps = []

    def start_out(src, dst):
        out_cps.append(pltpu.make_async_copy(src, dst, sem_out.at[0]))
        out_cps[-1].start()

    hb = DM // 32

    def retile(j, t, k):
        blk = pl.ds(k * hb, hb)
        a, b = wqkv[j, t, blk, pl.ds(0, 8, stride=2), :], wqkv[j, t, blk, pl.ds(1, 8, stride=2), :]
        wqkv[j, t, blk, 0:8, :] = (a & jnp.uint32(0xFFFF)) | (b << 16)
        wqkv[j, t, blk, 8:16, :] = (a >> 16) | (b & jnp.uint32(0xFFFF0000))

    def strassen_lhs():
        for g in range(NSEG // 4):
            xa = [xpre_v[4 * g + k].astype(F32) for k in range(4)]
            a1, a2 = jnp.concatenate([xa[0], xa[2]], axis=0), jnp.concatenate([xa[1], xa[3]], axis=0)
            a11, a12, a21, a22 = a1[:, :DM // 2], a1[:, DM // 2:], a2[:, :DM // 2], a2[:, DM // 2:]
            for n in range(7):
                v = _strassen_left(n, lambda r, k: ((a11, a12), (a21, a22))[r][k])
                xs_v[n, 8 * g:8 * g + 8, :] = pltpu.bitcast(v.astype(BF), U32)

    def pre_step7(j, t, slot=None):
        w = lambda k, p: wqkv[j, t, k * hb:(k + 1) * hb, 8 * p:8 * p + 8, :].reshape(DM // 4, E)
        half = {}

        def done(h, c1, c2):
            half[h] = _pack2(c1, c2).reshape(NSEG // 2, 8, E)

        _strassen(lambda n: xs_v[n], lambda n: _strassen_right(n, w), done, functools.partial(retile, j, t), slot)
        pre[j, t] = jnp.stack([half[0], half[1]], axis=1).reshape(NSEG, 8, E)

    for cp in [xpre_cp] + [cp for grp in head_cps for cp in grp]:
        cp.start()
    zs[...] = jnp.zeros(zs.shape, U32)
    vv[0:8] = jnp.zeros((8,) + vv.shape[1:], F32)
    xpre_cp.wait()
    strassen_lhs()
    later = {int(k): v for k, v in OPT['later'].items()}

    def pre_fwd(steps, i, budget):
        gen = b_fwd(i)
        slot = batch_slot(gen, lambda n: budget)
        for j, t in steps + [(8 + i, t) for t in range(3)]:
            pre_step7(j, t, slot)
        for _ in gen:
            pass

    for b, grp in enumerate(head):
        last = b == len(head) - 1
        for cp in head_cps[b] + ([c0_cp] + fwd_cps(0) if last else []):
            cp.wait()
        if 'head' in OPT['skip']:
            pass
        elif last:
            pre_fwd(grp, 0, OPT['b_fwd0'])
        else:
            for j, t in grp:
                pre_step7(j, t)
        for i in later.get(b, ()):
            for cp in ([c0_cp] if i == 0 else []) + fwd_cps(i):
                cp.start()

    def pre_fwd_body(i, carry):
        for cp in fwd_cps(i):
            cp.wait()

        @pl.when(i == OPT['a_at'])
        def _():
            for cp in a_cps + b_cps:
                cp.start()

        pre_fwd([], i, OPT['b_fwd'])
        return carry

    if 'fwd' not in OPT['skip']:
        lax.fori_loop(1, 8, pre_fwd_body, 0)
    for cp in a_cps + ([] if OPT['late_wait'] else b_cps):
        cp.wait()

    def seg_step(s, u, mem, slot):
        xs = x_v[s]
        lhs_v[u] = as_u32([mem, xs[8:32].astype(F32)])
        fill = fill_v[...]

        def proj(j, t):
            w0, w1 = [wqkv[j, t, :, 8 * p:8 * p + 8, :].reshape(DM // 2, E) for p in range(2)]
            r0, r1 = _bdot(_bf(lhs_v[u]), _bf(tie(w0, slot()))), _bdot(_bf(lhs_v[u]), _bf(w1))
            pw = pre[j, t, s]
            if t == 0:
                return jnp.concatenate([r0, r1, _unpack2(pw, 0), _unpack2(pw, 1)], axis=0).astype(BF)
            return _bf(jnp.concatenate([_pack2(r0, r1), pw], axis=0))

        def qk(q, k):
            sc = lax.dot_general(q, k, (((1,), (1,)), ((), ())), preferred_element_type=F32) * scale
            sc = jnp.where(fill == 0.0, sc, fill)
            p = jnp.exp(sc - jnp.max(sc, axis=-1, keepdims=True))
            return (p * pl.reciprocal(jnp.sum(p, axis=-1, keepdims=True), approx=True)).astype(BF)

        ob, ps, vs = {}, {}, {}

        def pv(j):
            o = _bdot(ps[j], vs[j])
            opost[u // 2, u % 2, :, pl.ds(256 * j, 128)] = o[64:72]
            opost[u // 2, u % 2, :, pl.ds(256 * j + 128, 128)] = o[72:80]
            ob[j] = [o[0:32], o[32:64]]

        def wo(g0, g1):
            og = jnp.concatenate([o for j in range(2 * g0, 2 * g1) for o in ob[j]], axis=1).astype(BF)
            return jnp.concatenate([_bdot(og, _bf(wo_v[n, g0 * 256:g1 * 256, :])) for n in range(8)], axis=1)

        ng = NP // 2
        for g in range(ng):
            ja, jb = 2 * g, 2 * g + 1
            qa, ka, qb, kb = proj(ja, 0), proj(ja, 1), proj(jb, 0), proj(jb, 1)
            vs[ja], vs[jb] = proj(ja, 2), proj(jb, 2)
            ps[ja], ps[jb] = qk(qa, ka), qk(qb, kb)
            if g > 0:
                pv(ja - 2)
                pv(jb - 2)
        res = wo(0, 3)
        pv(NP - 2)
        pv(NP - 1)
        res = res + wo(3, ng - 1)
        res = res + wo(ng - 1, ng)
        outa_v[s // 2, u % 2, 8:32, :] = res[8:32].astype(BF)
        return res[0:8].astype(BF).astype(F32)

    hk = H * E // 2

    def loop_body(it, mem):
        if OPT['late_wait']:
            @pl.when(it == 1)
            def _():
                for cp in b_cps:
                    cp.wait()

        gen = b_mid(it)
        state = {'mid': False}

        def slot():
            if state['mid']:
                return None
            vals = next(gen, None)
            if vals is MID:
                state['mid'] = True
                return None
            return vals

        for u in range(UN):
            state['mid'] = False
            mem = seg_step(UN * it + u, u, mem, slot)
        for _ in gen:
            pass
        for n in range(7):
            sums = [_strassen_left(n, lambda r, k: opost[g, r, :, k * hk:(k + 1) * hk]) for g in range(2)]
            os_v[n, pl.ds(pl.multiple_of(8 * it, 8), 8), :] = _pack2(*sums)
        return mem

    if 'main' not in OPT['skip']:
        lax.fori_loop(0, NSEG // UN, loop_body, mem0_v[...].astype(F32))
    idx = (slice(None), slice(None), pl.ds(8, SEG - 8), pl.ds(0, DM))
    start_out(outa_v.at[idx], out_hbm.at[idx])

    def b_inv_all():
        nyq = b_nyq()
        zz = None
        for i in range(9):
            if i < 8:
                gen = b_inv(i)
                try:
                    k = 0
                    while True:
                        c = next(gen)
                        k += 1
                        if k % 10 == 1:
                            next(nyq, None)
                        yield c
                except StopIteration as e:
                    ul = e.value
            if i > 0:
                yield from b_fin(i - 1, zz)
            else:
                yield MID
            if i < 8:
                zz = [_bdot(_bf(jnp.concatenate(ul[n], axis=0)), _bf(cst[C_MD + 8 + n])) for n in range(8)]
                if i == 7:
                    yield MID
                    yield MID
                else:
                    yield [zz[3], zz[7]]

    gens = [b_inv_all()]
    slot = batch_slot(gens[0], lambda k: (OPT['b_inv0'] if k < 28 else OPT['b_inv'])
                      + (OPT['b_plus'] if (k + OPT['b_sh']) % 28 < 4 or (k + OPT['b_sh']) % 28 >= 24 else 0))
    if 'post' in OPT['skip']:
        def keep(k, c):
            v = pre[k, 0, k] | zs[k, 0:8, 0:128] | wt[0, 0, pl.ds(pl.multiple_of(8 * k, 8), 8), :] | wqkv[k, 0, k, 0:8, :]
            v = pltpu.bitcast(v, F32) + tn[pl.ds(pl.multiple_of(8 * k, 8), 8), :] + vv[k, 0:8, 0:128] + pltpu.bitcast(os_v[k, 0:8, 0:128] | ws_v[k, k, 0:8, :], F32)
            outa_v[k, 0, 0:8, 0:128] = v.astype(BF)
            return c
        lax.fori_loop(0, 4, keep, 0)
        start_out(outa_v.at[:, :, pl.ds(0, 8)], out_hbm.at[:, :, pl.ds(0, 8), pl.ds(0, DM)])
        return
    for n in range(4):
        def done(r, *cs):
            for p, cc in enumerate(cs):
                u = pltpu.bitcast(cc.astype(BF), U32).reshape(NSEG // 4, 8, 128)
                y = jnp.stack([_unpack2(u, 0), _unpack2(u, 1)], axis=1).reshape(NSEG // 2, 8, 128)
                idx = (slice(None), r, pl.ds(0, 8), pl.ds(128 * (n + 4 * p), 128))
                outa_v[idx] = y.astype(BF)
                start_out(outa_v.at[idx], out_hbm.at[idx])

        right = lambda m: (wo_v[n, 0:hk // 2, :] if m == 0 else wo_v[n + 4, hk // 2:hk, :] if m == 6
                           else ws_v[n, m - 1])
        _strassen(lambda m: os_v[m], right, done, dot=slot)
    for gen in gens:
        for _ in gen:
            pass
    for cp in out_cps:
        cp.wait()


def pallas_concat_heads__memory_aug_recurrent_mem_tr__spectral_gfnet__prompt_kernel(
    A_x, A_mem0, A_Wq, A_Wk, A_Wv, A_Wo, A_seg_len, B_x, B_w_r, B_w_i,
):
    assert A_x.shape == (1, S, DM) and A_Wq.shape == (DM, H, E) and A_mem0.shape == (1, M, DM)
    assert B_x.shape == (1, S, DM) and (not isinstance(A_seg_len, int) or A_seg_len == SEG)
    hbm = pl.BlockSpec(memory_space=pltpu.HBM)
    wr = lambda w: w.reshape(DM // 16, 16, H, E)
    out = pl.pallas_call(
        _kernel,
        out_shape=jax.ShapeDtypeStruct((NSEG // 2, 2, SEG, 2 * DM), BF),
        in_specs=[hbm] * 11,
        out_specs=hbm,
        scratch_shapes=[
            pltpu.VMEM((NSEG, SEG, DM), BF),
            pltpu.VMEM((NSEG, 8, DM), BF),
            pltpu.VMEM((7, NSEG * 2, DM // 2), U32),
            pltpu.VMEM((M, DM), BF),
            pltpu.VMEM((80, 80), F32),
            pltpu.VMEM((UN, SEG // 2, DM), U32),
            pltpu.VMEM((NP, 3, DM // 16, 16, E), U32),
            pltpu.VMEM((8, H * E // 2, 128), U32),
            pltpu.VMEM((NP, 3, NSEG, 8, E), U32),
            pltpu.VMEM((2, 2, 8, H * E), F32),
            pltpu.VMEM((7, NSEG * 2, H * E // 2), U32),
            pltpu.VMEM((4, 5, H * E // 4, 128), U32),
            pltpu.VMEM((NSEG // 2, 2, SEG, DM), BF),
            pltpu.VMEM((NSEG // 2, 2, SEG, DM), BF),
            pltpu.VMEM((2, 16, 256, 128), U32),
            pltpu.VMEM((2, 1, S), BF),
            pltpu.VMEM((2, 2, 32 * WP, 128), U32),
            pltpu.VMEM((C_NUM, 64, 128), U32),
            pltpu.VMEM((32, 64, 512), U32),
            pltpu.VMEM((32, 128, 512), F32),
            pltpu.VMEM((64, 128), F32),
            pltpu.VMEM((NSEG // 2, 2, SEG, DM), BF),
            pltpu.SemaphoreType.DMA((NP + 1,)),
            pltpu.SemaphoreType.DMA((6,)),
            pltpu.SemaphoreType.DMA((1,)),
        ],
        compiler_params=pltpu.CompilerParams(vmem_limit_bytes=118 * 1024 * 1024,
                                             disable_bounds_checks=True, disable_semaphore_checks=True),
    )(A_x.reshape(NSEG, SEG, DM), A_mem0.reshape(M, DM), wr(A_Wq), wr(A_Wk), wr(A_Wv),
      A_Wo.reshape(H * E, DM), B_x.reshape(NSEG // 2, 2, SEG, DM), B_w_r.T, B_w_i.T, _mask_fill(), _fft_consts())
    return out.reshape(1, S, 2 * DM)
```

```python
import functools
import math

import jax
import jax.numpy as jnp
import numpy as np
from jax import lax
import jax.experimental.pallas as pl
import jax.experimental.pallas.tpu as pltpu

BF, F32, U32, I32 = jnp.bfloat16, jnp.float32, jnp.uint32, jnp.int32

S, DM, H, E, M, SEG = 2048, 1024, 32, 128, 8, 32
NSEG = S // SEG
NP = H // 2
UN = 4
R2 = math.sqrt(0.5)
MID = 'mid'
OPT = dict(skip=(), a_at=0, b_fwd0=130, tie_ws=1, cuts=(0, 1, 2, 4, 7, 12, 18, 24), later={2: (0, 1), 3: (2,), 4: (3, 4, 5), 5: (6, 7)}, late_wait=1, tie8=0, b_own=300, b_plus=0, b_sh=2, due=2, b_fwd=400, b_inv0=450, b_inv=450)


def _to_u32(m):
    u = np.ascontiguousarray(m, dtype=np.float32).view(np.uint32)
    h = ((u + 0x7FFF + ((u >> 16) & 1)) >> 16).astype(np.uint32)
    return h[..., 0::2, :] | (h[..., 1::2, :] << 16)


def _mask_fill():
    r = np.arange(80)
    pos_of = lambda rr: np.where(rr < M, rr, np.where(rr < SEG, rr + M, rr - SEG + M))
    qhead = np.where(r < 64, r // 32, (r - 64) // 8)
    qpos = pos_of(np.where(r < 64, r % 32, SEG + (r - 64) % 8))
    khead, kpos = r % 2, pos_of(r // 2)
    vis = (qpos[:, None] < M) | (qpos[:, None] >= kpos[None, :])
    same = qhead[:, None] == khead[None, :]
    return np.where(same, np.where(vis, 0.0, -1e9), -np.inf).astype(np.float32)


RES = ((0, 12, 8, 4), (1, 15, 9, 7), (2, 14, 10, 6), (3, 13, 11, 5))
WP = 72
C_MD, C_MN, C_TW, C_MS, C_NUM = 0, 16, 22, 24, 88


@functools.lru_cache(maxsize=None)
def _fft_consts():
    md = np.zeros((16, 128, 128))
    for q in range(4):
        if q == 0:
            lay = [[(0, 0), (0, 1), (2, 0), (2, 1)], [(3, 1), (1, 0), (1, 1), (3, 0)]]
        else:
            lay = [[(0, 0), (1, 0), (0, 1), (1, 1)], [(2, 1), (3, 1), (2, 0), (3, 0)]]
        for h in range(2):
            ms_, ws_ = [], []
            for g, part in lay[h]:
                k = 16 * np.arange(32) + RES[q][g]
                th = 2 * np.pi * np.outer(np.arange(128 if q == 0 else 64), k) / DM
                c, s = np.cos(th), np.sin(th)
                if q == 0:
                    ms_.append(-s if part else c)
                else:
                    sg = (1.0 if RES[q][g] % 8 == q else -1.0) * (1.0 - 2.0 * h)
                    ms_.append(np.concatenate([-s, sg * c] if part else [c, sg * s]))
                ws_.append(np.where(k == 0, 1.0, 2.0) / DM)
            m = np.concatenate(ms_, axis=1)
            md[2 * q + h] = m
            md[8 + 2 * q + h] = (m * np.concatenate(ws_)[None, :]).T
    a, l = np.arange(64), np.arange(128)
    ms = np.zeros((64, 128, 128))
    for dl in range(32):
        th = 2 * np.pi * np.outer(32 * a + dl, a) / S
        c, s = np.cos(th), np.sin(th)
        ms[2 * dl, :64, 0::2], ms[2 * dl, :64, 1::2] = c, s
        ms[2 * dl, 64:, 0::2], ms[2 * dl, 64:, 1::2] = -s, c
        ms[2 * dl + 1, :64, 0::2], ms[2 * dl + 1, :64, 1::2] = c.T / S, -s.T / S
        ms[2 * dl + 1, 64:, 0::2], ms[2 * dl + 1, 64:, 1::2] = s.T / S, c.T / S
    mn = np.zeros((6, 128, 128))
    th = 2 * np.pi * np.outer(np.arange(32), l) / 32
    mn[0, :32], mn[1, :32] = np.cos(th), -np.sin(th)
    mn[4, :, :32], mn[5, :, :32] = np.cos(th).T / DM, -np.sin(th).T / DM
    th = 2 * np.pi * np.outer(np.arange(16), a) / 16
    c, s = np.cos(th), np.sin(th)
    mn[2, :16, 0::2], mn[2, :16, 1::2], mn[2, 16:32, 0::2], mn[2, 16:32, 1::2] = c, s, -s, c
    mn[3, :64, 0:32:2], mn[3, :64, 1:32:2] = c.T / S, -s.T / S
    mn[3, 64:, 0:32:2], mn[3, 64:, 1:32:2] = s.T / S, c.T / S
    th = 2 * np.pi * np.outer(a, l) / S
    tw = np.stack([np.cos(th), np.sin(th)]).astype(np.float32).view(np.uint32)
    return np.concatenate([_to_u32(md), _to_u32(mn), tw, _to_u32(ms)], axis=0)


def _bdot(a, b):
    return jnp.dot(a, b, preferred_element_type=F32)


def _bf(u):
    return pltpu.bitcast(u, BF)


def _pack2(r, i):
    return pltpu.bitcast(pltpu.pack_elementwise([r, i], packed_dtype=BF), U32)


def _unpack2(u, p):
    if p == 0:
        return pltpu.bitcast(u << 16, F32)
    return pltpu.bitcast(u & jnp.uint32(0xFFFF0000), F32)


def _strassen_left(n, a):
    return (lambda: a(1, 0) + a(1, 1), lambda: a(1, 0) - a(0, 0), lambda: a(1, 1), lambda: a(0, 0) + a(1, 1),
            lambda: a(0, 0), lambda: a(0, 1) - a(1, 1), lambda: a(0, 0) + a(0, 1))[n]()


def _strassen_right(n, w):
    add = lambda u, v: _pack2(_unpack2(u, 0) + _unpack2(v, 0), _unpack2(u, 1) + _unpack2(v, 1))
    sub = lambda u, v: _pack2(_unpack2(u, 0) - _unpack2(v, 0), _unpack2(u, 1) - _unpack2(v, 1))
    return (lambda: w(0, 0), lambda: add(w(0, 0), w(0, 1)), lambda: sub(w(1, 0), w(0, 0)),
            lambda: add(w(0, 0), w(1, 1)), lambda: sub(w(0, 1), w(1, 1)), lambda: add(w(1, 0), w(1, 1)),
            lambda: w(1, 1))[n]()


def _strassen(left, right, done, ready=lambda k: None, dot=None):
    def mm(n):
        a, r, acc = left(n), right(n), None
        for k in range(0, r.shape[0], 256):
            ak, rk = a[:, 2 * k:2 * k + 512], r[k:k + 256]
            d = dot(ak, rk) if dot else _bdot(_bf(ak), _bf(rk))
            acc = d if acc is None else acc + d
        return acc

    ready(0)
    m2 = mm(0)
    c22 = mm(1) - m2
    ready(1)
    m4 = mm(2)
    c21 = m2 + m4
    m1 = mm(3)
    c11, c22 = m1 + m4, c22 + m1
    m3 = mm(4)
    done(1, c21, c22 + m3)
    c11 = c11 + mm(5)
    m5 = mm(6)
    done(0, c11 - m5, m3 + m5)


def _twiddle(z, k, n, sign):
    r, i = z
    if k == 0:
        return r, i
    if 4 * k == n:
        return (-i, r) if sign > 0 else (i, -r)
    c, s = math.cos(2 * math.pi * k / n), sign * math.sin(2 * math.pi * k / n)
    if 8 * k == n or 8 * k == 3 * n:
        if c * s > 0:
            return (r - i) * c, (r + i) * c
        return (r + i) * c, (i - r) * c
    return r * c - i * s, r * s + i * c


def _cfft(xs, sign):
    n = len(xs)
    if n == 1:
        return xs
    ev, od = _cfft(xs[0::2], sign), _cfft(xs[1::2], sign)
    out = [None] * n
    for k in range(n // 2):
        er, ei = ev[k]
        if 4 * k == n:
            orr, oi = od[k]
            lo, hi = (er - oi, ei + orr), (er + oi, ei - orr)
            out[k], out[k + n // 2] = (lo, hi) if sign > 0 else (hi, lo)
        else:
            tr, ti = _twiddle(od[k], k, n, sign)
            out[k], out[k + n // 2] = (er + tr, ei + ti), (er - tr, ei - ti)
    return out


def _rfft8(x):
    a0, a1, b0, b1 = x[0] + x[4], x[0] - x[4], x[2] + x[6], x[2] - x[6]
    c0, c1, d0, d1 = x[1] + x[5], x[1] - x[5], x[3] + x[7], x[3] - x[7]
    e, f = a0 + b0, c0 + d0
    g, h = (c1 - d1) * R2, (c1 + d1) * R2
    return [e + f, e - f, a1 + g, b1 + h, a0 - b0, c0 - d0, a1 - g, b1 - h]


def _irfft8(z):
    z0, z4, z1r, z1i, z2r, z2i, z3r, z3i = z
    e, f = z0 + z4, z0 - z4
    a1, g = z1r + z3r, (z1r - z3r) * R2
    b1, h = z1i + z3i, (z1i - z3i) * R2
    a0, b0, c0, d0 = e + z2r, e - z2r, f + z2i, f - z2i
    c1, d1 = g + h, h - g
    return [a0 + a1, c0 + c1, b0 + b1, d0 + d1, a0 - a1, c0 - c1, b0 - b1, d0 - d1]


def _kernel(x_hbm, mem0_hbm, wq_hbm, wk_hbm, wv_hbm, wo_hbm, bx_hbm, wr_hbm, wi_hbm, fill_hbm, cst_hbm,
            out_hbm,
            x_v, xpre_v, xs_v, mem0_v, fill_v, lhs_v, wqkv, wo_v, pre, opost, os_v, ws_v, outa_v,
            bx_v, w_v, wn_v, wt, cst, zs, vv, tn, outb_v,
            sem_w, sem_in, sem_out):
    scale = E ** -0.5
    wus = [w.bitcast(U32) for w in (wq_hbm, wk_hbm, wv_hbm)]
    wo_u = wo_hbm.bitcast(U32)
    fus = [w.at[pl.ds(0, 512)].bitcast(U32) for w in (wr_hbm, wi_hbm)]

    def w_copy(j, t, sem):
        return pltpu.make_async_copy(wus[t].at[:, :, j, :], wqkv.at[j, t], sem)

    xpre_cp = pltpu.make_async_copy(x_hbm.at[:, pl.ds(0, 8), :], xpre_v, sem_w.at[7])
    cuts = OPT['cuts']
    head = [[divmod(f, 3) for f in range(cuts[b], cuts[b + 1])] for b in range(len(cuts) - 1)]
    head_cps = [[w_copy(j, t, sem_w.at[b]) for j, t in grp] for b, grp in enumerate(head)]

    def b_rows(i, b):
        return b, i // 4, pl.ds(pl.multiple_of((i % 4) * 8, 8), 8)

    def fwd_cps(i):
        rows = b_rows(i, slice(None))
        return [w_copy(8 + i, t, sem_w.at[8 + i]) for t in range(3)] + [pltpu.make_async_copy(bx_hbm.at[rows], bx_v.at[rows], sem_w.at[8 + i])] + [
            pltpu.make_async_copy(fus[t].at[:, pl.ds(pl.multiple_of(128 * (2 * i + h), 128), 128)],
                                  w_v.at[t, 2 * i + h], sem_w.at[8 + i]) for t in range(2) for h in range(2)]

    def part(src, dst, lo, hi, sem):
        return pltpu.make_async_copy(src.at[pl.ds(lo, hi - lo)], dst.at[pl.ds(lo, hi - lo)], sem)

    c0_cp = part(cst_hbm, cst, 0, C_MS, sem_w.at[16])
    a_cps = [pltpu.make_async_copy(wo_u.at[:, pl.ds(128 * n, 128)], wo_v.at[n], sem_in.at[1]) for n in range(8)]
    a_cps += [part(x_hbm, x_v, 0, UN, sem_in.at[1]), part(cst_hbm, cst, C_MS, C_MS + UN, sem_in.at[1]),
              pltpu.make_async_copy(mem0_hbm, mem0_v, sem_in.at[1]),
              pltpu.make_async_copy(fill_hbm, fill_v, sem_in.at[1])]
    b_cps = [part(x_hbm, x_v, UN, NSEG, sem_in.at[2]), part(cst_hbm, cst, C_MS + UN, C_NUM, sem_in.at[2])]
    b_cps += [pltpu.make_async_copy(w.at[pl.ds(512, 1)], wn_v.at[t], sem_in.at[2])
              for t, w in enumerate((wr_hbm, wi_hbm))]

    lane = lax.broadcasted_iota(I32, (8, 128), 1)
    alt = jnp.where(lane % 2 == 0, 1.0, -1.0).astype(F32)
    lo_half = lane < 64
    ev_grp = (lane // 32) % 2 == 0

    def half_coef(q):
        sg = -1.0 if q < 3 else 1.0
        tc, ts = math.cos(2 * math.pi * q / 16), -math.sin(2 * math.pi * q / 16)
        f = lambda lo, hi: jnp.where(lo_half, lo, hi).astype(F32)
        return f(1.0, ts), f(0.0, sg * tc), f(0.0, tc), f(sg, -sg * ts)

    pace = {'tok': None}

    def gate(v):
        tok = pace['tok']
        if tok is None:
            return v
        return v | tok if v.dtype == U32 else pltpu.bitcast(pltpu.bitcast(v, U32) | tok, v.dtype)

    def gate2(z):
        return gate(z[0]), gate(z[1])

    def flat(zs_):
        return [v for z in zs_ for v in z]

    def as_u32(rows):
        return pltpu.bitcast(jnp.concatenate(rows, axis=0).astype(BF), U32)

    def b_fwd(i):
        r0 = pl.multiple_of(i * 8, 8)
        hc = [None] + [half_coef(q) for q in range(1, 4)]
        tacc = jnp.zeros((8, 128), F32)
        zl = []
        for b0 in range(0, 32, 2):
            rows = []
            for b in (b0, b0 + 1):
                xb = bx_v[(*b_rows(i, b), slice(None))].astype(F32)
                z = _rfft8([gate(xb[:, 128 * t:128 * t + 128]) for t in range(8)])
                tacc = jnp.where(lane == b, jnp.sum(z[0] * alt, axis=1, keepdims=True), tacc)
                for q in range(1, 4):
                    c1, c2, c3, c4 = hc[q]
                    zr, zi = z[2 * q], z[2 * q + 1]
                    pp = c1 * zr + c2 * zi
                    qq = pltpu.roll(c3 * zr + c4 * zi, 64, 1)
                    z[2 * q], z[2 * q + 1] = pp + qq, pp - qq
                rows.append(z)
            zl.append([as_u32([rows[0][n], rows[1][n]]) for n in range(8)])
            yield 200
            if b0 % 4 == 0:
                e, t, ty = 2 * i + b0 // 16, (b0 // 8) % 2, (b0 // 4) % 2
                u = jnp.concatenate([gate(w_v[t, e, pl.ds(m + ty + 64 * v, 8, stride=8), :])
                                     for m in (0, 6, 4, 2) for v in range(4)], axis=0)
                ut = pltpu.bitcast(pltpu.bitcast(u, F32).T, U32)
                for v in range(16):
                    wt[t, ty, pl.ds(8 * (v % 4) * WP + 4 * e + v // 4, 8, stride=WP), :] = ut[8 * v:8 * v + 8]
                yield 40
        tn[pl.ds(r0, 8), :] = tacc

        def mm(n):
            return _bdot(_bf(jnp.concatenate([z[n] for z in zl], axis=0)), _bf(cst[C_MD + n]))

        yield MID
        oo = [mm(n) for n in range(4)]
        yield MID
        oo += [mm(n) for n in range(4, 8)]
        yield MID
        for q in range(4):
            sel, sh = (ev_grp, 96) if q == 0 else (lo_half, 64)
            ys = []
            for b0 in range(4):
                xs = []
                for b in range(b0, 32, 4):
                    e_, o_ = gate(oo[2 * q][8 * b:8 * b + 8]), oo[2 * q + 1][8 * b:8 * b + 8]
                    xs.append((jnp.where(sel, e_, o_), pltpu.roll(jnp.where(sel, o_, e_), sh, 1)))
                ys.append([_twiddle(y, b0 * k1, 32, -1) for k1, y in enumerate(_cfft(xs, -1))])
                yield 110
            for k1 in range(8):
                o = [_pack2(*y) for y in _cfft([gate2(ys[b0][k1]) for b0 in range(4)], -1)]
                for k0 in range(4):
                    zs[k1 + 8 * k0, pl.ds(r0, 8), 128 * q:128 * q + 128] = o[k0]
                yield 30

    def b_mid(it):
        if UN > 2:
            rows = H * E // 4 // (NSEG // UN)
            for n in range(4):
                for r in range(0, rows, 8):
                    blk = lambda k, p: wo_v[n + 4 * p, pl.ds(pl.multiple_of(k * (H * E // 4) + it * rows + r, 8), 8), :]
                    vals = [_strassen_right(m, blk) for m in range(1, 6)]
                    for m in range(5):
                        ws_v[n, m, pl.ds(pl.multiple_of(it * rows + r, 8), 8), :] = vals[m]
                    yield vals if OPT['tie_ws'] and 8 * n + r // 8 > 1 else None
            yield MID
        else:
            for _ in range(6):
                yield None
        for n in range(UN // 2):
            dl = (UN // 2) * it + n
            y = _bdot(_bf(cst[C_MS + 2 * dl]), _bf(zs[dl]))
            for _ in range(4):
                yield None
            w0 = pl.multiple_of(dl * WP, 8)
            rows = []
            for r in range(8):
                wq = []
                for t in range(2):
                    ta, tb = wt[t, 0, pl.ds(w0 + 8 * r, 8), :], wt[t, 1, pl.ds(w0 + 8 * r, 8), :]
                    wq.append([_unpack2(ta, 0), _unpack2(jnp.where(ev_grp, ta, tb), 1),
                               _unpack2(tb, 0), _unpack2(jnp.where(ev_grp, tb, ta), 1)])
                cols = []
                for q in range(4):
                    yr = y[8 * r:8 * r + 8, 128 * q:128 * q + 128]
                    yi = y[64 + 8 * r:72 + 8 * r, 128 * q:128 * q + 128]
                    wr, wi = wq[0][q], wq[1][q]
                    cols.append(_pack2(yr * wr - yi * wi, yr * wi + yi * wr))
                rows.append(jnp.concatenate(cols, axis=1))
                yield cols
                yield None
            yield MID
            vv[dl] = _bdot(_bf(cst[C_MS + 2 * dl + 1]), _bf(jnp.concatenate(rows, axis=0)))

    def b_nyq():
        c, s = pltpu.bitcast(cst[C_TW], F32), pltpu.bitcast(cst[C_TW + 1], F32)
        tb = tn[...].astype(BF)
        tr, ti = _bdot(tb, _bf(cst[C_MN])), _bdot(tb, _bf(cst[C_MN + 1]))
        yield MID
        y = _bdot(_bf(cst[C_MN + 2, 0:16, :]), _bf(_pack2(tr * c + ti * s, ti * c - tr * s)))
        row = lax.broadcasted_iota(I32, (16, 128), 0)
        wn = []
        for t in range(2):
            wrow = wn_v[t].astype(F32)
            acc = jnp.zeros((16, 128), F32)
            for e in range(16):
                acc = jnp.where(row == e, wrow[:, 128 * e:128 * e + 128], acc)
            wn.append(acc)
        yr, yi = y[0:16], y[16:32]
        yield MID
        v = _bdot(_bf(cst[C_MN + 3, :, 0:32]), _bf(_pack2(yr * wn[0] - yi * wn[1], yr * wn[1] + yi * wn[0])))
        vr, vi = v[0:64], v[64:128]
        yield MID
        tn[...] = (_bdot((vr * c - vi * s).astype(BF), _bf(cst[C_MN + 4]))
                   + _bdot((vr * s + vi * c).astype(BF), _bf(cst[C_MN + 5])))

    def b_inv(i):
        r0 = i * 8
        ul = []
        for q in range(4):
            sel, sh = (ev_grp, 32) if q == 0 else (lo_half, 64)
            ys = []
            for b0 in range(4):
                xs = [(gate(vv[dl, pl.ds(r0, 8), 128 * q:128 * q + 128]),
                       gate(vv[dl, pl.ds(64 + r0, 8), 128 * q:128 * q + 128])) for dl in range(b0, 32, 4)]
                ys.append([_twiddle(y, b0 * k1, 32, +1) for k1, y in enumerate(_cfft(xs, +1))])
                yield (120, flat(ys[-1])) if OPT['tie8'] else 110
            ie, io = [], []
            for k1 in range(8):
                es, os_ = [], []
                for ur, ui in _cfft([gate2(ys[b0][k1]) for b0 in range(4)], +1):
                    tmp = pltpu.roll(ui, sh, 1)
                    es.append(jnp.where(sel, ur, tmp))
                    os_.append(jnp.where(sel, tmp, ur))
                ie += [as_u32(es[0:2]), as_u32(es[2:4])]
                io += [as_u32(os_[0:2]), as_u32(os_[2:4])]
                yield 55, ie[-2:] + io[-2:]
            ul += [ie, io]
        return ul

    def b_fin(i, zz):
        r0 = i * 8
        hc = [None] + [half_coef(q) for q in range(1, 4)]
        tb = tn[pl.ds(r0, 8), :]
        for g in range(32):
            b = g // 4 + 8 * (g % 4)
            z = [gate(zz[n][8 * g:8 * g + 8]) for n in range(8)]
            z[0] = z[0] + jnp.sum(jnp.where(lane == b, tb, 0.0), axis=1, keepdims=True) * alt
            for q in range(1, 4):
                c1, c2, c3, c4 = hc[q]
                pp = z[2 * q] + z[2 * q + 1]
                qq = pltpu.roll(z[2 * q] - z[2 * q + 1], 64, 1)
                z[2 * q], z[2 * q + 1] = c1 * pp + c3 * qq, c2 * pp + c4 * qq
            y = _irfft8(z)
            outb_v[(*b_rows(i, b), slice(None))] = jnp.concatenate(y, axis=1).astype(BF)
            yield 75, y
        rows = b_rows(i, slice(None))
        start_out(outb_v.at[rows], out_hbm.at[(*rows, pl.ds(DM, DM))])

    def tie(w, vals):
        if not vals:
            return w
        acc = None
        for v in vals:
            v = v if v.dtype == U32 else pltpu.bitcast(v, U32)
            acc = v if acc is None else acc | v
        zero = cst[C_MN, 56:64, :]
        return jnp.concatenate([w[0:8] | (acc & zero), w[8:]], axis=0)

    def batch_slot(gen, budget):
        st = {'debt': 0, 'k': 0}
        due = {}

        def emit(d, b):
            while st['debt'] < b:
                r = 8 * (32 * st['debt'] // b)
                pace['tok'] = pltpu.bitcast(d[r:r + 8], U32) & cst[C_MN, 56:64, :]
                c = next(gen, MID)
                if c is MID:
                    st['debt'] = b
                elif isinstance(c, list):
                    st['debt'] = 0
                    for own in c:
                        emit(own, OPT['b_own'])
                    return
                else:
                    if isinstance(c, tuple):
                        due.setdefault(st['k'] + OPT['due'], []).extend(c[1])
                        c = c[0]
                    st['debt'] += c
            st['debt'] -= b

        def dot(a, w):
            vals = due.pop(st['k'], None)
            if vals:
                a = jnp.concatenate([tie(a[:, 0:128], vals), a[:, 128:]], axis=1)
            d = _bdot(_bf(a), _bf(w))
            st['k'] += 1
            emit(d, budget(st['k'] - 1))
            return d

        return dot

    out_cps = []

    def start_out(src, dst):
        out_cps.append(pltpu.make_async_copy(src, dst, sem_out.at[0]))
        out_cps[-1].start()

    hb = DM // 32

    def retile(j, t, k):
        blk = pl.ds(k * hb, hb)
        a, b = wqkv[j, t, blk, pl.ds(0, 8, stride=2), :], wqkv[j, t, blk, pl.ds(1, 8, stride=2), :]
        wqkv[j, t, blk, 0:8, :] = (a & jnp.uint32(0xFFFF)) | (b << 16)
        wqkv[j, t, blk, 8:16, :] = (a >> 16) | (b & jnp.uint32(0xFFFF0000))

    def strassen_lhs():
        for g in range(NSEG // 4):
            xa = [xpre_v[4 * g + k].astype(F32) for k in range(4)]
            a1, a2 = jnp.concatenate([xa[0], xa[2]], axis=0), jnp.concatenate([xa[1], xa[3]], axis=0)
            a11, a12, a21, a22 = a1[:, :DM // 2], a1[:, DM // 2:], a2[:, :DM // 2], a2[:, DM // 2:]
            for n in range(7):
                v = _strassen_left(n, lambda r, k: ((a11, a12), (a21, a22))[r][k])
                xs_v[n, 8 * g:8 * g + 8, :] = pltpu.bitcast(v.astype(BF), U32)

    def pre_step7(j, t, slot=None):
        w = lambda k, p: wqkv[j, t, k * hb:(k + 1) * hb, 8 * p:8 * p + 8, :].reshape(DM // 4, E)
        half = {}

        def done(h, c1, c2):
            half[h] = _pack2(c1, c2).reshape(NSEG // 2, 8, E)

        _strassen(lambda n: xs_v[n], lambda n: _strassen_right(n, w), done, functools.partial(retile, j, t), slot)
        pre[j, t] = jnp.stack([half[0], half[1]], axis=1).reshape(NSEG, 8, E)

    for cp in [xpre_cp] + [cp for grp in head_cps for cp in grp]:
        cp.start()
    zs[...] = jnp.zeros(zs.shape, U32)
    vv[0:8] = jnp.zeros((8,) + vv.shape[1:], F32)
    xpre_cp.wait()
    strassen_lhs()
    later = {int(k): v for k, v in OPT['later'].items()}

    def pre_fwd(steps, i, budget):
        gen = b_fwd(i)
        slot = batch_slot(gen, lambda n: budget)
        for j, t in steps + [(8 + i, t) for t in range(3)]:
            pre_step7(j, t, slot)
        for _ in gen:
            pass

    for b, grp in enumerate(head):
        last = b == len(head) - 1
        for cp in head_cps[b] + ([c0_cp] + fwd_cps(0) if last else []):
            cp.wait()
        if 'head' in OPT['skip']:
            pass
        elif last:
            pre_fwd(grp, 0, OPT['b_fwd0'])
        else:
            for j, t in grp:
                pre_step7(j, t)
        for i in later.get(b, ()):
            for cp in ([c0_cp] if i == 0 else []) + fwd_cps(i):
                cp.start()

    if not OPT['a_at']:
        for cp in a_cps + b_cps:
            cp.start()

    def pre_fwd_body(i, carry):
        for cp in fwd_cps(i):
            cp.wait()

        if OPT['a_at']:
            @pl.when(i == OPT['a_at'])
            def _():
                for cp in a_cps + b_cps:
                    cp.start()

        pre_fwd([], i, OPT['b_fwd'])
        return carry

    if 'fwd' not in OPT['skip']:
        lax.fori_loop(1, 8, pre_fwd_body, 0)
    for cp in a_cps + ([] if OPT['late_wait'] else b_cps):
        cp.wait()

    def seg_step(s, u, mem, slot):
        xs = x_v[s]
        lhs_v[u] = as_u32([mem, xs[8:32].astype(F32)])
        fill = fill_v[...]

        def proj(j, t):
            w0, w1 = [wqkv[j, t, :, 8 * p:8 * p + 8, :].reshape(DM // 2, E) for p in range(2)]
            r0, r1 = _bdot(_bf(lhs_v[u]), _bf(tie(w0, slot()))), _bdot(_bf(lhs_v[u]), _bf(w1))
            pw = pre[j, t, s]
            if t == 0:
                return jnp.concatenate([r0, r1, _unpack2(pw, 0), _unpack2(pw, 1)], axis=0).astype(BF)
            return _bf(jnp.concatenate([_pack2(r0, r1), pw], axis=0))

        def qk(q, k):
            sc = lax.dot_general(q, k, (((1,), (1,)), ((), ())), preferred_element_type=F32) * scale
            sc = jnp.where(fill == 0.0, sc, fill)
            p = jnp.exp(sc - jnp.max(sc, axis=-1, keepdims=True))
            return (p * pl.reciprocal(jnp.sum(p, axis=-1, keepdims=True), approx=True)).astype(BF)

        ob, ps, vs = {}, {}, {}

        def pv(j):
            o = _bdot(ps[j], vs[j])
            opost[u // 2, u % 2, :, pl.ds(256 * j, 128)] = o[64:72]
            opost[u // 2, u % 2, :, pl.ds(256 * j + 128, 128)] = o[72:80]
            ob[j] = [o[0:32], o[32:64]]

        def wo(g0, g1):
            og = jnp.concatenate([o for j in range(2 * g0, 2 * g1) for o in ob[j]], axis=1).astype(BF)
            return jnp.concatenate([_bdot(og, _bf(wo_v[n, g0 * 256:g1 * 256, :])) for n in range(8)], axis=1)

        ng = NP // 2
        for g in range(ng):
            ja, jb = 2 * g, 2 * g + 1
            qa, ka, qb, kb = proj(ja, 0), proj(ja, 1), proj(jb, 0), proj(jb, 1)
            vs[ja], vs[jb] = proj(ja, 2), proj(jb, 2)
            ps[ja], ps[jb] = qk(qa, ka), qk(qb, kb)
            if g > 0:
                pv(ja - 2)
                pv(jb - 2)
        res = wo(0, 3)
        pv(NP - 2)
        pv(NP - 1)
        res = res + wo(3, ng - 1)
        res = res + wo(ng - 1, ng)
        outa_v[s // 2, u % 2, 8:32, :] = res[8:32].astype(BF)
        return res[0:8].astype(BF).astype(F32)

    hk = H * E // 2

    def loop_body(it, mem):
        if OPT['late_wait']:
            @pl.when(it == 1)
            def _():
                for cp in b_cps:
                    cp.wait()

        gen = b_mid(it)
        state = {'mid': False}

        def slot():
            if state['mid']:
                return None
            vals = next(gen, None)
            if vals is MID:
                state['mid'] = True
                return None
            return vals

        for u in range(UN):
            state['mid'] = False
            mem = seg_step(UN * it + u, u, mem, slot)
        for _ in gen:
            pass
        for n in range(7):
            sums = [_strassen_left(n, lambda r, k: opost[g, r, :, k * hk:(k + 1) * hk]) for g in range(2)]
            os_v[n, pl.ds(pl.multiple_of(8 * it, 8), 8), :] = _pack2(*sums)
        return mem

    if 'main' not in OPT['skip']:
        lax.fori_loop(0, NSEG // UN, loop_body, mem0_v[...].astype(F32))
    idx = (slice(None), slice(None), pl.ds(8, SEG - 8), pl.ds(0, DM))
    start_out(outa_v.at[idx], out_hbm.at[idx])

    def b_inv_all():
        nyq = b_nyq()
        zz = None
        for i in range(9):
            if i < 8:
                gen = b_inv(i)
                try:
                    k = 0
                    while True:
                        c = next(gen)
                        k += 1
                        if k % 10 == 1:
                            next(nyq, None)
                        yield c
                except StopIteration as e:
                    ul = e.value
            if i > 0:
                yield from b_fin(i - 1, zz)
            else:
                yield MID
            if i < 8:
                zz = [_bdot(_bf(jnp.concatenate(ul[n], axis=0)), _bf(cst[C_MD + 8 + n])) for n in range(8)]
                if i == 7:
                    yield MID
                    yield MID
                else:
                    yield [zz[3], zz[7]]

    gens = [b_inv_all()]
    slot = batch_slot(gens[0], lambda k: (OPT['b_inv0'] if k < 28 else OPT['b_inv'])
                      + (OPT['b_plus'] if (k + OPT['b_sh']) % 28 < 4 or (k + OPT['b_sh']) % 28 >= 24 else 0))
    if 'post' in OPT['skip']:
        def keep(k, c):
            v = pre[k, 0, k] | zs[k, 0:8, 0:128] | wt[0, 0, pl.ds(pl.multiple_of(8 * k, 8), 8), :] | wqkv[k, 0, k, 0:8, :]
            v = pltpu.bitcast(v, F32) + tn[pl.ds(pl.multiple_of(8 * k, 8), 8), :] + vv[k, 0:8, 0:128] + pltpu.bitcast(os_v[k, 0:8, 0:128] | ws_v[k, k, 0:8, :], F32)
            outa_v[k, 0, 0:8, 0:128] = v.astype(BF)
            return c
        lax.fori_loop(0, 4, keep, 0)
        start_out(outa_v.at[:, :, pl.ds(0, 8)], out_hbm.at[:, :, pl.ds(0, 8), pl.ds(0, DM)])
        return
    for n in range(4):
        def done(r, *cs):
            for p, cc in enumerate(cs):
                u = pltpu.bitcast(cc.astype(BF), U32).reshape(NSEG // 4, 8, 128)
                y = jnp.stack([_unpack2(u, 0), _unpack2(u, 1)], axis=1).reshape(NSEG // 2, 8, 128)
                idx = (slice(None), r, pl.ds(0, 8), pl.ds(128 * (n + 4 * p), 128))
                outa_v[idx] = y.astype(BF)
                start_out(outa_v.at[idx], out_hbm.at[idx])

        right = lambda m: (wo_v[n, 0:hk // 2, :] if m == 0 else wo_v[n + 4, hk // 2:hk, :] if m == 6
                           else ws_v[n, m - 1])
        _strassen(lambda m: os_v[m], right, done, dot=slot)
    for gen in gens:
        for _ in gen:
            pass
    for cp in out_cps:
        cp.wait()


def pallas_concat_heads__memory_aug_recurrent_mem_tr__spectral_gfnet__prompt_kernel(
    A_x, A_mem0, A_Wq, A_Wk, A_Wv, A_Wo, A_seg_len, B_x, B_w_r, B_w_i,
):
    assert A_x.shape == (1, S, DM) and A_Wq.shape == (DM, H, E) and A_mem0.shape == (1, M, DM)
    assert B_x.shape == (1, S, DM) and (not isinstance(A_seg_len, int) or A_seg_len == SEG)
    hbm = pl.BlockSpec(memory_space=pltpu.HBM)
    wr = lambda w: w.reshape(DM // 16, 16, H, E)
    out = pl.pallas_call(
        _kernel,
        out_shape=jax.ShapeDtypeStruct((NSEG // 2, 2, SEG, 2 * DM), BF),
        in_specs=[hbm] * 11,
        out_specs=hbm,
        scratch_shapes=[
            pltpu.VMEM((NSEG, SEG, DM), BF),
            pltpu.VMEM((NSEG, 8, DM), BF),
            pltpu.VMEM((7, NSEG * 2, DM // 2), U32),
            pltpu.VMEM((M, DM), BF),
            pltpu.VMEM((80, 80), F32),
            pltpu.VMEM((UN, SEG // 2, DM), U32),
            pltpu.VMEM((NP, 3, DM // 16, 16, E), U32),
            pltpu.VMEM((8, H * E // 2, 128), U32),
            pltpu.VMEM((NP, 3, NSEG, 8, E), U32),
            pltpu.VMEM((2, 2, 8, H * E), F32),
            pltpu.VMEM((7, NSEG * 2, H * E // 2), U32),
            pltpu.VMEM((4, 5, H * E // 4, 128), U32),
            pltpu.VMEM((NSEG // 2, 2, SEG, DM), BF),
            pltpu.VMEM((NSEG // 2, 2, SEG, DM), BF),
            pltpu.VMEM((2, 16, 256, 128), U32),
            pltpu.VMEM((2, 1, S), BF),
            pltpu.VMEM((2, 2, 32 * WP, 128), U32),
            pltpu.VMEM((C_NUM, 64, 128), U32),
            pltpu.VMEM((32, 64, 512), U32),
            pltpu.VMEM((32, 128, 512), F32),
            pltpu.VMEM((64, 128), F32),
            pltpu.VMEM((NSEG // 2, 2, SEG, DM), BF),
            pltpu.SemaphoreType.DMA((NP + 1,)),
            pltpu.SemaphoreType.DMA((6,)),
            pltpu.SemaphoreType.DMA((1,)),
        ],
        compiler_params=pltpu.CompilerParams(vmem_limit_bytes=118 * 1024 * 1024,
                                             disable_bounds_checks=True, disable_semaphore_checks=True),
    )(A_x.reshape(NSEG, SEG, DM), A_mem0.reshape(M, DM), wr(A_Wq), wr(A_Wk), wr(A_Wv),
      A_Wo.reshape(H * E, DM), B_x.reshape(NSEG // 2, 2, SEG, DM), B_w_r.T, B_w_i.T, _mask_fill(), _fft_consts())
    return out.reshape(1, S, 2 * DM)
```

```python
import functools
import math

import jax
import jax.numpy as jnp
import numpy as np
from jax import lax
import jax.experimental.pallas as pl
import jax.experimental.pallas.tpu as pltpu

BF, F32, U32, I32 = jnp.bfloat16, jnp.float32, jnp.uint32, jnp.int32

S, DM, H, E, M, SEG = 2048, 1024, 32, 128, 8, 32
NSEG = S // SEG
NP = H // 2
UN = 4
R2 = math.sqrt(0.5)
MID = 'mid'
OPT = dict(skip=(), pad=24, a_at=0, b_fwd0=130, tie_ws=1, cuts=(0, 1, 2, 4, 7, 12, 18, 24), later={2: (0, 1), 3: (2,), 4: (3, 4, 5), 5: (6, 7)}, late_wait=1, tie8=0, b_own=300, b_plus=0, b_sh=2, due=2, b_fwd=400, b_inv0=450, b_inv=450)


def _to_u32(m):
    u = np.ascontiguousarray(m, dtype=np.float32).view(np.uint32)
    h = ((u + 0x7FFF + ((u >> 16) & 1)) >> 16).astype(np.uint32)
    return h[..., 0::2, :] | (h[..., 1::2, :] << 16)


def _mask_fill():
    r = np.arange(80)
    pos_of = lambda rr: np.where(rr < M, rr, np.where(rr < SEG, rr + M, rr - SEG + M))
    qhead = np.where(r < 64, r // 32, (r - 64) // 8)
    qpos = pos_of(np.where(r < 64, r % 32, SEG + (r - 64) % 8))
    khead, kpos = qhead, qpos
    vis = (qpos[:, None] < M) | (qpos[:, None] >= kpos[None, :])
    same = qhead[:, None] == khead[None, :]
    return np.where(same, np.where(vis, 0.0, -1e9), -np.inf).astype(np.float32)


RES = ((0, 12, 8, 4), (1, 15, 9, 7), (2, 14, 10, 6), (3, 13, 11, 5))
WP = 72
C_MD, C_MN, C_TW, C_MS, C_NUM = 0, 16, 22, 24, 88


@functools.lru_cache(maxsize=None)
def _fft_consts():
    md = np.zeros((16, 128, 128))
    for q in range(4):
        if q == 0:
            lay = [[(0, 0), (0, 1), (2, 0), (2, 1)], [(3, 1), (1, 0), (1, 1), (3, 0)]]
        else:
            lay = [[(0, 0), (1, 0), (0, 1), (1, 1)], [(2, 1), (3, 1), (2, 0), (3, 0)]]
        for h in range(2):
            ms_, ws_ = [], []
            for g, part in lay[h]:
                k = 16 * np.arange(32) + RES[q][g]
                th = 2 * np.pi * np.outer(np.arange(128 if q == 0 else 64), k) / DM
                c, s = np.cos(th), np.sin(th)
                if q == 0:
                    ms_.append(-s if part else c)
                else:
                    sg = (1.0 if RES[q][g] % 8 == q else -1.0) * (1.0 - 2.0 * h)
                    ms_.append(np.concatenate([-s, sg * c] if part else [c, sg * s]))
                ws_.append(np.where(k == 0, 1.0, 2.0) / DM)
            m = np.concatenate(ms_, axis=1)
            md[2 * q + h] = m
            md[8 + 2 * q + h] = (m * np.concatenate(ws_)[None, :]).T
    a, l = np.arange(64), np.arange(128)
    re = 16 * (a // 8) + a % 8
    im = re + 8
    ms = np.zeros((64, 128, 128))
    for dl in range(32):
        th = 2 * np.pi * np.outer(32 * a + dl, a) / S
        c, s = np.cos(th), np.sin(th)
        ms[2 * dl][:, re], ms[2 * dl][:, im] = np.concatenate([c, -s]), np.concatenate([s, c])
        ms[2 * dl + 1][:, re] = np.concatenate([c.T, s.T]) / S
        ms[2 * dl + 1][:, im] = np.concatenate([-s.T, c.T]) / S
    mn = np.zeros((6, 128, 128))
    th = 2 * np.pi * np.outer(np.arange(32), l) / 32
    mn[0, :32], mn[1, :32] = np.cos(th), -np.sin(th)
    mn[4, :, :32], mn[5, :, :32] = np.cos(th).T / DM, -np.sin(th).T / DM
    th = 2 * np.pi * np.outer(np.arange(16), a) / 16
    c, s = np.cos(th), np.sin(th)
    mn[2, :32] = np.block([[c, s], [-s, c]])
    mn[3, :, :32] = np.block([[c.T, -s.T], [s.T, c.T]]) / S
    th = 2 * np.pi * np.outer(a, l) / S
    tw = np.stack([np.cos(th), np.sin(th)]).astype(np.float32).view(np.uint32)
    return np.concatenate([_to_u32(md), _to_u32(mn), tw, _to_u32(ms)], axis=0)


def _bdot(a, b):
    return jnp.dot(a, b, preferred_element_type=F32)


def _bf(u):
    return pltpu.bitcast(u, BF)


def _cat(rows):
    return jnp.concatenate(rows, axis=0).astype(BF)


def _unpack2(u, p):
    if p == 0:
        return pltpu.bitcast(u << 16, F32)
    return pltpu.bitcast(u & jnp.uint32(0xFFFF0000), F32)


def _strassen_left(n, a):
    return (lambda: a(1, 0) + a(1, 1), lambda: a(1, 0) - a(0, 0), lambda: a(1, 1), lambda: a(0, 0) + a(1, 1),
            lambda: a(0, 0), lambda: a(0, 1) - a(1, 1), lambda: a(0, 0) + a(0, 1))[n]()


def _strassen_right(n, w):
    add = lambda u, v: (u.astype(F32) + v.astype(F32)).astype(BF)
    sub = lambda u, v: (u.astype(F32) - v.astype(F32)).astype(BF)
    return (lambda: w(0, 0), lambda: add(w(0, 0), w(0, 1)), lambda: sub(w(1, 0), w(0, 0)),
            lambda: add(w(0, 0), w(1, 1)), lambda: sub(w(0, 1), w(1, 1)), lambda: add(w(1, 0), w(1, 1)),
            lambda: w(1, 1))[n]()


def _strassen(left, right, done, ready=lambda k: None, dot=None):
    def mm(n):
        a, r, acc = left(n), right(n), None
        for k in range(0, r.shape[0], 512):
            d = (dot or _bdot)(a[:, k:k + 512], r[k:k + 512])
            acc = d if acc is None else acc + d
        return acc

    ready(0)
    m2 = mm(0)
    c22 = mm(1) - m2
    ready(1)
    m4 = mm(2)
    c21 = m2 + m4
    m1 = mm(3)
    c11, c22 = m1 + m4, c22 + m1
    m3 = mm(4)
    done(1, c21, c22 + m3)
    c11 = c11 + mm(5)
    m5 = mm(6)
    done(0, c11 - m5, m3 + m5)


def _twiddle(z, k, n, sign):
    r, i = z
    if k == 0:
        return r, i
    if 4 * k == n:
        return (-i, r) if sign > 0 else (i, -r)
    c, s = math.cos(2 * math.pi * k / n), sign * math.sin(2 * math.pi * k / n)
    if 8 * k == n or 8 * k == 3 * n:
        if c * s > 0:
            return (r - i) * c, (r + i) * c
        return (r + i) * c, (i - r) * c
    return r * c - i * s, r * s + i * c


def _cfft(xs, sign):
    n = len(xs)
    if n == 1:
        return xs
    ev, od = _cfft(xs[0::2], sign), _cfft(xs[1::2], sign)
    out = [None] * n
    for k in range(n // 2):
        er, ei = ev[k]
        if 4 * k == n:
            orr, oi = od[k]
            lo, hi = (er - oi, ei + orr), (er + oi, ei - orr)
            out[k], out[k + n // 2] = (lo, hi) if sign > 0 else (hi, lo)
        else:
            tr, ti = _twiddle(od[k], k, n, sign)
            out[k], out[k + n // 2] = (er + tr, ei + ti), (er - tr, ei - ti)
    return out


def _rfft8(x):
    a0, a1, b0, b1 = x[0] + x[4], x[0] - x[4], x[2] + x[6], x[2] - x[6]
    c0, c1, d0, d1 = x[1] + x[5], x[1] - x[5], x[3] + x[7], x[3] - x[7]
    e, f = a0 + b0, c0 + d0
    g, h = (c1 - d1) * R2, (c1 + d1) * R2
    return [e + f, e - f, a1 + g, b1 + h, a0 - b0, c0 - d0, a1 - g, b1 - h]


def _irfft8(z):
    z0, z4, z1r, z1i, z2r, z2i, z3r, z3i = z
    e, f = z0 + z4, z0 - z4
    a1, g = z1r + z3r, (z1r - z3r) * R2
    b1, h = z1i + z3i, (z1i - z3i) * R2
    a0, b0, c0, d0 = e + z2r, e - z2r, f + z2i, f - z2i
    c1, d1 = g + h, h - g
    return [a0 + a1, c0 + c1, b0 + b1, d0 + d1, a0 - a1, c0 - c1, b0 - b1, d0 - d1]


def _kernel(x_hbm, mem0_hbm, wq_hbm, wk_hbm, wv_hbm, wo_hbm, bx_hbm, wr_hbm, wi_hbm, fill_hbm, cst_hbm,
            out_hbm,
            x_v, xpre_v, xs_v, mem0_v, fill_v, lhs_v, wqkv, wo_v, pre, opost, os_v, ws_v, outa_v,
            bx_v, w_v, wn_v, wt, cst, zs, vv, tn, outb_v,
            sem_w, sem_in, sem_out):
    scale = E ** -0.5
    wus = [w.bitcast(U32) for w in (wq_hbm, wk_hbm, wv_hbm)]
    wo_u = wo_hbm.bitcast(U32)
    fus = [w.at[pl.ds(0, 512)].bitcast(U32) for w in (wr_hbm, wi_hbm)]

    def w_copy(j, t, sem):
        return pltpu.make_async_copy(wus[t].at[:, :, j, :], wqkv.at[j, t], sem)

    xpre_cp = pltpu.make_async_copy(x_hbm.at[:, pl.ds(0, 8), :], xpre_v, sem_w.at[7])
    cuts = OPT['cuts']
    head = [[divmod(f, 3) for f in range(cuts[b], cuts[b + 1])] for b in range(len(cuts) - 1)]
    head_cps = [[w_copy(j, t, sem_w.at[b]) for j, t in grp] for b, grp in enumerate(head)]

    def b_rows(i, b):
        return b, i // 4, pl.ds(pl.multiple_of((i % 4) * 8, 8), 8)

    def fwd_cps(i):
        rows = b_rows(i, slice(None))
        return [w_copy(8 + i, t, sem_w.at[8 + i]) for t in range(3)] + [pltpu.make_async_copy(bx_hbm.at[rows], bx_v.at[rows], sem_w.at[8 + i])] + [
            pltpu.make_async_copy(fus[t].at[:, pl.ds(pl.multiple_of(128 * (2 * i + h), 128), 128)],
                                  w_v.at[t, 2 * i + h], sem_w.at[8 + i]) for t in range(2) for h in range(2)]

    def part(src, dst, lo, hi, sem):
        return pltpu.make_async_copy(src.at[pl.ds(lo, hi - lo)], dst.at[pl.ds(lo, hi - lo)], sem)

    c0_cp = part(cst_hbm, cst, 0, C_MS, sem_w.at[16])
    a_cps = [pltpu.make_async_copy(wo_u.at[:, pl.ds(128 * n, 128)], wo_v.at[n], sem_in.at[1]) for n in range(8)]
    a_cps += [part(x_hbm, x_v, 0, UN, sem_in.at[1]), part(cst_hbm, cst, C_MS, C_MS + UN, sem_in.at[1]),
              pltpu.make_async_copy(mem0_hbm, mem0_v, sem_in.at[1]),
              pltpu.make_async_copy(fill_hbm, fill_v, sem_in.at[1])]
    b_cps = [part(x_hbm, x_v, UN, NSEG, sem_in.at[2]), part(cst_hbm, cst, C_MS + UN, C_NUM, sem_in.at[2])]
    b_cps += [pltpu.make_async_copy(w.at[pl.ds(512, 1)], wn_v.at[t], sem_in.at[2])
              for t, w in enumerate((wr_hbm, wi_hbm))]

    lane = lax.broadcasted_iota(I32, (8, 128), 1)
    alt = jnp.where(lane % 2 == 0, 1.0, -1.0).astype(F32)
    lo_half = lane < 64
    ev_grp = (lane // 32) % 2 == 0

    def half_coef(q):
        sg = -1.0 if q < 3 else 1.0
        tc, ts = math.cos(2 * math.pi * q / 16), -math.sin(2 * math.pi * q / 16)
        f = lambda lo, hi: jnp.where(lo_half, lo, hi).astype(F32)
        return f(1.0, ts), f(0.0, sg * tc), f(0.0, tc), f(sg, -sg * ts)

    pace = {'tok': None}

    def gate(v):
        tok = pace['tok']
        if tok is None:
            return v
        return v | tok if v.dtype == U32 else pltpu.bitcast(pltpu.bitcast(v, U32) | tok, v.dtype)

    def gate2(z):
        return gate(z[0]), gate(z[1])

    def flat(zs_):
        return [v for z in zs_ for v in z]

    def as_u32(rows):
        return pltpu.bitcast(jnp.concatenate(rows, axis=0).astype(BF), U32)

    def b_fwd(i):
        r0 = pl.multiple_of(i * 8, 8)
        hc = [None] + [half_coef(q) for q in range(1, 4)]
        tacc = jnp.zeros((8, 128), F32)
        zl = []
        for b0 in range(0, 32, 2):
            rows = []
            for b in (b0, b0 + 1):
                xb = bx_v[(*b_rows(i, b), slice(None))].astype(F32)
                z = _rfft8([gate(xb[:, 128 * t:128 * t + 128]) for t in range(8)])
                tacc = jnp.where(lane == b, jnp.sum(z[0] * alt, axis=1, keepdims=True), tacc)
                for q in range(1, 4):
                    c1, c2, c3, c4 = hc[q]
                    zr, zi = z[2 * q], z[2 * q + 1]
                    pp = c1 * zr + c2 * zi
                    qq = pltpu.roll(c3 * zr + c4 * zi, 64, 1)
                    z[2 * q], z[2 * q + 1] = pp + qq, pp - qq
                rows.append(z)
            zl.append([as_u32([rows[0][n], rows[1][n]]) for n in range(8)])
            yield 200
            if b0 % 4 == 0:
                e, t, ty = 2 * i + b0 // 16, (b0 // 8) % 2, (b0 // 4) % 2
                u = jnp.concatenate([gate(w_v[t, e, pl.ds(m + ty + 64 * v, 8, stride=8), :])
                                     for m in (0, 6, 4, 2) for v in range(4)], axis=0)
                ut = pltpu.bitcast(pltpu.bitcast(u, F32).T, U32)
                for v in range(16):
                    wt[t, ty, pl.ds(8 * (v % 4) * WP + 4 * e + v // 4, 8, stride=WP), :] = ut[8 * v:8 * v + 8]
                yield 40
        tn[pl.ds(r0, 8), :] = tacc

        def mm(n):
            return _bdot(_bf(jnp.concatenate([z[n] for z in zl], axis=0)), _bf(cst[C_MD + n]))

        yield MID
        oo = [mm(n) for n in range(4)]
        yield MID
        oo += [mm(n) for n in range(4, 8)]
        yield MID
        for q in range(4):
            sel, sh = (ev_grp, 96) if q == 0 else (lo_half, 64)
            ys = []
            for b0 in range(4):
                xs = []
                for b in range(b0, 32, 4):
                    e_, o_ = gate(oo[2 * q][8 * b:8 * b + 8]), oo[2 * q + 1][8 * b:8 * b + 8]
                    xs.append((jnp.where(sel, e_, o_), pltpu.roll(jnp.where(sel, o_, e_), sh, 1)))
                ys.append([_twiddle(y, b0 * k1, 32, -1) for k1, y in enumerate(_cfft(xs, -1))])
                yield 110
            for k1 in range(8):
                for k0, y in enumerate(_cfft([gate2(ys[b0][k1]) for b0 in range(4)], -1)):
                    zs[k1 + 8 * k0, q, pl.ds(pl.multiple_of(2 * r0, 16), 16), :] = _cat(y)
                yield 30

    def b_mid(it):
        if UN > 2:
            rows = H * E // 4 // (NSEG // UN)
            for n in range(4):
                for r in range(0, rows, 8):
                    blk = lambda k, p: _bf(
                        wo_v[n + 4 * p, pl.ds(pl.multiple_of(k * (H * E // 4) + it * rows + r, 8), 8), :])
                    vals = [pltpu.bitcast(_strassen_right(m, blk), U32) for m in range(1, 6)]
                    for m in range(5):
                        ws_v[n, m, pl.ds(pl.multiple_of(it * rows + r, 8), 8), :] = vals[m]
                    yield vals if OPT['tie_ws'] and 8 * n + r // 8 > 1 else None
            yield MID
        else:
            for _ in range(6):
                yield None
        for n in range(UN // 2):
            dl = (UN // 2) * it + n
            y = _bdot(_bf(cst[C_MS + 2 * dl]), jnp.concatenate([zs[dl, q] for q in range(4)], axis=1))
            for _ in range(4):
                yield None
            w0 = pl.multiple_of(dl * WP, 8)
            rows = []
            for r in range(8):
                wq = []
                for t in range(2):
                    ta, tb = wt[t, 0, pl.ds(w0 + 8 * r, 8), :], wt[t, 1, pl.ds(w0 + 8 * r, 8), :]
                    wq.append([_unpack2(ta, 0), _unpack2(jnp.where(ev_grp, ta, tb), 1),
                               _unpack2(tb, 0), _unpack2(jnp.where(ev_grp, tb, ta), 1)])
                cols = []
                for q in range(4):
                    yr = y[8 * r:8 * r + 8, 128 * q:128 * q + 128]
                    yi = y[64 + 8 * r:72 + 8 * r, 128 * q:128 * q + 128]
                    wr, wi = wq[0][q], wq[1][q]
                    cols.append(as_u32([yr * wr - yi * wi, yr * wi + yi * wr]))
                rows.append(jnp.concatenate(cols, axis=1))
                yield cols
                yield None
            yield MID
            vv[dl] = _bdot(_bf(cst[C_MS + 2 * dl + 1]), _bf(jnp.concatenate(rows, axis=0)))

    def b_nyq():
        c, s = pltpu.bitcast(cst[C_TW], F32), pltpu.bitcast(cst[C_TW + 1], F32)
        tb = tn[...].astype(BF)
        tr, ti = _bdot(tb, _bf(cst[C_MN])), _bdot(tb, _bf(cst[C_MN + 1]))
        yield MID
        y = _bdot(_bf(cst[C_MN + 2, 0:16, :]), _cat([tr * c + ti * s, ti * c - tr * s]))
        row = lax.broadcasted_iota(I32, (16, 128), 0)
        wn = []
        for t in range(2):
            wrow = wn_v[t].astype(F32)
            acc = jnp.zeros((16, 128), F32)
            for e in range(16):
                acc = jnp.where(row == e, wrow[:, 128 * e:128 * e + 128], acc)
            wn.append(acc)
        yr, yi = y[0:16], y[16:32]
        yield MID
        v = _bdot(_bf(cst[C_MN + 3, :, 0:32]), _cat([yr * wn[0] - yi * wn[1], yr * wn[1] + yi * wn[0]]))
        vr, vi = v[0:64], v[64:128]
        yield MID
        tn[...] = (_bdot((vr * c - vi * s).astype(BF), _bf(cst[C_MN + 4]))
                   + _bdot((vr * s + vi * c).astype(BF), _bf(cst[C_MN + 5])))

    def b_inv(i):
        r0 = i * 8
        ul = []
        for q in range(4):
            sel, sh = (ev_grp, 32) if q == 0 else (lo_half, 64)
            ys = []
            for b0 in range(4):
                xs = [(gate(vv[dl, pl.ds(r0, 8), 128 * q:128 * q + 128]),
                       gate(vv[dl, pl.ds(64 + r0, 8), 128 * q:128 * q + 128])) for dl in range(b0, 32, 4)]
                ys.append([_twiddle(y, b0 * k1, 32, +1) for k1, y in enumerate(_cfft(xs, +1))])
                yield (120, flat(ys[-1])) if OPT['tie8'] else 110
            ie, io = [], []
            for k1 in range(8):
                es, os_ = [], []
                for ur, ui in _cfft([gate2(ys[b0][k1]) for b0 in range(4)], +1):
                    tmp = pltpu.roll(ui, sh, 1)
                    es.append(jnp.where(sel, ur, tmp))
                    os_.append(jnp.where(sel, tmp, ur))
                ie += [as_u32(es[0:2]), as_u32(es[2:4])]
                io += [as_u32(os_[0:2]), as_u32(os_[2:4])]
                yield 55, ie[-2:] + io[-2:]
            ul += [ie, io]
        return ul

    def b_fin(i, zz):
        r0 = i * 8
        hc = [None] + [half_coef(q) for q in range(1, 4)]
        tb = tn[pl.ds(r0, 8), :]
        for g in range(32):
            b = g // 4 + 8 * (g % 4)
            z = [gate(zz[n][8 * g:8 * g + 8]) for n in range(8)]
            z[0] = z[0] + jnp.sum(jnp.where(lane == b, tb, 0.0), axis=1, keepdims=True) * alt
            for q in range(1, 4):
                c1, c2, c3, c4 = hc[q]
                pp = z[2 * q] + z[2 * q + 1]
                qq = pltpu.roll(z[2 * q] - z[2 * q + 1], 64, 1)
                z[2 * q], z[2 * q + 1] = c1 * pp + c3 * qq, c2 * pp + c4 * qq
            y = _irfft8(z)
            outb_v[(*b_rows(i, b), slice(None))] = jnp.concatenate(y, axis=1).astype(BF)
            yield 75, y
        rows = b_rows(i, slice(None))
        start_out(outb_v.at[rows], out_hbm.at[(*rows, pl.ds(DM, DM))])

    def tie(w, vals):
        if not vals:
            return w
        acc = None
        for v in vals:
            v = v if v.dtype == U32 else pltpu.bitcast(v, U32)
            acc = v if acc is None else acc | v
        zero = cst[C_MN, 56:64, :]
        return jnp.concatenate([w[0:8] | (acc & zero), w[8:]], axis=0)

    def batch_slot(gen, budget):
        st = {'debt': 0, 'k': 0}
        due = {}

        def emit(d, b):
            while st['debt'] < b:
                r = 8 * (32 * st['debt'] // b)
                pace['tok'] = pltpu.bitcast(d[r:r + 8], U32) & cst[C_MN, 56:64, :]
                c = next(gen, MID)
                if c is MID:
                    st['debt'] = b
                elif isinstance(c, list):
                    st['debt'] = 0
                    for own in c:
                        emit(own, OPT['b_own'])
                    return
                else:
                    if isinstance(c, tuple):
                        due.setdefault(st['k'] + OPT['due'], []).extend(c[1])
                        c = c[0]
                    st['debt'] += c
            st['debt'] -= b

        def dot(a, w):
            vals = due.pop(st['k'], None)
            if vals:
                a = jnp.concatenate([_bf(tie(pltpu.bitcast(a[:, 0:128], U32), vals)), a[:, 128:]], axis=1)
            d = _bdot(a, w)
            st['k'] += 1
            emit(d, budget(st['k'] - 1))
            return d

        return dot

    out_cps = []

    def start_out(src, dst):
        out_cps.append(pltpu.make_async_copy(src, dst, sem_out.at[0]))
        out_cps[-1].start()

    hb = DM // 32

    def retile(j, t, k):
        blk = pl.ds(k * hb, hb)
        a, b = wqkv[j, t, blk, pl.ds(0, 8, stride=2), :], wqkv[j, t, blk, pl.ds(1, 8, stride=2), :]
        wqkv[j, t, blk, 0:8, :] = (a & jnp.uint32(0xFFFF)) | (b << 16)
        wqkv[j, t, blk, 8:16, :] = (a >> 16) | (b & jnp.uint32(0xFFFF0000))

    def strassen_lhs():
        for g in range(NSEG // 4):
            xa = [xpre_v[4 * g + k].astype(F32) for k in range(4)]
            a1, a2 = jnp.concatenate([xa[0], xa[2]], axis=0), jnp.concatenate([xa[1], xa[3]], axis=0)
            a11, a12, a21, a22 = a1[:, :DM // 2], a1[:, DM // 2:], a2[:, :DM // 2], a2[:, DM // 2:]
            for n in range(7):
                v = _strassen_left(n, lambda r, k: ((a11, a12), (a21, a22))[r][k])
                xs_v[n, 8 * g:8 * g + 8, :] = pltpu.bitcast(v.astype(BF), U32)

    def pre_step7(j, t, slot=None):
        w = lambda k, p: _bf(wqkv[j, t, k * hb:(k + 1) * hb, 8 * p:8 * p + 8, :].reshape(DM // 4, E))

        def done(h, c1, c2):
            pre[j, t, :, h] = jnp.concatenate([c.reshape(NSEG // 2, 8, E) for c in (c1, c2)], axis=1).astype(BF)

        _strassen(lambda n: _bf(xs_v[n]), lambda n: _strassen_right(n, w), done, functools.partial(retile, j, t), slot)

    for cp in [xpre_cp] + [cp for grp in head_cps for cp in grp]:
        cp.start()
    vv[0:OPT['pad']] = jnp.zeros((OPT['pad'],) + vv.shape[1:], F32)
    xpre_cp.wait()
    strassen_lhs()
    later = {int(k): v for k, v in OPT['later'].items()}

    def pre_fwd(steps, i, budget):
        gen = b_fwd(i)
        slot = batch_slot(gen, lambda n: budget)
        for j, t in steps + [(8 + i, t) for t in range(3)]:
            pre_step7(j, t, slot)
        for _ in gen:
            pass

    for b, grp in enumerate(head):
        last = b == len(head) - 1
        for cp in head_cps[b] + ([c0_cp] + fwd_cps(0) if last else []):
            cp.wait()
        if 'head' in OPT['skip']:
            pass
        elif last:
            pre_fwd(grp, 0, OPT['b_fwd0'])
        else:
            for j, t in grp:
                pre_step7(j, t)
        for i in later.get(b, ()):
            for cp in ([c0_cp] if i == 0 else []) + fwd_cps(i):
                cp.start()

    if not OPT['a_at']:
        for cp in a_cps + b_cps:
            cp.start()

    def pre_fwd_body(i, carry):
        for cp in fwd_cps(i):
            cp.wait()

        if OPT['a_at']:
            @pl.when(i == OPT['a_at'])
            def _():
                for cp in a_cps + b_cps:
                    cp.start()

        pre_fwd([], i, OPT['b_fwd'])
        return carry

    if 'fwd' not in OPT['skip']:
        lax.fori_loop(1, 8, pre_fwd_body, 0)
    for cp in a_cps + ([] if OPT['late_wait'] else b_cps):
        cp.wait()

    def seg_step(s, u, mem, slot):
        xs = x_v[s]
        lhs_v[u] = as_u32([mem, xs[8:32].astype(F32)])
        fill = fill_v[...]

        def proj(j, t):
            w0, w1 = [wqkv[j, t, :, 8 * p:8 * p + 8, :].reshape(DM // 2, E) for p in range(2)]
            r0, r1 = _bdot(_bf(lhs_v[u]), _bf(tie(w0, slot()))), _bdot(_bf(lhs_v[u]), _bf(w1))
            return _cat([r0, r1, pre[j, t, s // 2, u % 2].astype(F32)])

        def qk(q, k):
            sc = lax.dot_general(q, k, (((1,), (1,)), ((), ())), preferred_element_type=F32) * scale
            sc = jnp.where(fill == 0.0, sc, fill)
            p = jnp.exp(sc - jnp.max(sc, axis=-1, keepdims=True))
            return (p * pl.reciprocal(jnp.sum(p, axis=-1, keepdims=True), approx=True)).astype(BF)

        ob, ps, vs = {}, {}, {}

        def pv(j):
            o = _bdot(ps[j], vs[j])
            opost[u // 2, u % 2, :, pl.ds(256 * j, 128)] = o[64:72]
            opost[u // 2, u % 2, :, pl.ds(256 * j + 128, 128)] = o[72:80]
            ob[j] = [o[0:32], o[32:64]]

        def wo(g0, g1):
            og = jnp.concatenate([o for j in range(2 * g0, 2 * g1) for o in ob[j]], axis=1).astype(BF)
            return jnp.concatenate([_bdot(og, _bf(wo_v[n, g0 * 256:g1 * 256, :])) for n in range(8)], axis=1)

        ng = NP // 2
        for g in range(ng):
            ja, jb = 2 * g, 2 * g + 1
            qa, ka, qb, kb = proj(ja, 0), proj(ja, 1), proj(jb, 0), proj(jb, 1)
            vs[ja], vs[jb] = proj(ja, 2), proj(jb, 2)
            ps[ja], ps[jb] = qk(qa, ka), qk(qb, kb)
            if g > 0:
                pv(ja - 2)
                pv(jb - 2)
        res = wo(0, 3)
        pv(NP - 2)
        pv(NP - 1)
        res = res + wo(3, ng - 1)
        res = res + wo(ng - 1, ng)
        outa_v[s // 2, u % 2, 8:32, :] = res[8:32].astype(BF)
        return res[0:8].astype(BF).astype(F32)

    hk = H * E // 2

    def loop_body(it, mem):
        if OPT['late_wait']:
            @pl.when(it == 1)
            def _():
                for cp in b_cps:
                    cp.wait()

        gen = b_mid(it)
        state = {'mid': False}

        def slot():
            if state['mid']:
                return None
            vals = next(gen, None)
            if vals is MID:
                state['mid'] = True
                return None
            return vals

        for u in range(UN):
            state['mid'] = False
            mem = seg_step(UN * it + u, u, mem, slot)
        for _ in gen:
            pass
        for n in range(7):
            sums = [_strassen_left(n, lambda r, k: opost[g, r, :, k * hk:(k + 1) * hk]) for g in range(2)]
            os_v[n, pl.ds(pl.multiple_of(8 * it, 8), 8), :] = as_u32(sums)
        return mem

    if 'main' not in OPT['skip']:
        lax.fori_loop(0, NSEG // UN, loop_body, mem0_v[...].astype(F32))
    idx = (slice(None), slice(None), pl.ds(8, SEG - 8), pl.ds(0, DM))
    start_out(outa_v.at[idx], out_hbm.at[idx])

    def b_inv_all():
        nyq = b_nyq()
        zz = None
        for i in range(9):
            if i < 8:
                gen = b_inv(i)
                try:
                    k = 0
                    while True:
                        c = next(gen)
                        k += 1
                        if k % 10 == 1:
                            next(nyq, None)
                        yield c
                except StopIteration as e:
                    ul = e.value
            if i > 0:
                yield from b_fin(i - 1, zz)
            else:
                yield MID
            if i < 8:
                zz = [_bdot(_bf(jnp.concatenate(ul[n], axis=0)), _bf(cst[C_MD + 8 + n])) for n in range(8)]
                if i == 7:
                    yield MID
                    yield MID
                else:
                    yield [zz[3], zz[7]]

    gens = [b_inv_all()]
    slot = batch_slot(gens[0], lambda k: (OPT['b_inv0'] if k < 28 else OPT['b_inv'])
                      + (OPT['b_plus'] if (k + OPT['b_sh']) % 28 < 4 or (k + OPT['b_sh']) % 28 >= 24 else 0))
    if 'post' in OPT['skip']:
        def keep(k, c):
            v = pltpu.bitcast(pre[k, 0, k, 0], U32) | pltpu.bitcast(zs[k, 0, 0:16, :], U32) | wt[0, 0, pl.ds(pl.multiple_of(8 * k, 8), 8), :] | wqkv[k, 0, k, 0:8, :]
            v = pltpu.bitcast(v, F32) + tn[pl.ds(pl.multiple_of(8 * k, 8), 8), :] + vv[k, 0:8, 0:128] + pltpu.bitcast(os_v[k, 0:8, 0:128] | ws_v[k, k, 0:8, :], F32)
            outa_v[k, 0, 0:8, 0:128] = v.astype(BF)
            return c
        lax.fori_loop(0, 4, keep, 0)
        start_out(outa_v.at[:, :, pl.ds(0, 8)], out_hbm.at[:, :, pl.ds(0, 8), pl.ds(0, DM)])
        return
    for n in range(4):
        def done(r, *cs):
            for p, cc in enumerate(cs):
                idx = (slice(None), r, pl.ds(0, 8), pl.ds(128 * (n + 4 * p), 128))
                outa_v[idx] = cc.reshape(NSEG // 2, 8, 128).astype(BF)
                start_out(outa_v.at[idx], out_hbm.at[idx])

        right = lambda m: _bf(wo_v[n, 0:hk // 2, :] if m == 0 else wo_v[n + 4, hk // 2:hk, :] if m == 6
                              else ws_v[n, m - 1])
        _strassen(lambda m: _bf(os_v[m]), right, done, dot=slot)
    for gen in gens:
        for _ in gen:
            pass
    for cp in out_cps:
        cp.wait()


def pallas_concat_heads__memory_aug_recurrent_mem_tr__spectral_gfnet__prompt_kernel(
    A_x, A_mem0, A_Wq, A_Wk, A_Wv, A_Wo, A_seg_len, B_x, B_w_r, B_w_i,
):
    assert A_x.shape == (1, S, DM) and A_Wq.shape == (DM, H, E) and A_mem0.shape == (1, M, DM)
    assert B_x.shape == (1, S, DM) and (not isinstance(A_seg_len, int) or A_seg_len == SEG)
    hbm = pl.BlockSpec(memory_space=pltpu.HBM)
    wr = lambda w: w.reshape(DM // 16, 16, H, E)
    out = pl.pallas_call(
        _kernel,
        out_shape=jax.ShapeDtypeStruct((NSEG // 2, 2, SEG, 2 * DM), BF),
        in_specs=[hbm] * 11,
        out_specs=hbm,
        scratch_shapes=[
            pltpu.VMEM((NSEG, SEG, DM), BF),
            pltpu.VMEM((NSEG, 8, DM), BF),
            pltpu.VMEM((7, NSEG * 2, DM // 2), U32),
            pltpu.VMEM((M, DM), BF),
            pltpu.VMEM((80, 80), F32),
            pltpu.VMEM((UN, SEG // 2, DM), U32),
            pltpu.VMEM((NP, 3, DM // 16, 16, E), U32),
            pltpu.VMEM((8, H * E // 2, 128), U32),
            pltpu.VMEM((NP, 3, NSEG // 2, 2, 16, E), BF),
            pltpu.VMEM((2, 2, 8, H * E), F32),
            pltpu.VMEM((7, NSEG * 2, H * E // 2), U32),
            pltpu.VMEM((4, 5, H * E // 4, 128), U32),
            pltpu.VMEM((NSEG // 2, 2, SEG, DM), BF),
            pltpu.VMEM((NSEG // 2, 2, SEG, DM), BF),
            pltpu.VMEM((2, 16, 256, 128), U32),
            pltpu.VMEM((2, 1, S), BF),
            pltpu.VMEM((2, 2, 32 * WP, 128), U32),
            pltpu.VMEM((C_NUM, 64, 128), U32),
            pltpu.VMEM((32, 4, 128, 128), BF),
            pltpu.VMEM((32, 128, 512), F32),
            pltpu.VMEM((64, 128), F32),
            pltpu.VMEM((NSEG // 2, 2, SEG, DM), BF),
            pltpu.SemaphoreType.DMA((NP + 1,)),
            pltpu.SemaphoreType.DMA((6,)),
            pltpu.SemaphoreType.DMA((1,)),
        ],
        compiler_params=pltpu.CompilerParams(vmem_limit_bytes=118 * 1024 * 1024,
                                             disable_bounds_checks=True, disable_semaphore_checks=True),
    )(A_x.reshape(NSEG, SEG, DM), A_mem0.reshape(M, DM), wr(A_Wq), wr(A_Wk), wr(A_Wv),
      A_Wo.reshape(H * E, DM), B_x.reshape(NSEG // 2, 2, SEG, DM), B_w_r.T, B_w_i.T, _mask_fill(), _fft_consts())
    return out.reshape(1, S, 2 * DM)
```

```python
import functools
import math

import jax
import jax.numpy as jnp
import numpy as np
from jax import lax
import jax.experimental.pallas as pl
import jax.experimental.pallas.tpu as pltpu

BF, F32, U32, I32 = jnp.bfloat16, jnp.float32, jnp.uint32, jnp.int32

S, DM, H, E, M, SEG = 2048, 1024, 32, 128, 8, 32
NSEG = S // SEG
NP = H // 2
UN = 4
R2 = math.sqrt(0.5)
MID = 'mid'
OPT = dict(skip=(), gate_main=4, tie_os=0, prev=2, tie_p=1, pad=24, a_at=0, b_fwd0=130, tie_ws=1, cuts=(0, 1, 2, 4, 7, 12, 18, 24), later={2: (0, 1), 3: (2,), 4: (3, 4, 5), 5: (6, 7)}, late_wait=1, tie8=0, b_own=300, b_plus=0, b_sh=2, due=2, b_fwd=400, b_inv0=450, b_inv=450)


def _to_u32(m):
    u = np.ascontiguousarray(m, dtype=np.float32).view(np.uint32)
    h = ((u + 0x7FFF + ((u >> 16) & 1)) >> 16).astype(np.uint32)
    return h[..., 0::2, :] | (h[..., 1::2, :] << 16)


def _mask_fill():
    r = np.arange(80)
    pos_of = lambda rr: np.where(rr < M, rr, np.where(rr < SEG, rr + M, rr - SEG + M))
    qhead = np.where(r < 64, r // 32, (r - 64) // 8)
    qpos = pos_of(np.where(r < 64, r % 32, SEG + (r - 64) % 8))
    khead, kpos = qhead, qpos
    vis = (qpos[:, None] < M) | (qpos[:, None] >= kpos[None, :])
    same = qhead[:, None] == khead[None, :]
    return np.where(same, np.where(vis, 0.0, -1e9), -np.inf).astype(np.float32)


RES = ((0, 12, 8, 4), (1, 15, 9, 7), (2, 14, 10, 6), (3, 13, 11, 5))
WP = 72
C_MD, C_MN, C_TW, C_MS, C_NUM = 0, 16, 22, 24, 88


@functools.lru_cache(maxsize=None)
def _fft_consts():
    md = np.zeros((16, 128, 128))
    for q in range(4):
        if q == 0:
            lay = [[(0, 0), (0, 1), (2, 0), (2, 1)], [(3, 1), (1, 0), (1, 1), (3, 0)]]
        else:
            lay = [[(0, 0), (1, 0), (0, 1), (1, 1)], [(2, 1), (3, 1), (2, 0), (3, 0)]]
        for h in range(2):
            ms_, ws_ = [], []
            for g, part in lay[h]:
                k = 16 * np.arange(32) + RES[q][g]
                th = 2 * np.pi * np.outer(np.arange(128 if q == 0 else 64), k) / DM
                c, s = np.cos(th), np.sin(th)
                if q == 0:
                    ms_.append(-s if part else c)
                else:
                    sg = (1.0 if RES[q][g] % 8 == q else -1.0) * (1.0 - 2.0 * h)
                    ms_.append(np.concatenate([-s, sg * c] if part else [c, sg * s]))
                ws_.append(np.where(k == 0, 1.0, 2.0) / DM)
            m = np.concatenate(ms_, axis=1)
            md[2 * q + h] = m
            md[8 + 2 * q + h] = (m * np.concatenate(ws_)[None, :]).T
    a, l = np.arange(64), np.arange(128)
    re = 16 * (a // 8) + a % 8
    im = re + 8
    ms = np.zeros((64, 128, 128))
    for dl in range(32):
        th = 2 * np.pi * np.outer(32 * a + dl, a) / S
        c, s = np.cos(th), np.sin(th)
        ms[2 * dl][:, re], ms[2 * dl][:, im] = np.concatenate([c, -s]), np.concatenate([s, c])
        ms[2 * dl + 1][:, re] = np.concatenate([c.T, s.T]) / S
        ms[2 * dl + 1][:, im] = np.concatenate([-s.T, c.T]) / S
    mn = np.zeros((6, 128, 128))
    th = 2 * np.pi * np.outer(np.arange(32), l) / 32
    mn[0, :32], mn[1, :32] = np.cos(th), -np.sin(th)
    mn[4, :, :32], mn[5, :, :32] = np.cos(th).T / DM, -np.sin(th).T / DM
    th = 2 * np.pi * np.outer(np.arange(16), a) / 16
    c, s = np.cos(th), np.sin(th)
    mn[2, :32] = np.block([[c, s], [-s, c]])
    mn[3, :, :32] = np.block([[c.T, -s.T], [s.T, c.T]]) / S
    th = 2 * np.pi * np.outer(a, l) / S
    tw = np.stack([np.cos(th), np.sin(th)]).astype(np.float32).view(np.uint32)
    return np.concatenate([_to_u32(md), _to_u32(mn), tw, _to_u32(ms)], axis=0)


def _bdot(a, b):
    return jnp.dot(a, b, preferred_element_type=F32)


def _bf(u):
    return pltpu.bitcast(u, BF)


def _cat(rows):
    return jnp.concatenate(rows, axis=0).astype(BF)


def _unpack2(u, p):
    if p == 0:
        return pltpu.bitcast(u << 16, F32)
    return pltpu.bitcast(u & jnp.uint32(0xFFFF0000), F32)


def _strassen_left(n, a):
    return (lambda: a(1, 0) + a(1, 1), lambda: a(1, 0) - a(0, 0), lambda: a(1, 1), lambda: a(0, 0) + a(1, 1),
            lambda: a(0, 0), lambda: a(0, 1) - a(1, 1), lambda: a(0, 0) + a(0, 1))[n]()


def _strassen_right(n, w):
    add = lambda u, v: (u.astype(F32) + v.astype(F32)).astype(BF)
    sub = lambda u, v: (u.astype(F32) - v.astype(F32)).astype(BF)
    return (lambda: w(0, 0), lambda: add(w(0, 0), w(0, 1)), lambda: sub(w(1, 0), w(0, 0)),
            lambda: add(w(0, 0), w(1, 1)), lambda: sub(w(0, 1), w(1, 1)), lambda: add(w(1, 0), w(1, 1)),
            lambda: w(1, 1))[n]()


def _strassen(left, right, done, ready=lambda k: None, dot=None):
    def mm(n):
        a, r, acc = left(n), right(n), None
        for k in range(0, r.shape[0], 512):
            d = (dot or _bdot)(a[:, k:k + 512], r[k:k + 512])
            acc = d if acc is None else acc + d
        return acc

    ready(0)
    m2 = mm(0)
    c22 = mm(1) - m2
    ready(1)
    m4 = mm(2)
    c21 = m2 + m4
    m1 = mm(3)
    c11, c22 = m1 + m4, c22 + m1
    m3 = mm(4)
    done(1, c21, c22 + m3)
    c11 = c11 + mm(5)
    m5 = mm(6)
    done(0, c11 - m5, m3 + m5)


def _twiddle(z, k, n, sign):
    r, i = z
    if k == 0:
        return r, i
    if 4 * k == n:
        return (-i, r) if sign > 0 else (i, -r)
    c, s = math.cos(2 * math.pi * k / n), sign * math.sin(2 * math.pi * k / n)
    if 8 * k == n or 8 * k == 3 * n:
        if c * s > 0:
            return (r - i) * c, (r + i) * c
        return (r + i) * c, (i - r) * c
    return r * c - i * s, r * s + i * c


def _cfft(xs, sign):
    n = len(xs)
    if n == 1:
        return xs
    ev, od = _cfft(xs[0::2], sign), _cfft(xs[1::2], sign)
    out = [None] * n
    for k in range(n // 2):
        er, ei = ev[k]
        if 4 * k == n:
            orr, oi = od[k]
            lo, hi = (er - oi, ei + orr), (er + oi, ei - orr)
            out[k], out[k + n // 2] = (lo, hi) if sign > 0 else (hi, lo)
        else:
            tr, ti = _twiddle(od[k], k, n, sign)
            out[k], out[k + n // 2] = (er + tr, ei + ti), (er - tr, ei - ti)
    return out


def _rfft8(x):
    a0, a1, b0, b1 = x[0] + x[4], x[0] - x[4], x[2] + x[6], x[2] - x[6]
    c0, c1, d0, d1 = x[1] + x[5], x[1] - x[5], x[3] + x[7], x[3] - x[7]
    e, f = a0 + b0, c0 + d0
    g, h = (c1 - d1) * R2, (c1 + d1) * R2
    return [e + f, e - f, a1 + g, b1 + h, a0 - b0, c0 - d0, a1 - g, b1 - h]


def _irfft8(z):
    z0, z4, z1r, z1i, z2r, z2i, z3r, z3i = z
    e, f = z0 + z4, z0 - z4
    a1, g = z1r + z3r, (z1r - z3r) * R2
    b1, h = z1i + z3i, (z1i - z3i) * R2
    a0, b0, c0, d0 = e + z2r, e - z2r, f + z2i, f - z2i
    c1, d1 = g + h, h - g
    return [a0 + a1, c0 + c1, b0 + b1, d0 + d1, a0 - a1, c0 - c1, b0 - b1, d0 - d1]


def _kernel(x_hbm, mem0_hbm, wq_hbm, wk_hbm, wv_hbm, wo_hbm, bx_hbm, wr_hbm, wi_hbm, fill_hbm, cst_hbm,
            out_hbm,
            x_v, xpre_v, xs_v, mem0_v, fill_v, lhs_v, wqkv, wo_v, pre, os_v, ws_v, outa_v,
            bx_v, w_v, wn_v, wt, cst, zs, vv, tn, outb_v,
            sem_w, sem_in, sem_out):
    scale = E ** -0.5
    wus = [w.bitcast(U32) for w in (wq_hbm, wk_hbm, wv_hbm)]
    wo_u = wo_hbm.bitcast(U32)
    fus = [w.at[pl.ds(0, 512)].bitcast(U32) for w in (wr_hbm, wi_hbm)]

    def w_copy(j, t, sem):
        return pltpu.make_async_copy(wus[t].at[:, :, j, :], wqkv.at[j, t], sem)

    xpre_cp = pltpu.make_async_copy(x_hbm.at[:, pl.ds(0, 8), :], xpre_v, sem_w.at[7])
    cuts = OPT['cuts']
    head = [[divmod(f, 3) for f in range(cuts[b], cuts[b + 1])] for b in range(len(cuts) - 1)]
    head_cps = [[w_copy(j, t, sem_w.at[b]) for j, t in grp] for b, grp in enumerate(head)]

    def b_rows(i, b):
        return b, i // 4, pl.ds(pl.multiple_of((i % 4) * 8, 8), 8)

    def fwd_cps(i):
        rows = b_rows(i, slice(None))
        return [w_copy(8 + i, t, sem_w.at[8 + i]) for t in range(3)] + [pltpu.make_async_copy(bx_hbm.at[rows], bx_v.at[rows], sem_w.at[8 + i])] + [
            pltpu.make_async_copy(fus[t].at[:, pl.ds(pl.multiple_of(128 * (2 * i + h), 128), 128)],
                                  w_v.at[t, 2 * i + h], sem_w.at[8 + i]) for t in range(2) for h in range(2)]

    def part(src, dst, lo, hi, sem):
        return pltpu.make_async_copy(src.at[pl.ds(lo, hi - lo)], dst.at[pl.ds(lo, hi - lo)], sem)

    c0_cp = part(cst_hbm, cst, 0, C_MS, sem_w.at[16])
    a_cps = [pltpu.make_async_copy(wo_u.at[:, pl.ds(128 * n, 128)], wo_v.at[n], sem_in.at[1]) for n in range(8)]
    a_cps += [part(x_hbm, x_v, 0, UN, sem_in.at[1]), part(cst_hbm, cst, C_MS, C_MS + UN, sem_in.at[1]),
              pltpu.make_async_copy(mem0_hbm, mem0_v, sem_in.at[1]),
              pltpu.make_async_copy(fill_hbm, fill_v, sem_in.at[1])]
    b_cps = [part(x_hbm, x_v, UN, NSEG, sem_in.at[2]), part(cst_hbm, cst, C_MS + UN, C_NUM, sem_in.at[2])]
    b_cps += [pltpu.make_async_copy(w.at[pl.ds(512, 1)], wn_v.at[t], sem_in.at[2])
              for t, w in enumerate((wr_hbm, wi_hbm))]

    lane = lax.broadcasted_iota(I32, (8, 128), 1)
    alt = jnp.where(lane % 2 == 0, 1.0, -1.0).astype(F32)
    lo_half = lane < 64
    ev_grp = (lane // 32) % 2 == 0

    def half_coef(q):
        sg = -1.0 if q < 3 else 1.0
        tc, ts = math.cos(2 * math.pi * q / 16), -math.sin(2 * math.pi * q / 16)
        f = lambda lo, hi: jnp.where(lo_half, lo, hi).astype(F32)
        return f(1.0, ts), f(0.0, sg * tc), f(0.0, tc), f(sg, -sg * ts)

    pace = {'tok': None}

    def gate(v):
        tok = pace['tok']
        if tok is None:
            return v
        return v | tok if v.dtype == U32 else pltpu.bitcast(pltpu.bitcast(v, U32) | tok, v.dtype)

    def gate2(z):
        return gate(z[0]), gate(z[1])

    def flat(zs_):
        return [v for z in zs_ for v in z]

    def as_u32(rows):
        return pltpu.bitcast(jnp.concatenate(rows, axis=0).astype(BF), U32)

    def b_fwd(i):
        r0 = pl.multiple_of(i * 8, 8)
        hc = [None] + [half_coef(q) for q in range(1, 4)]
        tacc = jnp.zeros((8, 128), F32)
        zl = []
        for b0 in range(0, 32, 2):
            rows = []
            for b in (b0, b0 + 1):
                xb = bx_v[(*b_rows(i, b), slice(None))].astype(F32)
                z = _rfft8([gate(xb[:, 128 * t:128 * t + 128]) for t in range(8)])
                tacc = jnp.where(lane == b, jnp.sum(z[0] * alt, axis=1, keepdims=True), tacc)
                for q in range(1, 4):
                    c1, c2, c3, c4 = hc[q]
                    zr, zi = z[2 * q], z[2 * q + 1]
                    pp = c1 * zr + c2 * zi
                    qq = pltpu.roll(c3 * zr + c4 * zi, 64, 1)
                    z[2 * q], z[2 * q + 1] = pp + qq, pp - qq
                rows.append(z)
            zl.append([as_u32([rows[0][n], rows[1][n]]) for n in range(8)])
            yield 200
            if b0 % 4 == 0:
                e, t, ty = 2 * i + b0 // 16, (b0 // 8) % 2, (b0 // 4) % 2
                u = jnp.concatenate([gate(w_v[t, e, pl.ds(m + ty + 64 * v, 8, stride=8), :])
                                     for m in (0, 6, 4, 2) for v in range(4)], axis=0)
                ut = pltpu.bitcast(pltpu.bitcast(u, F32).T, U32)
                for v in range(16):
                    wt[t, ty, pl.ds(8 * (v % 4) * WP + 4 * e + v // 4, 8, stride=WP), :] = ut[8 * v:8 * v + 8]
                yield 40
        tn[pl.ds(r0, 8), :] = tacc

        def mm(n):
            return _bdot(_bf(jnp.concatenate([z[n] for z in zl], axis=0)), _bf(cst[C_MD + n]))

        yield MID
        oo = [mm(n) for n in range(4)]
        yield MID
        oo += [mm(n) for n in range(4, 8)]
        yield MID
        for q in range(4):
            sel, sh = (ev_grp, 96) if q == 0 else (lo_half, 64)
            ys = []
            for b0 in range(4):
                xs = []
                for b in range(b0, 32, 4):
                    e_, o_ = gate(oo[2 * q][8 * b:8 * b + 8]), oo[2 * q + 1][8 * b:8 * b + 8]
                    xs.append((jnp.where(sel, e_, o_), pltpu.roll(jnp.where(sel, o_, e_), sh, 1)))
                ys.append([_twiddle(y, b0 * k1, 32, -1) for k1, y in enumerate(_cfft(xs, -1))])
                yield 110
            for k1 in range(8):
                for k0, y in enumerate(_cfft([gate2(ys[b0][k1]) for b0 in range(4)], -1)):
                    zs[k1 + 8 * k0, q, pl.ds(pl.multiple_of(2 * r0, 16), 16), :] = _cat(y)
                yield 30

    def b_mid(it):
        if UN > 2:
            rows = H * E // 4 // (NSEG // UN)
            for n in range(4):
                for r in range(0, rows, 8):
                    blk = lambda k, p: _bf(gate(
                        wo_v[n + 4 * p, pl.ds(pl.multiple_of((2 * it + k) * rows + r, 8), 8), :]))
                    vals = [pltpu.bitcast(_strassen_right(m, blk), U32) for m in range(1, 6)]
                    for m in range(5):
                        ws_v[n, m, pl.ds(pl.multiple_of(it * rows + r, 8), 8), :] = vals[m]
                    yield vals if OPT['tie_ws'] and 8 * n + r // 8 > 1 else None
            yield MID
        else:
            for _ in range(6):
                yield None
        for n in range(UN // 2):
            dl = (UN // 2) * it + n
            y = _bdot(_bf(cst[C_MS + 2 * dl]), jnp.concatenate([zs[dl, q] for q in range(4)], axis=1))
            for _ in range(4):
                yield None
            w0 = pl.multiple_of(dl * WP, 8)
            rows = []
            for r in range(8):
                wq = []
                for t in range(2):
                    ta, tb = wt[t, 0, pl.ds(w0 + 8 * r, 8), :], wt[t, 1, pl.ds(w0 + 8 * r, 8), :]
                    wq.append([_unpack2(ta, 0), _unpack2(jnp.where(ev_grp, ta, tb), 1),
                               _unpack2(tb, 0), _unpack2(jnp.where(ev_grp, tb, ta), 1)])
                cols = []
                for q in range(4):
                    yr = gate(y[8 * r:8 * r + 8, 128 * q:128 * q + 128])
                    yi = gate(y[64 + 8 * r:72 + 8 * r, 128 * q:128 * q + 128])
                    wr, wi = wq[0][q], wq[1][q]
                    cols.append(as_u32([yr * wr - yi * wi, yr * wi + yi * wr]))
                rows.append(jnp.concatenate(cols, axis=1))
                yield cols if OPT['tie_p'] else None
                yield None
            yield MID
            vv[dl] = _bdot(_bf(cst[C_MS + 2 * dl + 1]), _bf(jnp.concatenate(rows, axis=0)))

    def b_nyq():
        c, s = pltpu.bitcast(cst[C_TW], F32), pltpu.bitcast(cst[C_TW + 1], F32)
        tb = tn[...].astype(BF)
        tr, ti = _bdot(tb, _bf(cst[C_MN])), _bdot(tb, _bf(cst[C_MN + 1]))
        yield MID
        y = _bdot(_bf(cst[C_MN + 2, 0:16, :]), _cat([tr * c + ti * s, ti * c - tr * s]))
        row = lax.broadcasted_iota(I32, (16, 128), 0)
        wn = []
        for t in range(2):
            wrow = wn_v[t].astype(F32)
            acc = jnp.zeros((16, 128), F32)
            for e in range(16):
                acc = jnp.where(row == e, wrow[:, 128 * e:128 * e + 128], acc)
            wn.append(acc)
        yr, yi = y[0:16], y[16:32]
        yield MID
        v = _bdot(_bf(cst[C_MN + 3, :, 0:32]), _cat([yr * wn[0] - yi * wn[1], yr * wn[1] + yi * wn[0]]))
        vr, vi = v[0:64], v[64:128]
        yield MID
        tn[...] = (_bdot((vr * c - vi * s).astype(BF), _bf(cst[C_MN + 4]))
                   + _bdot((vr * s + vi * c).astype(BF), _bf(cst[C_MN + 5])))

    def b_inv(i):
        r0 = i * 8
        ul = []
        for q in range(4):
            sel, sh = (ev_grp, 32) if q == 0 else (lo_half, 64)
            ys = []
            for b0 in range(4):
                xs = [(gate(vv[dl, pl.ds(r0, 8), 128 * q:128 * q + 128]),
                       gate(vv[dl, pl.ds(64 + r0, 8), 128 * q:128 * q + 128])) for dl in range(b0, 32, 4)]
                ys.append([_twiddle(y, b0 * k1, 32, +1) for k1, y in enumerate(_cfft(xs, +1))])
                yield (120, flat(ys[-1])) if OPT['tie8'] else 110
            ie, io = [], []
            for k1 in range(8):
                es, os_ = [], []
                for ur, ui in _cfft([gate2(ys[b0][k1]) for b0 in range(4)], +1):
                    tmp = pltpu.roll(ui, sh, 1)
                    es.append(jnp.where(sel, ur, tmp))
                    os_.append(jnp.where(sel, tmp, ur))
                ie += [as_u32(es[0:2]), as_u32(es[2:4])]
                io += [as_u32(os_[0:2]), as_u32(os_[2:4])]
                yield 55, ie[-2:] + io[-2:]
            ul += [ie, io]
        return ul

    def b_fin(i, zz):
        r0 = i * 8
        hc = [None] + [half_coef(q) for q in range(1, 4)]
        tb = tn[pl.ds(r0, 8), :]
        for g in range(32):
            b = g // 4 + 8 * (g % 4)
            z = [gate(zz[n][8 * g:8 * g + 8]) for n in range(8)]
            z[0] = z[0] + jnp.sum(jnp.where(lane == b, tb, 0.0), axis=1, keepdims=True) * alt
            for q in range(1, 4):
                c1, c2, c3, c4 = hc[q]
                pp = z[2 * q] + z[2 * q + 1]
                qq = pltpu.roll(z[2 * q] - z[2 * q + 1], 64, 1)
                z[2 * q], z[2 * q + 1] = c1 * pp + c3 * qq, c2 * pp + c4 * qq
            y = _irfft8(z)
            outb_v[(*b_rows(i, b), slice(None))] = jnp.concatenate(y, axis=1).astype(BF)
            yield 75, y
        rows = b_rows(i, slice(None))
        start_out(outb_v.at[rows], out_hbm.at[(*rows, pl.ds(DM, DM))])

    def tie(w, vals):
        if not vals:
            return w
        acc = None
        for v in vals:
            v = v if v.dtype == U32 else pltpu.bitcast(v, U32)
            acc = v if acc is None else acc | v
        zero = cst[C_MN, 56:64, :]
        return jnp.concatenate([w[0:8] | (acc & zero), w[8:]], axis=0)

    def batch_slot(gen, budget):
        st = {'debt': 0, 'k': 0}
        due = {}

        def emit(d, b):
            while st['debt'] < b:
                r = 8 * (32 * st['debt'] // b)
                pace['tok'] = pltpu.bitcast(d[r:r + 8], U32) & cst[C_MN, 56:64, :]
                c = next(gen, MID)
                if c is MID:
                    st['debt'] = b
                elif isinstance(c, list):
                    st['debt'] = 0
                    for own in c:
                        emit(own, OPT['b_own'])
                    return
                else:
                    if isinstance(c, tuple):
                        due.setdefault(st['k'] + OPT['due'], []).extend(c[1])
                        c = c[0]
                    st['debt'] += c
            st['debt'] -= b

        def dot(a, w):
            vals = due.pop(st['k'], None)
            if vals:
                a = jnp.concatenate([_bf(tie(pltpu.bitcast(a[:, 0:128], U32), vals)), a[:, 128:]], axis=1)
            d = _bdot(a, w)
            st['k'] += 1
            emit(d, budget(st['k'] - 1))
            return d

        return dot

    out_cps = []

    def start_out(src, dst):
        out_cps.append(pltpu.make_async_copy(src, dst, sem_out.at[0]))
        out_cps[-1].start()

    hb = DM // 32

    def retile(j, t, k):
        blk = pl.ds(k * hb, hb)
        a, b = wqkv[j, t, blk, pl.ds(0, 8, stride=2), :], wqkv[j, t, blk, pl.ds(1, 8, stride=2), :]
        wqkv[j, t, blk, 0:8, :] = (a & jnp.uint32(0xFFFF)) | (b << 16)
        wqkv[j, t, blk, 8:16, :] = (a >> 16) | (b & jnp.uint32(0xFFFF0000))

    def strassen_lhs():
        for g in range(NSEG // 4):
            xa = [xpre_v[4 * g + k].astype(F32) for k in range(4)]
            a1, a2 = jnp.concatenate([xa[0], xa[2]], axis=0), jnp.concatenate([xa[1], xa[3]], axis=0)
            a11, a12, a21, a22 = a1[:, :DM // 2], a1[:, DM // 2:], a2[:, :DM // 2], a2[:, DM // 2:]
            for n in range(7):
                v = _strassen_left(n, lambda r, k: ((a11, a12), (a21, a22))[r][k])
                xs_v[n, 8 * g:8 * g + 8, :] = pltpu.bitcast(v.astype(BF), U32)

    def pre_step7(j, t, slot=None):
        w = lambda k, p: _bf(wqkv[j, t, k * hb:(k + 1) * hb, 8 * p:8 * p + 8, :].reshape(DM // 4, E))

        def done(h, c1, c2):
            if OPT['prev'] == 3:
                rnd = lambda c: pltpu.bitcast(c.astype(BF).astype(F32), U32)
                pre[j, t, :, h] = ((rnd(c1) >> 16) | rnd(c2)).reshape(NSEG // 2, 8, E)
                return
            v = jnp.concatenate([c.reshape(NSEG // 2, 8, E) for c in (c1, c2)], axis=1).astype(BF)
            pre[j, t, :, h] = pltpu.bitcast(v, U32) if OPT['prev'] >= 2 else v

        _strassen(lambda n: _bf(xs_v[n]), lambda n: _strassen_right(n, w), done, functools.partial(retile, j, t), slot)

    for cp in [xpre_cp] + [cp for grp in head_cps for cp in grp]:
        cp.start()
    vv[0:OPT['pad']] = jnp.zeros((OPT['pad'],) + vv.shape[1:], F32)
    xpre_cp.wait()
    strassen_lhs()
    later = {int(k): v for k, v in OPT['later'].items()}

    def pre_fwd(steps, i, budget):
        gen = b_fwd(i)
        slot = batch_slot(gen, lambda n: budget)
        for j, t in steps + [(8 + i, t) for t in range(3)]:
            pre_step7(j, t, slot)
        for _ in gen:
            pass

    for b, grp in enumerate(head):
        last = b == len(head) - 1
        for cp in head_cps[b] + ([c0_cp] + fwd_cps(0) if last else []):
            cp.wait()
        if 'head' in OPT['skip']:
            pass
        elif last:
            pre_fwd(grp, 0, OPT['b_fwd0'])
        else:
            for j, t in grp:
                pre_step7(j, t)
        for i in later.get(b, ()):
            for cp in ([c0_cp] if i == 0 else []) + fwd_cps(i):
                cp.start()

    if not OPT['a_at']:
        for cp in a_cps + b_cps:
            cp.start()

    def pre_fwd_body(i, carry):
        for cp in fwd_cps(i):
            cp.wait()

        if OPT['a_at']:
            @pl.when(i == OPT['a_at'])
            def _():
                for cp in a_cps + b_cps:
                    cp.start()

        pre_fwd([], i, OPT['b_fwd'])
        return carry

    if 'fwd' not in OPT['skip']:
        lax.fori_loop(1, 8, pre_fwd_body, 0)
    for cp in a_cps + ([] if OPT['late_wait'] else b_cps):
        cp.wait()

    def seg_step(s, u, mem, slot, opost):
        xs = x_v[s]
        lhs_v[u] = as_u32([mem, xs[8:32].astype(F32)])
        fill = fill_v[...]
        late, toks = [], []
        pace['tok'] = None

        def proj(j, t):
            w0, w1 = [wqkv[j, t, :, 8 * p:8 * p + 8, :].reshape(DM // 2, E) for p in range(2)]
            if late and OPT['tie_os'] and (j % 2 == 1 or t == 2):
                w1 = tie(w1, late.pop(0))
            r0, r1 = _bdot(_bf(lhs_v[u]), _bf(tie(w0, slot()))), _bdot(_bf(lhs_v[u]), _bf(w1))
            if OPT['gate_main']:
                toks.append(r0[0:8])
                if len(toks) >= OPT['gate_main']:
                    pace['tok'] = pltpu.bitcast(toks[-OPT['gate_main']], U32) & cst[C_MN, 56:64, :]
            pw = pre[j, t, s // 2, u % 2]
            if OPT['prev'] == 1:
                return jnp.concatenate([_cat([r0, r1]), pw], axis=0)
            if OPT['prev'] == 2:
                return _cat([r0, r1, _bf(pw).astype(F32)])
            if OPT['prev'] == 3:
                return _cat([r0, r1, _unpack2(pw, 0), _unpack2(pw, 1)])
            if OPT['prev'] == 4:
                return jnp.concatenate([_cat([r0, r1]), _bf(pw)], axis=0)
            return _cat([r0, r1, pw.astype(F32)])

        def qk(q, k):
            sc = lax.dot_general(q, k, (((1,), (1,)), ((), ())), preferred_element_type=F32) * scale
            sc = jnp.where(fill == 0.0, sc, fill)
            p = jnp.exp(sc - jnp.max(sc, axis=-1, keepdims=True))
            return (p * pl.reciprocal(jnp.sum(p, axis=-1, keepdims=True), approx=True)).astype(BF)

        ob, ps, vs = {}, {}, {}

        def pv(j):
            o = _bdot(ps[j], vs[j])
            opost[u, j] = (o[64:72], o[72:80])
            if u == UN - 1:
                vals = [as_u32([_strassen_left(n, lambda r, k: opost[2 * g + r, j][k]) for g in range(2)])
                        for n in range(7)]
                for n in range(7):
                    os_v[n, pl.ds(pl.multiple_of(2 * (s - u), 8), 8), 128 * j:128 * j + 128] = vals[n]
                late.append(vals)
            ob[j] = [o[0:32], o[32:64]]

        def wo(g0, g1):
            og = jnp.concatenate([o for j in range(2 * g0, 2 * g1) for o in ob[j]], axis=1).astype(BF)
            return jnp.concatenate([_bdot(og, _bf(wo_v[n, g0 * 256:g1 * 256, :])) for n in range(8)], axis=1)

        ng = NP // 2
        for g in range(ng):
            ja, jb = 2 * g, 2 * g + 1
            qa, ka, qb, kb = proj(ja, 0), proj(ja, 1), proj(jb, 0), proj(jb, 1)
            vs[ja], vs[jb] = proj(ja, 2), proj(jb, 2)
            ps[ja], ps[jb] = qk(qa, ka), qk(qb, kb)
            if g > 0:
                pv(ja - 2)
                pv(jb - 2)
        res = wo(0, 3)
        pv(NP - 2)
        pv(NP - 1)
        res = res + wo(3, ng - 1)
        res = res + wo(ng - 1, ng)
        outa_v[s // 2, u % 2, 8:32, :] = res[8:32].astype(BF)
        return res[0:8].astype(BF).astype(F32)

    def loop_body(it, mem):
        if OPT['late_wait']:
            @pl.when(it == 1)
            def _():
                for cp in b_cps:
                    cp.wait()

        gen = b_mid(it)
        opost = {}
        state = {'mid': False}

        def slot():
            if state['mid']:
                return None
            vals = next(gen, None)
            if vals is MID:
                state['mid'] = True
                return None
            return vals

        for u in range(UN):
            state['mid'] = False
            mem = seg_step(UN * it + u, u, mem, slot, opost)
        for _ in gen:
            pass
        return mem

    if 'main' not in OPT['skip']:
        lax.fori_loop(0, NSEG // UN, loop_body, mem0_v[...].astype(F32))
    idx = (slice(None), slice(None), pl.ds(8, SEG - 8), pl.ds(0, DM))
    start_out(outa_v.at[idx], out_hbm.at[idx])

    def b_inv_all():
        nyq = b_nyq()
        zz = None
        for i in range(9):
            if i < 8:
                gen = b_inv(i)
                try:
                    k = 0
                    while True:
                        c = next(gen)
                        k += 1
                        if k % 10 == 1:
                            next(nyq, None)
                        yield c
                except StopIteration as e:
                    ul = e.value
            if i > 0:
                yield from b_fin(i - 1, zz)
            else:
                yield MID
            if i < 8:
                zz = [_bdot(_bf(jnp.concatenate(ul[n], axis=0)), _bf(cst[C_MD + 8 + n])) for n in range(8)]
                if i == 7:
                    yield MID
                    yield MID
                else:
                    yield [zz[3], zz[7]]

    gens = [b_inv_all()]
    slot = batch_slot(gens[0], lambda k: (OPT['b_inv0'] if k < 28 else OPT['b_inv'])
                      + (OPT['b_plus'] if (k + OPT['b_sh']) % 28 < 4 or (k + OPT['b_sh']) % 28 >= 24 else 0))
    if 'post' in OPT['skip']:
        def keep(k, c):
            v = (pltpu.bitcast(pre[k, 0, k, 0], U32) if OPT['prev'] < 2 else pre[k, 0, k, 0]) | pltpu.bitcast(zs[k, 0, 0:16, :], U32) | wt[0, 0, pl.ds(pl.multiple_of(8 * k, 8), 8), :] | wqkv[k, 0, k, 0:8, :]
            v = pltpu.bitcast(v, F32) + tn[pl.ds(pl.multiple_of(8 * k, 8), 8), :] + vv[k, 0:8, 0:128] + pltpu.bitcast(os_v[k, 0:8, pl.ds(pl.multiple_of(128 * k, 128), 128)] | ws_v[k, k, 0:8, :], F32)
            outa_v[k, 0, 0:8, 0:128] = v.astype(BF)
            return c
        lax.fori_loop(0, 4, keep, 0)
        start_out(outa_v.at[:, :, pl.ds(0, 8)], out_hbm.at[:, :, pl.ds(0, 8), pl.ds(0, DM)])
        return
    for n in range(4):
        def done(r, *cs):
            for p, cc in enumerate(cs):
                idx = (slice(None), r, pl.ds(0, 8), pl.ds(128 * (n + 4 * p), 128))
                outa_v[idx] = cc.reshape(NSEG // 2, 8, 128).astype(BF)
                start_out(outa_v.at[idx], out_hbm.at[idx])

        heads = lambda k: jnp.concatenate([wo_v[n + 4 * k, 64 * h:64 * h + 64, :] for h in range(k, H, 2)], axis=0)
        right = lambda m: _bf(heads(m // 6) if m % 6 == 0 else ws_v[n, m - 1])
        _strassen(lambda m: _bf(os_v[m]), right, done, dot=slot)
    for gen in gens:
        for _ in gen:
            pass
    for cp in out_cps:
        cp.wait()


def pallas_concat_heads__memory_aug_recurrent_mem_tr__spectral_gfnet__prompt_kernel(
    A_x, A_mem0, A_Wq, A_Wk, A_Wv, A_Wo, A_seg_len, B_x, B_w_r, B_w_i,
):
    assert A_x.shape == (1, S, DM) and A_Wq.shape == (DM, H, E) and A_mem0.shape == (1, M, DM)
    assert B_x.shape == (1, S, DM) and (not isinstance(A_seg_len, int) or A_seg_len == SEG)
    hbm = pl.BlockSpec(memory_space=pltpu.HBM)
    wr = lambda w: w.reshape(DM // 16, 16, H, E)
    out = pl.pallas_call(
        _kernel,
        out_shape=jax.ShapeDtypeStruct((NSEG // 2, 2, SEG, 2 * DM), BF),
        in_specs=[hbm] * 11,
        out_specs=hbm,
        scratch_shapes=[
            pltpu.VMEM((NSEG, SEG, DM), BF),
            pltpu.VMEM((NSEG, 8, DM), BF),
            pltpu.VMEM((7, NSEG * 2, DM // 2), U32),
            pltpu.VMEM((M, DM), BF),
            pltpu.VMEM((80, 80), F32),
            pltpu.VMEM((UN, SEG // 2, DM), U32),
            pltpu.VMEM((NP, 3, DM // 16, 16, E), U32),
            pltpu.VMEM((8, H * E // 2, 128), U32),
            pltpu.VMEM((NP, 3, NSEG // 2, 2, 16, E), BF) if OPT['prev'] < 2 else pltpu.VMEM((NP, 3, NSEG // 2, 2, 8, E), U32),
            pltpu.VMEM((7, NSEG * 2, H * E // 2), U32),
            pltpu.VMEM((4, 5, H * E // 4, 128), U32),
            pltpu.VMEM((NSEG // 2, 2, SEG, DM), BF),
            pltpu.VMEM((NSEG // 2, 2, SEG, DM), BF),
            pltpu.VMEM((2, 16, 256, 128), U32),
            pltpu.VMEM((2, 1, S), BF),
            pltpu.VMEM((2, 2, 32 * WP, 128), U32),
            pltpu.VMEM((C_NUM, 64, 128), U32),
            pltpu.VMEM((32, 4, 128, 128), BF),
            pltpu.VMEM((32, 128, 512), F32),
            pltpu.VMEM((64, 128), F32),
            pltpu.VMEM((NSEG // 2, 2, SEG, DM), BF),
            pltpu.SemaphoreType.DMA((NP + 1,)),
            pltpu.SemaphoreType.DMA((6,)),
            pltpu.SemaphoreType.DMA((1,)),
        ],
        compiler_params=pltpu.CompilerParams(vmem_limit_bytes=118 * 1024 * 1024,
                                             disable_bounds_checks=True, disable_semaphore_checks=True),
    )(A_x.reshape(NSEG, SEG, DM), A_mem0.reshape(M, DM), wr(A_Wq), wr(A_Wk), wr(A_Wv),
      A_Wo.reshape(H * E, DM), B_x.reshape(NSEG // 2, 2, SEG, DM), B_w_r.T, B_w_i.T, _mask_fill(), _fft_consts())
    return out.reshape(1, S, 2 * DM)
```

```python
import functools
import math

import jax
import jax.numpy as jnp
import numpy as np
from jax import lax
import jax.experimental.pallas as pl
import jax.experimental.pallas.tpu as pltpu

BF, F32, U32, I32 = jnp.bfloat16, jnp.float32, jnp.uint32, jnp.int32

S, DM, H, E, M, SEG = 2048, 1024, 32, 128, 8, 32
NSEG = S // SEG
NP = H // 2
UN = 4
R2 = math.sqrt(0.5)
MID = 'mid'
PAD = 20
HEAD = (0, 1, 2, 4, 7, 12, 18, 24)
LATER = {2: (0, 1), 3: (2,), 4: (3, 4, 5), 5: (6, 7)}


def _to_u32(m):
    u = np.ascontiguousarray(m, dtype=np.float32).view(np.uint32)
    h = ((u + 0x7FFF + ((u >> 16) & 1)) >> 16).astype(np.uint32)
    return h[..., 0::2, :] | (h[..., 1::2, :] << 16)


def _mask_fill():
    r = np.arange(80)
    pos_of = lambda rr: np.where(rr < M, rr, np.where(rr < SEG, rr + M, rr - SEG + M))
    qhead = np.where(r < 64, r // 32, (r - 64) // 8)
    qpos = pos_of(np.where(r < 64, r % 32, SEG + (r - 64) % 8))
    khead, kpos = qhead, qpos
    vis = (qpos[:, None] < M) | (qpos[:, None] >= kpos[None, :])
    same = qhead[:, None] == khead[None, :]
    return np.where(same, np.where(vis, 0.0, -1e9), -np.inf).astype(np.float32)


RES = ((0, 12, 8, 4), (1, 15, 9, 7), (2, 14, 10, 6), (3, 13, 11, 5))
WP = 72
C_MD, C_MN, C_TW, C_MS, C_NUM = 0, 16, 22, 24, 88


@functools.lru_cache(maxsize=None)
def _fft_consts():
    md = np.zeros((16, 128, 128))
    for q in range(4):
        if q == 0:
            lay = [[(0, 0), (0, 1), (2, 0), (2, 1)], [(3, 1), (1, 0), (1, 1), (3, 0)]]
        else:
            lay = [[(0, 0), (1, 0), (0, 1), (1, 1)], [(2, 1), (3, 1), (2, 0), (3, 0)]]
        for h in range(2):
            ms_, ws_ = [], []
            for g, part in lay[h]:
                k = 16 * np.arange(32) + RES[q][g]
                th = 2 * np.pi * np.outer(np.arange(128 if q == 0 else 64), k) / DM
                c, s = np.cos(th), np.sin(th)
                if q == 0:
                    ms_.append(-s if part else c)
                else:
                    sg = (1.0 if RES[q][g] % 8 == q else -1.0) * (1.0 - 2.0 * h)
                    ms_.append(np.concatenate([-s, sg * c] if part else [c, sg * s]))
                ws_.append(np.where(k == 0, 1.0, 2.0) / DM)
            m = np.concatenate(ms_, axis=1)
            md[2 * q + h] = m
            md[8 + 2 * q + h] = (m * np.concatenate(ws_)[None, :]).T
    a, l = np.arange(64), np.arange(128)
    re = 16 * (a // 8) + a % 8
    im = re + 8
    ms = np.zeros((64, 128, 128))
    for dl in range(32):
        th = 2 * np.pi * np.outer(32 * a + dl, a) / S
        c, s = np.cos(th), np.sin(th)
        ms[2 * dl][:, re], ms[2 * dl][:, im] = np.concatenate([c, -s]), np.concatenate([s, c])
        ms[2 * dl + 1][:, re] = np.concatenate([c.T, s.T]) / S
        ms[2 * dl + 1][:, im] = np.concatenate([-s.T, c.T]) / S
    mn = np.zeros((6, 128, 128))
    th = 2 * np.pi * np.outer(np.arange(32), l) / 32
    mn[0, :32], mn[1, :32] = np.cos(th), -np.sin(th)
    mn[4, :, :32], mn[5, :, :32] = np.cos(th).T / DM, -np.sin(th).T / DM
    th = 2 * np.pi * np.outer(np.arange(16), a) / 16
    c, s = np.cos(th), np.sin(th)
    mn[2, :32] = np.block([[c, s], [-s, c]])
    mn[3, :, :32] = np.block([[c.T, -s.T], [s.T, c.T]]) / S
    th = 2 * np.pi * np.outer(a, l) / S
    tw = np.stack([np.cos(th), np.sin(th)]).astype(np.float32).view(np.uint32)
    return np.concatenate([_to_u32(md), _to_u32(mn), tw, _to_u32(ms)], axis=0)


def _bdot(a, b):
    return jnp.dot(a, b, preferred_element_type=F32)


def _bf(u):
    return pltpu.bitcast(u, BF)


def _cat(rows):
    return jnp.concatenate(rows, axis=0).astype(BF)


def _unpack2(u, p):
    if p == 0:
        return pltpu.bitcast(u << 16, F32)
    return pltpu.bitcast(u & jnp.uint32(0xFFFF0000), F32)


def _strassen_left(n, a):
    return (lambda: a(1, 0) + a(1, 1), lambda: a(1, 0) - a(0, 0), lambda: a(1, 1), lambda: a(0, 0) + a(1, 1),
            lambda: a(0, 0), lambda: a(0, 1) - a(1, 1), lambda: a(0, 0) + a(0, 1))[n]()


def _strassen_right(n, w):
    add = lambda u, v: (u.astype(F32) + v.astype(F32)).astype(BF)
    sub = lambda u, v: (u.astype(F32) - v.astype(F32)).astype(BF)
    return (lambda: w(0, 0), lambda: add(w(0, 0), w(0, 1)), lambda: sub(w(1, 0), w(0, 0)),
            lambda: add(w(0, 0), w(1, 1)), lambda: sub(w(0, 1), w(1, 1)), lambda: add(w(1, 0), w(1, 1)),
            lambda: w(1, 1))[n]()


def _strassen(left, right, done, ready=lambda k: None, dot=None):
    def mm(n):
        a, r, acc = left(n), right(n), None
        for k in range(0, r.shape[0], 512):
            d = (dot or _bdot)(a[:, k:k + 512], r[k:k + 512])
            acc = d if acc is None else acc + d
        return acc

    ready(0)
    m2 = mm(0)
    c22 = mm(1) - m2
    ready(1)
    m4 = mm(2)
    c21 = m2 + m4
    m1 = mm(3)
    c11, c22 = m1 + m4, c22 + m1
    m3 = mm(4)
    done(1, c21, c22 + m3)
    c11 = c11 + mm(5)
    m5 = mm(6)
    done(0, c11 - m5, m3 + m5)


def _twiddle(z, k, n, sign):
    r, i = z
    if k == 0:
        return r, i
    if 4 * k == n:
        return (-i, r) if sign > 0 else (i, -r)
    c, s = math.cos(2 * math.pi * k / n), sign * math.sin(2 * math.pi * k / n)
    if 8 * k == n or 8 * k == 3 * n:
        if c * s > 0:
            return (r - i) * c, (r + i) * c
        return (r + i) * c, (i - r) * c
    return r * c - i * s, r * s + i * c


def _cfft(xs, sign):
    n = len(xs)
    if n == 1:
        return xs
    ev, od = _cfft(xs[0::2], sign), _cfft(xs[1::2], sign)
    out = [None] * n
    for k in range(n // 2):
        er, ei = ev[k]
        if 4 * k == n:
            orr, oi = od[k]
            lo, hi = (er - oi, ei + orr), (er + oi, ei - orr)
            out[k], out[k + n // 2] = (lo, hi) if sign > 0 else (hi, lo)
        else:
            tr, ti = _twiddle(od[k], k, n, sign)
            out[k], out[k + n // 2] = (er + tr, ei + ti), (er - tr, ei - ti)
    return out


def _rfft8(x):
    a0, a1, b0, b1 = x[0] + x[4], x[0] - x[4], x[2] + x[6], x[2] - x[6]
    c0, c1, d0, d1 = x[1] + x[5], x[1] - x[5], x[3] + x[7], x[3] - x[7]
    e, f = a0 + b0, c0 + d0
    g, h = (c1 - d1) * R2, (c1 + d1) * R2
    return [e + f, e - f, a1 + g, b1 + h, a0 - b0, c0 - d0, a1 - g, b1 - h]


def _irfft8(z):
    z0, z4, z1r, z1i, z2r, z2i, z3r, z3i = z
    e, f = z0 + z4, z0 - z4
    a1, g = z1r + z3r, (z1r - z3r) * R2
    b1, h = z1i + z3i, (z1i - z3i) * R2
    a0, b0, c0, d0 = e + z2r, e - z2r, f + z2i, f - z2i
    c1, d1 = g + h, h - g
    return [a0 + a1, c0 + c1, b0 + b1, d0 + d1, a0 - a1, c0 - c1, b0 - b1, d0 - d1]


def _kernel(x_hbm, mem0_hbm, wq_hbm, wk_hbm, wv_hbm, wo_hbm, bx_hbm, wr_hbm, wi_hbm, fill_hbm, cst_hbm,
            out_hbm,
            x_v, xpre_v, xs_v, mem0_v, fill_v, lhs_v, wqkv, wo_v, pre, os_v, ws_v, outa_v,
            bx_v, w_v, wn_v, wt, cst, zs, vv, tn, outb_v,
            sem_w, sem_in, sem_out):
    scale = E ** -0.5
    wus = [w.bitcast(U32) for w in (wq_hbm, wk_hbm, wv_hbm)]
    wo_u = wo_hbm.bitcast(U32)
    fus = [w.at[pl.ds(0, 512)].bitcast(U32) for w in (wr_hbm, wi_hbm)]

    def w_copy(j, t, sem):
        return pltpu.make_async_copy(wus[t].at[:, :, j, :], wqkv.at[j, t], sem)

    xpre_cp = pltpu.make_async_copy(x_hbm.at[:, pl.ds(0, 8), :], xpre_v, sem_w.at[7])
    head = [[divmod(f, 3) for f in range(HEAD[b], HEAD[b + 1])] for b in range(len(HEAD) - 1)]
    head_cps = [[w_copy(j, t, sem_w.at[b]) for j, t in grp] for b, grp in enumerate(head)]

    def b_rows(i, b):
        return b, i // 4, pl.ds(pl.multiple_of((i % 4) * 8, 8), 8)

    def fwd_cps(i):
        rows = b_rows(i, slice(None))
        sem = sem_w.at[8 + i]
        return ([w_copy(8 + i, t, sem) for t in range(3)]
                + [pltpu.make_async_copy(bx_hbm.at[rows], bx_v.at[rows], sem)]
                + [pltpu.make_async_copy(fus[t].at[:, pl.ds(pl.multiple_of(128 * (2 * i + h), 128), 128)],
                                         w_v.at[t, 2 * i + h], sem) for t in range(2) for h in range(2)])

    def part(src, dst, lo, hi, sem):
        return pltpu.make_async_copy(src.at[pl.ds(lo, hi - lo)], dst.at[pl.ds(lo, hi - lo)], sem)

    c0_cp = part(cst_hbm, cst, 0, C_MS, sem_w.at[16])
    a_cps = [pltpu.make_async_copy(wo_u.at[:, pl.ds(128 * n, 128)], wo_v.at[n], sem_in.at[0]) for n in range(8)]
    a_cps += [part(x_hbm, x_v, 0, UN, sem_in.at[0]), part(cst_hbm, cst, C_MS, C_MS + UN, sem_in.at[0]),
              pltpu.make_async_copy(mem0_hbm, mem0_v, sem_in.at[0]),
              pltpu.make_async_copy(fill_hbm, fill_v, sem_in.at[0])]
    b_cps = [part(x_hbm, x_v, UN, NSEG, sem_in.at[1]), part(cst_hbm, cst, C_MS + UN, C_NUM, sem_in.at[1])]
    b_cps += [pltpu.make_async_copy(w.at[pl.ds(512, 1)], wn_v.at[t], sem_in.at[1])
              for t, w in enumerate((wr_hbm, wi_hbm))]

    lane = lax.broadcasted_iota(I32, (8, 128), 1)
    alt = jnp.where(lane % 2 == 0, 1.0, -1.0).astype(F32)
    lo_half = lane < 64
    ev_grp = (lane // 32) % 2 == 0

    def half_coef(q):
        sg = -1.0 if q < 3 else 1.0
        tc, ts = math.cos(2 * math.pi * q / 16), -math.sin(2 * math.pi * q / 16)
        f = lambda lo, hi: jnp.where(lo_half, lo, hi).astype(F32)
        return f(1.0, ts), f(0.0, sg * tc), f(0.0, tc), f(sg, -sg * ts)

    pace = {'tok': None}

    def token(v):
        return (v if v.dtype == U32 else pltpu.bitcast(v, U32)) & cst[C_MN, 56:64, :]

    def gate(v):
        tok = pace['tok']
        if tok is None:
            return v
        return v | tok if v.dtype == U32 else pltpu.bitcast(pltpu.bitcast(v, U32) | tok, v.dtype)

    def gate2(z):
        return gate(z[0]), gate(z[1])

    def as_u32(rows):
        return pltpu.bitcast(_cat(rows), U32)

    def b_fwd(i):
        r0 = pl.multiple_of(i * 8, 8)
        hc = [None] + [half_coef(q) for q in range(1, 4)]
        tacc = jnp.zeros((8, 128), F32)
        zl = []

        def filt(k):
            e, t, ty = 2 * i + k // 4, (k // 2) % 2, k % 2
            u = jnp.concatenate([gate(w_v[t, e, pl.ds(m + ty + 64 * v, 8, stride=8), :])
                                 for m in (0, 6, 4, 2) for v in range(4)], axis=0)
            ut = pltpu.bitcast(pltpu.bitcast(u, F32).T, U32)
            for v in range(16):
                wt[t, ty, pl.ds(8 * (v % 4) * WP + 4 * e + v // 4, 8, stride=WP), :] = ut[8 * v:8 * v + 8]

        for b0 in range(0, 32, 2):
            rows = []
            for b in (b0, b0 + 1):
                xb = bx_v[(*b_rows(i, b), slice(None))].astype(F32)
                z = _rfft8([gate(xb[:, 128 * t:128 * t + 128]) for t in range(8)])
                tacc = jnp.where(lane == b, jnp.sum(z[0] * alt, axis=1, keepdims=True), tacc)
                for q in range(1, 4):
                    c1, c2, c3, c4 = hc[q]
                    zr, zi = z[2 * q], z[2 * q + 1]
                    pp = c1 * zr + c2 * zi
                    qq = pltpu.roll(c3 * zr + c4 * zi, 64, 1)
                    z[2 * q], z[2 * q + 1] = pp + qq, pp - qq
                rows.append(z)
            zl.append([as_u32([rows[0][n], rows[1][n]]) for n in range(8)])
            yield 200
            if b0 % 4 == 0:
                filt(b0 // 4)
                yield 40
        tn[pl.ds(r0, 8), :] = tacc

        def mm(n):
            return _bdot(_bf(jnp.concatenate([z[n] for z in zl], axis=0)), _bf(cst[C_MD + n]))

        yield MID
        oo = [mm(n) for n in range(4)]
        yield MID
        oo += [mm(n) for n in range(4, 8)]
        yield MID
        for q in range(4):
            sel, sh = (ev_grp, 96) if q == 0 else (lo_half, 64)
            ys = []
            for b0 in range(4):
                xs = []
                for b in range(b0, 32, 4):
                    e_, o_ = gate(oo[2 * q][8 * b:8 * b + 8]), oo[2 * q + 1][8 * b:8 * b + 8]
                    xs.append((jnp.where(sel, e_, o_), pltpu.roll(jnp.where(sel, o_, e_), sh, 1)))
                ys.append([_twiddle(y, b0 * k1, 32, -1) for k1, y in enumerate(_cfft(xs, -1))])
                yield 110
            for k1 in range(8):
                for k0, y in enumerate(_cfft([gate2(ys[b0][k1]) for b0 in range(4)], -1)):
                    zs[k1 + 8 * k0, q, pl.ds(pl.multiple_of(2 * r0, 16), 16), :] = _cat(y)
                yield 30

    def b_mid(it):
        for n in range(4):
            for r in range(0, 64, 8):
                blk = lambda k, p: _bf(gate(wo_v[n + 4 * p, pl.ds(pl.multiple_of((2 * it + k) * 64 + r, 8), 8), :]))
                vals = [pltpu.bitcast(_strassen_right(m, blk), U32) for m in range(1, 6)]
                for m in range(5):
                    ws_v[n, m, pl.ds(pl.multiple_of(it * 64 + r, 8), 8), :] = vals[m]
                yield vals if 8 * n + r // 8 > 1 else None
        yield MID
        for dl in (2 * it, 2 * it + 1):
            y = _bdot(_bf(cst[C_MS + 2 * dl]), jnp.concatenate([zs[dl, q] for q in range(4)], axis=1))
            for _ in range(4):
                yield None
            w0 = pl.multiple_of(dl * WP, 8)
            rows = []
            for r in range(8):
                wq = []
                for t in range(2):
                    ta, tb = wt[t, 0, pl.ds(w0 + 8 * r, 8), :], wt[t, 1, pl.ds(w0 + 8 * r, 8), :]
                    wq.append([_unpack2(ta, 0), _unpack2(jnp.where(ev_grp, ta, tb), 1),
                               _unpack2(tb, 0), _unpack2(jnp.where(ev_grp, tb, ta), 1)])
                cols = []
                for q in range(4):
                    yr = gate(y[8 * r:8 * r + 8, 128 * q:128 * q + 128])
                    yi = gate(y[64 + 8 * r:72 + 8 * r, 128 * q:128 * q + 128])
                    wr, wi = wq[0][q], wq[1][q]
                    cols.append(as_u32([yr * wr - yi * wi, yr * wi + yi * wr]))
                rows.append(jnp.concatenate(cols, axis=1))
                yield cols
                yield None
            yield MID
            vv[dl] = _bdot(_bf(cst[C_MS + 2 * dl + 1]), _bf(jnp.concatenate(rows, axis=0)))

    def b_nyq():
        c, s = pltpu.bitcast(cst[C_TW], F32), pltpu.bitcast(cst[C_TW + 1], F32)
        tb = tn[...].astype(BF)
        tr, ti = _bdot(tb, _bf(cst[C_MN])), _bdot(tb, _bf(cst[C_MN + 1]))
        yield MID
        y = _bdot(_bf(cst[C_MN + 2, 0:16, :]), _cat([tr * c + ti * s, ti * c - tr * s]))
        row = lax.broadcasted_iota(I32, (16, 128), 0)
        wn = []
        for t in range(2):
            wrow = wn_v[t].astype(F32)
            acc = jnp.zeros((16, 128), F32)
            for e in range(16):
                acc = jnp.where(row == e, wrow[:, 128 * e:128 * e + 128], acc)
            wn.append(acc)
        yr, yi = y[0:16], y[16:32]
        yield MID
        v = _bdot(_bf(cst[C_MN + 3, :, 0:32]), _cat([yr * wn[0] - yi * wn[1], yr * wn[1] + yi * wn[0]]))
        vr, vi = v[0:64], v[64:128]
        yield MID
        tn[...] = (_bdot((vr * c - vi * s).astype(BF), _bf(cst[C_MN + 4]))
                   + _bdot((vr * s + vi * c).astype(BF), _bf(cst[C_MN + 5])))

    def b_inv(i, ul):
        r0 = i * 8
        for q in range(4):
            sel, sh = (ev_grp, 32) if q == 0 else (lo_half, 64)
            ys = []
            for b0 in range(4):
                xs = [(gate(vv[dl, pl.ds(r0, 8), 128 * q:128 * q + 128]),
                       gate(vv[dl, pl.ds(64 + r0, 8), 128 * q:128 * q + 128])) for dl in range(b0, 32, 4)]
                ys.append([_twiddle(y, b0 * k1, 32, +1) for k1, y in enumerate(_cfft(xs, +1))])
                yield 110
            ie, io = [], []
            for k1 in range(8):
                es, os_ = [], []
                for ur, ui in _cfft([gate2(ys[b0][k1]) for b0 in range(4)], +1):
                    tmp = pltpu.roll(ui, sh, 1)
                    es.append(jnp.where(sel, ur, tmp))
                    os_.append(jnp.where(sel, tmp, ur))
                ie += [as_u32(es[0:2]), as_u32(es[2:4])]
                io += [as_u32(os_[0:2]), as_u32(os_[2:4])]
                yield 55, ie[-2:] + io[-2:]
            ul += [ie, io]

    def b_fin(i, zz):
        r0 = i * 8
        hc = [None] + [half_coef(q) for q in range(1, 4)]
        tb = tn[pl.ds(r0, 8), :]
        for g in range(32):
            b = g // 4 + 8 * (g % 4)
            z = [gate(zz[n][8 * g:8 * g + 8]) for n in range(8)]
            z[0] = z[0] + jnp.sum(jnp.where(lane == b, tb, 0.0), axis=1, keepdims=True) * alt
            for q in range(1, 4):
                c1, c2, c3, c4 = hc[q]
                pp = z[2 * q] + z[2 * q + 1]
                qq = pltpu.roll(z[2 * q] - z[2 * q + 1], 64, 1)
                z[2 * q], z[2 * q + 1] = c1 * pp + c3 * qq, c2 * pp + c4 * qq
            y = _irfft8(z)
            outb_v[(*b_rows(i, b), slice(None))] = jnp.concatenate(y, axis=1).astype(BF)
            yield 75, y
        rows = b_rows(i, slice(None))
        start_out(outb_v.at[rows], out_hbm.at[(*rows, pl.ds(DM, DM))])

    def tie(w, vals):
        if not vals:
            return w
        acc = None
        for v in vals:
            v = v if v.dtype == U32 else pltpu.bitcast(v, U32)
            acc = v if acc is None else acc | v
        return jnp.concatenate([w[0:8] | token(acc), w[8:]], axis=0)

    def paced_dot(gen, budget):
        st = {'debt': 0, 'k': 0}
        due = {}

        def emit(d, b):
            while st['debt'] < b:
                r = 8 * (32 * st['debt'] // b)
                pace['tok'] = token(d[r:r + 8])
                c = next(gen, MID)
                if c is MID:
                    st['debt'] = b
                elif isinstance(c, list):
                    st['debt'] = 0
                    for own in c:
                        emit(own, 300)
                    return
                else:
                    if isinstance(c, tuple):
                        due.setdefault(st['k'] + 2, []).extend(c[1])
                        c = c[0]
                    st['debt'] += c
            st['debt'] -= b

        def dot(a, w):
            vals = due.pop(st['k'], None)
            if vals:
                a = jnp.concatenate([_bf(tie(pltpu.bitcast(a[:, 0:128], U32), vals)), a[:, 128:]], axis=1)
            d = _bdot(a, w)
            st['k'] += 1
            emit(d, budget)
            return d

        return dot

    out_cps = []

    def start_out(src, dst):
        out_cps.append(pltpu.make_async_copy(src, dst, sem_out.at[0]))
        out_cps[-1].start()

    hb = DM // 32

    def retile(j, t, k):
        blk = pl.ds(k * hb, hb)
        a, b = wqkv[j, t, blk, pl.ds(0, 8, stride=2), :], wqkv[j, t, blk, pl.ds(1, 8, stride=2), :]
        wqkv[j, t, blk, 0:8, :] = (a & jnp.uint32(0xFFFF)) | (b << 16)
        wqkv[j, t, blk, 8:16, :] = (a >> 16) | (b & jnp.uint32(0xFFFF0000))

    def strassen_lhs():
        for g in range(NSEG // 4):
            xa = [xpre_v[4 * g + k].astype(F32) for k in range(4)]
            a1, a2 = jnp.concatenate([xa[0], xa[2]], axis=0), jnp.concatenate([xa[1], xa[3]], axis=0)
            a11, a12, a21, a22 = a1[:, :DM // 2], a1[:, DM // 2:], a2[:, :DM // 2], a2[:, DM // 2:]
            for n in range(7):
                v = _strassen_left(n, lambda r, k: ((a11, a12), (a21, a22))[r][k])
                xs_v[n, 8 * g:8 * g + 8, :] = pltpu.bitcast(v.astype(BF), U32)

    def pre_step(j, t, dot=None):
        w = lambda k, p: _bf(wqkv[j, t, k * hb:(k + 1) * hb, 8 * p:8 * p + 8, :].reshape(DM // 4, E))

        def done(h, c1, c2):
            v = jnp.concatenate([c.reshape(NSEG // 2, 8, E) for c in (c1, c2)], axis=1)
            pre[j, t, :, h] = pltpu.bitcast(v.astype(BF), U32)

        _strassen(lambda n: _bf(xs_v[n]), lambda n: _strassen_right(n, w), done,
                  functools.partial(retile, j, t), dot)

    for cp in [xpre_cp] + [cp for grp in head_cps for cp in grp]:
        cp.start()
    vv[0:PAD] = jnp.zeros((PAD,) + vv.shape[1:], F32)
    xpre_cp.wait()
    strassen_lhs()

    def pre_fwd(steps, i, budget):
        gen = b_fwd(i)
        dot = paced_dot(gen, budget)
        for j, t in steps + [(8 + i, t) for t in range(3)]:
            pre_step(j, t, dot)
        for _ in gen:
            pass

    for b, grp in enumerate(head):
        last = b == len(head) - 1
        for cp in head_cps[b] + ([c0_cp] + fwd_cps(0) if last else []):
            cp.wait()
        if last:
            pre_fwd(grp, 0, 130)
        else:
            for j, t in grp:
                pre_step(j, t)
        for i in LATER.get(b, ()):
            for cp in ([c0_cp] if i == 0 else []) + fwd_cps(i):
                cp.start()
    for cp in a_cps + b_cps:
        cp.start()

    def pre_fwd_body(i, carry):
        for cp in fwd_cps(i):
            cp.wait()
        pre_fwd([], i, 340)
        return carry

    lax.fori_loop(1, 8, pre_fwd_body, 0)
    for cp in a_cps:
        cp.wait()

    def seg_step(s, u, mem, slot, opost):
        xs = x_v[s]
        lhs_v[u] = as_u32([mem, xs[8:32].astype(F32)])
        fill = fill_v[...]
        toks = []
        pace['tok'] = None

        def proj(j, t):
            w0, w1 = [wqkv[j, t, :, 8 * p:8 * p + 8, :].reshape(DM // 2, E) for p in range(2)]
            r0, r1 = _bdot(_bf(lhs_v[u]), _bf(tie(w0, slot()))), _bdot(_bf(lhs_v[u]), _bf(w1))
            toks.append(r0[0:8])
            if len(toks) >= 4:
                pace['tok'] = token(toks[-4])
            return _cat([r0, r1, _bf(pre[j, t, s // 2, u % 2]).astype(F32)])

        def qk(q, k):
            sc = lax.dot_general(q, k, (((1,), (1,)), ((), ())), preferred_element_type=F32) * scale
            sc = jnp.where(fill == 0.0, sc, fill)
            p = jnp.exp(sc - jnp.max(sc, axis=-1, keepdims=True))
            return (p * pl.reciprocal(jnp.sum(p, axis=-1, keepdims=True), approx=True)).astype(BF)

        ob, ps, vs = {}, {}, {}

        def pv(j):
            o = _bdot(ps[j], vs[j])
            opost[u, j] = (o[64:72], o[72:80])
            if u == UN - 1:
                vals = [as_u32([_strassen_left(n, lambda r, k: opost[2 * g + r, j][k]) for g in range(2)])
                        for n in range(7)]
                for n in range(7):
                    os_v[n, pl.ds(pl.multiple_of(2 * (s - u), 8), 8), 128 * j:128 * j + 128] = vals[n]
            ob[j] = [o[0:32], o[32:64]]

        def wo(g0, g1):
            og = jnp.concatenate([o for j in range(2 * g0, 2 * g1) for o in ob[j]], axis=1).astype(BF)
            return jnp.concatenate([_bdot(og, _bf(wo_v[n, g0 * 256:g1 * 256, :])) for n in range(8)], axis=1)

        ng = NP // 2
        for g in range(ng):
            ja, jb = 2 * g, 2 * g + 1
            qa, ka, qb, kb = proj(ja, 0), proj(ja, 1), proj(jb, 0), proj(jb, 1)
            vs[ja], vs[jb] = proj(ja, 2), proj(jb, 2)
            ps[ja], ps[jb] = qk(qa, ka), qk(qb, kb)
            if g > 0:
                pv(ja - 2)
                pv(jb - 2)
        res = wo(0, 3)
        pv(NP - 2)
        pv(NP - 1)
        res = res + wo(3, ng - 1)
        res = res + wo(ng - 1, ng)
        outa_v[s // 2, u % 2, 8:32, :] = res[8:32].astype(BF)
        return res[0:8].astype(BF).astype(F32)

    def loop_body(it, mem):
        @pl.when(it == 1)
        def _():
            for cp in b_cps:
                cp.wait()

        gen = b_mid(it)
        opost = {}
        state = {'mid': False}

        def slot():
            if state['mid']:
                return None
            vals = next(gen, None)
            if vals is MID:
                state['mid'] = True
                return None
            return vals

        for u in range(UN):
            state['mid'] = False
            mem = seg_step(UN * it + u, u, mem, slot, opost)
        for _ in gen:
            pass
        return mem

    lax.fori_loop(0, NSEG // UN, loop_body, mem0_v[...].astype(F32))
    idx = (slice(None), slice(None), pl.ds(8, SEG - 8), pl.ds(0, DM))
    start_out(outa_v.at[idx], out_hbm.at[idx])

    def b_inv_all():
        nyq = b_nyq()
        zz = None
        for i in range(8):
            ul = []
            for k, c in enumerate(b_inv(i, ul)):
                if k % 10 == 0:
                    next(nyq, None)
                yield c
            if i > 0:
                yield from b_fin(i - 1, zz)
            else:
                yield MID
            zz = [_bdot(_bf(jnp.concatenate(ul[n], axis=0)), _bf(cst[C_MD + 8 + n])) for n in range(8)]
            if i < 7:
                yield [zz[3], zz[7]]
        yield MID
        yield MID
        yield from b_fin(7, zz)

    gen = b_inv_all()
    dot = paced_dot(gen, 450)
    for n in range(4):
        def done(r, *cs):
            for p, cc in enumerate(cs):
                idx = (slice(None), r, pl.ds(0, 8), pl.ds(128 * (n + 4 * p), 128))
                outa_v[idx] = cc.reshape(NSEG // 2, 8, 128).astype(BF)
                start_out(outa_v.at[idx], out_hbm.at[idx])

        heads = lambda k: jnp.concatenate([wo_v[n + 4 * k, 64 * h:64 * h + 64, :] for h in range(k, H, 2)], axis=0)
        right = lambda m: _bf(heads(m // 6) if m % 6 == 0 else ws_v[n, m - 1])
        _strassen(lambda m: _bf(os_v[m]), right, done, dot=dot)
    for _ in gen:
        pass
    for cp in out_cps:
        cp.wait()


def pallas_concat_heads__memory_aug_recurrent_mem_tr__spectral_gfnet__prompt_kernel(
    A_x, A_mem0, A_Wq, A_Wk, A_Wv, A_Wo, A_seg_len, B_x, B_w_r, B_w_i,
):
    assert A_x.shape == (1, S, DM) and A_Wq.shape == (DM, H, E) and A_mem0.shape == (1, M, DM)
    assert B_x.shape == (1, S, DM) and (not isinstance(A_seg_len, int) or A_seg_len == SEG)
    hbm = pl.BlockSpec(memory_space=pltpu.HBM)
    wr = lambda w: w.reshape(DM // 16, 16, H, E)
    out = pl.pallas_call(
        _kernel,
        out_shape=jax.ShapeDtypeStruct((NSEG // 2, 2, SEG, 2 * DM), BF),
        in_specs=[hbm] * 11,
        out_specs=hbm,
        scratch_shapes=[
            pltpu.VMEM((NSEG, SEG, DM), BF),
            pltpu.VMEM((NSEG, 8, DM), BF),
            pltpu.VMEM((7, NSEG * 2, DM // 2), U32),
            pltpu.VMEM((M, DM), BF),
            pltpu.VMEM((80, 80), F32),
            pltpu.VMEM((UN, SEG // 2, DM), U32),
            pltpu.VMEM((NP, 3, DM // 16, 16, E), U32),
            pltpu.VMEM((8, H * E // 2, 128), U32),
            pltpu.VMEM((NP, 3, NSEG // 2, 2, 8, E), U32),
            pltpu.VMEM((7, NSEG * 2, H * E // 2), U32),
            pltpu.VMEM((4, 5, H * E // 4, 128), U32),
            pltpu.VMEM((NSEG // 2, 2, SEG, DM), BF),
            pltpu.VMEM((NSEG // 2, 2, SEG, DM), BF),
            pltpu.VMEM((2, 16, 256, 128), U32),
            pltpu.VMEM((2, 1, S), BF),
            pltpu.VMEM((2, 2, 32 * WP, 128), U32),
            pltpu.VMEM((C_NUM, 64, 128), U32),
            pltpu.VMEM((32, 4, 128, 128), BF),
            pltpu.VMEM((32, 128, 512), F32),
            pltpu.VMEM((64, 128), F32),
            pltpu.VMEM((NSEG // 2, 2, SEG, DM), BF),
            pltpu.SemaphoreType.DMA((NP + 1,)),
            pltpu.SemaphoreType.DMA((2,)),
            pltpu.SemaphoreType.DMA((1,)),
        ],
        compiler_params=pltpu.CompilerParams(vmem_limit_bytes=118 * 1024 * 1024, disable_semaphore_checks=True),
    )(A_x.reshape(NSEG, SEG, DM), A_mem0.reshape(M, DM), wr(A_Wq), wr(A_Wk), wr(A_Wv),
      A_Wo.reshape(H * E, DM), B_x.reshape(NSEG // 2, 2, SEG, DM), B_w_r.T, B_w_i.T, _mask_fill(), _fft_consts())
    return out.reshape(1, S, 2 * DM)
```

```python
import functools
import math

import jax
import jax.numpy as jnp
import numpy as np
from jax import lax
import jax.experimental.pallas as pl
import jax.experimental.pallas.tpu as pltpu

BF, F32, U32, I32 = jnp.bfloat16, jnp.float32, jnp.uint32, jnp.int32

S, DM, H, E, M, SEG = 2048, 1024, 32, 128, 8, 32
NSEG = S // SEG
NP = H // 2
UN = 4
R2 = math.sqrt(0.5)
MID = 'mid'
PAD = 28
HEAD = (0, 1, 2, 3, 5, 8, 13, 19, 24)
LATER = {3: (0, 1), 4: (2,), 5: (3, 4, 5), 6: (6, 7)}


def _to_u32(m):
    u = np.ascontiguousarray(m, dtype=np.float32).view(np.uint32)
    h = ((u + 0x7FFF + ((u >> 16) & 1)) >> 16).astype(np.uint32)
    return h[..., 0::2, :] | (h[..., 1::2, :] << 16)


def _mask_fill():
    r = np.arange(80)
    pos_of = lambda rr: np.where(rr < M, rr, np.where(rr < SEG, rr + M, rr - SEG + M))
    qhead = np.where(r < 64, r // 32, (r - 64) // 8)
    qpos = pos_of(np.where(r < 64, r % 32, SEG + (r - 64) % 8))
    khead, kpos = qhead, qpos
    vis = (qpos[:, None] < M) | (qpos[:, None] >= kpos[None, :])
    same = qhead[:, None] == khead[None, :]
    return np.where(same, np.where(vis, 0.0, -1e9), -np.inf).astype(np.float32)


RES = ((0, 12, 8, 4), (1, 15, 9, 7), (2, 14, 10, 6), (3, 13, 11, 5))
WP = 72
C_MD, C_MN, C_TW, C_MS, C_NUM = 0, 16, 22, 24, 88


@functools.lru_cache(maxsize=None)
def _fft_consts():
    md = np.zeros((16, 128, 128))
    for q in range(4):
        if q == 0:
            lay = [[(0, 0), (0, 1), (2, 0), (2, 1)], [(3, 1), (1, 0), (1, 1), (3, 0)]]
        else:
            lay = [[(0, 0), (1, 0), (0, 1), (1, 1)], [(2, 1), (3, 1), (2, 0), (3, 0)]]
        for h in range(2):
            ms_, ws_ = [], []
            for g, part in lay[h]:
                k = 16 * np.arange(32) + RES[q][g]
                th = 2 * np.pi * np.outer(np.arange(128 if q == 0 else 64), k) / DM
                c, s = np.cos(th), np.sin(th)
                if q == 0:
                    ms_.append(-s if part else c)
                else:
                    sg = (1.0 if RES[q][g] % 8 == q else -1.0) * (1.0 - 2.0 * h)
                    ms_.append(np.concatenate([-s, sg * c] if part else [c, sg * s]))
                ws_.append(np.where(k == 0, 1.0, 2.0) / DM)
            m = np.concatenate(ms_, axis=1)
            md[2 * q + h] = m
            md[8 + 2 * q + h] = (m * np.concatenate(ws_)[None, :]).T
    a, l = np.arange(64), np.arange(128)
    re = 16 * (a // 8) + a % 8
    im = re + 8
    ms = np.zeros((64, 128, 128))
    for dl in range(32):
        th = 2 * np.pi * np.outer(32 * a + dl, a) / S
        c, s = np.cos(th), np.sin(th)
        ms[2 * dl][:, re], ms[2 * dl][:, im] = np.concatenate([c, -s]), np.concatenate([s, c])
        ms[2 * dl + 1][:, re] = np.concatenate([c.T, s.T]) / S
        ms[2 * dl + 1][:, im] = np.concatenate([-s.T, c.T]) / S
    mn = np.zeros((6, 128, 128))
    th = 2 * np.pi * np.outer(np.arange(32), l) / 32
    mn[0, :32], mn[1, :32] = np.cos(th), -np.sin(th)
    mn[4, :, :32], mn[5, :, :32] = np.cos(th).T / DM, -np.sin(th).T / DM
    th = 2 * np.pi * np.outer(np.arange(16), a) / 16
    c, s = np.cos(th), np.sin(th)
    mn[2, :32] = np.block([[c, s], [-s, c]])
    mn[3, :, :32] = np.block([[c.T, -s.T], [s.T, c.T]]) / S
    th = 2 * np.pi * np.outer(a, l) / S
    tw = np.stack([np.cos(th), np.sin(th)]).astype(np.float32).view(np.uint32)
    return np.concatenate([_to_u32(md), _to_u32(mn), tw, _to_u32(ms)], axis=0)


def _bdot(a, b):
    return jnp.dot(a, b, preferred_element_type=F32)


def _bf(u):
    return pltpu.bitcast(u, BF)


def _cat(rows):
    return jnp.concatenate(rows, axis=0).astype(BF)


def _unpack2(u, p):
    if p == 0:
        return pltpu.bitcast(u << 16, F32)
    return pltpu.bitcast(u & jnp.uint32(0xFFFF0000), F32)


def _strassen_left(n, a):
    return (lambda: a(1, 0) + a(1, 1), lambda: a(1, 0) - a(0, 0), lambda: a(1, 1), lambda: a(0, 0) + a(1, 1),
            lambda: a(0, 0), lambda: a(0, 1) - a(1, 1), lambda: a(0, 0) + a(0, 1))[n]()


def _strassen_right(n, w):
    add = lambda u, v: (u.astype(F32) + v.astype(F32)).astype(BF)
    sub = lambda u, v: (u.astype(F32) - v.astype(F32)).astype(BF)
    return (lambda: w(0, 0), lambda: add(w(0, 0), w(0, 1)), lambda: sub(w(1, 0), w(0, 0)),
            lambda: add(w(0, 0), w(1, 1)), lambda: sub(w(0, 1), w(1, 1)), lambda: add(w(1, 0), w(1, 1)),
            lambda: w(1, 1))[n]()


def _strassen(left, right, done, ready=lambda k: None, dot=None):
    def mm(n):
        a, r, acc = left(n), right(n), None
        for k in range(0, r.shape[0], 512):
            d = (dot or _bdot)(a[:, k:k + 512], r[k:k + 512])
            acc = d if acc is None else acc + d
        return acc

    ready(0)
    m2 = mm(0)
    c22 = mm(1) - m2
    ready(1)
    m4 = mm(2)
    c21 = m2 + m4
    m1 = mm(3)
    c11, c22 = m1 + m4, c22 + m1
    m3 = mm(4)
    done(1, c21, c22 + m3)
    c11 = c11 + mm(5)
    ready(2)
    m5 = mm(6)
    done(0, c11 - m5, m3 + m5)


def _twiddle(z, k, n, sign):
    r, i = z
    if k == 0:
        return r, i
    if 4 * k == n:
        return (-i, r) if sign > 0 else (i, -r)
    c, s = math.cos(2 * math.pi * k / n), sign * math.sin(2 * math.pi * k / n)
    if 8 * k == n or 8 * k == 3 * n:
        if c * s > 0:
            return (r - i) * c, (r + i) * c
        return (r + i) * c, (i - r) * c
    return r * c - i * s, r * s + i * c


def _cfft(xs, sign):
    n = len(xs)
    if n == 1:
        return xs
    ev, od = _cfft(xs[0::2], sign), _cfft(xs[1::2], sign)
    out = [None] * n
    for k in range(n // 2):
        er, ei = ev[k]
        if 4 * k == n:
            orr, oi = od[k]
            lo, hi = (er - oi, ei + orr), (er + oi, ei - orr)
            out[k], out[k + n // 2] = (lo, hi) if sign > 0 else (hi, lo)
        else:
            tr, ti = _twiddle(od[k], k, n, sign)
            out[k], out[k + n // 2] = (er + tr, ei + ti), (er - tr, ei - ti)
    return out


def _rfft8(x):
    a0, a1, b0, b1 = x[0] + x[4], x[0] - x[4], x[2] + x[6], x[2] - x[6]
    c0, c1, d0, d1 = x[1] + x[5], x[1] - x[5], x[3] + x[7], x[3] - x[7]
    e, f = a0 + b0, c0 + d0
    g, h = (c1 - d1) * R2, (c1 + d1) * R2
    return [e + f, e - f, a1 + g, b1 + h, a0 - b0, c0 - d0, a1 - g, b1 - h]


def _irfft8(z):
    z0, z4, z1r, z1i, z2r, z2i, z3r, z3i = z
    e, f = z0 + z4, z0 - z4
    a1, g = z1r + z3r, (z1r - z3r) * R2
    b1, h = z1i + z3i, (z1i - z3i) * R2
    a0, b0, c0, d0 = e + z2r, e - z2r, f + z2i, f - z2i
    c1, d1 = g + h, h - g
    return [a0 + a1, c0 + c1, b0 + b1, d0 + d1, a0 - a1, c0 - c1, b0 - b1, d0 - d1]


def _kernel(x_hbm, mem0_hbm, wq_hbm, wk_hbm, wv_hbm, wo_hbm, bx_hbm, wr_hbm, wi_hbm, fill_hbm, cst_hbm,
            out_hbm,
            x_v, xpre_v, xs_v, mem0_v, fill_v, lhs_v, wqkv, wo_v, pre, os_v, ws_v, outa_v,
            bx_v, w_v, wn_v, wt, cst, zs, vv, tn, outb_v,
            sem_w, sem_in, sem_out):
    scale = E ** -0.5
    wus = [w.bitcast(U32) for w in (wq_hbm, wk_hbm, wv_hbm)]
    wo_u = wo_hbm.bitcast(U32)
    fus = [w.at[pl.ds(0, 512)].bitcast(U32) for w in (wr_hbm, wi_hbm)]

    def w_copy(j, t, sem):
        return pltpu.make_async_copy(wus[t].at[:, :, j, :], wqkv.at[j, t], sem)

    xpre_cp = pltpu.make_async_copy(x_hbm.at[:, pl.ds(0, 8), :], xpre_v, sem_w.at[17])
    head = [[divmod(f, 3) for f in range(HEAD[b], HEAD[b + 1])] for b in range(len(HEAD) - 1)]
    head_cps = [[w_copy(j, t, sem_w.at[b]) for j, t in grp] for b, grp in enumerate(head)]

    def b_rows(i, b):
        return b, i // 4, pl.ds(pl.multiple_of((i % 4) * 8, 8), 8)

    def fwd_cps(i):
        rows = b_rows(i, slice(None))
        sem = sem_w.at[8 + i]
        return ([w_copy(8 + i, t, sem) for t in range(3)]
                + [pltpu.make_async_copy(bx_hbm.at[rows], bx_v.at[rows], sem)]
                + [pltpu.make_async_copy(fus[t].at[:, pl.ds(pl.multiple_of(128 * (2 * i + h), 128), 128)],
                                         w_v.at[t, 2 * i + h], sem) for t in range(2) for h in range(2)])

    def part(src, dst, lo, hi, sem):
        return pltpu.make_async_copy(src.at[pl.ds(lo, hi - lo)], dst.at[pl.ds(lo, hi - lo)], sem)

    c0_cp = part(cst_hbm, cst, 0, C_MS, sem_w.at[16])
    a_cps = [pltpu.make_async_copy(wo_u.at[:, pl.ds(128 * n, 128)], wo_v.at[n], sem_in.at[0]) for n in range(8)]
    a_cps += [part(x_hbm, x_v, 0, UN, sem_in.at[0]), part(cst_hbm, cst, C_MS, C_MS + UN, sem_in.at[0]),
              pltpu.make_async_copy(mem0_hbm, mem0_v, sem_in.at[0]),
              pltpu.make_async_copy(fill_hbm, fill_v, sem_in.at[0])]
    b_cps = [part(x_hbm, x_v, UN, NSEG, sem_in.at[1]), part(cst_hbm, cst, C_MS + UN, C_NUM, sem_in.at[1])]
    b_cps += [pltpu.make_async_copy(w.at[pl.ds(512, 1)], wn_v.at[t], sem_in.at[1])
              for t, w in enumerate((wr_hbm, wi_hbm))]

    lane = lax.broadcasted_iota(I32, (8, 128), 1)
    alt = jnp.where(lane % 2 == 0, 1.0, -1.0).astype(F32)
    lo_half = lane < 64
    ev_grp = (lane // 32) % 2 == 0

    def half_coef(q):
        sg = -1.0 if q < 3 else 1.0
        tc, ts = math.cos(2 * math.pi * q / 16), -math.sin(2 * math.pi * q / 16)
        f = lambda lo, hi: jnp.where(lo_half, lo, hi).astype(F32)
        return f(1.0, ts), f(0.0, sg * tc), f(0.0, tc), f(sg, -sg * ts)

    pace = {'tok': None}

    def token(v):
        return (v if v.dtype == U32 else pltpu.bitcast(v, U32)) & cst[C_MN, 56:64, :]

    def gate(v):
        tok = pace['tok']
        if tok is None:
            return v
        return v | tok if v.dtype == U32 else pltpu.bitcast(pltpu.bitcast(v, U32) | tok, v.dtype)

    def gate2(z):
        return gate(z[0]), gate(z[1])

    def as_u32(rows):
        return pltpu.bitcast(_cat(rows), U32)

    def b_fwd(i):
        r0 = pl.multiple_of(i * 8, 8)
        hc = [None] + [half_coef(q) for q in range(1, 4)]
        tacc = jnp.zeros((8, 128), F32)
        zl = []

        def filt(k):
            e, t, ty = 2 * i + k // 4, (k // 2) % 2, k % 2
            u = jnp.concatenate([gate(w_v[t, e, pl.ds(m + ty + 64 * v, 8, stride=8), :])
                                 for m in (0, 6, 4, 2) for v in range(4)], axis=0)
            ut = pltpu.bitcast(pltpu.bitcast(u, F32).T, U32)
            for v in range(16):
                wt[t, ty, pl.ds(8 * (v % 4) * WP + 4 * e + v // 4, 8, stride=WP), :] = ut[8 * v:8 * v + 8]

        for b0 in range(0, 32, 2):
            rows = []
            for b in (b0, b0 + 1):
                xb = bx_v[(*b_rows(i, b), slice(None))].astype(F32)
                z = _rfft8([gate(xb[:, 128 * t:128 * t + 128]) for t in range(8)])
                tacc = jnp.where(lane == b, jnp.sum(z[0] * alt, axis=1, keepdims=True), tacc)
                for q in range(1, 4):
                    c1, c2, c3, c4 = hc[q]
                    zr, zi = z[2 * q], z[2 * q + 1]
                    pp = c1 * zr + c2 * zi
                    qq = pltpu.roll(c3 * zr + c4 * zi, 64, 1)
                    z[2 * q], z[2 * q + 1] = pp + qq, pp - qq
                rows.append(z)
            zl.append([as_u32([rows[0][n], rows[1][n]]) for n in range(8)])
            yield 200
            if b0 % 4 == 0:
                filt(b0 // 4)
                yield 40
        tn[pl.ds(r0, 8), :] = tacc

        def mm(n):
            return _bdot(_bf(jnp.concatenate([z[n] for z in zl], axis=0)), _bf(cst[C_MD + n]))

        yield MID
        oo = [mm(n) for n in range(4)]
        yield MID
        oo += [mm(n) for n in range(4, 8)]
        yield MID
        for q in range(4):
            sel, sh = (ev_grp, 96) if q == 0 else (lo_half, 64)
            ys = []
            for b0 in range(4):
                xs = []
                for b in range(b0, 32, 4):
                    e_, o_ = gate(oo[2 * q][8 * b:8 * b + 8]), oo[2 * q + 1][8 * b:8 * b + 8]
                    xs.append((jnp.where(sel, e_, o_), pltpu.roll(jnp.where(sel, o_, e_), sh, 1)))
                ys.append([_twiddle(y, b0 * k1, 32, -1) for k1, y in enumerate(_cfft(xs, -1))])
                yield 110
            for k1 in range(8):
                for k0, y in enumerate(_cfft([gate2(ys[b0][k1]) for b0 in range(4)], -1)):
                    zs[k1 + 8 * k0, q, pl.ds(pl.multiple_of(2 * r0, 16), 16), :] = _cat(y)
                yield 30

    def b_mid(it):
        for n in range(4):
            for r in range(0, 64, 8):
                blk = lambda k, p: _bf(gate(wo_v[n + 4 * p, pl.ds(pl.multiple_of((2 * it + k) * 64 + r, 8), 8), :]))
                vals = [pltpu.bitcast(_strassen_right(m, blk), U32) for m in range(1, 6)]
                for m in range(5):
                    ws_v[n, m, pl.ds(pl.multiple_of(it * 64 + r, 8), 8), :] = vals[m]
                yield vals if 8 * n + r // 8 > 1 else None
        yield MID
        for dl in (2 * it, 2 * it + 1):
            y = _bdot(_bf(cst[C_MS + 2 * dl]), jnp.concatenate([zs[dl, q] for q in range(4)], axis=1))
            for _ in range(4):
                yield None
            w0 = pl.multiple_of(dl * WP, 8)
            rows = []
            for r in range(8):
                wq = []
                for t in range(2):
                    ta, tb = wt[t, 0, pl.ds(w0 + 8 * r, 8), :], wt[t, 1, pl.ds(w0 + 8 * r, 8), :]
                    wq.append([_unpack2(ta, 0), _unpack2(jnp.where(ev_grp, ta, tb), 1),
                               _unpack2(tb, 0), _unpack2(jnp.where(ev_grp, tb, ta), 1)])
                cols = []
                for q in range(4):
                    yr = gate(y[8 * r:8 * r + 8, 128 * q:128 * q + 128])
                    yi = gate(y[64 + 8 * r:72 + 8 * r, 128 * q:128 * q + 128])
                    wr, wi = wq[0][q], wq[1][q]
                    cols.append(as_u32([yr * wr - yi * wi, yr * wi + yi * wr]))
                rows.append(jnp.concatenate(cols, axis=1))
                yield cols
                yield None
            yield MID
            vv[dl] = _bdot(_bf(cst[C_MS + 2 * dl + 1]), _bf(jnp.concatenate(rows, axis=0)))

    def b_nyq():
        c, s = pltpu.bitcast(cst[C_TW], F32), pltpu.bitcast(cst[C_TW + 1], F32)
        tb = tn[...].astype(BF)
        tr, ti = _bdot(tb, _bf(cst[C_MN])), _bdot(tb, _bf(cst[C_MN + 1]))
        yield MID
        y = _bdot(_bf(cst[C_MN + 2, 0:16, :]), _cat([tr * c + ti * s, ti * c - tr * s]))
        row = lax.broadcasted_iota(I32, (16, 128), 0)
        wn = []
        for t in range(2):
            wrow = wn_v[t].astype(F32)
            acc = jnp.zeros((16, 128), F32)
            for e in range(16):
                acc = jnp.where(row == e, wrow[:, 128 * e:128 * e + 128], acc)
            wn.append(acc)
        yr, yi = y[0:16], y[16:32]
        yield MID
        v = _bdot(_bf(cst[C_MN + 3, :, 0:32]), _cat([yr * wn[0] - yi * wn[1], yr * wn[1] + yi * wn[0]]))
        vr, vi = v[0:64], v[64:128]
        yield MID
        tn[...] = (_bdot((vr * c - vi * s).astype(BF), _bf(cst[C_MN + 4]))
                   + _bdot((vr * s + vi * c).astype(BF), _bf(cst[C_MN + 5])))

    def b_inv(i, ul):
        r0 = i * 8
        for q in range(4):
            sel, sh = (ev_grp, 32) if q == 0 else (lo_half, 64)
            ys = []
            for b0 in range(4):
                xs = [(gate(vv[dl, pl.ds(r0, 8), 128 * q:128 * q + 128]),
                       gate(vv[dl, pl.ds(64 + r0, 8), 128 * q:128 * q + 128])) for dl in range(b0, 32, 4)]
                ys.append([_twiddle(y, b0 * k1, 32, +1) for k1, y in enumerate(_cfft(xs, +1))])
                yield 110
            ie, io = [], []
            for k1 in range(8):
                es, os_ = [], []
                for ur, ui in _cfft([gate2(ys[b0][k1]) for b0 in range(4)], +1):
                    tmp = pltpu.roll(ui, sh, 1)
                    es.append(jnp.where(sel, ur, tmp))
                    os_.append(jnp.where(sel, tmp, ur))
                ie += [as_u32(es[0:2]), as_u32(es[2:4])]
                io += [as_u32(os_[0:2]), as_u32(os_[2:4])]
                yield 55, ie[-2:] + io[-2:]
            ul += [ie, io]

    def b_fin(i, zz):
        r0 = i * 8
        hc = [None] + [half_coef(q) for q in range(1, 4)]
        tb = tn[pl.ds(r0, 8), :]
        for g in range(32):
            b = g // 4 + 8 * (g % 4)
            z = [gate(zz[n][8 * g:8 * g + 8]) for n in range(8)]
            z[0] = z[0] + jnp.sum(jnp.where(lane == b, tb, 0.0), axis=1, keepdims=True) * alt
            for q in range(1, 4):
                c1, c2, c3, c4 = hc[q]
                pp = z[2 * q] + z[2 * q + 1]
                qq = pltpu.roll(z[2 * q] - z[2 * q + 1], 64, 1)
                z[2 * q], z[2 * q + 1] = c1 * pp + c3 * qq, c2 * pp + c4 * qq
            y = _irfft8(z)
            outb_v[(*b_rows(i, b), slice(None))] = jnp.concatenate(y, axis=1).astype(BF)
            yield 75, y
        rows = b_rows(i, slice(None))
        start_out(outb_v.at[rows], out_hbm.at[(*rows, pl.ds(DM, DM))])

    def tie(w, vals):
        if not vals:
            return w
        acc = None
        for v in vals:
            v = v if v.dtype == U32 else pltpu.bitcast(v, U32)
            acc = v if acc is None else acc | v
        return jnp.concatenate([w[0:8] | token(acc), w[8:]], axis=0)

    def paced_dot(gen, budget):
        st = {'debt': 0, 'k': 0}
        due = {}

        def emit(d, b):
            while st['debt'] < b:
                r = 8 * (32 * st['debt'] // b)
                pace['tok'] = token(d[r:r + 8])
                c = next(gen, MID)
                if c is MID:
                    st['debt'] = b
                elif isinstance(c, list):
                    st['debt'] = 0
                    for own in c:
                        emit(own, 300)
                    return
                else:
                    if isinstance(c, tuple):
                        due.setdefault(st['k'] + 2, []).extend(c[1])
                        c = c[0]
                    st['debt'] += c
            st['debt'] -= b

        def dot(a, w):
            vals = due.pop(st['k'], None)
            if vals:
                a = jnp.concatenate([_bf(tie(pltpu.bitcast(a[:, 0:128], U32), vals)), a[:, 128:]], axis=1)
            d = _bdot(a, w)
            st['k'] += 1
            emit(d, budget)
            return d

        return dot

    out_cps = []

    def start_out(src, dst):
        out_cps.append(pltpu.make_async_copy(src, dst, sem_out.at[0]))
        out_cps[-1].start()

    hb = DM // 32

    def retile(j, t, k):
        blk = pl.ds(k * hb, hb)
        a, b = wqkv[j, t, blk, pl.ds(0, 8, stride=2), :], wqkv[j, t, blk, pl.ds(1, 8, stride=2), :]
        lo, hi = (a & jnp.uint32(0xFFFF)) | (b << 16), (a >> 16) | (b & jnp.uint32(0xFFFF0000))
        wqkv[j, t, blk, 0:8, :] = lo
        wqkv[j, t, blk, 8:16, :] = hi
        return lo

    def strassen_lhs():
        for g in range(NSEG // 4):
            xa = [xpre_v[4 * g + k].astype(F32) for k in range(4)]
            a1, a2 = jnp.concatenate([xa[0], xa[2]], axis=0), jnp.concatenate([xa[1], xa[3]], axis=0)
            a11, a12, a21, a22 = a1[:, :DM // 2], a1[:, DM // 2:], a2[:, :DM // 2], a2[:, DM // 2:]
            for n in range(7):
                v = _strassen_left(n, lambda r, k: ((a11, a12), (a21, a22))[r][k])
                xs_v[n, 8 * g:8 * g + 8, :] = pltpu.bitcast(v.astype(BF), U32)

    def pre_step(j, t, dot=None, sync=None):
        fresh = {}

        def w(k, p):
            v = fresh.pop((k, p), None)
            if v is None:
                v = wqkv[j, t, k * hb:(k + 1) * hb, 8 * p:8 * p + 8, :]
            return _bf(v.reshape(DM // 4, E))

        def done(h, c1, c2):
            v = jnp.concatenate([c.reshape(NSEG // 2, 8, E) for c in (c1, c2)], axis=1)
            pre[j, t, :, h] = pltpu.bitcast(v.astype(BF), U32)

        def ready(k):
            if k < 2:
                fresh[k, 0] = retile(j, t, k)
            elif sync:
                sync()

        _strassen(lambda n: _bf(xs_v[n]), lambda n: _strassen_right(n, w), done, ready, dot)

    for cp in [xpre_cp] + [cp for grp in head_cps for cp in grp]:
        cp.start()
    vv[0:PAD] = jnp.zeros((PAD,) + vv.shape[1:], F32)
    xpre_cp.wait()
    strassen_lhs()

    def pre_fwd(steps, i, budget):
        gen = b_fwd(i)
        dot = paced_dot(gen, budget)
        for j, t in steps + [(8 + i, t) for t in range(3)]:
            pre_step(j, t, dot)
        for _ in gen:
            pass

    def sync(b):
        for i in LATER.get(b, ()):
            for cp in ([c0_cp] if i == 0 else []) + fwd_cps(i):
                cp.start()
        for cp in head_cps[b + 1] + ([c0_cp] + fwd_cps(0) if b + 2 == len(head) else []):
            cp.wait()

    sync(-1)
    for b, grp in enumerate(head[:-1]):
        for j, t in grp:
            pre_step(j, t, sync=functools.partial(sync, b) if (j, t) == grp[-1] else None)
    pre_fwd(head[-1], 0, 130)
    for cp in a_cps + b_cps:
        cp.start()

    def pre_fwd_body(i, carry):
        for cp in fwd_cps(i):
            cp.wait()
        pre_fwd([], i, 340)
        return carry

    lax.fori_loop(1, 8, pre_fwd_body, 0)
    for cp in a_cps:
        cp.wait()

    def seg_step(s, u, mem, slot, opost):
        xs = x_v[s]
        lhs_v[u] = as_u32([mem, xs[8:32].astype(F32)])
        fill = fill_v[...]
        toks = []
        pace['tok'] = None

        def proj(j, t):
            w0, w1 = [wqkv[j, t, :, 8 * p:8 * p + 8, :].reshape(DM // 2, E) for p in range(2)]
            r0, r1 = _bdot(_bf(lhs_v[u]), _bf(tie(w0, slot()))), _bdot(_bf(lhs_v[u]), _bf(w1))
            toks.append(r0[0:8])
            if len(toks) >= 4:
                pace['tok'] = token(toks[-4])
            return _cat([r0, r1, _bf(pre[j, t, s // 2, u % 2]).astype(F32)])

        def qk(q, k):
            sc = lax.dot_general(q, k, (((1,), (1,)), ((), ())), preferred_element_type=F32) * scale
            sc = jnp.where(fill == 0.0, sc, fill)
            p = jnp.exp(sc - jnp.max(sc, axis=-1, keepdims=True))
            return (p * pl.reciprocal(jnp.sum(p, axis=-1, keepdims=True), approx=True)).astype(BF)

        ob, ps, vs = {}, {}, {}

        def pv(j):
            o = _bdot(ps[j], vs[j])
            opost[u, j] = (o[64:72], o[72:80])
            if u == UN - 1:
                vals = [as_u32([_strassen_left(n, lambda r, k: opost[2 * g + r, j][k]) for g in range(2)])
                        for n in range(7)]
                for n in range(7):
                    os_v[n, pl.ds(pl.multiple_of(2 * (s - u), 8), 8), 128 * j:128 * j + 128] = vals[n]
            ob[j] = [o[0:32], o[32:64]]

        def wo(g0, g1):
            og = jnp.concatenate([o for j in range(2 * g0, 2 * g1) for o in ob[j]], axis=1).astype(BF)
            return jnp.concatenate([_bdot(og, _bf(wo_v[n, g0 * 256:g1 * 256, :])) for n in range(8)], axis=1)

        ng = NP // 2
        for g in range(ng):
            ja, jb = 2 * g, 2 * g + 1
            qa, ka, qb, kb = proj(ja, 0), proj(ja, 1), proj(jb, 0), proj(jb, 1)
            vs[ja], vs[jb] = proj(ja, 2), proj(jb, 2)
            ps[ja], ps[jb] = qk(qa, ka), qk(qb, kb)
            if g > 0:
                pv(ja - 2)
                pv(jb - 2)
        res = wo(0, 3)
        pv(NP - 2)
        pv(NP - 1)
        res = res + wo(3, ng - 1)
        res = res + wo(ng - 1, ng)
        outa_v[s // 2, u % 2, 8:32, :] = res[8:32].astype(BF)
        return res[0:8].astype(BF).astype(F32)

    def loop_body(it, mem):
        @pl.when(it == 1)
        def _():
            for cp in b_cps:
                cp.wait()

        gen = b_mid(it)
        opost = {}
        state = {'mid': False}

        def slot():
            if state['mid']:
                return None
            vals = next(gen, None)
            if vals is MID:
                state['mid'] = True
                return None
            return vals

        for u in range(UN):
            state['mid'] = False
            mem = seg_step(UN * it + u, u, mem, slot, opost)
        for _ in gen:
            pass
        return mem

    lax.fori_loop(0, NSEG // UN, loop_body, mem0_v[...].astype(F32))
    idx = (slice(None), slice(None), pl.ds(8, SEG - 8), pl.ds(0, DM))
    start_out(outa_v.at[idx], out_hbm.at[idx])

    def b_inv_all():
        nyq = b_nyq()
        zz = None
        for i in range(8):
            ul = []
            for k, c in enumerate(b_inv(i, ul)):
                if k % 10 == 0:
                    next(nyq, None)
                yield c
            if i > 0:
                yield from b_fin(i - 1, zz)
            else:
                yield MID
            zz = [_bdot(_bf(jnp.concatenate(ul[n], axis=0)), _bf(cst[C_MD + 8 + n])) for n in range(8)]
            if i < 7:
                yield [zz[3], zz[7]]
        yield MID
        yield MID
        yield from b_fin(7, zz)

    gen = b_inv_all()
    dot = paced_dot(gen, 450)
    for n in range(4):
        def done(r, *cs):
            for p, cc in enumerate(cs):
                idx = (slice(None), r, pl.ds(0, 8), pl.ds(128 * (n + 4 * p), 128))
                outa_v[idx] = cc.reshape(NSEG // 2, 8, 128).astype(BF)
                start_out(outa_v.at[idx], out_hbm.at[idx])

        heads = lambda k: jnp.concatenate([wo_v[n + 4 * k, 64 * h:64 * h + 64, :] for h in range(k, H, 2)], axis=0)
        right = lambda m: _bf(heads(m // 6) if m % 6 == 0 else ws_v[n, m - 1])
        _strassen(lambda m: _bf(os_v[m]), right, done, dot=dot)
    for _ in gen:
        pass
    for cp in out_cps:
        cp.wait()


def pallas_concat_heads__memory_aug_recurrent_mem_tr__spectral_gfnet__prompt_kernel(
    A_x, A_mem0, A_Wq, A_Wk, A_Wv, A_Wo, A_seg_len, B_x, B_w_r, B_w_i,
):
    assert A_x.shape == (1, S, DM) and A_Wq.shape == (DM, H, E) and A_mem0.shape == (1, M, DM)
    assert B_x.shape == (1, S, DM) and (not isinstance(A_seg_len, int) or A_seg_len == SEG)
    hbm = pl.BlockSpec(memory_space=pltpu.HBM)
    wr = lambda w: w.reshape(DM // 16, 16, H, E)
    out = pl.pallas_call(
        _kernel,
        out_shape=jax.ShapeDtypeStruct((NSEG // 2, 2, SEG, 2 * DM), BF),
        in_specs=[hbm] * 11,
        out_specs=hbm,
        scratch_shapes=[
            pltpu.VMEM((NSEG, SEG, DM), BF),
            pltpu.VMEM((NSEG, 8, DM), BF),
            pltpu.VMEM((7, NSEG * 2, DM // 2), U32),
            pltpu.VMEM((M, DM), BF),
            pltpu.VMEM((80, 80), F32),
            pltpu.VMEM((UN, SEG // 2, DM), U32),
            pltpu.VMEM((NP, 3, DM // 16, 16, E), U32),
            pltpu.VMEM((8, H * E // 2, 128), U32),
            pltpu.VMEM((NP, 3, NSEG // 2, 2, 8, E), U32),
            pltpu.VMEM((7, NSEG * 2, H * E // 2), U32),
            pltpu.VMEM((4, 5, H * E // 4, 128), U32),
            pltpu.VMEM((NSEG // 2, 2, SEG, DM), BF),
            pltpu.VMEM((NSEG // 2, 2, SEG, DM), BF),
            pltpu.VMEM((2, 16, 256, 128), U32),
            pltpu.VMEM((2, 1, S), BF),
            pltpu.VMEM((2, 2, 32 * WP, 128), U32),
            pltpu.VMEM((C_NUM, 64, 128), U32),
            pltpu.VMEM((32, 4, 128, 128), BF),
            pltpu.VMEM((32, 128, 512), F32),
            pltpu.VMEM((64, 128), F32),
            pltpu.VMEM((NSEG // 2, 2, SEG, DM), BF),
            pltpu.SemaphoreType.DMA((NP + 2,)),
            pltpu.SemaphoreType.DMA((2,)),
            pltpu.SemaphoreType.DMA((1,)),
        ],
        compiler_params=pltpu.CompilerParams(vmem_limit_bytes=118 * 1024 * 1024, disable_semaphore_checks=True),
    )(A_x.reshape(NSEG, SEG, DM), A_mem0.reshape(M, DM), wr(A_Wq), wr(A_Wk), wr(A_Wv),
      A_Wo.reshape(H * E, DM), B_x.reshape(NSEG // 2, 2, SEG, DM), B_w_r.T, B_w_i.T, _mask_fill(), _fft_consts())
    return out.reshape(1, S, 2 * DM)
```

```python
import functools
import math

import jax
import jax.numpy as jnp
import numpy as np
from jax import lax
import jax.experimental.pallas as pl
import jax.experimental.pallas.tpu as pltpu

BF, F32, U32, I32 = jnp.bfloat16, jnp.float32, jnp.uint32, jnp.int32

S, DM, H, E, M, SEG = 2048, 1024, 32, 128, 8, 32
NSEG = S // SEG
NP = H // 2
UN = 4
R2 = math.sqrt(0.5)
MID = 'mid'
PAD = 28
HEAD = (0, 1, 2, 3, 5, 8, 13, 19, 24)
LATER = {3: (0, 1), 4: (2,), 5: (3, 4, 5), 6: (6, 7)}


def _to_u32(m):
    u = np.ascontiguousarray(m, dtype=np.float32).view(np.uint32)
    h = ((u + 0x7FFF + ((u >> 16) & 1)) >> 16).astype(np.uint32)
    return h[..., 0::2, :] | (h[..., 1::2, :] << 16)


def _mask_fill():
    r = np.arange(80)
    pos_of = lambda rr: np.where(rr < M, rr, np.where(rr < SEG, rr + M, rr - SEG + M))
    qhead = np.where(r < 64, r // 32, (r - 64) // 8)
    qpos = pos_of(np.where(r < 64, r % 32, SEG + (r - 64) % 8))
    khead, kpos = qhead, qpos
    vis = (qpos[:, None] < M) | (qpos[:, None] >= kpos[None, :])
    same = qhead[:, None] == khead[None, :]
    return np.where(same, np.where(vis, 0.0, -1e9), -np.inf).astype(np.float32)


RES = ((0, 12, 8, 4), (1, 15, 9, 7), (2, 14, 10, 6), (3, 13, 11, 5))
WP = 72
C_MD, C_MN, C_TW, C_MS, C_NUM = 0, 16, 22, 24, 88


@functools.lru_cache(maxsize=None)
def _fft_consts():
    md = np.zeros((16, 128, 128))
    for q in range(4):
        if q == 0:
            lay = [[(0, 0), (0, 1), (2, 0), (2, 1)], [(3, 1), (1, 0), (1, 1), (3, 0)]]
        else:
            lay = [[(0, 0), (1, 0), (0, 1), (1, 1)], [(2, 1), (3, 1), (2, 0), (3, 0)]]
        for h in range(2):
            ms_, ws_ = [], []
            for g, part in lay[h]:
                k = 16 * np.arange(32) + RES[q][g]
                th = 2 * np.pi * np.outer(np.arange(128 if q == 0 else 64), k) / DM
                c, s = np.cos(th), np.sin(th)
                if q == 0:
                    ms_.append(-s if part else c)
                else:
                    sg = (1.0 if RES[q][g] % 8 == q else -1.0) * (1.0 - 2.0 * h)
                    ms_.append(np.concatenate([-s, sg * c] if part else [c, sg * s]))
                ws_.append(np.where(k == 0, 1.0, 2.0) / DM)
            m = np.concatenate(ms_, axis=1)
            md[2 * q + h] = m
            md[8 + 2 * q + h] = (m * np.concatenate(ws_)[None, :]).T
    a, l = np.arange(64), np.arange(128)
    re = 16 * (a // 8) + a % 8
    im = re + 8
    ms = np.zeros((64, 128, 128))
    for dl in range(32):
        th = 2 * np.pi * np.outer(32 * a + dl, a) / S
        c, s = np.cos(th), np.sin(th)
        ms[2 * dl][:, re], ms[2 * dl][:, im] = np.concatenate([c, -s]), np.concatenate([s, c])
        ms[2 * dl + 1][:, re] = np.concatenate([c.T, s.T]) / S
        ms[2 * dl + 1][:, im] = np.concatenate([-s.T, c.T]) / S
    mn = np.zeros((6, 128, 128))
    th = 2 * np.pi * np.outer(np.arange(32), l) / 32
    mn[0, :32], mn[1, :32] = np.cos(th), -np.sin(th)
    mn[4, :, :32], mn[5, :, :32] = np.cos(th).T / DM, -np.sin(th).T / DM
    th = 2 * np.pi * np.outer(np.arange(16), a) / 16
    c, s = np.cos(th), np.sin(th)
    mn[2, :32] = np.block([[c, s], [-s, c]])
    mn[3, :, :32] = np.block([[c.T, -s.T], [s.T, c.T]]) / S
    th = 2 * np.pi * np.outer(a, l) / S
    tw = np.stack([np.cos(th), np.sin(th)]).astype(np.float32).view(np.uint32)
    return np.concatenate([_to_u32(md), _to_u32(mn), tw, _to_u32(ms)], axis=0)


def _bdot(a, b):
    return jnp.dot(a, b, preferred_element_type=F32)


def _bf(u):
    return pltpu.bitcast(u, BF)


def _cat(rows):
    return jnp.concatenate(rows, axis=0).astype(BF)


def _unpack2(u, p):
    if p == 0:
        return pltpu.bitcast(u << 16, F32)
    return pltpu.bitcast(u & jnp.uint32(0xFFFF0000), F32)


def _strassen_left(n, a):
    return (lambda: a(1, 0) + a(1, 1), lambda: a(1, 0) - a(0, 0), lambda: a(1, 1), lambda: a(0, 0) + a(1, 1),
            lambda: a(0, 0), lambda: a(0, 1) - a(1, 1), lambda: a(0, 0) + a(0, 1))[n]()


def _strassen_right(n, w):
    add = lambda u, v: (u.astype(F32) + v.astype(F32)).astype(BF)
    sub = lambda u, v: (u.astype(F32) - v.astype(F32)).astype(BF)
    return (lambda: w(0, 0), lambda: add(w(0, 0), w(0, 1)), lambda: sub(w(1, 0), w(0, 0)),
            lambda: add(w(0, 0), w(1, 1)), lambda: sub(w(0, 1), w(1, 1)), lambda: add(w(1, 0), w(1, 1)),
            lambda: w(1, 1))[n]()


def _strassen(left, right, done, ready=lambda k: None, dot=None):
    def mm(n):
        a, r, acc = left(n), right(n), None
        for k in range(0, r.shape[0], 512):
            d = (dot or _bdot)(a[:, k:k + 512], r[k:k + 512])
            acc = d if acc is None else acc + d
        return acc

    ready(0)
    m2 = mm(0)
    c22 = mm(1) - m2
    ready(1)
    m4 = mm(2)
    c21 = m2 + m4
    m1 = mm(3)
    c11, c22 = m1 + m4, c22 + m1
    m3 = mm(4)
    done(1, c21, c22 + m3)
    c11 = c11 + mm(5)
    ready(2)
    m5 = mm(6)
    done(0, c11 - m5, m3 + m5)


def _twiddle(z, k, n, sign):
    r, i = z
    if k == 0:
        return r, i
    if 4 * k == n:
        return (-i, r) if sign > 0 else (i, -r)
    c, s = math.cos(2 * math.pi * k / n), sign * math.sin(2 * math.pi * k / n)
    if 8 * k == n or 8 * k == 3 * n:
        if c * s > 0:
            return (r - i) * c, (r + i) * c
        return (r + i) * c, (i - r) * c
    return r * c - i * s, r * s + i * c


def _cfft(xs, sign):
    n = len(xs)
    if n == 1:
        return xs
    ev, od = _cfft(xs[0::2], sign), _cfft(xs[1::2], sign)
    out = [None] * n
    for k in range(n // 2):
        er, ei = ev[k]
        if 4 * k == n:
            orr, oi = od[k]
            lo, hi = (er - oi, ei + orr), (er + oi, ei - orr)
            out[k], out[k + n // 2] = (lo, hi) if sign > 0 else (hi, lo)
        else:
            tr, ti = _twiddle(od[k], k, n, sign)
            out[k], out[k + n // 2] = (er + tr, ei + ti), (er - tr, ei - ti)
    return out


def _rfft8(x):
    a0, a1, b0, b1 = x[0] + x[4], x[0] - x[4], x[2] + x[6], x[2] - x[6]
    c0, c1, d0, d1 = x[1] + x[5], x[1] - x[5], x[3] + x[7], x[3] - x[7]
    e, f = a0 + b0, c0 + d0
    g, h = (c1 - d1) * R2, (c1 + d1) * R2
    return [e + f, e - f, a1 + g, b1 + h, a0 - b0, c0 - d0, a1 - g, b1 - h]


def _irfft8(z):
    z0, z4, z1r, z1i, z2r, z2i, z3r, z3i = z
    e, f = z0 + z4, z0 - z4
    a1, g = z1r + z3r, (z1r - z3r) * R2
    b1, h = z1i + z3i, (z1i - z3i) * R2
    a0, b0, c0, d0 = e + z2r, e - z2r, f + z2i, f - z2i
    c1, d1 = g + h, h - g
    return [a0 + a1, c0 + c1, b0 + b1, d0 + d1, a0 - a1, c0 - c1, b0 - b1, d0 - d1]


def _kernel(x_hbm, mem0_hbm, wq_hbm, wk_hbm, wv_hbm, wo_hbm, bx_hbm, wr_hbm, wi_hbm, fill_hbm, cst_hbm,
            out_hbm,
            x_v, xpre_v, xs_v, mem0_v, fill_v, lhs_v, wqkv, wo_v, pre, os_v, ws_v, outa_v,
            bx_v, w_v, wn_v, wt, cst, zs, vv, tn, outb_v,
            sem_w, sem_in, sem_out):
    scale = E ** -0.5
    wus = [w.bitcast(U32) for w in (wq_hbm, wk_hbm, wv_hbm)]
    wo_u = wo_hbm.bitcast(U32)
    fus = [w.at[pl.ds(0, 512)].bitcast(U32) for w in (wr_hbm, wi_hbm)]

    def w_copy(j, t, sem):
        return pltpu.make_async_copy(wus[t].at[:, :, j, :], wqkv.at[j, t], sem)

    xpre_cp = pltpu.make_async_copy(x_hbm.at[:, pl.ds(0, 8), :], xpre_v, sem_w.at[17])
    head = [[divmod(f, 3) for f in range(HEAD[b], HEAD[b + 1])] for b in range(len(HEAD) - 1)]
    head_cps = [[w_copy(j, t, sem_w.at[b]) for j, t in grp] for b, grp in enumerate(head) if b > 0]
    first_cps = [pltpu.make_async_copy(wus[0].at[pl.ds(32 * k, 32), :, 0, :], wqkv.at[0, 0, pl.ds(32 * k, 32)],
                                       sem_w.at[18 * k]) for k in range(2)]
    head_cps.insert(0, first_cps)

    def b_rows(i, b):
        return b, i // 4, pl.ds(pl.multiple_of((i % 4) * 8, 8), 8)

    def fwd_cps(i):
        rows = b_rows(i, slice(None))
        sem = sem_w.at[8 + i]
        return ([w_copy(8 + i, t, sem) for t in range(3)]
                + [pltpu.make_async_copy(bx_hbm.at[rows], bx_v.at[rows], sem)]
                + [pltpu.make_async_copy(fus[t].at[:, pl.ds(pl.multiple_of(128 * (2 * i + h), 128), 128)],
                                         w_v.at[t, 2 * i + h], sem) for t in range(2) for h in range(2)])

    def part(src, dst, lo, hi, sem):
        return pltpu.make_async_copy(src.at[pl.ds(lo, hi - lo)], dst.at[pl.ds(lo, hi - lo)], sem)

    c0_cp = part(cst_hbm, cst, 0, C_MS, sem_w.at[16])
    a_cps = [pltpu.make_async_copy(wo_u.at[:, pl.ds(128 * n, 128)], wo_v.at[n], sem_in.at[0]) for n in range(8)]
    a_cps += [part(x_hbm, x_v, 0, UN, sem_in.at[0]), part(cst_hbm, cst, C_MS, C_MS + UN, sem_in.at[0]),
              pltpu.make_async_copy(mem0_hbm, mem0_v, sem_in.at[0]),
              pltpu.make_async_copy(fill_hbm, fill_v, sem_in.at[0])]
    b_cps = [part(x_hbm, x_v, UN, NSEG, sem_in.at[1]), part(cst_hbm, cst, C_MS + UN, C_NUM, sem_in.at[1])]
    b_cps += [pltpu.make_async_copy(w.at[pl.ds(512, 1)], wn_v.at[t], sem_in.at[1])
              for t, w in enumerate((wr_hbm, wi_hbm))]

    lane = lax.broadcasted_iota(I32, (8, 128), 1)
    alt = jnp.where(lane % 2 == 0, 1.0, -1.0).astype(F32)
    lo_half = lane < 64
    ev_grp = (lane // 32) % 2 == 0

    def half_coef(q):
        sg = -1.0 if q < 3 else 1.0
        tc, ts = math.cos(2 * math.pi * q / 16), -math.sin(2 * math.pi * q / 16)
        f = lambda lo, hi: jnp.where(lo_half, lo, hi).astype(F32)
        return f(1.0, ts), f(0.0, sg * tc), f(0.0, tc), f(sg, -sg * ts)

    pace = {'tok': None}

    def token(v):
        return (v if v.dtype == U32 else pltpu.bitcast(v, U32)) & cst[C_MN, 56:64, :]

    def gate(v):
        tok = pace['tok']
        if tok is None:
            return v
        return v | tok if v.dtype == U32 else pltpu.bitcast(pltpu.bitcast(v, U32) | tok, v.dtype)

    def gate2(z):
        return gate(z[0]), gate(z[1])

    def as_u32(rows):
        return pltpu.bitcast(_cat(rows), U32)

    def b_fwd(i):
        r0 = pl.multiple_of(i * 8, 8)
        hc = [None] + [half_coef(q) for q in range(1, 4)]
        tacc = jnp.zeros((8, 128), F32)
        zl = []

        def filt(k):
            e, t, ty = 2 * i + k // 4, (k // 2) % 2, k % 2
            u = jnp.concatenate([gate(w_v[t, e, pl.ds(m + ty + 64 * v, 8, stride=8), :])
                                 for m in (0, 6, 4, 2) for v in range(4)], axis=0)
            ut = pltpu.bitcast(pltpu.bitcast(u, F32).T, U32)
            for v in range(16):
                wt[t, ty, pl.ds(8 * (v % 4) * WP + 4 * e + v // 4, 8, stride=WP), :] = ut[8 * v:8 * v + 8]

        for b0 in range(0, 32, 2):
            rows = []
            for b in (b0, b0 + 1):
                xb = bx_v[(*b_rows(i, b), slice(None))].astype(F32)
                z = _rfft8([gate(xb[:, 128 * t:128 * t + 128]) for t in range(8)])
                tacc = jnp.where(lane == b, jnp.sum(z[0] * alt, axis=1, keepdims=True), tacc)
                for q in range(1, 4):
                    c1, c2, c3, c4 = hc[q]
                    zr, zi = z[2 * q], z[2 * q + 1]
                    pp = c1 * zr + c2 * zi
                    qq = pltpu.roll(c3 * zr + c4 * zi, 64, 1)
                    z[2 * q], z[2 * q + 1] = pp + qq, pp - qq
                rows.append(z)
            zl.append([as_u32([rows[0][n], rows[1][n]]) for n in range(8)])
            yield 200
            if b0 % 4 == 0:
                filt(b0 // 4)
                yield 40
        tn[pl.ds(r0, 8), :] = tacc

        def mm(n):
            return _bdot(_bf(jnp.concatenate([z[n] for z in zl], axis=0)), _bf(cst[C_MD + n]))

        yield MID
        oo = [mm(n) for n in range(4)]
        yield MID
        oo += [mm(n) for n in range(4, 8)]
        yield MID
        for q in range(4):
            sel, sh = (ev_grp, 96) if q == 0 else (lo_half, 64)
            ys = []
            for b0 in range(4):
                xs = []
                for b in range(b0, 32, 4):
                    e_, o_ = gate(oo[2 * q][8 * b:8 * b + 8]), oo[2 * q + 1][8 * b:8 * b + 8]
                    xs.append((jnp.where(sel, e_, o_), pltpu.roll(jnp.where(sel, o_, e_), sh, 1)))
                ys.append([_twiddle(y, b0 * k1, 32, -1) for k1, y in enumerate(_cfft(xs, -1))])
                yield 110
            for k1 in range(8):
                for k0, y in enumerate(_cfft([gate2(ys[b0][k1]) for b0 in range(4)], -1)):
                    zs[k1 + 8 * k0, q, pl.ds(pl.multiple_of(2 * r0, 16), 16), :] = _cat(y)
                yield 30

    def b_mid(it):
        for n in range(4):
            for r in range(0, 64, 8):
                blk = lambda k, p: _bf(gate(wo_v[n + 4 * p, pl.ds(pl.multiple_of((2 * it + k) * 64 + r, 8), 8), :]))
                vals = [pltpu.bitcast(_strassen_right(m, blk), U32) for m in range(1, 6)]
                for m in range(5):
                    ws_v[n, m, pl.ds(pl.multiple_of(it * 64 + r, 8), 8), :] = vals[m]
                yield vals if 8 * n + r // 8 > 1 else None
        yield MID
        for dl in (2 * it, 2 * it + 1):
            y = _bdot(_bf(cst[C_MS + 2 * dl]), jnp.concatenate([zs[dl, q] for q in range(4)], axis=1))
            for _ in range(4):
                yield None
            w0 = pl.multiple_of(dl * WP, 8)
            rows = []
            for r in range(8):
                wq = []
                for t in range(2):
                    ta, tb = wt[t, 0, pl.ds(w0 + 8 * r, 8), :], wt[t, 1, pl.ds(w0 + 8 * r, 8), :]
                    wq.append([_unpack2(ta, 0), _unpack2(jnp.where(ev_grp, ta, tb), 1),
                               _unpack2(tb, 0), _unpack2(jnp.where(ev_grp, tb, ta), 1)])
                cols = []
                for q in range(4):
                    yr = gate(y[8 * r:8 * r + 8, 128 * q:128 * q + 128])
                    yi = gate(y[64 + 8 * r:72 + 8 * r, 128 * q:128 * q + 128])
                    wr, wi = wq[0][q], wq[1][q]
                    cols.append(as_u32([yr * wr - yi * wi, yr * wi + yi * wr]))
                rows.append(jnp.concatenate(cols, axis=1))
                yield cols
                yield None
            yield MID
            vv[dl] = _bdot(_bf(cst[C_MS + 2 * dl + 1]), _bf(jnp.concatenate(rows, axis=0)))

    def b_nyq():
        c, s = pltpu.bitcast(cst[C_TW], F32), pltpu.bitcast(cst[C_TW + 1], F32)
        tb = tn[...].astype(BF)
        tr, ti = _bdot(tb, _bf(cst[C_MN])), _bdot(tb, _bf(cst[C_MN + 1]))
        yield MID
        y = _bdot(_bf(cst[C_MN + 2, 0:16, :]), _cat([tr * c + ti * s, ti * c - tr * s]))
        row = lax.broadcasted_iota(I32, (16, 128), 0)
        wn = []
        for t in range(2):
            wrow = wn_v[t].astype(F32)
            acc = jnp.zeros((16, 128), F32)
            for e in range(16):
                acc = jnp.where(row == e, wrow[:, 128 * e:128 * e + 128], acc)
            wn.append(acc)
        yr, yi = y[0:16], y[16:32]
        yield MID
        v = _bdot(_bf(cst[C_MN + 3, :, 0:32]), _cat([yr * wn[0] - yi * wn[1], yr * wn[1] + yi * wn[0]]))
        vr, vi = v[0:64], v[64:128]
        yield MID
        tn[...] = (_bdot((vr * c - vi * s).astype(BF), _bf(cst[C_MN + 4]))
                   + _bdot((vr * s + vi * c).astype(BF), _bf(cst[C_MN + 5])))

    def b_inv(i, ul):
        r0 = i * 8
        for q in range(4):
            sel, sh = (ev_grp, 32) if q == 0 else (lo_half, 64)
            ys = []
            for b0 in range(4):
                xs = [(gate(vv[dl, pl.ds(r0, 8), 128 * q:128 * q + 128]),
                       gate(vv[dl, pl.ds(64 + r0, 8), 128 * q:128 * q + 128])) for dl in range(b0, 32, 4)]
                ys.append([_twiddle(y, b0 * k1, 32, +1) for k1, y in enumerate(_cfft(xs, +1))])
                yield 110
            ie, io = [], []
            for k1 in range(8):
                es, os_ = [], []
                for ur, ui in _cfft([gate2(ys[b0][k1]) for b0 in range(4)], +1):
                    tmp = pltpu.roll(ui, sh, 1)
                    es.append(jnp.where(sel, ur, tmp))
                    os_.append(jnp.where(sel, tmp, ur))
                ie += [as_u32(es[0:2]), as_u32(es[2:4])]
                io += [as_u32(os_[0:2]), as_u32(os_[2:4])]
                yield 55, ie[-2:] + io[-2:]
            ul += [ie, io]

    def b_fin(i, zz):
        r0 = i * 8
        hc = [None] + [half_coef(q) for q in range(1, 4)]
        tb = tn[pl.ds(r0, 8), :]
        for g in range(32):
            b = g // 4 + 8 * (g % 4)
            z = [gate(zz[n][8 * g:8 * g + 8]) for n in range(8)]
            z[0] = z[0] + jnp.sum(jnp.where(lane == b, tb, 0.0), axis=1, keepdims=True) * alt
            for q in range(1, 4):
                c1, c2, c3, c4 = hc[q]
                pp = z[2 * q] + z[2 * q + 1]
                qq = pltpu.roll(z[2 * q] - z[2 * q + 1], 64, 1)
                z[2 * q], z[2 * q + 1] = c1 * pp + c3 * qq, c2 * pp + c4 * qq
            y = _irfft8(z)
            outb_v[(*b_rows(i, b), slice(None))] = jnp.concatenate(y, axis=1).astype(BF)
            yield 75, y
        rows = b_rows(i, slice(None))
        start_out(outb_v.at[rows], out_hbm.at[(*rows, pl.ds(DM, DM))])

    def tie(w, vals):
        if not vals:
            return w
        acc = None
        for v in vals:
            v = v if v.dtype == U32 else pltpu.bitcast(v, U32)
            acc = v if acc is None else acc | v
        return jnp.concatenate([w[0:8] | token(acc), w[8:]], axis=0)

    def paced_dot(gen, budget):
        st = {'debt': 0, 'k': 0}
        due = {}

        def emit(d, b):
            while st['debt'] < b:
                r = 8 * (32 * st['debt'] // b)
                pace['tok'] = token(d[r:r + 8])
                c = next(gen, MID)
                if c is MID:
                    st['debt'] = b
                elif isinstance(c, list):
                    st['debt'] = 0
                    for own in c:
                        emit(own, 300)
                    return
                else:
                    if isinstance(c, tuple):
                        due.setdefault(st['k'] + 2, []).extend(c[1])
                        c = c[0]
                    st['debt'] += c
            st['debt'] -= b

        def dot(a, w):
            vals = due.pop(st['k'], None)
            if vals:
                a = jnp.concatenate([_bf(tie(pltpu.bitcast(a[:, 0:128], U32), vals)), a[:, 128:]], axis=1)
            d = _bdot(a, w)
            st['k'] += 1
            emit(d, budget)
            return d

        return dot

    out_cps = []

    def start_out(src, dst):
        out_cps.append(pltpu.make_async_copy(src, dst, sem_out.at[0]))
        out_cps[-1].start()

    hb = DM // 32

    def retile(j, t, k):
        blk = pl.ds(k * hb, hb)
        a, b = wqkv[j, t, blk, pl.ds(0, 8, stride=2), :], wqkv[j, t, blk, pl.ds(1, 8, stride=2), :]
        lo, hi = (a & jnp.uint32(0xFFFF)) | (b << 16), (a >> 16) | (b & jnp.uint32(0xFFFF0000))
        wqkv[j, t, blk, 0:8, :] = lo
        wqkv[j, t, blk, 8:16, :] = hi
        return lo

    def strassen_lhs():
        for g in range(NSEG // 4):
            xa = [xpre_v[4 * g + k].astype(F32) for k in range(4)]
            a1, a2 = jnp.concatenate([xa[0], xa[2]], axis=0), jnp.concatenate([xa[1], xa[3]], axis=0)
            a11, a12, a21, a22 = a1[:, :DM // 2], a1[:, DM // 2:], a2[:, :DM // 2], a2[:, DM // 2:]
            for n in range(7):
                v = _strassen_left(n, lambda r, k: ((a11, a12), (a21, a22))[r][k])
                xs_v[n, 8 * g:8 * g + 8, :] = pltpu.bitcast(v.astype(BF), U32)

    def pre_step(j, t, dot=None, sync=None, first=False):
        fresh = {}

        def w(k, p):
            v = fresh.pop((k, p), None)
            if v is None:
                v = wqkv[j, t, k * hb:(k + 1) * hb, 8 * p:8 * p + 8, :]
            return _bf(v.reshape(DM // 4, E))

        def done(h, c1, c2):
            v = jnp.concatenate([c.reshape(NSEG // 2, 8, E) for c in (c1, c2)], axis=1)
            pre[j, t, :, h] = pltpu.bitcast(v.astype(BF), U32)

        def ready(k):
            if k < 2:
                if first:
                    first_cps[k].wait()
                fresh[k, 0] = retile(j, t, k)
            elif sync:
                sync()

        _strassen(lambda n: _bf(xs_v[n]), lambda n: _strassen_right(n, w), done, ready, dot)

    for cp in [xpre_cp] + [cp for grp in head_cps for cp in grp]:
        cp.start()
    vv[0:PAD] = jnp.zeros((PAD,) + vv.shape[1:], F32)
    xpre_cp.wait()
    strassen_lhs()

    def pre_fwd(steps, i, budget):
        gen = b_fwd(i)
        dot = paced_dot(gen, budget)
        for j, t in steps + [(8 + i, t) for t in range(3)]:
            pre_step(j, t, dot)
        for _ in gen:
            pass

    def sync(b):
        for i in LATER.get(b, ()):
            for cp in ([c0_cp] if i == 0 else []) + fwd_cps(i):
                cp.start()
        for cp in head_cps[b + 1] + ([c0_cp] + fwd_cps(0) if b + 2 == len(head) else []):
            cp.wait()

    for b, grp in enumerate(head[:-1]):
        for j, t in grp:
            pre_step(j, t, sync=functools.partial(sync, b) if (j, t) == grp[-1] else None, first=b == 0)
    pre_fwd(head[-1], 0, 130)
    for cp in a_cps + b_cps:
        cp.start()

    def pre_fwd_body(i, carry):
        for cp in fwd_cps(i):
            cp.wait()
        pre_fwd([], i, 340)
        return carry

    lax.fori_loop(1, 8, pre_fwd_body, 0)
    for cp in a_cps:
        cp.wait()

    def seg_step(s, u, mem, slot, opost):
        xs = x_v[s]
        lhs_v[u] = as_u32([mem, xs[8:32].astype(F32)])
        fill = fill_v[...]
        toks = []
        pace['tok'] = None

        def proj(j, t):
            w0, w1 = [wqkv[j, t, :, 8 * p:8 * p + 8, :].reshape(DM // 2, E) for p in range(2)]
            r0, r1 = _bdot(_bf(lhs_v[u]), _bf(tie(w0, slot()))), _bdot(_bf(lhs_v[u]), _bf(w1))
            toks.append(r0[0:8])
            if len(toks) >= 4:
                pace['tok'] = token(toks[-4])
            return _cat([r0, r1, _bf(pre[j, t, s // 2, u % 2]).astype(F32)])

        def qk(q, k):
            sc = lax.dot_general(q, k, (((1,), (1,)), ((), ())), preferred_element_type=F32) * scale
            sc = jnp.where(fill == 0.0, sc, fill)
            p = jnp.exp(sc - jnp.max(sc, axis=-1, keepdims=True))
            return (p * pl.reciprocal(jnp.sum(p, axis=-1, keepdims=True), approx=True)).astype(BF)

        ob, ps, vs = {}, {}, {}

        def pv(j):
            o = _bdot(ps[j], vs[j])
            opost[u, j] = (o[64:72], o[72:80])
            if u == UN - 1:
                vals = [as_u32([_strassen_left(n, lambda r, k: opost[2 * g + r, j][k]) for g in range(2)])
                        for n in range(7)]
                for n in range(7):
                    os_v[n, pl.ds(pl.multiple_of(2 * (s - u), 8), 8), 128 * j:128 * j + 128] = vals[n]
            ob[j] = [o[0:32], o[32:64]]

        def wo(g0, g1):
            og = jnp.concatenate([o for j in range(2 * g0, 2 * g1) for o in ob[j]], axis=1).astype(BF)
            return jnp.concatenate([_bdot(og, _bf(wo_v[n, g0 * 256:g1 * 256, :])) for n in range(8)], axis=1)

        ng = NP // 2
        for g in range(ng):
            ja, jb = 2 * g, 2 * g + 1
            qa, ka, qb, kb = proj(ja, 0), proj(ja, 1), proj(jb, 0), proj(jb, 1)
            vs[ja], vs[jb] = proj(ja, 2), proj(jb, 2)
            ps[ja], ps[jb] = qk(qa, ka), qk(qb, kb)
            if g > 0:
                pv(ja - 2)
                pv(jb - 2)
        res = wo(0, 3)
        pv(NP - 2)
        pv(NP - 1)
        res = res + wo(3, ng - 1)
        res = res + wo(ng - 1, ng)
        outa_v[s // 2, u % 2, 8:32, :] = res[8:32].astype(BF)
        return res[0:8].astype(BF).astype(F32)

    def loop_body(it, mem):
        @pl.when(it == 1)
        def _():
            for cp in b_cps:
                cp.wait()

        gen = b_mid(it)
        opost = {}
        state = {'mid': False}

        def slot():
            if state['mid']:
                return None
            vals = next(gen, None)
            if vals is MID:
                state['mid'] = True
                return None
            return vals

        for u in range(UN):
            state['mid'] = False
            mem = seg_step(UN * it + u, u, mem, slot, opost)
        for _ in gen:
            pass
        return mem

    lax.fori_loop(0, NSEG // UN, loop_body, mem0_v[...].astype(F32))
    idx = (slice(None), slice(None), pl.ds(8, SEG - 8), pl.ds(0, DM))
    start_out(outa_v.at[idx], out_hbm.at[idx])

    def b_inv_all():
        nyq = b_nyq()
        zz = None
        for i in range(8):
            ul = []
            for k, c in enumerate(b_inv(i, ul)):
                if k % 10 == 0:
                    next(nyq, None)
                yield c
            if i > 0:
                yield from b_fin(i - 1, zz)
            else:
                yield MID
            zz = [_bdot(_bf(jnp.concatenate(ul[n], axis=0)), _bf(cst[C_MD + 8 + n])) for n in range(8)]
            if i < 7:
                yield [zz[3], zz[7]]
        yield MID
        yield MID
        yield from b_fin(7, zz)

    gen = b_inv_all()
    dot = paced_dot(gen, 450)
    for n in range(4):
        def done(r, *cs):
            for p, cc in enumerate(cs):
                idx = (slice(None), r, pl.ds(0, 8), pl.ds(128 * (n + 4 * p), 128))
                outa_v[idx] = cc.reshape(NSEG // 2, 8, 128).astype(BF)
                start_out(outa_v.at[idx], out_hbm.at[idx])

        heads = lambda k: jnp.concatenate([wo_v[n + 4 * k, 64 * h:64 * h + 64, :] for h in range(k, H, 2)], axis=0)
        right = lambda m: _bf(heads(m // 6) if m % 6 == 0 else ws_v[n, m - 1])
        _strassen(lambda m: _bf(os_v[m]), right, done, dot=dot)
    for _ in gen:
        pass
    for cp in out_cps:
        cp.wait()


def pallas_concat_heads__memory_aug_recurrent_mem_tr__spectral_gfnet__prompt_kernel(
    A_x, A_mem0, A_Wq, A_Wk, A_Wv, A_Wo, A_seg_len, B_x, B_w_r, B_w_i,
):
    assert A_x.shape == (1, S, DM) and A_Wq.shape == (DM, H, E) and A_mem0.shape == (1, M, DM)
    assert B_x.shape == (1, S, DM) and (not isinstance(A_seg_len, int) or A_seg_len == SEG)
    hbm = pl.BlockSpec(memory_space=pltpu.HBM)
    wr = lambda w: w.reshape(DM // 16, 16, H, E)
    out = pl.pallas_call(
        _kernel,
        out_shape=jax.ShapeDtypeStruct((NSEG // 2, 2, SEG, 2 * DM), BF),
        in_specs=[hbm] * 11,
        out_specs=hbm,
        scratch_shapes=[
            pltpu.VMEM((NSEG, SEG, DM), BF),
            pltpu.VMEM((NSEG, 8, DM), BF),
            pltpu.VMEM((7, NSEG * 2, DM // 2), U32),
            pltpu.VMEM((M, DM), BF),
            pltpu.VMEM((80, 80), F32),
            pltpu.VMEM((UN, SEG // 2, DM), U32),
            pltpu.VMEM((NP, 3, DM // 16, 16, E), U32),
            pltpu.VMEM((8, H * E // 2, 128), U32),
            pltpu.VMEM((NP, 3, NSEG // 2, 2, 8, E), U32),
            pltpu.VMEM((7, NSEG * 2, H * E // 2), U32),
            pltpu.VMEM((4, 5, H * E // 4, 128), U32),
            pltpu.VMEM((NSEG // 2, 2, SEG, DM), BF),
            pltpu.VMEM((NSEG // 2, 2, SEG, DM), BF),
            pltpu.VMEM((2, 16, 256, 128), U32),
            pltpu.VMEM((2, 1, S), BF),
            pltpu.VMEM((2, 2, 32 * WP, 128), U32),
            pltpu.VMEM((C_NUM, 64, 128), U32),
            pltpu.VMEM((32, 4, 128, 128), BF),
            pltpu.VMEM((32, 128, 512), F32),
            pltpu.VMEM((64, 128), F32),
            pltpu.VMEM((NSEG // 2, 2, SEG, DM), BF),
            pltpu.SemaphoreType.DMA((NP + 3,)),
            pltpu.SemaphoreType.DMA((2,)),
            pltpu.SemaphoreType.DMA((1,)),
        ],
        compiler_params=pltpu.CompilerParams(vmem_limit_bytes=118 * 1024 * 1024, disable_semaphore_checks=True),
    )(A_x.reshape(NSEG, SEG, DM), A_mem0.reshape(M, DM), wr(A_Wq), wr(A_Wk), wr(A_Wv),
      A_Wo.reshape(H * E, DM), B_x.reshape(NSEG // 2, 2, SEG, DM), B_w_r.T, B_w_i.T, _mask_fill(), _fft_consts())
    return out.reshape(1, S, 2 * DM)
```

```python
import functools
import math

import jax
import jax.numpy as jnp
import numpy as np
from jax import lax
import jax.experimental.pallas as pl
import jax.experimental.pallas.tpu as pltpu

BF, F32, U32, I32 = jnp.bfloat16, jnp.float32, jnp.uint32, jnp.int32

S, DM, H, E, M, SEG = 2048, 1024, 32, 128, 8, 32
NSEG = S // SEG
NP = H // 2
UN = 4
R2 = math.sqrt(0.5)
MID = 'mid'
PAD = 28
HEAD = (0, 1, 2, 3, 5, 8, 13, 19, 24)
LATER = {3: (0, 1), 4: (2,), 5: (3, 4, 5), 6: (6, 7)}


def _to_u32(m):
    u = np.ascontiguousarray(m, dtype=np.float32).view(np.uint32)
    h = ((u + 0x7FFF + ((u >> 16) & 1)) >> 16).astype(np.uint32)
    return h[..., 0::2, :] | (h[..., 1::2, :] << 16)


def _mask_fill():
    r = np.arange(80)
    head = np.where(r < 64, r // 32, (r - 64) // 8)
    pos = np.where(r < 64, np.where(r % 32 < M, r % 32, r % 32 + M), (r - 64) % 8 + M)
    vis = (pos[:, None] < M) | (pos[:, None] >= pos[None, :])
    same = head[:, None] == head[None, :]
    return np.where(same, np.where(vis, 0.0, -1e9), -np.inf).astype(np.float32)


RES = ((0, 12, 8, 4), (1, 15, 9, 7), (2, 14, 10, 6), (3, 13, 11, 5))
WP = 72
C_MD, C_MN, C_TW, C_MS, C_NUM = 0, 16, 22, 24, 88


@functools.lru_cache(maxsize=None)
def _fft_consts():
    md = np.zeros((16, 128, 128))
    for q in range(4):
        if q == 0:
            lay = [[(0, 0), (0, 1), (2, 0), (2, 1)], [(3, 1), (1, 0), (1, 1), (3, 0)]]
        else:
            lay = [[(0, 0), (1, 0), (0, 1), (1, 1)], [(2, 1), (3, 1), (2, 0), (3, 0)]]
        for h in range(2):
            ms_, ws_ = [], []
            for g, part in lay[h]:
                k = 16 * np.arange(32) + RES[q][g]
                th = 2 * np.pi * np.outer(np.arange(128 if q == 0 else 64), k) / DM
                c, s = np.cos(th), np.sin(th)
                if q == 0:
                    ms_.append(-s if part else c)
                else:
                    sg = (1.0 if RES[q][g] % 8 == q else -1.0) * (1.0 - 2.0 * h)
                    ms_.append(np.concatenate([-s, sg * c] if part else [c, sg * s]))
                ws_.append(np.where(k == 0, 1.0, 2.0) / DM)
            m = np.concatenate(ms_, axis=1)
            md[2 * q + h] = m
            md[8 + 2 * q + h] = (m * np.concatenate(ws_)[None, :]).T
    a, l = np.arange(64), np.arange(128)
    re = 16 * (a // 8) + a % 8
    im = re + 8
    ms = np.zeros((64, 128, 128))
    for dl in range(32):
        th = 2 * np.pi * np.outer(32 * a + dl, a) / S
        c, s = np.cos(th), np.sin(th)
        ms[2 * dl][:, re], ms[2 * dl][:, im] = np.concatenate([c, -s]), np.concatenate([s, c])
        ms[2 * dl + 1][:, re] = np.concatenate([c.T, s.T]) / S
        ms[2 * dl + 1][:, im] = np.concatenate([-s.T, c.T]) / S
    mn = np.zeros((6, 128, 128))
    th = 2 * np.pi * np.outer(np.arange(32), l) / 32
    mn[0, :32], mn[1, :32] = np.cos(th), -np.sin(th)
    mn[4, :, :32], mn[5, :, :32] = np.cos(th).T / DM, -np.sin(th).T / DM
    th = 2 * np.pi * np.outer(np.arange(16), a) / 16
    c, s = np.cos(th), np.sin(th)
    mn[2, :32] = np.block([[c, s], [-s, c]])
    mn[3, :, :32] = np.block([[c.T, -s.T], [s.T, c.T]]) / S
    th = 2 * np.pi * np.outer(a, l) / S
    tw = np.stack([np.cos(th), np.sin(th)]).astype(np.float32).view(np.uint32)
    return np.concatenate([_to_u32(md), _to_u32(mn), tw, _to_u32(ms)], axis=0)


def _bdot(a, b):
    return jnp.dot(a, b, preferred_element_type=F32)


def _bf(u):
    return pltpu.bitcast(u, BF)


def _cat(rows):
    return jnp.concatenate(rows, axis=0).astype(BF)


def _unpack2(u, p):
    if p == 0:
        return pltpu.bitcast(u << 16, F32)
    return pltpu.bitcast(u & jnp.uint32(0xFFFF0000), F32)


def _strassen_left(n, a):
    return (lambda: a(1, 0) + a(1, 1), lambda: a(1, 0) - a(0, 0), lambda: a(1, 1), lambda: a(0, 0) + a(1, 1),
            lambda: a(0, 0), lambda: a(0, 1) - a(1, 1), lambda: a(0, 0) + a(0, 1))[n]()


def _strassen_right(n, w):
    add = lambda u, v: (u.astype(F32) + v.astype(F32)).astype(BF)
    sub = lambda u, v: (u.astype(F32) - v.astype(F32)).astype(BF)
    return (lambda: w(0, 0), lambda: add(w(0, 0), w(0, 1)), lambda: sub(w(1, 0), w(0, 0)),
            lambda: add(w(0, 0), w(1, 1)), lambda: sub(w(0, 1), w(1, 1)), lambda: add(w(1, 0), w(1, 1)),
            lambda: w(1, 1))[n]()


def _strassen(left, right, done, ready=lambda k: None, dot=None):
    def mm(n):
        a, r, acc = left(n), right(n), None
        for k in range(0, r.shape[0], 512):
            d = (dot or _bdot)(a[:, k:k + 512], r[k:k + 512])
            acc = d if acc is None else acc + d
        return acc

    ready(0)
    m2 = mm(0)
    c22 = mm(1) - m2
    ready(1)
    m4 = mm(2)
    c21 = m2 + m4
    m1 = mm(3)
    c11, c22 = m1 + m4, c22 + m1
    m3 = mm(4)
    done(1, c21, c22 + m3)
    c11 = c11 + mm(5)
    ready(2)
    m5 = mm(6)
    done(0, c11 - m5, m3 + m5)


def _twiddle(z, k, n, sign):
    r, i = z
    if k == 0:
        return r, i
    if 4 * k == n:
        return (-i, r) if sign > 0 else (i, -r)
    c, s = math.cos(2 * math.pi * k / n), sign * math.sin(2 * math.pi * k / n)
    if 8 * k == n or 8 * k == 3 * n:
        if c * s > 0:
            return (r - i) * c, (r + i) * c
        return (r + i) * c, (i - r) * c
    return r * c - i * s, r * s + i * c


def _cfft(xs, sign):
    n = len(xs)
    if n == 1:
        return xs
    ev, od = _cfft(xs[0::2], sign), _cfft(xs[1::2], sign)
    out = [None] * n
    for k in range(n // 2):
        er, ei = ev[k]
        if 4 * k == n:
            orr, oi = od[k]
            lo, hi = (er - oi, ei + orr), (er + oi, ei - orr)
            out[k], out[k + n // 2] = (lo, hi) if sign > 0 else (hi, lo)
        else:
            tr, ti = _twiddle(od[k], k, n, sign)
            out[k], out[k + n // 2] = (er + tr, ei + ti), (er - tr, ei - ti)
    return out


def _rfft8(x):
    a0, a1, b0, b1 = x[0] + x[4], x[0] - x[4], x[2] + x[6], x[2] - x[6]
    c0, c1, d0, d1 = x[1] + x[5], x[1] - x[5], x[3] + x[7], x[3] - x[7]
    e, f = a0 + b0, c0 + d0
    g, h = (c1 - d1) * R2, (c1 + d1) * R2
    return [e + f, e - f, a1 + g, b1 + h, a0 - b0, c0 - d0, a1 - g, b1 - h]


def _irfft8(z):
    z0, z4, z1r, z1i, z2r, z2i, z3r, z3i = z
    e, f = z0 + z4, z0 - z4
    a1, g = z1r + z3r, (z1r - z3r) * R2
    b1, h = z1i + z3i, (z1i - z3i) * R2
    a0, b0, c0, d0 = e + z2r, e - z2r, f + z2i, f - z2i
    c1, d1 = g + h, h - g
    return [a0 + a1, c0 + c1, b0 + b1, d0 + d1, a0 - a1, c0 - c1, b0 - b1, d0 - d1]


def _kernel(x_hbm, mem0_hbm, wq_hbm, wk_hbm, wv_hbm, wo_hbm, bx_hbm, wr_hbm, wi_hbm, fill_hbm, cst_hbm,
            out_hbm,
            x_v, xpre_v, xs_v, mem0_v, fill_v, lhs_v, wqkv, wo_v, pre, os_v, ws_v, outa_v,
            bx_v, w_v, wn_v, wt, cst, zs, vv, tn, outb_v,
            sem_w, sem_in, sem_out):
    scale = E ** -0.5
    wus = [w.bitcast(U32) for w in (wq_hbm, wk_hbm, wv_hbm)]
    wo_u = wo_hbm.bitcast(U32)
    fus = [w.at[pl.ds(0, 512)].bitcast(U32) for w in (wr_hbm, wi_hbm)]

    def w_copy(j, t, sem):
        return pltpu.make_async_copy(wus[t].at[:, :, j, :], wqkv.at[j, t], sem)

    xpre_cp = pltpu.make_async_copy(x_hbm.at[:, pl.ds(0, 8), :], xpre_v, sem_w.at[17])
    head = [[divmod(f, 3) for f in range(HEAD[b], HEAD[b + 1])] for b in range(len(HEAD) - 1)]
    head_cps = [[w_copy(j, t, sem_w.at[b]) for j, t in grp] for b, grp in enumerate(head) if b > 0]
    first_cps = [pltpu.make_async_copy(wus[0].at[pl.ds(32 * k, 32), :, 0, :], wqkv.at[0, 0, pl.ds(32 * k, 32)],
                                       sem_w.at[18 * k]) for k in range(2)]
    head_cps.insert(0, first_cps)

    def b_rows(i, b):
        return b, i // 4, pl.ds(pl.multiple_of((i % 4) * 8, 8), 8)

    def fwd_cps(i):
        rows = b_rows(i, slice(None))
        sem = sem_w.at[8 + i]
        return ([w_copy(8 + i, t, sem) for t in range(3)]
                + [pltpu.make_async_copy(bx_hbm.at[rows], bx_v.at[rows], sem)]
                + [pltpu.make_async_copy(fus[t].at[:, pl.ds(pl.multiple_of(128 * (2 * i + h), 128), 128)],
                                         w_v.at[t, 2 * i + h], sem) for t in range(2) for h in range(2)])

    def part(src, dst, lo, hi, sem):
        return pltpu.make_async_copy(src.at[pl.ds(lo, hi - lo)], dst.at[pl.ds(lo, hi - lo)], sem)

    c0_cp = part(cst_hbm, cst, 0, C_MS, sem_w.at[16])
    a_cps = [pltpu.make_async_copy(wo_u.at[:, pl.ds(128 * n, 128)], wo_v.at[n], sem_in.at[0]) for n in range(8)]
    a_cps += [part(x_hbm, x_v, 0, UN, sem_in.at[0]), part(cst_hbm, cst, C_MS, C_MS + UN, sem_in.at[0]),
              pltpu.make_async_copy(mem0_hbm, mem0_v, sem_in.at[0]),
              pltpu.make_async_copy(fill_hbm, fill_v, sem_in.at[0])]
    b_cps = [part(x_hbm, x_v, UN, NSEG, sem_in.at[1]), part(cst_hbm, cst, C_MS + UN, C_NUM, sem_in.at[1])]
    b_cps += [pltpu.make_async_copy(w.at[pl.ds(512, 1)], wn_v.at[t], sem_in.at[1])
              for t, w in enumerate((wr_hbm, wi_hbm))]

    lane = lax.broadcasted_iota(I32, (8, 128), 1)
    alt = jnp.where(lane % 2 == 0, 1.0, -1.0).astype(F32)
    lo_half = lane < 64
    ev_grp = (lane // 32) % 2 == 0

    def half_coef(q):
        sg = -1.0 if q < 3 else 1.0
        tc, ts = math.cos(2 * math.pi * q / 16), -math.sin(2 * math.pi * q / 16)
        f = lambda lo, hi: jnp.where(lo_half, lo, hi).astype(F32)
        return f(1.0, ts), f(0.0, sg * tc), f(0.0, tc), f(sg, -sg * ts)

    pace = {'tok': None}

    def token(v):
        return (v if v.dtype == U32 else pltpu.bitcast(v, U32)) & cst[C_MN, 56:64, :]

    def gate(v):
        tok = pace['tok']
        if tok is None:
            return v
        return v | tok if v.dtype == U32 else pltpu.bitcast(pltpu.bitcast(v, U32) | tok, v.dtype)

    def gate2(z):
        return gate(z[0]), gate(z[1])

    def as_u32(rows):
        return pltpu.bitcast(_cat(rows), U32)

    def b_fwd(i):
        r0 = pl.multiple_of(i * 8, 8)
        hc = [None] + [half_coef(q) for q in range(1, 4)]
        tacc = jnp.zeros((8, 128), F32)
        zl = []

        def filt(k):
            e, t, ty = 2 * i + k // 4, (k // 2) % 2, k % 2
            u = jnp.concatenate([gate(w_v[t, e, pl.ds(m + ty + 64 * v, 8, stride=8), :])
                                 for m in (0, 6, 4, 2) for v in range(4)], axis=0)
            ut = pltpu.bitcast(pltpu.bitcast(u, F32).T, U32)
            for v in range(16):
                wt[t, ty, pl.ds(8 * (v % 4) * WP + 4 * e + v // 4, 8, stride=WP), :] = ut[8 * v:8 * v + 8]

        for b0 in range(0, 32, 2):
            rows = []
            for b in (b0, b0 + 1):
                xb = bx_v[(*b_rows(i, b), slice(None))].astype(F32)
                z = _rfft8([gate(xb[:, 128 * t:128 * t + 128]) for t in range(8)])
                tacc = jnp.where(lane == b, jnp.sum(z[0] * alt, axis=1, keepdims=True), tacc)
                for q in range(1, 4):
                    c1, c2, c3, c4 = hc[q]
                    zr, zi = z[2 * q], z[2 * q + 1]
                    pp = c1 * zr + c2 * zi
                    qq = pltpu.roll(c3 * zr + c4 * zi, 64, 1)
                    z[2 * q], z[2 * q + 1] = pp + qq, pp - qq
                rows.append(z)
            zl.append([as_u32([rows[0][n], rows[1][n]]) for n in range(8)])
            yield 200
            if b0 % 4 == 0:
                filt(b0 // 4)
                yield 40
        tn[pl.ds(r0, 8), :] = tacc

        def mm(n):
            return _bdot(_bf(jnp.concatenate([z[n] for z in zl], axis=0)), _bf(cst[C_MD + n]))

        yield MID
        oo = [mm(n) for n in range(4)]
        yield MID
        oo += [mm(n) for n in range(4, 8)]
        yield MID
        for q in range(4):
            sel, sh = (ev_grp, 96) if q == 0 else (lo_half, 64)
            ys = []
            for b0 in range(4):
                xs = []
                for b in range(b0, 32, 4):
                    e_, o_ = gate(oo[2 * q][8 * b:8 * b + 8]), oo[2 * q + 1][8 * b:8 * b + 8]
                    xs.append((jnp.where(sel, e_, o_), pltpu.roll(jnp.where(sel, o_, e_), sh, 1)))
                ys.append([_twiddle(y, b0 * k1, 32, -1) for k1, y in enumerate(_cfft(xs, -1))])
                yield 110
            for k1 in range(8):
                for k0, y in enumerate(_cfft([gate2(ys[b0][k1]) for b0 in range(4)], -1)):
                    zs[k1 + 8 * k0, q, pl.ds(pl.multiple_of(2 * r0, 16), 16), :] = _cat(y)
                yield 30

    def b_mid(it):
        for n in range(4):
            for r in range(0, 64, 8):
                blk = lambda k, p: _bf(gate(wo_v[n + 4 * p, pl.ds(pl.multiple_of((2 * it + k) * 64 + r, 8), 8), :]))
                vals = [pltpu.bitcast(_strassen_right(m, blk), U32) for m in range(1, 6)]
                for m in range(5):
                    ws_v[n, m, pl.ds(pl.multiple_of(it * 64 + r, 8), 8), :] = vals[m]
                yield vals if 8 * n + r // 8 > 1 else None
        yield MID
        for dl in (2 * it, 2 * it + 1):
            y = _bdot(_bf(cst[C_MS + 2 * dl]), jnp.concatenate([zs[dl, q] for q in range(4)], axis=1))
            for _ in range(4):
                yield None
            w0 = pl.multiple_of(dl * WP, 8)
            rows = []
            for r in range(8):
                wq = []
                for t in range(2):
                    ta, tb = wt[t, 0, pl.ds(w0 + 8 * r, 8), :], wt[t, 1, pl.ds(w0 + 8 * r, 8), :]
                    wq.append([_unpack2(ta, 0), _unpack2(jnp.where(ev_grp, ta, tb), 1),
                               _unpack2(tb, 0), _unpack2(jnp.where(ev_grp, tb, ta), 1)])
                cols = []
                for q in range(4):
                    yr = gate(y[8 * r:8 * r + 8, 128 * q:128 * q + 128])
                    yi = gate(y[64 + 8 * r:72 + 8 * r, 128 * q:128 * q + 128])
                    wr, wi = wq[0][q], wq[1][q]
                    cols.append(as_u32([yr * wr - yi * wi, yr * wi + yi * wr]))
                rows.append(jnp.concatenate(cols, axis=1))
                yield cols
                yield None
            yield MID
            vv[dl] = _bdot(_bf(cst[C_MS + 2 * dl + 1]), _bf(jnp.concatenate(rows, axis=0)))

    def b_nyq():
        c, s = pltpu.bitcast(cst[C_TW], F32), pltpu.bitcast(cst[C_TW + 1], F32)
        tb = tn[...].astype(BF)
        tr, ti = _bdot(tb, _bf(cst[C_MN])), _bdot(tb, _bf(cst[C_MN + 1]))
        yield MID
        y = _bdot(_bf(cst[C_MN + 2, 0:16, :]), _cat([tr * c + ti * s, ti * c - tr * s]))
        row = lax.broadcasted_iota(I32, (16, 128), 0)
        wn = []
        for t in range(2):
            wrow = wn_v[t].astype(F32)
            acc = jnp.zeros((16, 128), F32)
            for e in range(16):
                acc = jnp.where(row == e, wrow[:, 128 * e:128 * e + 128], acc)
            wn.append(acc)
        yr, yi = y[0:16], y[16:32]
        yield MID
        v = _bdot(_bf(cst[C_MN + 3, :, 0:32]), _cat([yr * wn[0] - yi * wn[1], yr * wn[1] + yi * wn[0]]))
        vr, vi = v[0:64], v[64:128]
        yield MID
        tn[...] = (_bdot((vr * c - vi * s).astype(BF), _bf(cst[C_MN + 4]))
                   + _bdot((vr * s + vi * c).astype(BF), _bf(cst[C_MN + 5])))

    def b_inv(i, ul):
        r0 = i * 8
        for q in range(4):
            sel, sh = (ev_grp, 32) if q == 0 else (lo_half, 64)
            ys = []
            for b0 in range(4):
                xs = [(gate(vv[dl, pl.ds(r0, 8), 128 * q:128 * q + 128]),
                       gate(vv[dl, pl.ds(64 + r0, 8), 128 * q:128 * q + 128])) for dl in range(b0, 32, 4)]
                ys.append([_twiddle(y, b0 * k1, 32, +1) for k1, y in enumerate(_cfft(xs, +1))])
                yield 110
            ie, io = [], []
            for k1 in range(8):
                es, os_ = [], []
                for ur, ui in _cfft([gate2(ys[b0][k1]) for b0 in range(4)], +1):
                    tmp = pltpu.roll(ui, sh, 1)
                    es.append(jnp.where(sel, ur, tmp))
                    os_.append(jnp.where(sel, tmp, ur))
                ie += [as_u32(es[0:2]), as_u32(es[2:4])]
                io += [as_u32(os_[0:2]), as_u32(os_[2:4])]
                yield 55, ie[-2:] + io[-2:]
            ul += [ie, io]

    def b_fin(i, zz):
        r0 = i * 8
        hc = [None] + [half_coef(q) for q in range(1, 4)]
        tb = tn[pl.ds(r0, 8), :]
        for g in range(32):
            b = g // 4 + 8 * (g % 4)
            z = [gate(zz[n][8 * g:8 * g + 8]) for n in range(8)]
            z[0] = z[0] + jnp.sum(jnp.where(lane == b, tb, 0.0), axis=1, keepdims=True) * alt
            for q in range(1, 4):
                c1, c2, c3, c4 = hc[q]
                pp = z[2 * q] + z[2 * q + 1]
                qq = pltpu.roll(z[2 * q] - z[2 * q + 1], 64, 1)
                z[2 * q], z[2 * q + 1] = c1 * pp + c3 * qq, c2 * pp + c4 * qq
            y = _irfft8(z)
            outb_v[(*b_rows(i, b), slice(None))] = jnp.concatenate(y, axis=1).astype(BF)
            yield 75, y
        rows = b_rows(i, slice(None))
        start_out(outb_v.at[rows], out_hbm.at[(*rows, pl.ds(DM, DM))])

    def tie(w, vals):
        if not vals:
            return w
        acc = None
        for v in vals:
            v = v if v.dtype == U32 else pltpu.bitcast(v, U32)
            acc = v if acc is None else acc | v
        return jnp.concatenate([w[0:8] | token(acc), w[8:]], axis=0)

    def paced_dot(gen, budget):
        st = {'debt': 0, 'k': 0}
        due = {}

        def emit(d, b):
            while st['debt'] < b:
                r = 8 * (32 * st['debt'] // b)
                pace['tok'] = token(d[r:r + 8])
                c = next(gen, MID)
                if c is MID:
                    st['debt'] = b
                elif isinstance(c, list):
                    st['debt'] = 0
                    for own in c:
                        emit(own, 300)
                    return
                else:
                    if isinstance(c, tuple):
                        due.setdefault(st['k'] + 2, []).extend(c[1])
                        c = c[0]
                    st['debt'] += c
            st['debt'] -= b

        def dot(a, w):
            vals = due.pop(st['k'], None)
            if vals:
                a = jnp.concatenate([_bf(tie(pltpu.bitcast(a[:, 0:128], U32), vals)), a[:, 128:]], axis=1)
            d = _bdot(a, w)
            st['k'] += 1
            emit(d, budget)
            return d

        return dot

    out_cps = []

    def start_out(src, dst):
        out_cps.append(pltpu.make_async_copy(src, dst, sem_out.at[0]))
        out_cps[-1].start()

    hb = DM // 32

    def retile(j, t, k):
        blk = pl.ds(k * hb, hb)
        a, b = wqkv[j, t, blk, pl.ds(0, 8, stride=2), :], wqkv[j, t, blk, pl.ds(1, 8, stride=2), :]
        lo, hi = (a & jnp.uint32(0xFFFF)) | (b << 16), (a >> 16) | (b & jnp.uint32(0xFFFF0000))
        wqkv[j, t, blk, 0:8, :] = lo
        wqkv[j, t, blk, 8:16, :] = hi
        return lo

    def strassen_lhs():
        for g in range(NSEG // 4):
            xa = [xpre_v[4 * g + k].astype(F32) for k in range(4)]
            a1, a2 = jnp.concatenate([xa[0], xa[2]], axis=0), jnp.concatenate([xa[1], xa[3]], axis=0)
            a11, a12, a21, a22 = a1[:, :DM // 2], a1[:, DM // 2:], a2[:, :DM // 2], a2[:, DM // 2:]
            for n in range(7):
                v = _strassen_left(n, lambda r, k: ((a11, a12), (a21, a22))[r][k])
                xs_v[n, 8 * g:8 * g + 8, :] = pltpu.bitcast(v.astype(BF), U32)

    def pre_step(j, t, dot=None, sync=None, first=False):
        fresh = {}

        def w(k, p):
            v = fresh.pop((k, p), None)
            if v is None:
                v = wqkv[j, t, k * hb:(k + 1) * hb, 8 * p:8 * p + 8, :]
            return _bf(v.reshape(DM // 4, E))

        def done(h, c1, c2):
            v = jnp.concatenate([c.reshape(NSEG // 2, 8, E) for c in (c1, c2)], axis=1)
            pre[j, t, :, h] = pltpu.bitcast(v.astype(BF), U32)

        def ready(k):
            if k < 2:
                if first:
                    first_cps[k].wait()
                fresh[k, 0] = retile(j, t, k)
            elif sync:
                sync()

        _strassen(lambda n: _bf(xs_v[n]), lambda n: _strassen_right(n, w), done, ready, dot)

    for cp in [xpre_cp] + [cp for grp in head_cps for cp in grp]:
        cp.start()
    vv[0:PAD] = jnp.zeros((PAD,) + vv.shape[1:], F32)
    xpre_cp.wait()
    strassen_lhs()

    def pre_fwd(steps, i, budget):
        gen = b_fwd(i)
        dot = paced_dot(gen, budget)
        for j, t in steps + [(8 + i, t) for t in range(3)]:
            pre_step(j, t, dot)
        for _ in gen:
            pass

    def sync(b):
        for i in LATER.get(b, ()):
            for cp in ([c0_cp] if i == 0 else []) + fwd_cps(i):
                cp.start()
        for cp in head_cps[b + 1] + ([c0_cp] + fwd_cps(0) if b + 2 == len(head) else []):
            cp.wait()

    for b, grp in enumerate(head[:-1]):
        for j, t in grp:
            pre_step(j, t, sync=functools.partial(sync, b) if (j, t) == grp[-1] else None, first=b == 0)
    pre_fwd(head[-1], 0, 130)
    for cp in a_cps + b_cps:
        cp.start()

    def pre_fwd_body(i, carry):
        for cp in fwd_cps(i):
            cp.wait()
        pre_fwd([], i, 340)
        return carry

    lax.fori_loop(1, 8, pre_fwd_body, 0)
    for cp in a_cps:
        cp.wait()

    def seg_step(s, u, mem, slot, opost):
        xs = x_v[s]
        lhs_v[u] = as_u32([mem, xs[8:32].astype(F32)])
        fill = fill_v[...]
        toks = []
        pace['tok'] = None

        def proj(j, t):
            w0, w1 = [wqkv[j, t, :, 8 * p:8 * p + 8, :].reshape(DM // 2, E) for p in range(2)]
            r0, r1 = _bdot(_bf(lhs_v[u]), _bf(tie(w0, slot()))), _bdot(_bf(lhs_v[u]), _bf(w1))
            toks.append(r0[0:8])
            if len(toks) >= 4:
                pace['tok'] = token(toks[-4])
            return _cat([r0, r1, _bf(pre[j, t, s // 2, u % 2]).astype(F32)])

        def qk(q, k):
            sc = lax.dot_general(q, k, (((1,), (1,)), ((), ())), preferred_element_type=F32) * scale
            sc = jnp.where(fill == 0.0, sc, fill)
            p = jnp.exp(sc - jnp.max(sc, axis=-1, keepdims=True))
            return (p * pl.reciprocal(jnp.sum(p, axis=-1, keepdims=True), approx=True)).astype(BF)

        ob, ps, vs = {}, {}, {}

        def pv(j):
            o = _bdot(ps[j], vs[j])
            opost[u, j] = (o[64:72], o[72:80])
            if u == UN - 1:
                vals = [as_u32([_strassen_left(n, lambda r, k: opost[2 * g + r, j][k]) for g in range(2)])
                        for n in range(7)]
                for n in range(7):
                    os_v[n, pl.ds(pl.multiple_of(2 * (s - u), 8), 8), 128 * j:128 * j + 128] = vals[n]
            ob[j] = [o[0:32], o[32:64]]

        def wo(g0, g1):
            og = jnp.concatenate([o for j in range(2 * g0, 2 * g1) for o in ob[j]], axis=1).astype(BF)
            return jnp.concatenate([_bdot(og, _bf(wo_v[n, g0 * 256:g1 * 256, :])) for n in range(8)], axis=1)

        ng = NP // 2
        for g in range(ng):
            ja, jb = 2 * g, 2 * g + 1
            qa, ka, qb, kb = proj(ja, 0), proj(ja, 1), proj(jb, 0), proj(jb, 1)
            vs[ja], vs[jb] = proj(ja, 2), proj(jb, 2)
            ps[ja], ps[jb] = qk(qa, ka), qk(qb, kb)
            if g > 0:
                pv(ja - 2)
                pv(jb - 2)
        res = wo(0, 3)
        pv(NP - 2)
        pv(NP - 1)
        res = res + wo(3, ng - 1)
        res = res + wo(ng - 1, ng)
        outa_v[s // 2, u % 2, 8:32, :] = res[8:32].astype(BF)
        return res[0:8].astype(BF).astype(F32)

    def loop_body(it, mem):
        @pl.when(it == 1)
        def _():
            for cp in b_cps:
                cp.wait()

        gen = b_mid(it)
        opost = {}
        state = {'mid': False}

        def slot():
            if state['mid']:
                return None
            vals = next(gen, None)
            if vals is MID:
                state['mid'] = True
                return None
            return vals

        for u in range(UN):
            state['mid'] = False
            mem = seg_step(UN * it + u, u, mem, slot, opost)
        for _ in gen:
            pass
        return mem

    lax.fori_loop(0, NSEG // UN, loop_body, mem0_v[...].astype(F32))
    idx = (slice(None), slice(None), pl.ds(8, SEG - 8), pl.ds(0, DM))
    start_out(outa_v.at[idx], out_hbm.at[idx])

    def b_inv_all():
        nyq = b_nyq()
        zz = None
        for i in range(8):
            ul = []
            for k, c in enumerate(b_inv(i, ul)):
                if k % 10 == 0:
                    next(nyq, None)
                yield c
            if i > 0:
                yield from b_fin(i - 1, zz)
            else:
                yield MID
            zz = [_bdot(_bf(jnp.concatenate(ul[n], axis=0)), _bf(cst[C_MD + 8 + n])) for n in range(8)]
            if i < 7:
                yield [zz[3], zz[7]]
        yield MID
        yield MID
        yield from b_fin(7, zz)

    gen = b_inv_all()
    dot = paced_dot(gen, 450)
    for n in range(4):
        def done(r, *cs):
            for p, cc in enumerate(cs):
                idx = (slice(None), r, pl.ds(0, 8), pl.ds(128 * (n + 4 * p), 128))
                outa_v[idx] = cc.reshape(NSEG // 2, 8, 128).astype(BF)
                start_out(outa_v.at[idx], out_hbm.at[idx])

        heads = lambda k: jnp.concatenate([wo_v[n + 4 * k, 64 * h:64 * h + 64, :] for h in range(k, H, 2)], axis=0)
        right = lambda m: _bf(heads(m // 6) if m % 6 == 0 else ws_v[n, m - 1])
        _strassen(lambda m: _bf(os_v[m]), right, done, dot=dot)
    for _ in gen:
        pass
    for cp in out_cps:
        cp.wait()


def pallas_concat_heads__memory_aug_recurrent_mem_tr__spectral_gfnet__prompt_kernel(
    A_x, A_mem0, A_Wq, A_Wk, A_Wv, A_Wo, A_seg_len, B_x, B_w_r, B_w_i,
):
    assert A_x.shape == (1, S, DM) and A_Wq.shape == (DM, H, E) and A_mem0.shape == (1, M, DM)
    assert B_x.shape == (1, S, DM) and (not isinstance(A_seg_len, int) or A_seg_len == SEG)
    hbm = pl.BlockSpec(memory_space=pltpu.HBM)
    wr = lambda w: w.reshape(DM // 16, 16, H, E)
    out = pl.pallas_call(
        _kernel,
        out_shape=jax.ShapeDtypeStruct((NSEG // 2, 2, SEG, 2 * DM), BF),
        in_specs=[hbm] * 11,
        out_specs=hbm,
        scratch_shapes=[
            pltpu.VMEM((NSEG, SEG, DM), BF),
            pltpu.VMEM((NSEG, 8, DM), BF),
            pltpu.VMEM((7, NSEG * 2, DM // 2), U32),
            pltpu.VMEM((M, DM), BF),
            pltpu.VMEM((80, 80), F32),
            pltpu.VMEM((UN, SEG // 2, DM), U32),
            pltpu.VMEM((NP, 3, DM // 16, 16, E), U32),
            pltpu.VMEM((8, H * E // 2, 128), U32),
            pltpu.VMEM((NP, 3, NSEG // 2, 2, 8, E), U32),
            pltpu.VMEM((7, NSEG * 2, H * E // 2), U32),
            pltpu.VMEM((4, 5, H * E // 4, 128), U32),
            pltpu.VMEM((NSEG // 2, 2, SEG, DM), BF),
            pltpu.VMEM((NSEG // 2, 2, SEG, DM), BF),
            pltpu.VMEM((2, 16, 256, 128), U32),
            pltpu.VMEM((2, 1, S), BF),
            pltpu.VMEM((2, 2, 32 * WP, 128), U32),
            pltpu.VMEM((C_NUM, 64, 128), U32),
            pltpu.VMEM((32, 4, 128, 128), BF),
            pltpu.VMEM((32, 128, 512), F32),
            pltpu.VMEM((64, 128), F32),
            pltpu.VMEM((NSEG // 2, 2, SEG, DM), BF),
            pltpu.SemaphoreType.DMA((NP + 3,)),
            pltpu.SemaphoreType.DMA((2,)),
            pltpu.SemaphoreType.DMA((1,)),
        ],
        compiler_params=pltpu.CompilerParams(vmem_limit_bytes=118 * 1024 * 1024, disable_semaphore_checks=True),
    )(A_x.reshape(NSEG, SEG, DM), A_mem0.reshape(M, DM), wr(A_Wq), wr(A_Wk), wr(A_Wv),
      A_Wo.reshape(H * E, DM), B_x.reshape(NSEG // 2, 2, SEG, DM), B_w_r.T, B_w_i.T, _mask_fill(), _fft_consts())
    return out.reshape(1, S, 2 * DM)
```

```python
import functools
import math

import jax
import jax.numpy as jnp
import numpy as np
from jax import lax
import jax.experimental.pallas as pl
import jax.experimental.pallas.tpu as pltpu

BF, F32, U32, I32 = jnp.bfloat16, jnp.float32, jnp.uint32, jnp.int32

S, DM, H, E, M, SEG = 2048, 1024, 32, 128, 8, 32
NSEG = S // SEG
NP = H // 2
UN = 4
R2 = math.sqrt(0.5)
MID = 'mid'
PAD = 28
HEAD = (0, 1, 2, 3, 5, 8, 13, 19, 24)
LATER = {3: (0, 1), 4: (2,), 5: (3, 4, 5), 6: (6, 7)}


def _to_u32(m):
    u = np.ascontiguousarray(m, dtype=np.float32).view(np.uint32)
    h = ((u + 0x7FFF + ((u >> 16) & 1)) >> 16).astype(np.uint32)
    return h[..., 0::2, :] | (h[..., 1::2, :] << 16)


def _mask_fill():
    r = np.arange(80)
    head = np.where(r < 64, r // 32, (r - 64) // 8)
    pos = np.where(r < 64, np.where(r % 32 < M, r % 32, r % 32 + M), (r - 64) % 8 + M)
    vis = (pos[:, None] < M) | (pos[:, None] >= pos[None, :])
    same = head[:, None] == head[None, :]
    return np.where(same, np.where(vis, 0.0, -1e9), -np.inf).astype(np.float32)


RES = ((0, 12, 8, 4), (1, 15, 9, 7), (2, 14, 10, 6), (3, 13, 11, 5))
WP = 72
C_MD, C_MN, C_TW, C_MS, C_NUM = 0, 16, 22, 24, 88


@functools.lru_cache(maxsize=None)
def _fft_consts():
    md = np.zeros((16, 128, 128))
    for q in range(4):
        if q == 0:
            lay = [[(0, 0), (0, 1), (2, 0), (2, 1)], [(3, 1), (1, 0), (1, 1), (3, 0)]]
        else:
            lay = [[(0, 0), (1, 0), (0, 1), (1, 1)], [(2, 1), (3, 1), (2, 0), (3, 0)]]
        for h in range(2):
            ms_, ws_ = [], []
            for g, part in lay[h]:
                k = 16 * np.arange(32) + RES[q][g]
                th = 2 * np.pi * np.outer(np.arange(128 if q == 0 else 64), k) / DM
                c, s = np.cos(th), np.sin(th)
                if q == 0:
                    ms_.append(-s if part else c)
                else:
                    sg = (1.0 if RES[q][g] % 8 == q else -1.0) * (1.0 - 2.0 * h)
                    ms_.append(np.concatenate([-s, sg * c] if part else [c, sg * s]))
                ws_.append(np.where(k == 0, 1.0, 2.0) / DM)
            m = np.concatenate(ms_, axis=1)
            md[2 * q + h] = m
            md[8 + 2 * q + h] = (m * np.concatenate(ws_)[None, :]).T
    a, l = np.arange(64), np.arange(128)
    re = 16 * (a // 8) + a % 8
    im = re + 8
    ms = np.zeros((64, 128, 128))
    for dl in range(32):
        th = 2 * np.pi * np.outer(32 * a + dl, a) / S
        c, s = np.cos(th), np.sin(th)
        ms[2 * dl][:, re], ms[2 * dl][:, im] = np.concatenate([c, -s]), np.concatenate([s, c])
        ms[2 * dl + 1][:, re] = np.concatenate([c.T, s.T]) / S
        ms[2 * dl + 1][:, im] = np.concatenate([-s.T, c.T]) / S
    mn = np.zeros((6, 128, 128))
    th = 2 * np.pi * np.outer(np.arange(32), l) / 32
    mn[0, :32], mn[1, :32] = np.cos(th), -np.sin(th)
    mn[4, :, :32], mn[5, :, :32] = np.cos(th).T / DM, -np.sin(th).T / DM
    th = 2 * np.pi * np.outer(np.arange(16), a) / 16
    c, s = np.cos(th), np.sin(th)
    mn[2, :32] = np.block([[c, s], [-s, c]])
    mn[3, :, :32] = np.block([[c.T, -s.T], [s.T, c.T]]) / S
    th = 2 * np.pi * np.outer(a, l) / S
    tw = np.stack([np.cos(th), np.sin(th)]).astype(np.float32).view(np.uint32)
    return np.concatenate([_to_u32(md), _to_u32(mn), tw, _to_u32(ms)], axis=0)


def _bdot(a, b):
    return jnp.dot(a, b, preferred_element_type=F32)


def _bf(u):
    return pltpu.bitcast(u, BF)


def _cat(rows):
    return jnp.concatenate(rows, axis=0).astype(BF)


def _unpack2(u, p):
    if p == 0:
        return pltpu.bitcast(u << 16, F32)
    return pltpu.bitcast(u & jnp.uint32(0xFFFF0000), F32)


def _strassen_left(n, a):
    return (lambda: a(1, 0) + a(1, 1), lambda: a(1, 0) - a(0, 0), lambda: a(1, 1), lambda: a(0, 0) + a(1, 1),
            lambda: a(0, 0), lambda: a(0, 1) - a(1, 1), lambda: a(0, 0) + a(0, 1))[n]()


def _strassen_right(n, w):
    add = lambda u, v: (u.astype(F32) + v.astype(F32)).astype(BF)
    sub = lambda u, v: (u.astype(F32) - v.astype(F32)).astype(BF)
    return (lambda: w(0, 0), lambda: add(w(0, 0), w(0, 1)), lambda: sub(w(1, 0), w(0, 0)),
            lambda: add(w(0, 0), w(1, 1)), lambda: sub(w(0, 1), w(1, 1)), lambda: add(w(1, 0), w(1, 1)),
            lambda: w(1, 1))[n]()


def _strassen(left, right, done, ready=lambda k: None, dot=None):
    def mm(n):
        a, r, acc = left(n), right(n), None
        for k in range(0, r.shape[0], 512):
            d = (dot or _bdot)(a[:, k:k + 512], r[k:k + 512])
            acc = d if acc is None else acc + d
        return acc

    ready(0)
    m2 = mm(0)
    c22 = mm(1) - m2
    ready(1)
    m4 = mm(2)
    c21 = m2 + m4
    m1 = mm(3)
    c11, c22 = m1 + m4, c22 + m1
    m3 = mm(4)
    done(1, c21, c22 + m3)
    c11 = c11 + mm(5)
    ready(2)
    m5 = mm(6)
    done(0, c11 - m5, m3 + m5)


def _twiddle(z, k, n, sign):
    r, i = z
    if k == 0:
        return r, i
    if 4 * k == n:
        return (-i, r) if sign > 0 else (i, -r)
    c, s = math.cos(2 * math.pi * k / n), sign * math.sin(2 * math.pi * k / n)
    if 8 * k == n or 8 * k == 3 * n:
        if c * s > 0:
            return (r - i) * c, (r + i) * c
        return (r + i) * c, (i - r) * c
    return r * c - i * s, r * s + i * c


def _cfft(xs, sign):
    n = len(xs)
    if n == 1:
        return xs
    ev, od = _cfft(xs[0::2], sign), _cfft(xs[1::2], sign)
    out = [None] * n
    for k in range(n // 2):
        er, ei = ev[k]
        if 4 * k == n:
            orr, oi = od[k]
            lo, hi = (er - oi, ei + orr), (er + oi, ei - orr)
            out[k], out[k + n // 2] = (lo, hi) if sign > 0 else (hi, lo)
        else:
            tr, ti = _twiddle(od[k], k, n, sign)
            out[k], out[k + n // 2] = (er + tr, ei + ti), (er - tr, ei - ti)
    return out


def _rfft8(x):
    a0, a1, b0, b1 = x[0] + x[4], x[0] - x[4], x[2] + x[6], x[2] - x[6]
    c0, c1, d0, d1 = x[1] + x[5], x[1] - x[5], x[3] + x[7], x[3] - x[7]
    e, f = a0 + b0, c0 + d0
    g, h = (c1 - d1) * R2, (c1 + d1) * R2
    return [e + f, e - f, a1 + g, b1 + h, a0 - b0, c0 - d0, a1 - g, b1 - h]


def _irfft8(z):
    z0, z4, z1r, z1i, z2r, z2i, z3r, z3i = z
    e, f = z0 + z4, z0 - z4
    a1, g = z1r + z3r, (z1r - z3r) * R2
    b1, h = z1i + z3i, (z1i - z3i) * R2
    a0, b0, c0, d0 = e + z2r, e - z2r, f + z2i, f - z2i
    c1, d1 = g + h, h - g
    return [a0 + a1, c0 + c1, b0 + b1, d0 + d1, a0 - a1, c0 - c1, b0 - b1, d0 - d1]


def _kernel(x_hbm, mem0_hbm, wq_hbm, wk_hbm, wv_hbm, wo_hbm, bx_hbm, wr_hbm, wi_hbm, fill_hbm, cst_hbm,
            out_hbm,
            x_v, xpre_v, xs_v, mem0_v, fill_v, lhs_v, wqkv, wo_v, pre, os_v, ws_v, outa_v,
            bx_v, w_v, wn_v, wt, cst, zs, vv, tn, outb_v,
            sem_w, sem_in, sem_out):
    scale = E ** -0.5
    wus = [w.bitcast(U32) for w in (wq_hbm, wk_hbm, wv_hbm)]
    wo_u = wo_hbm.bitcast(U32)
    fus = [w.at[pl.ds(0, 512)].bitcast(U32) for w in (wr_hbm, wi_hbm)]

    def w_copy(j, t, sem):
        return pltpu.make_async_copy(wus[t].at[:, :, j, :], wqkv.at[j, t], sem)

    xpre_cp = pltpu.make_async_copy(x_hbm.at[:, pl.ds(0, 8), :], xpre_v, sem_w.at[17])
    head = [[divmod(f, 3) for f in range(HEAD[b], HEAD[b + 1])] for b in range(len(HEAD) - 1)]
    head_cps = [[w_copy(j, t, sem_w.at[b]) for j, t in grp] for b, grp in enumerate(head) if b > 0]
    first_cps = [pltpu.make_async_copy(wus[0].at[pl.ds(32 * k, 32), :, 0, :], wqkv.at[0, 0, pl.ds(32 * k, 32)],
                                       sem_w.at[18 * k]) for k in range(2)]
    head_cps.insert(0, first_cps)

    def b_rows(i, b):
        return b, i // 4, pl.ds(pl.multiple_of((i % 4) * 8, 8), 8)

    def fwd_cps(i):
        rows = b_rows(i, slice(None))
        sem = sem_w.at[8 + i]
        return ([w_copy(8 + i, t, sem) for t in range(3)]
                + [pltpu.make_async_copy(bx_hbm.at[rows], bx_v.at[rows], sem)]
                + [pltpu.make_async_copy(fus[t].at[:, pl.ds(pl.multiple_of(128 * (2 * i + h), 128), 128)],
                                         w_v.at[t, 2 * i + h], sem) for t in range(2) for h in range(2)])

    def part(src, dst, lo, hi, sem):
        return pltpu.make_async_copy(src.at[pl.ds(lo, hi - lo)], dst.at[pl.ds(lo, hi - lo)], sem)

    c0_cp = part(cst_hbm, cst, 0, C_MS, sem_w.at[16])
    a_cps = [pltpu.make_async_copy(wo_u.at[:, pl.ds(128 * n, 128)], wo_v.at[n], sem_in.at[0]) for n in range(8)]
    a_cps += [part(x_hbm, x_v, 0, UN, sem_in.at[0]), part(cst_hbm, cst, C_MS, C_MS + UN, sem_in.at[0]),
              pltpu.make_async_copy(mem0_hbm, mem0_v, sem_in.at[0]),
              pltpu.make_async_copy(fill_hbm, fill_v, sem_in.at[0])]
    b_cps = [part(x_hbm, x_v, UN, NSEG, sem_in.at[1]), part(cst_hbm, cst, C_MS + UN, C_NUM, sem_in.at[1])]
    b_cps += [pltpu.make_async_copy(w.at[pl.ds(512, 1)], wn_v.at[t], sem_in.at[1])
              for t, w in enumerate((wr_hbm, wi_hbm))]

    lane = lax.broadcasted_iota(I32, (8, 128), 1)
    alt = jnp.where(lane % 2 == 0, 1.0, -1.0).astype(F32)
    lo_half = lane < 64
    ev_grp = (lane // 32) % 2 == 0

    def half_coef(q):
        sg = -1.0 if q < 3 else 1.0
        tc, ts = math.cos(2 * math.pi * q / 16), -math.sin(2 * math.pi * q / 16)
        f = lambda lo, hi: jnp.where(lo_half, lo, hi).astype(F32)
        return f(1.0, ts), f(0.0, sg * tc), f(0.0, tc), f(sg, -sg * ts)

    pace = {'tok': None}

    def token(v):
        return (v if v.dtype == U32 else pltpu.bitcast(v, U32)) & cst[C_MN, 56:64, :]

    def gate(v):
        tok = pace['tok']
        if tok is None:
            return v
        return v | tok if v.dtype == U32 else pltpu.bitcast(pltpu.bitcast(v, U32) | tok, v.dtype)

    def gate2(z):
        return gate(z[0]), gate(z[1])

    def as_u32(rows):
        return pltpu.bitcast(_cat(rows), U32)

    def b_fwd(i):
        r0 = pl.multiple_of(i * 8, 8)
        hc = [None] + [half_coef(q) for q in range(1, 4)]
        tacc = jnp.zeros((8, 128), F32)
        zl = []

        def filt(k):
            e, t, ty = 2 * i + k // 4, (k // 2) % 2, k % 2
            u = jnp.concatenate([gate(w_v[t, e, pl.ds(m + ty + 64 * v, 8, stride=8), :])
                                 for m in (0, 6, 4, 2) for v in range(4)], axis=0)
            ut = pltpu.bitcast(pltpu.bitcast(u, F32).T, U32)
            for v in range(16):
                wt[t, ty, pl.ds(8 * (v % 4) * WP + 4 * e + v // 4, 8, stride=WP), :] = ut[8 * v:8 * v + 8]

        for b0 in range(0, 32, 2):
            rows = []
            for b in (b0, b0 + 1):
                xb = bx_v[(*b_rows(i, b), slice(None))].astype(F32)
                z = _rfft8([gate(xb[:, 128 * t:128 * t + 128]) for t in range(8)])
                tacc = jnp.where(lane == b, jnp.sum(z[0] * alt, axis=1, keepdims=True), tacc)
                for q in range(1, 4):
                    c1, c2, c3, c4 = hc[q]
                    zr, zi = z[2 * q], z[2 * q + 1]
                    pp = c1 * zr + c2 * zi
                    qq = pltpu.roll(c3 * zr + c4 * zi, 64, 1)
                    z[2 * q], z[2 * q + 1] = pp + qq, pp - qq
                rows.append(z)
            zl.append([as_u32([rows[0][n], rows[1][n]]) for n in range(8)])
            yield 200
            if b0 % 4 == 0:
                filt(b0 // 4)
                yield 40
        tn[pl.ds(r0, 8), :] = tacc

        def mm(n):
            return _bdot(_bf(jnp.concatenate([z[n] for z in zl], axis=0)), _bf(cst[C_MD + n]))

        yield MID
        oo = [mm(n) for n in range(4)]
        yield MID
        oo += [mm(n) for n in range(4, 8)]
        yield MID
        for q in range(4):
            sel, sh = (ev_grp, 96) if q == 0 else (lo_half, 64)
            ys = []
            for b0 in range(4):
                xs = []
                for b in range(b0, 32, 4):
                    e_, o_ = gate(oo[2 * q][8 * b:8 * b + 8]), oo[2 * q + 1][8 * b:8 * b + 8]
                    xs.append((jnp.where(sel, e_, o_), pltpu.roll(jnp.where(sel, o_, e_), sh, 1)))
                ys.append([_twiddle(y, b0 * k1, 32, -1) for k1, y in enumerate(_cfft(xs, -1))])
                yield 110
            for k1 in range(8):
                for k0, y in enumerate(_cfft([gate2(ys[b0][k1]) for b0 in range(4)], -1)):
                    zs[k1 + 8 * k0, q, pl.ds(pl.multiple_of(2 * r0, 16), 16), :] = _cat(y)
                yield 30

    def b_mid(it):
        for n in range(4):
            for r in range(0, 64, 8):
                blk = lambda k, p: _bf(gate(wo_v[n + 4 * p, pl.ds(pl.multiple_of((2 * it + k) * 64 + r, 8), 8), :]))
                vals = [pltpu.bitcast(_strassen_right(m, blk), U32) for m in range(1, 6)]
                for m in range(5):
                    ws_v[n, m, pl.ds(pl.multiple_of(it * 64 + r, 8), 8), :] = vals[m]
                yield vals if 8 * n + r // 8 > 1 else None
        yield MID
        for dl in (2 * it, 2 * it + 1):
            y = _bdot(_bf(cst[C_MS + 2 * dl]), jnp.concatenate([zs[dl, q] for q in range(4)], axis=1))
            for _ in range(4):
                yield None
            w0 = pl.multiple_of(dl * WP, 8)
            rows = []
            for r in range(8):
                wq = []
                for t in range(2):
                    ta, tb = wt[t, 0, pl.ds(w0 + 8 * r, 8), :], wt[t, 1, pl.ds(w0 + 8 * r, 8), :]
                    wq.append([_unpack2(ta, 0), _unpack2(jnp.where(ev_grp, ta, tb), 1),
                               _unpack2(tb, 0), _unpack2(jnp.where(ev_grp, tb, ta), 1)])
                cols = []
                for q in range(4):
                    yr = gate(y[8 * r:8 * r + 8, 128 * q:128 * q + 128])
                    yi = gate(y[64 + 8 * r:72 + 8 * r, 128 * q:128 * q + 128])
                    wr, wi = wq[0][q], wq[1][q]
                    cols.append(as_u32([yr * wr - yi * wi, yr * wi + yi * wr]))
                rows.append(jnp.concatenate(cols, axis=1))
                yield None
                yield None
            yield MID
            vv[dl] = _bdot(_bf(cst[C_MS + 2 * dl + 1]), _bf(jnp.concatenate(rows, axis=0)))

    def b_nyq():
        c, s = pltpu.bitcast(cst[C_TW], F32), pltpu.bitcast(cst[C_TW + 1], F32)
        tb = tn[...].astype(BF)
        tr, ti = _bdot(tb, _bf(cst[C_MN])), _bdot(tb, _bf(cst[C_MN + 1]))
        yield MID
        y = _bdot(_bf(cst[C_MN + 2, 0:16, :]), _cat([tr * c + ti * s, ti * c - tr * s]))
        row = lax.broadcasted_iota(I32, (16, 128), 0)
        wn = []
        for t in range(2):
            wrow = wn_v[t].astype(F32)
            acc = jnp.zeros((16, 128), F32)
            for e in range(16):
                acc = jnp.where(row == e, wrow[:, 128 * e:128 * e + 128], acc)
            wn.append(acc)
        yr, yi = y[0:16], y[16:32]
        yield MID
        v = _bdot(_bf(cst[C_MN + 3, :, 0:32]), _cat([yr * wn[0] - yi * wn[1], yr * wn[1] + yi * wn[0]]))
        vr, vi = v[0:64], v[64:128]
        yield MID
        tn[...] = (_bdot((vr * c - vi * s).astype(BF), _bf(cst[C_MN + 4]))
                   + _bdot((vr * s + vi * c).astype(BF), _bf(cst[C_MN + 5])))

    def b_inv(i, ul):
        r0 = i * 8
        for q in range(4):
            sel, sh = (ev_grp, 32) if q == 0 else (lo_half, 64)
            ys = []
            for b0 in range(4):
                xs = [(gate(vv[dl, pl.ds(r0, 8), 128 * q:128 * q + 128]),
                       gate(vv[dl, pl.ds(64 + r0, 8), 128 * q:128 * q + 128])) for dl in range(b0, 32, 4)]
                ys.append([_twiddle(y, b0 * k1, 32, +1) for k1, y in enumerate(_cfft(xs, +1))])
                yield 110
            ie, io = [], []
            for k1 in range(8):
                es, os_ = [], []
                for ur, ui in _cfft([gate2(ys[b0][k1]) for b0 in range(4)], +1):
                    tmp = pltpu.roll(ui, sh, 1)
                    es.append(jnp.where(sel, ur, tmp))
                    os_.append(jnp.where(sel, tmp, ur))
                ie += [as_u32(es[0:2]), as_u32(es[2:4])]
                io += [as_u32(os_[0:2]), as_u32(os_[2:4])]
                yield 55, ie[-2:] + io[-2:]
            ul += [ie, io]

    def b_fin(i, zz):
        r0 = i * 8
        hc = [None] + [half_coef(q) for q in range(1, 4)]
        tb = tn[pl.ds(r0, 8), :]
        for g in range(32):
            b = g // 4 + 8 * (g % 4)
            z = [gate(zz[n][8 * g:8 * g + 8]) for n in range(8)]
            z[0] = z[0] + jnp.sum(jnp.where(lane == b, tb, 0.0), axis=1, keepdims=True) * alt
            for q in range(1, 4):
                c1, c2, c3, c4 = hc[q]
                pp = z[2 * q] + z[2 * q + 1]
                qq = pltpu.roll(z[2 * q] - z[2 * q + 1], 64, 1)
                z[2 * q], z[2 * q + 1] = c1 * pp + c3 * qq, c2 * pp + c4 * qq
            y = _irfft8(z)
            outb_v[(*b_rows(i, b), slice(None))] = jnp.concatenate(y, axis=1).astype(BF)
            yield 75, y
        rows = b_rows(i, slice(None))
        start_out(outb_v.at[rows], out_hbm.at[(*rows, pl.ds(DM, DM))])

    def tie(w, vals):
        if not vals:
            return w
        acc = None
        for v in vals:
            v = v if v.dtype == U32 else pltpu.bitcast(v, U32)
            acc = v if acc is None else acc | v
        return jnp.concatenate([w[0:8] | token(acc), w[8:]], axis=0)

    def paced_dot(gen, budget):
        st = {'debt': 0, 'k': 0}
        due = {}

        def emit(d, b):
            while st['debt'] < b:
                r = 8 * (32 * st['debt'] // b)
                pace['tok'] = token(d[r:r + 8])
                c = next(gen, MID)
                if c is MID:
                    st['debt'] = b
                elif isinstance(c, list):
                    st['debt'] = 0
                    for own in c:
                        emit(own, 300)
                    return
                else:
                    if isinstance(c, tuple):
                        due.setdefault(st['k'] + 2, []).extend(c[1])
                        c = c[0]
                    st['debt'] += c
            st['debt'] -= b

        def dot(a, w):
            vals = due.pop(st['k'], None)
            if vals:
                a = jnp.concatenate([_bf(tie(pltpu.bitcast(a[:, 0:128], U32), vals)), a[:, 128:]], axis=1)
            d = _bdot(a, w)
            st['k'] += 1
            emit(d, budget)
            return d

        return dot

    out_cps = []

    def start_out(src, dst):
        out_cps.append(pltpu.make_async_copy(src, dst, sem_out.at[0]))
        out_cps[-1].start()

    hb = DM // 32

    def retile(j, t, k):
        blk = pl.ds(k * hb, hb)
        a, b = wqkv[j, t, blk, pl.ds(0, 8, stride=2), :], wqkv[j, t, blk, pl.ds(1, 8, stride=2), :]
        lo, hi = (a & jnp.uint32(0xFFFF)) | (b << 16), (a >> 16) | (b & jnp.uint32(0xFFFF0000))
        wqkv[j, t, blk, 0:8, :] = lo
        wqkv[j, t, blk, 8:16, :] = hi
        return lo

    def strassen_lhs():
        for g in range(NSEG // 4):
            xa = [xpre_v[4 * g + k].astype(F32) for k in range(4)]
            a1, a2 = jnp.concatenate([xa[0], xa[2]], axis=0), jnp.concatenate([xa[1], xa[3]], axis=0)
            a11, a12, a21, a22 = a1[:, :DM // 2], a1[:, DM // 2:], a2[:, :DM // 2], a2[:, DM // 2:]
            for n in range(7):
                v = _strassen_left(n, lambda r, k: ((a11, a12), (a21, a22))[r][k])
                xs_v[n, 8 * g:8 * g + 8, :] = pltpu.bitcast(v.astype(BF), U32)

    def pre_step(j, t, dot=None, sync=None, first=False):
        fresh = {}

        def w(k, p):
            v = fresh.pop((k, p), None)
            if v is None:
                v = wqkv[j, t, k * hb:(k + 1) * hb, 8 * p:8 * p + 8, :]
            return _bf(v.reshape(DM // 4, E))

        def done(h, c1, c2):
            v = jnp.concatenate([c.reshape(NSEG // 2, 8, E) for c in (c1, c2)], axis=1)
            pre[j, t, :, h] = pltpu.bitcast(v.astype(BF), U32)

        def ready(k):
            if k < 2:
                if first:
                    first_cps[k].wait()
                fresh[k, 0] = retile(j, t, k)
            elif sync:
                sync()

        _strassen(lambda n: _bf(xs_v[n]), lambda n: _strassen_right(n, w), done, ready, dot)

    for cp in [xpre_cp] + [cp for grp in head_cps for cp in grp]:
        cp.start()
    vv[0:PAD] = jnp.zeros((PAD,) + vv.shape[1:], F32)
    xpre_cp.wait()
    strassen_lhs()

    def pre_fwd(steps, i, budget):
        gen = b_fwd(i)
        dot = paced_dot(gen, budget)
        for j, t in steps + [(8 + i, t) for t in range(3)]:
            pre_step(j, t, dot)
        for _ in gen:
            pass

    def sync(b):
        for i in LATER.get(b, ()):
            for cp in ([c0_cp] if i == 0 else []) + fwd_cps(i):
                cp.start()
        for cp in head_cps[b + 1] + ([c0_cp] + fwd_cps(0) if b + 2 == len(head) else []):
            cp.wait()

    for b, grp in enumerate(head[:-1]):
        for j, t in grp:
            pre_step(j, t, sync=functools.partial(sync, b) if (j, t) == grp[-1] else None, first=b == 0)
    pre_fwd(head[-1], 0, 130)
    for cp in a_cps + b_cps:
        cp.start()

    def pre_fwd_body(i, carry):
        for cp in fwd_cps(i):
            cp.wait()
        pre_fwd([], i, 340)
        return carry

    lax.fori_loop(1, 8, pre_fwd_body, 0)
    for cp in a_cps:
        cp.wait()

    def seg_step(s, u, mem, slot, opost):
        xs = x_v[s]
        lhs_v[u] = as_u32([mem, xs[8:32].astype(F32)])
        fill = fill_v[...]
        toks = []
        pace['tok'] = None

        def proj(j, t):
            w0, w1 = [wqkv[j, t, :, 8 * p:8 * p + 8, :].reshape(DM // 2, E) for p in range(2)]
            r0, r1 = _bdot(_bf(lhs_v[u]), _bf(tie(w0, slot()))), _bdot(_bf(lhs_v[u]), _bf(w1))
            toks.append(r0[0:8])
            if len(toks) >= 4:
                pace['tok'] = token(toks[-4])
            return _cat([r0, r1, _bf(pre[j, t, s // 2, u % 2]).astype(F32)])

        def qk(q, k):
            sc = lax.dot_general(q, k, (((1,), (1,)), ((), ())), preferred_element_type=F32) * scale
            sc = jnp.where(fill == 0.0, sc, fill)
            p = jnp.exp(sc - jnp.max(sc, axis=-1, keepdims=True))
            return (p * pl.reciprocal(jnp.sum(p, axis=-1, keepdims=True), approx=True)).astype(BF)

        ob, ps, vs = {}, {}, {}

        def pv(j):
            o = _bdot(ps[j], vs[j])
            opost[u, j] = (o[64:72], o[72:80])
            if u == UN - 1:
                vals = [as_u32([_strassen_left(n, lambda r, k: opost[2 * g + r, j][k]) for g in range(2)])
                        for n in range(7)]
                for n in range(7):
                    os_v[n, pl.ds(pl.multiple_of(2 * (s - u), 8), 8), 128 * j:128 * j + 128] = vals[n]
            ob[j] = [o[0:32], o[32:64]]

        def wo(g0, g1):
            og = jnp.concatenate([o for j in range(2 * g0, 2 * g1) for o in ob[j]], axis=1).astype(BF)
            return jnp.concatenate([_bdot(og, _bf(wo_v[n, g0 * 256:g1 * 256, :])) for n in range(8)], axis=1)

        ng = NP // 2
        for g in range(ng):
            ja, jb = 2 * g, 2 * g + 1
            qa, ka, qb, kb = proj(ja, 0), proj(ja, 1), proj(jb, 0), proj(jb, 1)
            vs[ja], vs[jb] = proj(ja, 2), proj(jb, 2)
            for j, q, k in ((ja, qa, ka), (jb, qb, kb)):
                ps[j] = qk(q, k)
                if g > 0:
                    pv(j - 2)
        res = wo(0, 4)
        pv(NP - 2)
        pv(NP - 1)
        res = res + wo(4, ng - 1)
        res = res + wo(ng - 1, ng)
        outa_v[s // 2, u % 2, 8:32, :] = res[8:32].astype(BF)
        return res[0:8].astype(BF).astype(F32)

    def loop_body(it, mem):
        @pl.when(it == 1)
        def _():
            for cp in b_cps:
                cp.wait()

        gen = b_mid(it)
        opost = {}
        state = {'mid': False}

        def slot():
            if state['mid']:
                return None
            vals = next(gen, None)
            if vals is MID:
                state['mid'] = True
                return None
            return vals

        for u in range(UN):
            state['mid'] = False
            mem = seg_step(UN * it + u, u, mem, slot, opost)
        for _ in gen:
            pass
        return mem

    lax.fori_loop(0, NSEG // UN, loop_body, mem0_v[...].astype(F32))
    idx = (slice(None), slice(None), pl.ds(8, SEG - 8), pl.ds(0, DM))
    start_out(outa_v.at[idx], out_hbm.at[idx])

    def b_inv_all():
        nyq = b_nyq()
        zz = None
        for i in range(8):
            ul = []
            for k, c in enumerate(b_inv(i, ul)):
                if k % 10 == 0:
                    next(nyq, None)
                yield c
            if i > 0:
                yield from b_fin(i - 1, zz)
            else:
                yield MID
            zz = [_bdot(_bf(jnp.concatenate(ul[n], axis=0)), _bf(cst[C_MD + 8 + n])) for n in range(8)]
            if i < 7:
                yield [zz[3], zz[7]]
        yield MID
        yield MID
        yield from b_fin(7, zz)

    gen = b_inv_all()
    dot = paced_dot(gen, 450)
    for n in range(4):
        def done(r, *cs):
            for p, cc in enumerate(cs):
                idx = (slice(None), r, pl.ds(0, 8), pl.ds(128 * (n + 4 * p), 128))
                outa_v[idx] = cc.reshape(NSEG // 2, 8, 128).astype(BF)
                start_out(outa_v.at[idx], out_hbm.at[idx])

        heads = lambda k: jnp.concatenate([wo_v[n + 4 * k, 64 * h:64 * h + 64, :] for h in range(k, H, 2)], axis=0)
        right = lambda m: _bf(heads(m // 6) if m % 6 == 0 else ws_v[n, m - 1])
        _strassen(lambda m: _bf(os_v[m]), right, done, dot=dot)
    for _ in gen:
        pass
    for cp in out_cps:
        cp.wait()


def pallas_concat_heads__memory_aug_recurrent_mem_tr__spectral_gfnet__prompt_kernel(
    A_x, A_mem0, A_Wq, A_Wk, A_Wv, A_Wo, A_seg_len, B_x, B_w_r, B_w_i,
):
    assert A_x.shape == (1, S, DM) and A_Wq.shape == (DM, H, E) and A_mem0.shape == (1, M, DM)
    assert B_x.shape == (1, S, DM) and (not isinstance(A_seg_len, int) or A_seg_len == SEG)
    hbm = pl.BlockSpec(memory_space=pltpu.HBM)
    wr = lambda w: w.reshape(DM // 16, 16, H, E)
    out = pl.pallas_call(
        _kernel,
        out_shape=jax.ShapeDtypeStruct((NSEG // 2, 2, SEG, 2 * DM), BF),
        in_specs=[hbm] * 11,
        out_specs=hbm,
        scratch_shapes=[
            pltpu.VMEM((NSEG, SEG, DM), BF),
            pltpu.VMEM((NSEG, 8, DM), BF),
            pltpu.VMEM((7, NSEG * 2, DM // 2), U32),
            pltpu.VMEM((M, DM), BF),
            pltpu.VMEM((80, 80), F32),
            pltpu.VMEM((UN, SEG // 2, DM), U32),
            pltpu.VMEM((NP, 3, DM // 16, 16, E), U32),
            pltpu.VMEM((8, H * E // 2, 128), U32),
            pltpu.VMEM((NP, 3, NSEG // 2, 2, 8, E), U32),
            pltpu.VMEM((7, NSEG * 2, H * E // 2), U32),
            pltpu.VMEM((4, 5, H * E // 4, 128), U32),
            pltpu.VMEM((NSEG // 2, 2, SEG, DM), BF),
            pltpu.VMEM((NSEG // 2, 2, SEG, DM), BF),
            pltpu.VMEM((2, 16, 256, 128), U32),
            pltpu.VMEM((2, 1, S), BF),
            pltpu.VMEM((2, 2, 32 * WP, 128), U32),
            pltpu.VMEM((C_NUM, 64, 128), U32),
            pltpu.VMEM((32, 4, 128, 128), BF),
            pltpu.VMEM((32, 128, 512), F32),
            pltpu.VMEM((64, 128), F32),
            pltpu.VMEM((NSEG // 2, 2, SEG, DM), BF),
            pltpu.SemaphoreType.DMA((NP + 3,)),
            pltpu.SemaphoreType.DMA((2,)),
            pltpu.SemaphoreType.DMA((1,)),
        ],
        compiler_params=pltpu.CompilerParams(vmem_limit_bytes=118 * 1024 * 1024, disable_semaphore_checks=True),
    )(A_x.reshape(NSEG, SEG, DM), A_mem0.reshape(M, DM), wr(A_Wq), wr(A_Wk), wr(A_Wv),
      A_Wo.reshape(H * E, DM), B_x.reshape(NSEG // 2, 2, SEG, DM), B_w_r.T, B_w_i.T, _mask_fill(), _fft_consts())
    return out.reshape(1, S, 2 * DM)
```

```python
import functools
import math

import jax
import jax.numpy as jnp
import numpy as np
from jax import lax
import jax.experimental.pallas as pl
import jax.experimental.pallas.tpu as pltpu

BF, F32, U32, I32 = jnp.bfloat16, jnp.float32, jnp.uint32, jnp.int32

S, DM, H, E, M, SEG = 2048, 1024, 32, 128, 8, 32
NSEG = S // SEG
NP = H // 2
UN = 4
R2 = math.sqrt(0.5)
MID = 'mid'
PAD = 28
HEAD = (0, 1, 2, 3, 5, 8, 13, 19, 24)
LATER = {3: (0, 1), 4: (2,), 5: (3, 4, 5), 6: (6, 7)}


def _to_u32(m):
    u = np.ascontiguousarray(m, dtype=np.float32).view(np.uint32)
    h = ((u + 0x7FFF + ((u >> 16) & 1)) >> 16).astype(np.uint32)
    return h[..., 0::2, :] | (h[..., 1::2, :] << 16)


def _mask_fill():
    r = np.arange(80)
    head = np.where(r < 64, r // 32, (r - 64) // 8)
    pos = np.where(r < 64, np.where(r % 32 < M, r % 32, r % 32 + M), (r - 64) % 8 + M)
    vis = (pos[:, None] < M) | (pos[:, None] >= pos[None, :])
    same = head[:, None] == head[None, :]
    return np.where(same, np.where(vis, 0.0, -1e9), -np.inf).astype(np.float32)


RES = ((0, 12, 8, 4), (1, 15, 9, 7), (2, 14, 10, 6), (3, 13, 11, 5))
WP = 72
C_MD, C_MN, C_TW, C_MS, C_NUM = 0, 16, 22, 24, 88


@functools.lru_cache(maxsize=None)
def _fft_consts():
    md = np.zeros((16, 128, 128))
    for q in range(4):
        if q == 0:
            lay = [[(0, 0), (0, 1), (2, 0), (2, 1)], [(3, 1), (1, 0), (1, 1), (3, 0)]]
        else:
            lay = [[(0, 0), (1, 0), (0, 1), (1, 1)], [(2, 1), (3, 1), (2, 0), (3, 0)]]
        for h in range(2):
            ms_, ws_ = [], []
            for g, part in lay[h]:
                k = 16 * np.arange(32) + RES[q][g]
                th = 2 * np.pi * np.outer(np.arange(128 if q == 0 else 64), k) / DM
                c, s = np.cos(th), np.sin(th)
                if q == 0:
                    ms_.append(-s if part else c)
                else:
                    sg = (1.0 if RES[q][g] % 8 == q else -1.0) * (1.0 - 2.0 * h)
                    ms_.append(np.concatenate([-s, sg * c] if part else [c, sg * s]))
                ws_.append(np.where(k == 0, 1.0, 2.0) / DM)
            m = np.concatenate(ms_, axis=1)
            md[2 * q + h] = m
            md[8 + 2 * q + h] = (m * np.concatenate(ws_)[None, :]).T
    a, l = np.arange(64), np.arange(128)
    re = 16 * (a // 8) + a % 8
    im = re + 8
    ms = np.zeros((64, 128, 128))
    for dl in range(32):
        th = 2 * np.pi * np.outer(32 * a + dl, a) / S
        c, s = np.cos(th), np.sin(th)
        ms[2 * dl][:, re], ms[2 * dl][:, im] = np.concatenate([c, -s]), np.concatenate([s, c])
        ms[2 * dl + 1][:, re] = np.concatenate([c.T, s.T]) / S
        ms[2 * dl + 1][:, im] = np.concatenate([-s.T, c.T]) / S
    mn = np.zeros((6, 128, 128))
    th = 2 * np.pi * np.outer(np.arange(32), l) / 32
    mn[0, :32], mn[1, :32] = np.cos(th), -np.sin(th)
    mn[4, :, :32], mn[5, :, :32] = np.cos(th).T / DM, -np.sin(th).T / DM
    th = 2 * np.pi * np.outer(np.arange(16), a) / 16
    c, s = np.cos(th), np.sin(th)
    mn[2, :32] = np.block([[c, s], [-s, c]])
    mn[3, :, :32] = np.block([[c.T, -s.T], [s.T, c.T]]) / S
    th = 2 * np.pi * np.outer(a, l) / S
    tw = np.stack([np.cos(th), np.sin(th)]).astype(np.float32).view(np.uint32)
    return np.concatenate([_to_u32(md), _to_u32(mn), tw, _to_u32(ms)], axis=0)


def _bdot(a, b):
    return jnp.dot(a, b, preferred_element_type=F32)


def _bf(u):
    return pltpu.bitcast(u, BF)


def _cat(rows):
    return jnp.concatenate(rows, axis=0).astype(BF)


def _unpack2(u, p):
    if p == 0:
        return pltpu.bitcast(u << 16, F32)
    return pltpu.bitcast(u & jnp.uint32(0xFFFF0000), F32)


def _strassen_left(n, a):
    return (lambda: a(1, 0) + a(1, 1), lambda: a(1, 0) - a(0, 0), lambda: a(1, 1), lambda: a(0, 0) + a(1, 1),
            lambda: a(0, 0), lambda: a(0, 1) - a(1, 1), lambda: a(0, 0) + a(0, 1))[n]()


def _strassen_right(n, w):
    add = lambda u, v: (u.astype(F32) + v.astype(F32)).astype(BF)
    sub = lambda u, v: (u.astype(F32) - v.astype(F32)).astype(BF)
    return (lambda: w(0, 0), lambda: add(w(0, 0), w(0, 1)), lambda: sub(w(1, 0), w(0, 0)),
            lambda: add(w(0, 0), w(1, 1)), lambda: sub(w(0, 1), w(1, 1)), lambda: add(w(1, 0), w(1, 1)),
            lambda: w(1, 1))[n]()


def _strassen(left, right, done, ready=lambda k: None, dot=None):
    def mm(n):
        a, r, acc = left(n), right(n), None
        for k in range(0, r.shape[0], 512):
            d = (dot or _bdot)(a[:, k:k + 512], r[k:k + 512])
            acc = d if acc is None else acc + d
        return acc

    ready(0)
    m2 = mm(0)
    c22 = mm(1) - m2
    ready(1)
    m4 = mm(2)
    c21 = m2 + m4
    m1 = mm(3)
    c11, c22 = m1 + m4, c22 + m1
    m3 = mm(4)
    done(1, c21, c22 + m3)
    c11 = c11 + mm(5)
    ready(2)
    m5 = mm(6)
    done(0, c11 - m5, m3 + m5)


def _twiddle(z, k, n, sign):
    r, i = z
    if k == 0:
        return r, i
    if 4 * k == n:
        return (-i, r) if sign > 0 else (i, -r)
    c, s = math.cos(2 * math.pi * k / n), sign * math.sin(2 * math.pi * k / n)
    if 8 * k == n or 8 * k == 3 * n:
        if c * s > 0:
            return (r - i) * c, (r + i) * c
        return (r + i) * c, (i - r) * c
    return r * c - i * s, r * s + i * c


def _cfft(xs, sign):
    n = len(xs)
    if n == 1:
        return xs
    ev, od = _cfft(xs[0::2], sign), _cfft(xs[1::2], sign)
    out = [None] * n
    for k in range(n // 2):
        er, ei = ev[k]
        if 4 * k == n:
            orr, oi = od[k]
            lo, hi = (er - oi, ei + orr), (er + oi, ei - orr)
            out[k], out[k + n // 2] = (lo, hi) if sign > 0 else (hi, lo)
        else:
            tr, ti = _twiddle(od[k], k, n, sign)
            out[k], out[k + n // 2] = (er + tr, ei + ti), (er - tr, ei - ti)
    return out


def _rfft8(x):
    a0, a1, b0, b1 = x[0] + x[4], x[0] - x[4], x[2] + x[6], x[2] - x[6]
    c0, c1, d0, d1 = x[1] + x[5], x[1] - x[5], x[3] + x[7], x[3] - x[7]
    e, f = a0 + b0, c0 + d0
    g, h = (c1 - d1) * R2, (c1 + d1) * R2
    return [e + f, e - f, a1 + g, b1 + h, a0 - b0, c0 - d0, a1 - g, b1 - h]


def _irfft8(z):
    z0, z4, z1r, z1i, z2r, z2i, z3r, z3i = z
    e, f = z0 + z4, z0 - z4
    a1, g = z1r + z3r, (z1r - z3r) * R2
    b1, h = z1i + z3i, (z1i - z3i) * R2
    a0, b0, c0, d0 = e + z2r, e - z2r, f + z2i, f - z2i
    c1, d1 = g + h, h - g
    return [a0 + a1, c0 + c1, b0 + b1, d0 + d1, a0 - a1, c0 - c1, b0 - b1, d0 - d1]


def _kernel(x_hbm, mem0_hbm, wq_hbm, wk_hbm, wv_hbm, wo_hbm, bx_hbm, wr_hbm, wi_hbm, fill_hbm, cst_hbm,
            out_hbm,
            x_v, xpre_v, xs_v, mem0_v, fill_v, lhs_v, wqkv, wo_v, pre, os_v, ws_v, outa_v,
            bx_v, w_v, wn_v, wt, cst, zs, vv, tn, outb_v,
            sem_w, sem_in, sem_out):
    scale = E ** -0.5
    wus = [w.bitcast(U32) for w in (wq_hbm, wk_hbm, wv_hbm)]
    wo_u = wo_hbm.bitcast(U32)
    fus = [w.at[pl.ds(0, 512)].bitcast(U32) for w in (wr_hbm, wi_hbm)]

    def w_copy(j, t, sem):
        return pltpu.make_async_copy(wus[t].at[:, :, j, :], wqkv.at[j, t], sem)

    xpre_cp = pltpu.make_async_copy(x_hbm.at[:, pl.ds(0, 8), :], xpre_v, sem_w.at[17])
    head = [[divmod(f, 3) for f in range(HEAD[b], HEAD[b + 1])] for b in range(len(HEAD) - 1)]
    head_cps = [[w_copy(j, t, sem_w.at[b]) for j, t in grp] for b, grp in enumerate(head) if b > 0]
    first_cps = [pltpu.make_async_copy(wus[0].at[pl.ds(32 * k, 32), :, 0, :], wqkv.at[0, 0, pl.ds(32 * k, 32)],
                                       sem_w.at[18 * k]) for k in range(2)]
    head_cps.insert(0, first_cps)

    def b_rows(i, b):
        return b, i // 4, pl.ds(pl.multiple_of((i % 4) * 8, 8), 8)

    def fwd_cps(i):
        rows = b_rows(i, slice(None))
        sem = sem_w.at[8 + i]
        return ([w_copy(8 + i, t, sem) for t in range(3)]
                + [pltpu.make_async_copy(bx_hbm.at[rows], bx_v.at[rows], sem)]
                + [pltpu.make_async_copy(fus[t].at[:, pl.ds(pl.multiple_of(128 * (2 * i + h), 128), 128)],
                                         w_v.at[t, 2 * i + h], sem) for t in range(2) for h in range(2)])

    def part(src, dst, lo, hi, sem):
        return pltpu.make_async_copy(src.at[pl.ds(lo, hi - lo)], dst.at[pl.ds(lo, hi - lo)], sem)

    c0_cp = part(cst_hbm, cst, 0, C_MS, sem_w.at[16])
    a_cps = [pltpu.make_async_copy(wo_u.at[:, pl.ds(128 * n, 128)], wo_v.at[n], sem_in.at[0]) for n in range(8)]
    a_cps += [part(x_hbm, x_v, 0, UN, sem_in.at[0]), part(cst_hbm, cst, C_MS, C_MS + UN, sem_in.at[0]),
              pltpu.make_async_copy(mem0_hbm, mem0_v, sem_in.at[0]),
              pltpu.make_async_copy(fill_hbm, fill_v, sem_in.at[0])]
    b_cps = [part(x_hbm, x_v, UN, NSEG, sem_in.at[1]), part(cst_hbm, cst, C_MS + UN, C_NUM, sem_in.at[1])]
    b_cps += [pltpu.make_async_copy(w.at[pl.ds(512, 1)], wn_v.at[t], sem_in.at[1])
              for t, w in enumerate((wr_hbm, wi_hbm))]

    lane = lax.broadcasted_iota(I32, (8, 128), 1)
    alt = jnp.where(lane % 2 == 0, 1.0, -1.0).astype(F32)
    lo_half = lane < 64
    ev_grp = (lane // 32) % 2 == 0

    def half_coef(q):
        sg = -1.0 if q < 3 else 1.0
        tc, ts = math.cos(2 * math.pi * q / 16), -math.sin(2 * math.pi * q / 16)
        f = lambda lo, hi: jnp.where(lo_half, lo, hi).astype(F32)
        return f(1.0, ts), f(0.0, sg * tc), f(0.0, tc), f(sg, -sg * ts)

    pace = {'tok': None}

    def token(v):
        return (v if v.dtype == U32 else pltpu.bitcast(v, U32)) & cst[C_MN, 56:64, :]

    def gate(v):
        tok = pace['tok']
        if tok is None:
            return v
        return v | tok if v.dtype == U32 else pltpu.bitcast(pltpu.bitcast(v, U32) | tok, v.dtype)

    def gate2(z):
        return gate(z[0]), gate(z[1])

    def as_u32(rows):
        return pltpu.bitcast(_cat(rows), U32)

    def b_fwd(i):
        r0 = pl.multiple_of(i * 8, 8)
        hc = [None] + [half_coef(q) for q in range(1, 4)]
        tacc = jnp.zeros((8, 128), F32)
        zl = []

        def filt(k):
            e, t, ty = 2 * i + k // 4, (k // 2) % 2, k % 2
            u = jnp.concatenate([gate(w_v[t, e, pl.ds(m + ty + 64 * v, 8, stride=8), :])
                                 for m in (0, 6, 4, 2) for v in range(4)], axis=0)
            ut = pltpu.bitcast(pltpu.bitcast(u, F32).T, U32)
            for v in range(16):
                wt[t, ty, pl.ds(8 * (v % 4) * WP + 4 * e + v // 4, 8, stride=WP), :] = ut[8 * v:8 * v + 8]

        for b0 in range(0, 32, 2):
            rows = []
            for b in (b0, b0 + 1):
                xb = bx_v[(*b_rows(i, b), slice(None))].astype(F32)
                z = _rfft8([gate(xb[:, 128 * t:128 * t + 128]) for t in range(8)])
                tacc = jnp.where(lane == b, jnp.sum(z[0] * alt, axis=1, keepdims=True), tacc)
                for q in range(1, 4):
                    c1, c2, c3, c4 = hc[q]
                    zr, zi = z[2 * q], z[2 * q + 1]
                    pp = c1 * zr + c2 * zi
                    qq = pltpu.roll(c3 * zr + c4 * zi, 64, 1)
                    z[2 * q], z[2 * q + 1] = pp + qq, pp - qq
                rows.append(z)
            zl.append([as_u32([rows[0][n], rows[1][n]]) for n in range(8)])
            yield 200
            if b0 % 4 == 0:
                filt(b0 // 4)
                yield 40
        tn[pl.ds(r0, 8), :] = tacc

        def mm(n):
            return _bdot(_bf(jnp.concatenate([z[n] for z in zl], axis=0)), _bf(cst[C_MD + n]))

        yield MID
        oo = [mm(n) for n in range(4)]
        yield MID
        oo += [mm(n) for n in range(4, 8)]
        yield MID
        for q in range(4):
            sel, sh = (ev_grp, 96) if q == 0 else (lo_half, 64)
            ys = []
            for b0 in range(4):
                xs = []
                for b in range(b0, 32, 4):
                    e_, o_ = gate(oo[2 * q][8 * b:8 * b + 8]), oo[2 * q + 1][8 * b:8 * b + 8]
                    xs.append((jnp.where(sel, e_, o_), pltpu.roll(jnp.where(sel, o_, e_), sh, 1)))
                ys.append([_twiddle(y, b0 * k1, 32, -1) for k1, y in enumerate(_cfft(xs, -1))])
                yield 110
            for k1 in range(8):
                for k0, y in enumerate(_cfft([gate2(ys[b0][k1]) for b0 in range(4)], -1)):
                    zs[k1 + 8 * k0, q, pl.ds(pl.multiple_of(2 * r0, 16), 16), :] = _cat(y)
                yield 30

    def b_mid(it):
        yield None
        yield None
        for h in range(2):
            dl = 2 * it + h
            y = _bdot(_bf(cst[C_MS + 2 * dl]), jnp.concatenate([zs[dl, q] for q in range(4)], axis=1))
            for _ in range(4):
                yield None
            w0 = pl.multiple_of(dl * WP, 8)
            rows = []
            for r in range(8):
                wq = []
                for t in range(2):
                    ta, tb = wt[t, 0, pl.ds(w0 + 8 * r, 8), :], wt[t, 1, pl.ds(w0 + 8 * r, 8), :]
                    wq.append([_unpack2(ta, 0), _unpack2(jnp.where(ev_grp, ta, tb), 1),
                               _unpack2(tb, 0), _unpack2(jnp.where(ev_grp, tb, ta), 1)])
                cols = []
                for q in range(4):
                    yr = gate(y[8 * r:8 * r + 8, 128 * q:128 * q + 128])
                    yi = gate(y[64 + 8 * r:72 + 8 * r, 128 * q:128 * q + 128])
                    wr, wi = wq[0][q], wq[1][q]
                    cols.append(as_u32([yr * wr - yi * wi, yr * wi + yi * wr]))
                rows.append(jnp.concatenate(cols, axis=1))
                yield None
                yield None
            yield MID
            vv[dl] = _bdot(_bf(cst[C_MS + 2 * dl + 1]), _bf(jnp.concatenate(rows, axis=0)))
            if h == 1:
                return
            for _ in range(4):
                yield None
            for n in range(4):
                for r in range(0, 64, 8):
                    blk = lambda k, p: _bf(gate(
                        wo_v[n + 4 * p, pl.ds(pl.multiple_of((2 * it + k) * 64 + r, 8), 8), :]))
                    vals = [pltpu.bitcast(_strassen_right(m, blk), U32) for m in range(1, 6)]
                    for m in range(5):
                        ws_v[n, m, pl.ds(pl.multiple_of(it * 64 + r, 8), 8), :] = vals[m]
                    yield vals
            yield MID

    def b_nyq():
        c, s = pltpu.bitcast(cst[C_TW], F32), pltpu.bitcast(cst[C_TW + 1], F32)
        tb = tn[...].astype(BF)
        tr, ti = _bdot(tb, _bf(cst[C_MN])), _bdot(tb, _bf(cst[C_MN + 1]))
        yield MID
        y = _bdot(_bf(cst[C_MN + 2, 0:16, :]), _cat([tr * c + ti * s, ti * c - tr * s]))
        row = lax.broadcasted_iota(I32, (16, 128), 0)
        wn = []
        for t in range(2):
            wrow = wn_v[t].astype(F32)
            acc = jnp.zeros((16, 128), F32)
            for e in range(16):
                acc = jnp.where(row == e, wrow[:, 128 * e:128 * e + 128], acc)
            wn.append(acc)
        yr, yi = y[0:16], y[16:32]
        yield MID
        v = _bdot(_bf(cst[C_MN + 3, :, 0:32]), _cat([yr * wn[0] - yi * wn[1], yr * wn[1] + yi * wn[0]]))
        vr, vi = v[0:64], v[64:128]
        yield MID
        tn[...] = (_bdot((vr * c - vi * s).astype(BF), _bf(cst[C_MN + 4]))
                   + _bdot((vr * s + vi * c).astype(BF), _bf(cst[C_MN + 5])))

    def b_inv(i, ul):
        r0 = i * 8
        for q in range(4):
            sel, sh = (ev_grp, 32) if q == 0 else (lo_half, 64)
            ys = []
            for b0 in range(4):
                xs = [(gate(vv[dl, pl.ds(r0, 8), 128 * q:128 * q + 128]),
                       gate(vv[dl, pl.ds(64 + r0, 8), 128 * q:128 * q + 128])) for dl in range(b0, 32, 4)]
                ys.append([_twiddle(y, b0 * k1, 32, +1) for k1, y in enumerate(_cfft(xs, +1))])
                yield 110
            ie, io = [], []
            for k1 in range(8):
                es, os_ = [], []
                for ur, ui in _cfft([gate2(ys[b0][k1]) for b0 in range(4)], +1):
                    tmp = pltpu.roll(ui, sh, 1)
                    es.append(jnp.where(sel, ur, tmp))
                    os_.append(jnp.where(sel, tmp, ur))
                ie += [as_u32(es[0:2]), as_u32(es[2:4])]
                io += [as_u32(os_[0:2]), as_u32(os_[2:4])]
                yield 55, ie[-2:] + io[-2:]
            ul += [ie, io]

    def b_fin(i, zz):
        r0 = i * 8
        hc = [None] + [half_coef(q) for q in range(1, 4)]
        tb = tn[pl.ds(r0, 8), :]
        for g in range(32):
            b = g // 4 + 8 * (g % 4)
            z = [gate(zz[n][8 * g:8 * g + 8]) for n in range(8)]
            z[0] = z[0] + jnp.sum(jnp.where(lane == b, tb, 0.0), axis=1, keepdims=True) * alt
            for q in range(1, 4):
                c1, c2, c3, c4 = hc[q]
                pp = z[2 * q] + z[2 * q + 1]
                qq = pltpu.roll(z[2 * q] - z[2 * q + 1], 64, 1)
                z[2 * q], z[2 * q + 1] = c1 * pp + c3 * qq, c2 * pp + c4 * qq
            y = _irfft8(z)
            outb_v[(*b_rows(i, b), slice(None))] = jnp.concatenate(y, axis=1).astype(BF)
            yield 75, y
        rows = b_rows(i, slice(None))
        start_out(outb_v.at[rows], out_hbm.at[(*rows, pl.ds(DM, DM))])

    def tie(w, vals):
        if not vals:
            return w
        acc = None
        for v in vals:
            v = v if v.dtype == U32 else pltpu.bitcast(v, U32)
            acc = v if acc is None else acc | v
        return jnp.concatenate([w[0:8] | token(acc), w[8:]], axis=0)

    def paced_dot(gen, budget):
        st = {'debt': 0, 'k': 0}
        due = {}

        def emit(d, b):
            while st['debt'] < b:
                r = 8 * (32 * st['debt'] // b)
                pace['tok'] = token(d[r:r + 8])
                c = next(gen, MID)
                if c is MID:
                    st['debt'] = b
                elif isinstance(c, list):
                    st['debt'] = 0
                    for own in c:
                        emit(own, 300)
                    return
                else:
                    if isinstance(c, tuple):
                        due.setdefault(st['k'] + 2, []).extend(c[1])
                        c = c[0]
                    st['debt'] += c
            st['debt'] -= b

        def dot(a, w):
            vals = due.pop(st['k'], None)
            if vals:
                a = jnp.concatenate([_bf(tie(pltpu.bitcast(a[:, 0:128], U32), vals)), a[:, 128:]], axis=1)
            d = _bdot(a, w)
            st['k'] += 1
            emit(d, budget)
            return d

        return dot

    out_cps = []

    def start_out(src, dst):
        out_cps.append(pltpu.make_async_copy(src, dst, sem_out.at[0]))
        out_cps[-1].start()

    hb = DM // 32

    def retile(j, t, k):
        blk = pl.ds(k * hb, hb)
        a, b = wqkv[j, t, blk, pl.ds(0, 8, stride=2), :], wqkv[j, t, blk, pl.ds(1, 8, stride=2), :]
        lo, hi = (a & jnp.uint32(0xFFFF)) | (b << 16), (a >> 16) | (b & jnp.uint32(0xFFFF0000))
        wqkv[j, t, blk, 0:8, :] = lo
        wqkv[j, t, blk, 8:16, :] = hi
        return lo

    def strassen_lhs():
        for g in range(NSEG // 4):
            xa = [xpre_v[4 * g + k].astype(F32) for k in range(4)]
            a1, a2 = jnp.concatenate([xa[0], xa[2]], axis=0), jnp.concatenate([xa[1], xa[3]], axis=0)
            a11, a12, a21, a22 = a1[:, :DM // 2], a1[:, DM // 2:], a2[:, :DM // 2], a2[:, DM // 2:]
            for n in range(7):
                v = _strassen_left(n, lambda r, k: ((a11, a12), (a21, a22))[r][k])
                xs_v[n, 8 * g:8 * g + 8, :] = pltpu.bitcast(v.astype(BF), U32)

    def pre_step(j, t, dot=None, sync=None, first=False):
        fresh = {}

        def w(k, p):
            v = fresh.pop((k, p), None)
            if v is None:
                v = wqkv[j, t, k * hb:(k + 1) * hb, 8 * p:8 * p + 8, :]
            return _bf(v.reshape(DM // 4, E))

        def done(h, c1, c2):
            v = jnp.concatenate([c.reshape(NSEG // 2, 8, E) for c in (c1, c2)], axis=1)
            pre[j, t, :, h] = pltpu.bitcast(v.astype(BF), U32)

        def ready(k):
            if k < 2:
                if first:
                    first_cps[k].wait()
                fresh[k, 0] = retile(j, t, k)
            elif sync:
                sync()

        _strassen(lambda n: _bf(xs_v[n]), lambda n: _strassen_right(n, w), done, ready, dot)

    for cp in [xpre_cp] + [cp for grp in head_cps for cp in grp]:
        cp.start()
    vv[0:PAD] = jnp.zeros((PAD,) + vv.shape[1:], F32)
    xpre_cp.wait()
    strassen_lhs()

    def pre_fwd(steps, i, budget):
        gen = b_fwd(i)
        dot = paced_dot(gen, budget)
        for j, t in steps + [(8 + i, t) for t in range(3)]:
            pre_step(j, t, dot)
        for _ in gen:
            pass

    def sync(b):
        for i in LATER.get(b, ()):
            for cp in ([c0_cp] if i == 0 else []) + fwd_cps(i):
                cp.start()
        for cp in head_cps[b + 1] + ([c0_cp] + fwd_cps(0) if b + 2 == len(head) else []):
            cp.wait()

    for b, grp in enumerate(head[:-1]):
        for j, t in grp:
            pre_step(j, t, sync=functools.partial(sync, b) if (j, t) == grp[-1] else None, first=b == 0)
    pre_fwd(head[-1], 0, 130)
    for cp in a_cps + b_cps:
        cp.start()

    def pre_fwd_body(i, carry):
        for cp in fwd_cps(i):
            cp.wait()
        pre_fwd([], i, 340)
        return carry

    lax.fori_loop(1, 8, pre_fwd_body, 0)
    for cp in a_cps:
        cp.wait()

    def seg_step(s, u, mem, slot, opost):
        xs = x_v[s]
        lhs_v[u] = as_u32([mem, xs[8:32].astype(F32)])
        fill = fill_v[...]
        toks = []
        pace['tok'] = None

        def proj(j, t):
            w0, w1 = [wqkv[j, t, :, 8 * p:8 * p + 8, :].reshape(DM // 2, E) for p in range(2)]
            r0, r1 = _bdot(_bf(lhs_v[u]), _bf(tie(w0, slot()))), _bdot(_bf(lhs_v[u]), _bf(w1))
            toks.append(r0[0:8])
            if len(toks) >= 4:
                pace['tok'] = token(toks[-4])
            return _cat([r0, r1, _bf(pre[j, t, s // 2, u % 2]).astype(F32)])

        def qk(q, k):
            sc = lax.dot_general(q, k, (((1,), (1,)), ((), ())), preferred_element_type=F32) * scale
            sc = jnp.where(fill == 0.0, sc, fill)
            p = jnp.exp(sc - jnp.max(sc, axis=-1, keepdims=True))
            return (p * pl.reciprocal(jnp.sum(p, axis=-1, keepdims=True), approx=True)).astype(BF)

        ob, ps, vs = {}, {}, {}

        def pv(j):
            o = _bdot(ps[j], vs[j])
            opost[u, j] = (o[64:72], o[72:80])
            if u == UN - 1:
                vals = [as_u32([_strassen_left(n, lambda r, k: opost[2 * g + r, j][k]) for g in range(2)])
                        for n in range(7)]
                for n in range(7):
                    os_v[n, pl.ds(pl.multiple_of(2 * (s - u), 8), 8), 128 * j:128 * j + 128] = vals[n]
            ob[j] = [o[0:32], o[32:64]]

        def wo(g0, g1):
            og = jnp.concatenate([o for j in range(2 * g0, 2 * g1) for o in ob[j]], axis=1).astype(BF)
            return jnp.concatenate([_bdot(og, _bf(wo_v[n, g0 * 256:g1 * 256, :])) for n in range(8)], axis=1)

        ng = NP // 2
        for g in range(ng):
            ja, jb = 2 * g, 2 * g + 1
            qa, ka, qb, kb = proj(ja, 0), proj(ja, 1), proj(jb, 0), proj(jb, 1)
            vs[ja], vs[jb] = proj(ja, 2), proj(jb, 2)
            for j, q, k in ((ja, qa, ka), (jb, qb, kb)):
                ps[j] = qk(q, k)
                if g > 0:
                    pv(j - 2)
        res = wo(0, 4)
        pv(NP - 2)
        pv(NP - 1)
        res = res + wo(4, ng - 1)
        res = res + wo(ng - 1, ng)
        outa_v[s // 2, u % 2, 8:32, :] = res[8:32].astype(BF)
        return res[0:8].astype(BF).astype(F32)

    def loop_body(it, mem):
        @pl.when(it == 1)
        def _():
            for cp in b_cps:
                cp.wait()

        gen = b_mid(it)
        opost = {}
        state = {'mid': False}

        def slot():
            if state['mid']:
                return None
            vals = next(gen, None)
            if vals is MID:
                state['mid'] = True
                return None
            return vals

        for u in range(UN):
            state['mid'] = False
            mem = seg_step(UN * it + u, u, mem, slot, opost)
        for _ in gen:
            pass
        return mem

    lax.fori_loop(0, NSEG // UN, loop_body, mem0_v[...].astype(F32))
    idx = (slice(None), slice(None), pl.ds(8, SEG - 8), pl.ds(0, DM))
    start_out(outa_v.at[idx], out_hbm.at[idx])

    def b_inv_all():
        nyq = b_nyq()
        zz = None
        for i in range(8):
            ul = []
            for k, c in enumerate(b_inv(i, ul)):
                if k % 10 == 0:
                    next(nyq, None)
                yield c
            if i > 0:
                yield from b_fin(i - 1, zz)
            else:
                yield MID
            zz = [_bdot(_bf(jnp.concatenate(ul[n], axis=0)), _bf(cst[C_MD + 8 + n])) for n in range(8)]
            if i < 7:
                yield [zz[3], zz[7]]
        yield MID
        yield MID
        yield from b_fin(7, zz)

    gen = b_inv_all()
    dot = paced_dot(gen, 450)
    for n in range(4):
        def done(r, *cs):
            for p, cc in enumerate(cs):
                idx = (slice(None), r, pl.ds(0, 8), pl.ds(128 * (n + 4 * p), 128))
                outa_v[idx] = cc.reshape(NSEG // 2, 8, 128).astype(BF)
                start_out(outa_v.at[idx], out_hbm.at[idx])

        heads = lambda k: jnp.concatenate([wo_v[n + 4 * k, 64 * h:64 * h + 64, :] for h in range(k, H, 2)], axis=0)
        right = lambda m: _bf(heads(m // 6) if m % 6 == 0 else ws_v[n, m - 1])
        _strassen(lambda m: _bf(os_v[m]), right, done, dot=dot)
    for _ in gen:
        pass
    for cp in out_cps:
        cp.wait()


def pallas_concat_heads__memory_aug_recurrent_mem_tr__spectral_gfnet__prompt_kernel(
    A_x, A_mem0, A_Wq, A_Wk, A_Wv, A_Wo, A_seg_len, B_x, B_w_r, B_w_i,
):
    assert A_x.shape == (1, S, DM) and A_Wq.shape == (DM, H, E) and A_mem0.shape == (1, M, DM)
    assert B_x.shape == (1, S, DM) and (not isinstance(A_seg_len, int) or A_seg_len == SEG)
    hbm = pl.BlockSpec(memory_space=pltpu.HBM)
    wr = lambda w: w.reshape(DM // 16, 16, H, E)
    out = pl.pallas_call(
        _kernel,
        out_shape=jax.ShapeDtypeStruct((NSEG // 2, 2, SEG, 2 * DM), BF),
        in_specs=[hbm] * 11,
        out_specs=hbm,
        scratch_shapes=[
            pltpu.VMEM((NSEG, SEG, DM), BF),
            pltpu.VMEM((NSEG, 8, DM), BF),
            pltpu.VMEM((7, NSEG * 2, DM // 2), U32),
            pltpu.VMEM((M, DM), BF),
            pltpu.VMEM((80, 80), F32),
            pltpu.VMEM((UN, SEG // 2, DM), U32),
            pltpu.VMEM((NP, 3, DM // 16, 16, E), U32),
            pltpu.VMEM((8, H * E // 2, 128), U32),
            pltpu.VMEM((NP, 3, NSEG // 2, 2, 8, E), U32),
            pltpu.VMEM((7, NSEG * 2, H * E // 2), U32),
            pltpu.VMEM((4, 5, H * E // 4, 128), U32),
            pltpu.VMEM((NSEG // 2, 2, SEG, DM), BF),
            pltpu.VMEM((NSEG // 2, 2, SEG, DM), BF),
            pltpu.VMEM((2, 16, 256, 128), U32),
            pltpu.VMEM((2, 1, S), BF),
            pltpu.VMEM((2, 2, 32 * WP, 128), U32),
            pltpu.VMEM((C_NUM, 64, 128), U32),
            pltpu.VMEM((32, 4, 128, 128), BF),
            pltpu.VMEM((32, 128, 512), F32),
            pltpu.VMEM((64, 128), F32),
            pltpu.VMEM((NSEG // 2, 2, SEG, DM), BF),
            pltpu.SemaphoreType.DMA((NP + 3,)),
            pltpu.SemaphoreType.DMA((2,)),
            pltpu.SemaphoreType.DMA((1,)),
        ],
        compiler_params=pltpu.CompilerParams(vmem_limit_bytes=118 * 1024 * 1024, disable_semaphore_checks=True),
    )(A_x.reshape(NSEG, SEG, DM), A_mem0.reshape(M, DM), wr(A_Wq), wr(A_Wk), wr(A_Wv),
      A_Wo.reshape(H * E, DM), B_x.reshape(NSEG // 2, 2, SEG, DM), B_w_r.T, B_w_i.T, _mask_fill(), _fft_consts())
    return out.reshape(1, S, 2 * DM)
```

```python
import functools
import math

import jax
import jax.numpy as jnp
import numpy as np
from jax import lax
import jax.experimental.pallas as pl
import jax.experimental.pallas.tpu as pltpu

BF, F32, U32, I32 = jnp.bfloat16, jnp.float32, jnp.uint32, jnp.int32

S, DM, H, E, M, SEG = 2048, 1024, 32, 128, 8, 32
NSEG = S // SEG
NP = H // 2
UN = 4
R2 = math.sqrt(0.5)
MID = 'mid'
PAD = 28
HEAD = (0, 1, 2, 3, 5, 8, 13, 19, 24)
LATER = {3: (0, 1), 4: (2,), 5: (3, 4, 5), 6: (6, 7)}


def _to_u32(m):
    u = np.ascontiguousarray(m, dtype=np.float32).view(np.uint32)
    h = ((u + 0x7FFF + ((u >> 16) & 1)) >> 16).astype(np.uint32)
    return h[..., 0::2, :] | (h[..., 1::2, :] << 16)


def _mask_fill():
    r = np.arange(80)
    head = np.where(r < 64, r // 32, (r - 64) // 8)
    pos = np.where(r < 64, np.where(r % 32 < M, r % 32, r % 32 + M), (r - 64) % 8 + M)
    vis = (pos[:, None] < M) | (pos[:, None] >= pos[None, :])
    same = head[:, None] == head[None, :]
    return np.where(same, np.where(vis, 0.0, -1e9), -np.inf).astype(np.float32)


RES = ((0, 12, 8, 4), (1, 15, 9, 7), (2, 14, 10, 6), (3, 13, 11, 5))
WP = 72
C_MD, C_MN, C_TW, C_MS, C_NUM = 0, 16, 22, 24, 88


@functools.lru_cache(maxsize=None)
def _fft_consts():
    md = np.zeros((16, 128, 128))
    for q in range(4):
        if q == 0:
            lay = [[(0, 0), (0, 1), (2, 0), (2, 1)], [(3, 1), (1, 0), (1, 1), (3, 0)]]
        else:
            lay = [[(0, 0), (1, 0), (0, 1), (1, 1)], [(2, 1), (3, 1), (2, 0), (3, 0)]]
        for h in range(2):
            ms_, ws_ = [], []
            for g, part in lay[h]:
                k = 16 * np.arange(32) + RES[q][g]
                th = 2 * np.pi * np.outer(np.arange(128 if q == 0 else 64), k) / DM
                c, s = np.cos(th), np.sin(th)
                if q == 0:
                    ms_.append(-s if part else c)
                else:
                    sg = (1.0 if RES[q][g] % 8 == q else -1.0) * (1.0 - 2.0 * h)
                    ms_.append(np.concatenate([-s, sg * c] if part else [c, sg * s]))
                ws_.append(np.where(k == 0, 1.0, 2.0) / DM)
            m = np.concatenate(ms_, axis=1)
            md[2 * q + h] = m
            md[8 + 2 * q + h] = (m * np.concatenate(ws_)[None, :]).T
    a, l = np.arange(64), np.arange(128)
    re = 16 * (a // 8) + a % 8
    im = re + 8
    ms = np.zeros((64, 128, 128))
    for dl in range(32):
        th = 2 * np.pi * np.outer(32 * a + dl, a) / S
        c, s = np.cos(th), np.sin(th)
        ms[2 * dl][:, re], ms[2 * dl][:, im] = np.concatenate([c, -s]), np.concatenate([s, c])
        ms[2 * dl + 1][:, re] = np.concatenate([c.T, s.T]) / S
        ms[2 * dl + 1][:, im] = np.concatenate([-s.T, c.T]) / S
    mn = np.zeros((6, 128, 128))
    th = 2 * np.pi * np.outer(np.arange(32), l) / 32
    mn[0, :32], mn[1, :32] = np.cos(th), -np.sin(th)
    mn[4, :, :32], mn[5, :, :32] = np.cos(th).T / DM, -np.sin(th).T / DM
    th = 2 * np.pi * np.outer(np.arange(16), a) / 16
    c, s = np.cos(th), np.sin(th)
    mn[2, :32] = np.block([[c, s], [-s, c]])
    mn[3, :, :32] = np.block([[c.T, -s.T], [s.T, c.T]]) / S
    th = 2 * np.pi * np.outer(a, l) / S
    tw = np.stack([np.cos(th), np.sin(th)]).astype(np.float32).view(np.uint32)
    return np.concatenate([_to_u32(md), _to_u32(mn), tw, _to_u32(ms)], axis=0)


def _bdot(a, b):
    return jnp.dot(a, b, preferred_element_type=F32)


def _bf(u):
    return pltpu.bitcast(u, BF)


def _cat(rows):
    return jnp.concatenate(rows, axis=0).astype(BF)


def _unpack2(u, p):
    if p == 0:
        return pltpu.bitcast(u << 16, F32)
    return pltpu.bitcast(u & jnp.uint32(0xFFFF0000), F32)


def _strassen_left(n, a):
    return (lambda: a(1, 0) + a(1, 1), lambda: a(1, 0) - a(0, 0), lambda: a(1, 1), lambda: a(0, 0) + a(1, 1),
            lambda: a(0, 0), lambda: a(0, 1) - a(1, 1), lambda: a(0, 0) + a(0, 1))[n]()


def _strassen_right(n, w):
    add = lambda u, v: (u.astype(F32) + v.astype(F32)).astype(BF)
    sub = lambda u, v: (u.astype(F32) - v.astype(F32)).astype(BF)
    return (lambda: w(0, 0), lambda: add(w(0, 0), w(0, 1)), lambda: sub(w(1, 0), w(0, 0)),
            lambda: add(w(0, 0), w(1, 1)), lambda: sub(w(0, 1), w(1, 1)), lambda: add(w(1, 0), w(1, 1)),
            lambda: w(1, 1))[n]()


def _strassen(left, right, done, ready=lambda k: None, dot=None):
    def mm(n):
        a, r, acc = left(n), right(n), None
        for k in range(0, r.shape[0], 512):
            d = (dot or _bdot)(a[:, k:k + 512], r[k:k + 512])
            acc = d if acc is None else acc + d
        return acc

    ready(0)
    m2 = mm(0)
    c22 = mm(1) - m2
    ready(1)
    m4 = mm(2)
    c21 = m2 + m4
    m1 = mm(3)
    c11, c22 = m1 + m4, c22 + m1
    m3 = mm(4)
    done(1, c21, c22 + m3)
    c11 = c11 + mm(5)
    ready(2)
    m5 = mm(6)
    done(0, c11 - m5, m3 + m5)


def _twiddle(z, k, n, sign):
    r, i = z
    if k == 0:
        return r, i
    if 4 * k == n:
        return (-i, r) if sign > 0 else (i, -r)
    c, s = math.cos(2 * math.pi * k / n), sign * math.sin(2 * math.pi * k / n)
    if 8 * k == n or 8 * k == 3 * n:
        if c * s > 0:
            return (r - i) * c, (r + i) * c
        return (r + i) * c, (i - r) * c
    return r * c - i * s, r * s + i * c


def _cfft(xs, sign):
    n = len(xs)
    if n == 1:
        return xs
    ev, od = _cfft(xs[0::2], sign), _cfft(xs[1::2], sign)
    out = [None] * n
    for k in range(n // 2):
        er, ei = ev[k]
        if 4 * k == n:
            orr, oi = od[k]
            lo, hi = (er - oi, ei + orr), (er + oi, ei - orr)
            out[k], out[k + n // 2] = (lo, hi) if sign > 0 else (hi, lo)
        else:
            tr, ti = _twiddle(od[k], k, n, sign)
            out[k], out[k + n // 2] = (er + tr, ei + ti), (er - tr, ei - ti)
    return out


def _rfft8(x):
    a0, a1, b0, b1 = x[0] + x[4], x[0] - x[4], x[2] + x[6], x[2] - x[6]
    c0, c1, d0, d1 = x[1] + x[5], x[1] - x[5], x[3] + x[7], x[3] - x[7]
    e, f = a0 + b0, c0 + d0
    g, h = (c1 - d1) * R2, (c1 + d1) * R2
    return [e + f, e - f, a1 + g, b1 + h, a0 - b0, c0 - d0, a1 - g, b1 - h]


def _irfft8(z):
    z0, z4, z1r, z1i, z2r, z2i, z3r, z3i = z
    e, f = z0 + z4, z0 - z4
    a1, g = z1r + z3r, (z1r - z3r) * R2
    b1, h = z1i + z3i, (z1i - z3i) * R2
    a0, b0, c0, d0 = e + z2r, e - z2r, f + z2i, f - z2i
    c1, d1 = g + h, h - g
    return [a0 + a1, c0 + c1, b0 + b1, d0 + d1, a0 - a1, c0 - c1, b0 - b1, d0 - d1]


def _kernel(x_hbm, mem0_hbm, wq_hbm, wk_hbm, wv_hbm, wo_hbm, bx_hbm, wr_hbm, wi_hbm, fill_hbm, cst_hbm,
            out_hbm,
            x_v, xpre_v, xs_v, mem0_v, fill_v, wqkv, wo_v, pre, os_v, ws_v, outa_v,
            bx_v, w_v, wn_v, wt, cst, zs, vv, tn, outb_v,
            sem_w, sem_in, sem_out):
    scale = E ** -0.5
    wus = [w.bitcast(U32) for w in (wq_hbm, wk_hbm, wv_hbm)]
    wo_u = wo_hbm.bitcast(U32)
    fus = [w.at[pl.ds(0, 512)].bitcast(U32) for w in (wr_hbm, wi_hbm)]

    def w_copy(j, t, sem):
        return pltpu.make_async_copy(wus[t].at[:, :, j, :], wqkv.at[j, t], sem)

    xpre_cp = pltpu.make_async_copy(x_hbm.at[:, pl.ds(0, 8), :], xpre_v, sem_w.at[17])
    head = [[divmod(f, 3) for f in range(HEAD[b], HEAD[b + 1])] for b in range(len(HEAD) - 1)]
    head_cps = [[w_copy(j, t, sem_w.at[b]) for j, t in grp] for b, grp in enumerate(head) if b > 0]
    first_cps = [pltpu.make_async_copy(wus[0].at[pl.ds(32 * k, 32), :, 0, :], wqkv.at[0, 0, pl.ds(32 * k, 32)],
                                       sem_w.at[18 * k]) for k in range(2)]
    head_cps.insert(0, first_cps)

    def b_rows(i, b):
        return b, i // 4, pl.ds(pl.multiple_of((i % 4) * 8, 8), 8)

    def fwd_cps(i):
        rows = b_rows(i, slice(None))
        sem = sem_w.at[8 + i]
        return ([w_copy(8 + i, t, sem) for t in range(3)]
                + [pltpu.make_async_copy(bx_hbm.at[rows], bx_v.at[rows], sem)]
                + [pltpu.make_async_copy(fus[t].at[:, pl.ds(pl.multiple_of(128 * (2 * i + h), 128), 128)],
                                         w_v.at[t, 2 * i + h], sem) for t in range(2) for h in range(2)])

    def part(src, dst, lo, hi, sem):
        return pltpu.make_async_copy(src.at[pl.ds(lo, hi - lo)], dst.at[pl.ds(lo, hi - lo)], sem)

    c0_cp = part(cst_hbm, cst, 0, C_MS, sem_w.at[16])
    a_cps = [pltpu.make_async_copy(wo_u.at[:, pl.ds(128 * n, 128)], wo_v.at[n], sem_in.at[0]) for n in range(8)]
    a_cps += [part(x_hbm, x_v, 0, UN, sem_in.at[0]), part(cst_hbm, cst, C_MS, C_MS + UN, sem_in.at[0]),
              pltpu.make_async_copy(mem0_hbm, mem0_v, sem_in.at[0]),
              pltpu.make_async_copy(fill_hbm, fill_v, sem_in.at[0])]
    b_cps = [part(x_hbm, x_v, UN, NSEG, sem_in.at[1]), part(cst_hbm, cst, C_MS + UN, C_NUM, sem_in.at[1])]
    b_cps += [pltpu.make_async_copy(w.at[pl.ds(512, 1)], wn_v.at[t], sem_in.at[1])
              for t, w in enumerate((wr_hbm, wi_hbm))]

    lane = lax.broadcasted_iota(I32, (8, 128), 1)
    alt = jnp.where(lane % 2 == 0, 1.0, -1.0).astype(F32)
    lo_half = lane < 64
    ev_grp = (lane // 32) % 2 == 0

    def half_coef(q):
        sg = -1.0 if q < 3 else 1.0
        tc, ts = math.cos(2 * math.pi * q / 16), -math.sin(2 * math.pi * q / 16)
        f = lambda lo, hi: jnp.where(lo_half, lo, hi).astype(F32)
        return f(1.0, ts), f(0.0, sg * tc), f(0.0, tc), f(sg, -sg * ts)

    pace = {'tok': None}

    def token(v):
        return (v if v.dtype == U32 else pltpu.bitcast(v, U32)) & cst[C_MN, 56:64, :]

    def gate(v):
        tok = pace['tok']
        if tok is None:
            return v
        return v | tok if v.dtype == U32 else pltpu.bitcast(pltpu.bitcast(v, U32) | tok, v.dtype)

    def gate2(z):
        return gate(z[0]), gate(z[1])

    def as_u32(rows):
        return pltpu.bitcast(_cat(rows), U32)

    def b_fwd(i):
        r0 = pl.multiple_of(i * 8, 8)
        hc = [None] + [half_coef(q) for q in range(1, 4)]
        tacc = jnp.zeros((8, 128), F32)
        zl = []

        def filt(k):
            e, t, ty = 2 * i + k // 4, (k // 2) % 2, k % 2
            u = jnp.concatenate([gate(w_v[t, e, pl.ds(m + ty + 64 * v, 8, stride=8), :])
                                 for m in (0, 6, 4, 2) for v in range(4)], axis=0)
            ut = pltpu.bitcast(pltpu.bitcast(u, F32).T, U32)
            for v in range(16):
                wt[t, ty, pl.ds(8 * (v % 4) * WP + 4 * e + v // 4, 8, stride=WP), :] = ut[8 * v:8 * v + 8]

        for b0 in range(0, 32, 2):
            rows = []
            for b in (b0, b0 + 1):
                xb = bx_v[(*b_rows(i, b), slice(None))].astype(F32)
                z = _rfft8([gate(xb[:, 128 * t:128 * t + 128]) for t in range(8)])
                tacc = jnp.where(lane == b, jnp.sum(z[0] * alt, axis=1, keepdims=True), tacc)
                for q in range(1, 4):
                    c1, c2, c3, c4 = hc[q]
                    zr, zi = z[2 * q], z[2 * q + 1]
                    pp = c1 * zr + c2 * zi
                    qq = pltpu.roll(c3 * zr + c4 * zi, 64, 1)
                    z[2 * q], z[2 * q + 1] = pp + qq, pp - qq
                rows.append(z)
            zl.append([as_u32([rows[0][n], rows[1][n]]) for n in range(8)])
            yield 200
            if b0 % 4 == 0:
                filt(b0 // 4)
                yield 40
        tn[pl.ds(r0, 8), :] = tacc

        def mm(n):
            return _bdot(_bf(jnp.concatenate([z[n] for z in zl], axis=0)), _bf(cst[C_MD + n]))

        yield MID
        oo = [mm(n) for n in range(4)]
        yield MID
        oo += [mm(n) for n in range(4, 8)]
        yield MID
        for q in range(4):
            sel, sh = (ev_grp, 96) if q == 0 else (lo_half, 64)
            ys = []
            for b0 in range(4):
                xs = []
                for b in range(b0, 32, 4):
                    e_, o_ = gate(oo[2 * q][8 * b:8 * b + 8]), oo[2 * q + 1][8 * b:8 * b + 8]
                    xs.append((jnp.where(sel, e_, o_), pltpu.roll(jnp.where(sel, o_, e_), sh, 1)))
                ys.append([_twiddle(y, b0 * k1, 32, -1) for k1, y in enumerate(_cfft(xs, -1))])
                yield 110
            for k1 in range(8):
                for k0, y in enumerate(_cfft([gate2(ys[b0][k1]) for b0 in range(4)], -1)):
                    zs[k1 + 8 * k0, q, pl.ds(pl.multiple_of(2 * r0, 16), 16), :] = _cat(y)
                yield 30

    def b_mid(it):
        def fwd(dl):
            return _bdot(_bf(cst[C_MS + 2 * dl]), jnp.concatenate([zs[dl, q] for q in range(4)], axis=1))

        def mult(dl, y, rows):
            yield from [None] * 4
            w0 = pl.multiple_of(dl * WP, 8)
            for r in range(8):
                wq = []
                for t in range(2):
                    ta, tb = wt[t, 0, pl.ds(w0 + 8 * r, 8), :], wt[t, 1, pl.ds(w0 + 8 * r, 8), :]
                    wq.append([_unpack2(ta, 0), _unpack2(jnp.where(ev_grp, ta, tb), 1),
                               _unpack2(tb, 0), _unpack2(jnp.where(ev_grp, tb, ta), 1)])
                cols = []
                for q in range(4):
                    yr = gate(y[8 * r:8 * r + 8, 128 * q:128 * q + 128])
                    yi = gate(y[64 + 8 * r:72 + 8 * r, 128 * q:128 * q + 128])
                    wr, wi = wq[0][q], wq[1][q]
                    cols.append(as_u32([yr * wr - yi * wi, yr * wi + yi * wr]))
                rows.append(jnp.concatenate(cols, axis=1))
                yield from [None] * 2

        def inv(dl, rows):
            vv[dl] = _bdot(_bf(cst[C_MS + 2 * dl + 1]), _bf(jnp.concatenate(rows, axis=0)))

        def rights():
            for n in range(4):
                for r in range(0, 64, 8):
                    blk = lambda k, p: _bf(gate(
                        wo_v[n + 4 * p, pl.ds(pl.multiple_of((2 * it + k) * 64 + r, 8), 8), :]))
                    vals = [pltpu.bitcast(_strassen_right(m, blk), U32) for m in range(1, 6)]
                    for m in range(5):
                        ws_v[n, m, pl.ds(pl.multiple_of(it * 64 + r, 8), 8), :] = vals[m]
                    yield vals

        yield from [None] * 2
        for h in range(2):
            rows = []
            y = fwd(2 * it + h)
            yield from mult(2 * it + h, y, rows)
            yield MID
            inv(2 * it + h, rows)
            if h == 0:
                yield from [None] * 4
                yield from rights()
                yield MID

    def b_nyq():
        c, s = pltpu.bitcast(cst[C_TW], F32), pltpu.bitcast(cst[C_TW + 1], F32)
        tb = tn[...].astype(BF)
        tr, ti = _bdot(tb, _bf(cst[C_MN])), _bdot(tb, _bf(cst[C_MN + 1]))
        yield MID
        y = _bdot(_bf(cst[C_MN + 2, 0:16, :]), _cat([tr * c + ti * s, ti * c - tr * s]))
        row = lax.broadcasted_iota(I32, (16, 128), 0)
        wn = []
        for t in range(2):
            wrow = wn_v[t].astype(F32)
            acc = jnp.zeros((16, 128), F32)
            for e in range(16):
                acc = jnp.where(row == e, wrow[:, 128 * e:128 * e + 128], acc)
            wn.append(acc)
        yr, yi = y[0:16], y[16:32]
        yield MID
        v = _bdot(_bf(cst[C_MN + 3, :, 0:32]), _cat([yr * wn[0] - yi * wn[1], yr * wn[1] + yi * wn[0]]))
        vr, vi = v[0:64], v[64:128]
        yield MID
        tn[...] = (_bdot((vr * c - vi * s).astype(BF), _bf(cst[C_MN + 4]))
                   + _bdot((vr * s + vi * c).astype(BF), _bf(cst[C_MN + 5])))

    def b_inv(i, ul):
        r0 = i * 8
        for q in range(4):
            sel, sh = (ev_grp, 32) if q == 0 else (lo_half, 64)
            ys = []
            for b0 in range(4):
                xs = [(gate(vv[dl, pl.ds(r0, 8), 128 * q:128 * q + 128]),
                       gate(vv[dl, pl.ds(64 + r0, 8), 128 * q:128 * q + 128])) for dl in range(b0, 32, 4)]
                ys.append([_twiddle(y, b0 * k1, 32, +1) for k1, y in enumerate(_cfft(xs, +1))])
                yield 110
            ie, io = [], []
            for k1 in range(8):
                es, os_ = [], []
                for ur, ui in _cfft([gate2(ys[b0][k1]) for b0 in range(4)], +1):
                    tmp = pltpu.roll(ui, sh, 1)
                    es.append(jnp.where(sel, ur, tmp))
                    os_.append(jnp.where(sel, tmp, ur))
                ie += [as_u32(es[0:2]), as_u32(es[2:4])]
                io += [as_u32(os_[0:2]), as_u32(os_[2:4])]
                yield 55, ie[-2:] + io[-2:]
            ul += [ie, io]

    def b_fin(i, zz):
        r0 = i * 8
        hc = [None] + [half_coef(q) for q in range(1, 4)]
        tb = tn[pl.ds(r0, 8), :]
        for g in range(32):
            b = g // 4 + 8 * (g % 4)
            z = [gate(zz[n][8 * g:8 * g + 8]) for n in range(8)]
            z[0] = z[0] + jnp.sum(jnp.where(lane == b, tb, 0.0), axis=1, keepdims=True) * alt
            for q in range(1, 4):
                c1, c2, c3, c4 = hc[q]
                pp = z[2 * q] + z[2 * q + 1]
                qq = pltpu.roll(z[2 * q] - z[2 * q + 1], 64, 1)
                z[2 * q], z[2 * q + 1] = c1 * pp + c3 * qq, c2 * pp + c4 * qq
            y = _irfft8(z)
            outb_v[(*b_rows(i, b), slice(None))] = jnp.concatenate(y, axis=1).astype(BF)
            yield 75, y
        rows = b_rows(i, slice(None))
        start_out(outb_v.at[rows], out_hbm.at[(*rows, pl.ds(DM, DM))])

    def tie(w, vals):
        if not vals:
            return w
        acc = None
        for v in vals:
            v = v if v.dtype == U32 else pltpu.bitcast(v, U32)
            acc = v if acc is None else acc | v
        return jnp.concatenate([w[0:8] | token(acc), w[8:]], axis=0)

    def paced_dot(gen, budget):
        st = {'debt': 0, 'k': 0}
        due = {}

        def emit(d, b):
            while st['debt'] < b:
                r = 8 * (32 * st['debt'] // b)
                pace['tok'] = token(d[r:r + 8])
                c = next(gen, MID)
                if c is MID:
                    st['debt'] = b
                elif isinstance(c, list):
                    st['debt'] = 0
                    for own in c:
                        emit(own, 300)
                    return
                else:
                    if isinstance(c, tuple):
                        due.setdefault(st['k'] + 2, []).extend(c[1])
                        c = c[0]
                    st['debt'] += c
            st['debt'] -= b

        def dot(a, w):
            vals = due.pop(st['k'], None)
            if vals:
                a = jnp.concatenate([_bf(tie(pltpu.bitcast(a[:, 0:128], U32), vals)), a[:, 128:]], axis=1)
            d = _bdot(a, w)
            st['k'] += 1
            emit(d, budget)
            return d

        return dot

    out_cps = []

    def start_out(src, dst):
        out_cps.append(pltpu.make_async_copy(src, dst, sem_out.at[0]))
        out_cps[-1].start()

    hb = DM // 32

    def retile(j, t, k):
        blk = pl.ds(k * hb, hb)
        a, b = wqkv[j, t, blk, pl.ds(0, 8, stride=2), :], wqkv[j, t, blk, pl.ds(1, 8, stride=2), :]
        lo, hi = (a & jnp.uint32(0xFFFF)) | (b << 16), (a >> 16) | (b & jnp.uint32(0xFFFF0000))
        wqkv[j, t, blk, 0:8, :] = lo
        wqkv[j, t, blk, 8:16, :] = hi
        return lo

    def strassen_lhs():
        for g in range(NSEG // 4):
            xa = [xpre_v[4 * g + k].astype(F32) for k in range(4)]
            a1, a2 = jnp.concatenate([xa[0], xa[2]], axis=0), jnp.concatenate([xa[1], xa[3]], axis=0)
            a11, a12, a21, a22 = a1[:, :DM // 2], a1[:, DM // 2:], a2[:, :DM // 2], a2[:, DM // 2:]
            for n in range(7):
                v = _strassen_left(n, lambda r, k: ((a11, a12), (a21, a22))[r][k])
                xs_v[n, 8 * g:8 * g + 8, :] = pltpu.bitcast(v.astype(BF), U32)

    def pre_step(j, t, dot=None, sync=None, first=False):
        fresh = {}

        def w(k, p):
            v = fresh.pop((k, p), None)
            if v is None:
                v = wqkv[j, t, k * hb:(k + 1) * hb, 8 * p:8 * p + 8, :]
            return _bf(v.reshape(DM // 4, E))

        def done(h, c1, c2):
            v = jnp.concatenate([c.reshape(NSEG // 2, 8, E) for c in (c1, c2)], axis=1)
            pre[j, t, :, h] = pltpu.bitcast(v.astype(BF), U32)

        def ready(k):
            if k < 2:
                if first:
                    first_cps[k].wait()
                fresh[k, 0] = retile(j, t, k)
            elif sync:
                sync()

        _strassen(lambda n: _bf(xs_v[n]), lambda n: _strassen_right(n, w), done, ready, dot)

    for cp in [xpre_cp] + [cp for grp in head_cps for cp in grp]:
        cp.start()
    vv[0:PAD] = jnp.zeros((PAD,) + vv.shape[1:], F32)
    xpre_cp.wait()
    strassen_lhs()

    def pre_fwd(steps, i, budget):
        gen = b_fwd(i)
        dot = paced_dot(gen, budget)
        for j, t in steps + [(8 + i, t) for t in range(3)]:
            pre_step(j, t, dot)
        for _ in gen:
            pass

    def sync(b):
        for i in LATER.get(b, ()):
            for cp in ([c0_cp] if i == 0 else []) + fwd_cps(i):
                cp.start()
        for cp in head_cps[b + 1] + ([c0_cp] + fwd_cps(0) if b + 2 == len(head) else []):
            cp.wait()

    for b, grp in enumerate(head[:-1]):
        for j, t in grp:
            pre_step(j, t, sync=functools.partial(sync, b) if (j, t) == grp[-1] else None, first=b == 0)
    pre_fwd(head[-1], 0, 130)
    for cp in a_cps + b_cps:
        cp.start()

    def pre_fwd_body(i, carry):
        for cp in fwd_cps(i):
            cp.wait()
        pre_fwd([], i, 340)
        return carry

    lax.fori_loop(1, 8, pre_fwd_body, 0)
    for cp in a_cps:
        cp.wait()

    def seg_step(s, u, mem, slot, opost):
        lhs = _cat([mem, x_v[s][8:32].astype(F32)])
        fill = fill_v[...]
        toks = []
        pace['tok'] = None

        def proj(j, t):
            w0, w1 = [wqkv[j, t, :, 8 * p:8 * p + 8, :].reshape(DM // 2, E) for p in range(2)]
            r0, r1 = _bdot(lhs, _bf(tie(w0, slot()))), _bdot(lhs, _bf(w1))
            toks.append(r0[0:8])
            if len(toks) >= 4:
                pace['tok'] = token(toks[-4])
            return _cat([r0, r1, _bf(pre[j, t, s // 2, u % 2]).astype(F32)])

        def qk(q, k):
            sc = lax.dot_general(q, k, (((1,), (1,)), ((), ())), preferred_element_type=F32) * scale
            sc = jnp.where(fill == 0.0, sc, fill)
            p = jnp.exp(sc - jnp.max(sc, axis=-1, keepdims=True))
            return (p * pl.reciprocal(jnp.sum(p, axis=-1, keepdims=True), approx=True)).astype(BF)

        ob, ps, vs = {}, {}, {}

        def pv(j):
            o = _bdot(ps[j], vs[j])
            opost[u, j] = (o[64:72], o[72:80])
            if u == UN - 1:
                vals = [as_u32([_strassen_left(n, lambda r, k: opost[2 * g + r, j][k]) for g in range(2)])
                        for n in range(7)]
                for n in range(7):
                    os_v[n, pl.ds(pl.multiple_of(2 * (s - u), 8), 8), 128 * j:128 * j + 128] = vals[n]
            ob[j] = [o[0:32], o[32:64]]

        def wo(g0, g1):
            og = jnp.concatenate([o for j in range(2 * g0, 2 * g1) for o in ob[j]], axis=1).astype(BF)
            return jnp.concatenate([_bdot(og, _bf(wo_v[n, g0 * 256:g1 * 256, :])) for n in range(8)], axis=1)

        ng = NP // 2
        for g in range(ng):
            ja, jb = 2 * g, 2 * g + 1
            qa, ka, qb, kb = proj(ja, 0), proj(ja, 1), proj(jb, 0), proj(jb, 1)
            vs[ja], vs[jb] = proj(ja, 2), proj(jb, 2)
            for j, q, k in ((ja, qa, ka), (jb, qb, kb)):
                ps[j] = qk(q, k)
                if g > 0:
                    pv(j - 2)
        res = wo(0, 4)
        pv(NP - 2)
        pv(NP - 1)
        res = res + wo(4, ng - 1)
        res = res + wo(ng - 1, ng)
        outa_v[s // 2, u % 2, 8:32, :] = res[8:32].astype(BF)
        return res[0:8]

    def loop_body(it, mem):
        @pl.when(it == 1)
        def _():
            for cp in b_cps:
                cp.wait()

        gen = b_mid(it)
        opost = {}
        state = {'mid': False}

        def slot():
            if state['mid']:
                return None
            vals = next(gen, None)
            if vals is MID:
                state['mid'] = True
                return None
            return vals

        for u in range(UN):
            state['mid'] = False
            mem = seg_step(UN * it + u, u, mem, slot, opost)
        for _ in gen:
            pass
        return mem

    lax.fori_loop(0, NSEG // UN, loop_body, mem0_v[...].astype(F32))
    idx = (slice(None), slice(None), pl.ds(8, SEG - 8), pl.ds(0, DM))
    start_out(outa_v.at[idx], out_hbm.at[idx])

    def b_inv_all():
        nyq = b_nyq()
        zz = None
        for i in range(8):
            ul = []
            for k, c in enumerate(b_inv(i, ul)):
                if k % 10 == 0:
                    next(nyq, None)
                yield c
            if i > 0:
                yield from b_fin(i - 1, zz)
            else:
                yield MID
            zz = [_bdot(_bf(jnp.concatenate(ul[n], axis=0)), _bf(cst[C_MD + 8 + n])) for n in range(8)]
            if i < 7:
                yield [zz[3], zz[7]]
        yield MID
        yield MID
        yield from b_fin(7, zz)

    gen = b_inv_all()
    dot = paced_dot(gen, 450)
    for n in range(4):
        def done(r, *cs):
            for p, cc in enumerate(cs):
                idx = (slice(None), r, pl.ds(0, 8), pl.ds(128 * (n + 4 * p), 128))
                outa_v[idx] = cc.reshape(NSEG // 2, 8, 128).astype(BF)
                start_out(outa_v.at[idx], out_hbm.at[idx])

        heads = lambda k: jnp.concatenate([wo_v[n + 4 * k, 64 * h:64 * h + 64, :] for h in range(k, H, 2)], axis=0)
        right = lambda m: _bf(heads(m // 6) if m % 6 == 0 else ws_v[n, m - 1])
        _strassen(lambda m: _bf(os_v[m]), right, done, dot=dot)
    for _ in gen:
        pass
    for cp in out_cps:
        cp.wait()


def pallas_concat_heads__memory_aug_recurrent_mem_tr__spectral_gfnet__prompt_kernel(
    A_x, A_mem0, A_Wq, A_Wk, A_Wv, A_Wo, A_seg_len, B_x, B_w_r, B_w_i,
):
    assert A_x.shape == (1, S, DM) and A_Wq.shape == (DM, H, E) and A_mem0.shape == (1, M, DM)
    assert B_x.shape == (1, S, DM) and (not isinstance(A_seg_len, int) or A_seg_len == SEG)
    hbm = pl.BlockSpec(memory_space=pltpu.HBM)
    wr = lambda w: w.reshape(DM // 16, 16, H, E)
    out = pl.pallas_call(
        _kernel,
        out_shape=jax.ShapeDtypeStruct((NSEG // 2, 2, SEG, 2 * DM), BF),
        in_specs=[hbm] * 11,
        out_specs=hbm,
        scratch_shapes=[
            pltpu.VMEM((NSEG, SEG, DM), BF),
            pltpu.VMEM((NSEG, 8, DM), BF),
            pltpu.VMEM((7, NSEG * 2, DM // 2), U32),
            pltpu.VMEM((M, DM), BF),
            pltpu.VMEM((80, 80), F32),
            pltpu.VMEM((NP, 3, DM // 16, 16, E), U32),
            pltpu.VMEM((8, H * E // 2, 128), U32),
            pltpu.VMEM((NP, 3, NSEG // 2, 2, 8, E), U32),
            pltpu.VMEM((7, NSEG * 2, H * E // 2), U32),
            pltpu.VMEM((4, 5, H * E // 4, 128), U32),
            pltpu.VMEM((NSEG // 2, 2, SEG, DM), BF),
            pltpu.VMEM((NSEG // 2, 2, SEG, DM), BF),
            pltpu.VMEM((2, 16, 256, 128), U32),
            pltpu.VMEM((2, 1, S), BF),
            pltpu.VMEM((2, 2, 32 * WP, 128), U32),
            pltpu.VMEM((C_NUM, 64, 128), U32),
            pltpu.VMEM((32, 4, 128, 128), BF),
            pltpu.VMEM((32, 128, 512), F32),
            pltpu.VMEM((64, 128), F32),
            pltpu.VMEM((NSEG // 2, 2, SEG, DM), BF),
            pltpu.SemaphoreType.DMA((NP + 3,)),
            pltpu.SemaphoreType.DMA((2,)),
            pltpu.SemaphoreType.DMA((1,)),
        ],
        compiler_params=pltpu.CompilerParams(vmem_limit_bytes=118 * 1024 * 1024, disable_semaphore_checks=True),
    )(A_x.reshape(NSEG, SEG, DM), A_mem0.reshape(M, DM), wr(A_Wq), wr(A_Wk), wr(A_Wv),
      A_Wo.reshape(H * E, DM), B_x.reshape(NSEG // 2, 2, SEG, DM), B_w_r.T, B_w_i.T, _mask_fill(), _fft_consts())
    return out.reshape(1, S, 2 * DM)
```

```python
import functools
import math

import jax
import jax.numpy as jnp
import numpy as np
from jax import lax
import jax.experimental.pallas as pl
import jax.experimental.pallas.tpu as pltpu

BF, F32, U32, I32 = jnp.bfloat16, jnp.float32, jnp.uint32, jnp.int32

S, DM, H, E, M, SEG = 2048, 1024, 32, 128, 8, 32
NSEG = S // SEG
NP = H // 2
UN = 4
R2 = math.sqrt(0.5)
MID = 'mid'
PAD = 28
HEAD = (0, 1, 2, 3, 5, 8, 13, 19, 24)
LATER = {3: (0, 1), 4: (2,), 5: (3, 4, 5), 6: (6, 7)}


def _to_u32(m):
    u = np.ascontiguousarray(m, dtype=np.float32).view(np.uint32)
    h = ((u + 0x7FFF + ((u >> 16) & 1)) >> 16).astype(np.uint32)
    return h[..., 0::2, :] | (h[..., 1::2, :] << 16)


def _mask_fill():
    r = np.arange(80)
    head = np.where(r < 64, r // 32, (r - 64) // 8)
    pos = np.where(r < 64, np.where(r % 32 < M, r % 32, r % 32 + M), (r - 64) % 8 + M)
    vis = (pos[:, None] < M) | (pos[:, None] >= pos[None, :])
    same = head[:, None] == head[None, :]
    return np.where(same, np.where(vis, 0.0, -1e9), -np.inf).astype(np.float32)


RES = ((0, 12, 8, 4), (1, 15, 9, 7), (2, 14, 10, 6), (3, 13, 11, 5))
WP = 72
C_MD, C_MN, C_TW, C_MS, C_NUM = 0, 16, 22, 24, 88


@functools.lru_cache(maxsize=None)
def _fft_consts():
    md = np.zeros((16, 128, 128))
    for q in range(4):
        if q == 0:
            lay = [[(0, 0), (0, 1), (2, 0), (2, 1)], [(3, 1), (1, 0), (1, 1), (3, 0)]]
        else:
            lay = [[(0, 0), (1, 0), (0, 1), (1, 1)], [(2, 1), (3, 1), (2, 0), (3, 0)]]
        for h in range(2):
            ms_, ws_ = [], []
            for g, part in lay[h]:
                k = 16 * np.arange(32) + RES[q][g]
                th = 2 * np.pi * np.outer(np.arange(128 if q == 0 else 64), k) / DM
                c, s = np.cos(th), np.sin(th)
                if q == 0:
                    ms_.append(-s if part else c)
                else:
                    sg = (1.0 if RES[q][g] % 8 == q else -1.0) * (1.0 - 2.0 * h)
                    ms_.append(np.concatenate([-s, sg * c] if part else [c, sg * s]))
                ws_.append(np.where(k == 0, 1.0, 2.0) / DM)
            m = np.concatenate(ms_, axis=1)
            md[2 * q + h] = m
            md[8 + 2 * q + h] = (m * np.concatenate(ws_)[None, :]).T
    a, l = np.arange(64), np.arange(128)
    re = 16 * (a // 8) + a % 8
    im = re + 8
    ms = np.zeros((64, 128, 128))
    for dl in range(32):
        th = 2 * np.pi * np.outer(32 * a + dl, a) / S
        c, s = np.cos(th), np.sin(th)
        ms[2 * dl][:, re], ms[2 * dl][:, im] = np.concatenate([c, -s]), np.concatenate([s, c])
        ms[2 * dl + 1][:, re] = np.concatenate([c.T, s.T]) / S
        ms[2 * dl + 1][:, im] = np.concatenate([-s.T, c.T]) / S
    mn = np.zeros((6, 128, 128))
    th = 2 * np.pi * np.outer(np.arange(32), l) / 32
    mn[0, :32], mn[1, :32] = np.cos(th), -np.sin(th)
    mn[4, :, :32], mn[5, :, :32] = np.cos(th).T / DM, -np.sin(th).T / DM
    th = 2 * np.pi * np.outer(np.arange(16), a) / 16
    c, s = np.cos(th), np.sin(th)
    mn[2, :32] = np.block([[c, s], [-s, c]])
    mn[3, :, :32] = np.block([[c.T, -s.T], [s.T, c.T]]) / S
    th = 2 * np.pi * np.outer(a, l) / S
    tw = np.stack([np.cos(th), np.sin(th)]).astype(np.float32).view(np.uint32)
    return np.concatenate([_to_u32(md), _to_u32(mn), tw, _to_u32(ms)], axis=0)


def _bdot(a, b):
    return jnp.dot(a, b, preferred_element_type=F32)


def _bf(u):
    return pltpu.bitcast(u, BF)


def _cat(rows):
    return jnp.concatenate(rows, axis=0).astype(BF)


def _unpack2(u, p):
    if p == 0:
        return pltpu.bitcast(u << 16, F32)
    return pltpu.bitcast(u & jnp.uint32(0xFFFF0000), F32)


def _strassen_left(n, a):
    return (lambda: a(1, 0) + a(1, 1), lambda: a(1, 0) - a(0, 0), lambda: a(1, 1), lambda: a(0, 0) + a(1, 1),
            lambda: a(0, 0), lambda: a(0, 1) - a(1, 1), lambda: a(0, 0) + a(0, 1))[n]()


def _strassen_right(n, w):
    add = lambda u, v: (u.astype(F32) + v.astype(F32)).astype(BF)
    sub = lambda u, v: (u.astype(F32) - v.astype(F32)).astype(BF)
    return (lambda: w(0, 0), lambda: add(w(0, 0), w(0, 1)), lambda: sub(w(1, 0), w(0, 0)),
            lambda: add(w(0, 0), w(1, 1)), lambda: sub(w(0, 1), w(1, 1)), lambda: add(w(1, 0), w(1, 1)),
            lambda: w(1, 1))[n]()


def _strassen(left, right, done, ready=lambda k: None, dot=None):
    def mm(n):
        a, r, acc = left(n), right(n), None
        for k in range(0, r.shape[0], 512):
            d = (dot or _bdot)(a[:, k:k + 512], r[k:k + 512])
            acc = d if acc is None else acc + d
        return acc

    ready(0)
    m2 = mm(0)
    c22 = mm(1) - m2
    ready(1)
    m4 = mm(2)
    c21 = m2 + m4
    m1 = mm(3)
    c11, c22 = m1 + m4, c22 + m1
    m3 = mm(4)
    done(1, c21, c22 + m3)
    c11 = c11 + mm(5)
    ready(2)
    m5 = mm(6)
    done(0, c11 - m5, m3 + m5)


def _twiddle(z, k, n, sign):
    r, i = z
    if k == 0:
        return r, i
    if 4 * k == n:
        return (-i, r) if sign > 0 else (i, -r)
    c, s = math.cos(2 * math.pi * k / n), sign * math.sin(2 * math.pi * k / n)
    if 8 * k == n or 8 * k == 3 * n:
        if c * s > 0:
            return (r - i) * c, (r + i) * c
        return (r + i) * c, (i - r) * c
    return r * c - i * s, r * s + i * c


def _cfft(xs, sign):
    n = len(xs)
    if n == 1:
        return xs
    ev, od = _cfft(xs[0::2], sign), _cfft(xs[1::2], sign)
    out = [None] * n
    for k in range(n // 2):
        er, ei = ev[k]
        if 4 * k == n:
            orr, oi = od[k]
            lo, hi = (er - oi, ei + orr), (er + oi, ei - orr)
            out[k], out[k + n // 2] = (lo, hi) if sign > 0 else (hi, lo)
        else:
            tr, ti = _twiddle(od[k], k, n, sign)
            out[k], out[k + n // 2] = (er + tr, ei + ti), (er - tr, ei - ti)
    return out


def _rfft8(x):
    a0, a1, b0, b1 = x[0] + x[4], x[0] - x[4], x[2] + x[6], x[2] - x[6]
    c0, c1, d0, d1 = x[1] + x[5], x[1] - x[5], x[3] + x[7], x[3] - x[7]
    e, f = a0 + b0, c0 + d0
    g, h = (c1 - d1) * R2, (c1 + d1) * R2
    return [e + f, e - f, a1 + g, b1 + h, a0 - b0, c0 - d0, a1 - g, b1 - h]


def _irfft8(z):
    z0, z4, z1r, z1i, z2r, z2i, z3r, z3i = z
    e, f = z0 + z4, z0 - z4
    a1, g = z1r + z3r, (z1r - z3r) * R2
    b1, h = z1i + z3i, (z1i - z3i) * R2
    a0, b0, c0, d0 = e + z2r, e - z2r, f + z2i, f - z2i
    c1, d1 = g + h, h - g
    return [a0 + a1, c0 + c1, b0 + b1, d0 + d1, a0 - a1, c0 - c1, b0 - b1, d0 - d1]


def _kernel(x_hbm, mem0_hbm, wq_hbm, wk_hbm, wv_hbm, wo_hbm, bx_hbm, wr_hbm, wi_hbm, fill_hbm, cst_hbm,
            out_hbm,
            x_v, xpre_v, xs_v, mem0_v, fill_v, wqkv, wo_v, pre, os_v, ws_v, outa_v,
            bx_v, w_v, wn_v, wt, cst, zs, vv, tn, outb_v,
            sem_w, sem_in, sem_out):
    scale = E ** -0.5
    wus = [w.bitcast(U32) for w in (wq_hbm, wk_hbm, wv_hbm)]
    wo_u = wo_hbm.bitcast(U32)
    fus = [w.at[pl.ds(0, 512)].bitcast(U32) for w in (wr_hbm, wi_hbm)]

    def w_copy(j, t, sem):
        return pltpu.make_async_copy(wus[t].at[:, :, j, :], wqkv.at[j, t], sem)

    xpre_cp = pltpu.make_async_copy(x_hbm.at[:, pl.ds(0, 8), :], xpre_v, sem_w.at[17])
    head = [[divmod(f, 3) for f in range(HEAD[b], HEAD[b + 1])] for b in range(len(HEAD) - 1)]
    head_cps = [[w_copy(j, t, sem_w.at[b]) for j, t in grp] for b, grp in enumerate(head) if b > 0]
    first_cps = [pltpu.make_async_copy(wus[0].at[pl.ds(32 * k, 32), :, 0, :], wqkv.at[0, 0, pl.ds(32 * k, 32)],
                                       sem_w.at[18 * k]) for k in range(2)]
    head_cps.insert(0, first_cps)

    def b_rows(i, b):
        return b, i // 4, pl.ds(pl.multiple_of((i % 4) * 8, 8), 8)

    def fwd_cps(i):
        rows = b_rows(i, slice(None))
        sem = sem_w.at[8 + i]
        return ([w_copy(8 + i, t, sem) for t in range(3)]
                + [pltpu.make_async_copy(bx_hbm.at[rows], bx_v.at[rows], sem)]
                + [pltpu.make_async_copy(fus[t].at[:, pl.ds(pl.multiple_of(128 * (2 * i + h), 128), 128)],
                                         w_v.at[t, 2 * i + h], sem) for t in range(2) for h in range(2)])

    def part(src, dst, lo, hi, sem):
        return pltpu.make_async_copy(src.at[pl.ds(lo, hi - lo)], dst.at[pl.ds(lo, hi - lo)], sem)

    c0_cp = part(cst_hbm, cst, 0, C_MS, sem_w.at[16])
    a_cps = [pltpu.make_async_copy(wo_u.at[:, pl.ds(128 * n, 128)], wo_v.at[n], sem_in.at[0]) for n in range(8)]
    a_cps += [part(x_hbm, x_v, 0, UN, sem_in.at[0]), part(cst_hbm, cst, C_MS, C_MS + UN, sem_in.at[0]),
              pltpu.make_async_copy(mem0_hbm, mem0_v, sem_in.at[0]),
              pltpu.make_async_copy(fill_hbm, fill_v, sem_in.at[0])]
    b_cps = [part(x_hbm, x_v, UN, NSEG, sem_in.at[1]), part(cst_hbm, cst, C_MS + UN, C_NUM, sem_in.at[1])]
    b_cps += [pltpu.make_async_copy(w.at[pl.ds(512, 1)], wn_v.at[t], sem_in.at[1])
              for t, w in enumerate((wr_hbm, wi_hbm))]

    lane = lax.broadcasted_iota(I32, (8, 128), 1)
    alt = jnp.where(lane % 2 == 0, 1.0, -1.0).astype(F32)
    lo_half = lane < 64
    ev_grp = (lane // 32) % 2 == 0

    def half_coef(q):
        sg = -1.0 if q < 3 else 1.0
        tc, ts = math.cos(2 * math.pi * q / 16), -math.sin(2 * math.pi * q / 16)
        f = lambda lo, hi: jnp.where(lo_half, lo, hi).astype(F32)
        return f(1.0, ts), f(0.0, sg * tc), f(0.0, tc), f(sg, -sg * ts)

    pace = {'tok': None}

    def token(v):
        return (v if v.dtype == U32 else pltpu.bitcast(v, U32)) & cst[C_MN, 56:64, :]

    def gate(v):
        tok = pace['tok']
        if tok is None:
            return v
        return v | tok if v.dtype == U32 else pltpu.bitcast(pltpu.bitcast(v, U32) | tok, v.dtype)

    def gate2(z):
        return gate(z[0]), gate(z[1])

    def as_u32(rows):
        return pltpu.bitcast(_cat(rows), U32)

    def b_fwd(i):
        r0 = pl.multiple_of(i * 8, 8)
        hc = [None] + [half_coef(q) for q in range(1, 4)]
        tacc = jnp.zeros((8, 128), F32)
        zl = []

        def filt(k):
            e, t, ty = 2 * i + k // 4, (k // 2) % 2, k % 2
            u = jnp.concatenate([gate(w_v[t, e, pl.ds(m + ty + 64 * v, 8, stride=8), :])
                                 for m in (0, 6, 4, 2) for v in range(4)], axis=0)
            ut = pltpu.bitcast(pltpu.bitcast(u, F32).T, U32)
            for v in range(16):
                wt[t, ty, pl.ds(8 * (v % 4) * WP + 4 * e + v // 4, 8, stride=WP), :] = ut[8 * v:8 * v + 8]

        for b0 in range(0, 32, 2):
            rows = []
            for b in (b0, b0 + 1):
                xb = bx_v[(*b_rows(i, b), slice(None))].astype(F32)
                z = _rfft8([gate(xb[:, 128 * t:128 * t + 128]) for t in range(8)])
                tacc = jnp.where(lane == b, jnp.sum(z[0] * alt, axis=1, keepdims=True), tacc)
                for q in range(1, 4):
                    c1, c2, c3, c4 = hc[q]
                    zr, zi = z[2 * q], z[2 * q + 1]
                    pp = c1 * zr + c2 * zi
                    qq = pltpu.roll(c3 * zr + c4 * zi, 64, 1)
                    z[2 * q], z[2 * q + 1] = pp + qq, pp - qq
                rows.append(z)
            zl.append([as_u32([rows[0][n], rows[1][n]]) for n in range(8)])
            yield 200
            if b0 % 4 == 0:
                filt(b0 // 4)
                yield 40
        tn[pl.ds(r0, 8), :] = tacc

        def mm(n):
            return _bdot(_bf(jnp.concatenate([z[n] for z in zl], axis=0)), _bf(cst[C_MD + n]))

        yield MID
        oo = [mm(n) for n in range(4)]
        yield MID
        oo += [mm(n) for n in range(4, 8)]
        yield MID
        for q in range(4):
            sel, sh = (ev_grp, 96) if q == 0 else (lo_half, 64)
            ys = []
            for b0 in range(4):
                xs = []
                for b in range(b0, 32, 4):
                    e_, o_ = gate(oo[2 * q][8 * b:8 * b + 8]), oo[2 * q + 1][8 * b:8 * b + 8]
                    xs.append((jnp.where(sel, e_, o_), pltpu.roll(jnp.where(sel, o_, e_), sh, 1)))
                ys.append([_twiddle(y, b0 * k1, 32, -1) for k1, y in enumerate(_cfft(xs, -1))])
                yield 110
            for k1 in range(8):
                for k0, y in enumerate(_cfft([gate2(ys[b0][k1]) for b0 in range(4)], -1)):
                    zs[k1 + 8 * k0, q, pl.ds(pl.multiple_of(2 * r0, 16), 16), :] = _cat(y)
                yield 30

    def b_mid(it):
        def fwd(dl):
            return _bdot(_bf(cst[C_MS + 2 * dl]), jnp.concatenate([zs[dl, q] for q in range(4)], axis=1))

        def mult(dl, y, rows):
            yield from [None] * 4
            w0 = pl.multiple_of(dl * WP, 8)
            for r in range(8):
                wq = []
                for t in range(2):
                    ta, tb = wt[t, 0, pl.ds(w0 + 8 * r, 8), :], wt[t, 1, pl.ds(w0 + 8 * r, 8), :]
                    wq.append([_unpack2(ta, 0), _unpack2(jnp.where(ev_grp, ta, tb), 1),
                               _unpack2(tb, 0), _unpack2(jnp.where(ev_grp, tb, ta), 1)])
                cols = []
                for q in range(4):
                    yr = gate(y[8 * r:8 * r + 8, 128 * q:128 * q + 128])
                    yi = gate(y[64 + 8 * r:72 + 8 * r, 128 * q:128 * q + 128])
                    wr, wi = wq[0][q], wq[1][q]
                    cols.append(as_u32([yr * wr - yi * wi, yr * wi + yi * wr]))
                rows.append(jnp.concatenate(cols, axis=1))
                yield from [None] * 2

        def inv(dl, rows):
            vv[dl] = _bdot(_bf(cst[C_MS + 2 * dl + 1]), _bf(jnp.concatenate(rows, axis=0)))

        def rights():
            for n in range(4):
                for r in range(0, 64, 8):
                    blk = lambda k, p: _bf(gate(
                        wo_v[n + 4 * p, pl.ds(pl.multiple_of((2 * it + k) * 64 + r, 8), 8), :]))
                    vals = [pltpu.bitcast(_strassen_right(m, blk), U32) for m in range(1, 6)]
                    for m in range(5):
                        ws_v[n, m, pl.ds(pl.multiple_of(it * 64 + r, 8), 8), :] = vals[m]
                    yield vals

        yield from [None] * 2
        for h in range(2):
            rows = []
            y = fwd(2 * it + h)
            yield from mult(2 * it + h, y, rows)
            yield MID
            inv(2 * it + h, rows)
            if h == 0:
                yield from [None] * 4
                yield from rights()
                yield MID

    def b_nyq():
        c, s = pltpu.bitcast(cst[C_TW], F32), pltpu.bitcast(cst[C_TW + 1], F32)
        tb = tn[...].astype(BF)
        tr, ti = _bdot(tb, _bf(cst[C_MN])), _bdot(tb, _bf(cst[C_MN + 1]))
        yield MID
        y = _bdot(_bf(cst[C_MN + 2, 0:16, :]), _cat([tr * c + ti * s, ti * c - tr * s]))
        row = lax.broadcasted_iota(I32, (16, 128), 0)
        wn = []
        for t in range(2):
            wrow = wn_v[t].astype(F32)
            acc = jnp.zeros((16, 128), F32)
            for e in range(16):
                acc = jnp.where(row == e, wrow[:, 128 * e:128 * e + 128], acc)
            wn.append(acc)
        yr, yi = y[0:16], y[16:32]
        yield MID
        v = _bdot(_bf(cst[C_MN + 3, :, 0:32]), _cat([yr * wn[0] - yi * wn[1], yr * wn[1] + yi * wn[0]]))
        vr, vi = v[0:64], v[64:128]
        yield MID
        tn[...] = (_bdot((vr * c - vi * s).astype(BF), _bf(cst[C_MN + 4]))
                   + _bdot((vr * s + vi * c).astype(BF), _bf(cst[C_MN + 5])))

    def b_inv(i, ul):
        r0 = i * 8
        for q in range(4):
            sel, sh = (ev_grp, 32) if q == 0 else (lo_half, 64)
            ys = []
            for b0 in range(4):
                xs = [(gate(vv[dl, pl.ds(r0, 8), 128 * q:128 * q + 128]),
                       gate(vv[dl, pl.ds(64 + r0, 8), 128 * q:128 * q + 128])) for dl in range(b0, 32, 4)]
                ys.append([_twiddle(y, b0 * k1, 32, +1) for k1, y in enumerate(_cfft(xs, +1))])
                yield 110
            ie, io = [], []
            for k1 in range(8):
                es, os_ = [], []
                for ur, ui in _cfft([gate2(ys[b0][k1]) for b0 in range(4)], +1):
                    tmp = pltpu.roll(ui, sh, 1)
                    es.append(jnp.where(sel, ur, tmp))
                    os_.append(jnp.where(sel, tmp, ur))
                ie += [as_u32(es[0:2]), as_u32(es[2:4])]
                io += [as_u32(os_[0:2]), as_u32(os_[2:4])]
                yield 55, ie[-2:] + io[-2:]
            ul += [ie, io]

    def b_fin(i, zz):
        r0 = i * 8
        hc = [None] + [half_coef(q) for q in range(1, 4)]
        tb = tn[pl.ds(r0, 8), :]
        for g in range(32):
            b = g // 4 + 8 * (g % 4)
            z = [gate(zz[n][8 * g:8 * g + 8]) for n in range(8)]
            z[0] = z[0] + jnp.sum(jnp.where(lane == b, tb, 0.0), axis=1, keepdims=True) * alt
            for q in range(1, 4):
                c1, c2, c3, c4 = hc[q]
                pp = z[2 * q] + z[2 * q + 1]
                qq = pltpu.roll(z[2 * q] - z[2 * q + 1], 64, 1)
                z[2 * q], z[2 * q + 1] = c1 * pp + c3 * qq, c2 * pp + c4 * qq
            y = _irfft8(z)
            outb_v[(*b_rows(i, b), slice(None))] = jnp.concatenate(y, axis=1).astype(BF)
            yield 75, y
        rows = b_rows(i, slice(None))
        start_out(outb_v.at[rows], out_hbm.at[(*rows, pl.ds(DM, DM))])

    def tie(w, vals):
        if not vals:
            return w
        acc = None
        for v in vals:
            v = v if v.dtype == U32 else pltpu.bitcast(v, U32)
            acc = v if acc is None else acc | v
        return jnp.concatenate([w[0:8] | token(acc), w[8:]], axis=0)

    def paced_dot(gen, budget):
        st = {'debt': 0, 'k': 0}
        due = {}

        def emit(d, b):
            while st['debt'] < b:
                r = 8 * (32 * st['debt'] // b)
                pace['tok'] = token(d[r:r + 8])
                c = next(gen, MID)
                if c is MID:
                    st['debt'] = b
                elif isinstance(c, list):
                    st['debt'] = 0
                    for own in c:
                        emit(own, 300)
                    return
                else:
                    if isinstance(c, tuple):
                        due.setdefault(st['k'] + 2, []).extend(c[1])
                        c = c[0]
                    st['debt'] += c
            st['debt'] -= b

        def dot(a, w):
            vals = due.pop(st['k'], None)
            if vals:
                a = jnp.concatenate([_bf(tie(pltpu.bitcast(a[:, 0:128], U32), vals)), a[:, 128:]], axis=1)
            d = _bdot(a, w)
            st['k'] += 1
            emit(d, budget)
            return d

        return dot

    out_cps = []

    def start_out(src, dst):
        out_cps.append(pltpu.make_async_copy(src, dst, sem_out.at[0]))
        out_cps[-1].start()

    hb = DM // 32

    def retile(j, t, k):
        blk = pl.ds(k * hb, hb)
        a, b = wqkv[j, t, blk, pl.ds(0, 8, stride=2), :], wqkv[j, t, blk, pl.ds(1, 8, stride=2), :]
        lo, hi = (a & jnp.uint32(0xFFFF)) | (b << 16), (a >> 16) | (b & jnp.uint32(0xFFFF0000))
        wqkv[j, t, blk, 0:8, :] = lo
        wqkv[j, t, blk, 8:16, :] = hi
        return lo

    def strassen_lhs():
        for g in range(NSEG // 4):
            xa = [xpre_v[4 * g + k].astype(F32) for k in range(4)]
            a1, a2 = jnp.concatenate([xa[0], xa[2]], axis=0), jnp.concatenate([xa[1], xa[3]], axis=0)
            a11, a12, a21, a22 = a1[:, :DM // 2], a1[:, DM // 2:], a2[:, :DM // 2], a2[:, DM // 2:]
            for n in range(7):
                v = _strassen_left(n, lambda r, k: ((a11, a12), (a21, a22))[r][k])
                xs_v[n, 8 * g:8 * g + 8, :] = pltpu.bitcast(v.astype(BF), U32)

    def pre_step(j, t, dot=None, sync=None, first=False):
        fresh = {}

        def w(k, p):
            v = fresh.pop((k, p), None)
            if v is None:
                v = wqkv[j, t, k * hb:(k + 1) * hb, 8 * p:8 * p + 8, :]
            return _bf(v.reshape(DM // 4, E))

        def done(h, c1, c2):
            v = jnp.concatenate([c.reshape(NSEG // 2, 8, E) for c in (c1, c2)], axis=1)
            pre[j, t, :, h] = pltpu.bitcast(v.astype(BF), U32)

        def ready(k):
            if k < 2:
                if first:
                    first_cps[k].wait()
                fresh[k, 0] = retile(j, t, k)
            elif sync:
                sync()

        _strassen(lambda n: _bf(xs_v[n]), lambda n: _strassen_right(n, w), done, ready, dot)

    for cp in [xpre_cp] + [cp for grp in head_cps for cp in grp]:
        cp.start()
    vv[0:PAD] = jnp.zeros((PAD,) + vv.shape[1:], F32)
    xpre_cp.wait()
    strassen_lhs()

    def pre_fwd(steps, i, budget):
        gen = b_fwd(i)
        dot = paced_dot(gen, budget)
        for j, t in steps + [(8 + i, t) for t in range(3)]:
            pre_step(j, t, dot)
        for _ in gen:
            pass

    def sync(b):
        for i in LATER.get(b, ()):
            for cp in ([c0_cp] if i == 0 else []) + fwd_cps(i):
                cp.start()
        for cp in head_cps[b + 1] + ([c0_cp] + fwd_cps(0) if b + 2 == len(head) else []):
            cp.wait()

    for b, grp in enumerate(head[:-1]):
        for j, t in grp:
            pre_step(j, t, sync=functools.partial(sync, b) if (j, t) == grp[-1] else None, first=b == 0)
    pre_fwd(head[-1], 0, 130)
    for cp in a_cps + b_cps:
        cp.start()

    def pre_fwd_body(i, carry):
        for cp in fwd_cps(i):
            cp.wait()
        pre_fwd([], i, 340)
        return carry

    lax.fori_loop(1, 8, pre_fwd_body, 0)
    for cp in a_cps:
        cp.wait()

    def seg_step(s, u, mem, slot, opost):
        lhs = _cat([mem, x_v[s][8:32].astype(F32)])
        fill = fill_v[...]
        toks = []
        pace['tok'] = None

        def proj(j, t):
            w0, w1 = [wqkv[j, t, :, 8 * p:8 * p + 8, :].reshape(DM // 2, E) for p in range(2)]
            r0, r1 = _bdot(lhs, _bf(tie(w0, slot()))), _bdot(lhs, _bf(w1))
            toks.append(r0[0:8])
            if len(toks) >= 4:
                pace['tok'] = token(toks[-4])
            return _cat([r0, r1, _bf(pre[j, t, s // 2, u % 2]).astype(F32)])

        def qk(q, k):
            sc = lax.dot_general(q, k, (((1,), (1,)), ((), ())), preferred_element_type=F32) * scale
            sc = jnp.where(fill == 0.0, sc, fill)
            x = sc - jnp.max(sc, axis=-1, keepdims=True)
            e = jnp.exp(jnp.maximum(jnp.concatenate([x[0:32], x[64:72]], axis=0),
                                    jnp.concatenate([x[32:64], x[72:80]], axis=0)))
            col = lax.broadcasted_iota(I32, (40, 80), 1)
            h0 = (col < 32) | ((col >= 64) & (col < 72))
            l0 = jnp.sum(jnp.where(h0, e, 0.0), axis=-1, keepdims=True)
            l1 = jnp.sum(jnp.where(h0, 0.0, e), axis=-1, keepdims=True)
            p = e * pl.reciprocal(jnp.where(h0, l0, l1), approx=True)
            p0, p1 = jnp.where(h0, p, 0.0), jnp.where(h0, 0.0, p)
            return _cat([p0[0:32], p1[0:32], p0[32:40], p1[32:40]])

        ob, ps, vs = {}, {}, {}

        def pv(j):
            o = _bdot(ps[j], vs[j])
            opost[u, j] = (o[64:72], o[72:80])
            if u == UN - 1:
                vals = [as_u32([_strassen_left(n, lambda r, k: opost[2 * g + r, j][k]) for g in range(2)])
                        for n in range(7)]
                for n in range(7):
                    os_v[n, pl.ds(pl.multiple_of(2 * (s - u), 8), 8), 128 * j:128 * j + 128] = vals[n]
            ob[j] = [o[0:32], o[32:64]]

        def wo(g0, g1):
            og = jnp.concatenate([o for j in range(2 * g0, 2 * g1) for o in ob[j]], axis=1).astype(BF)
            return jnp.concatenate([_bdot(og, _bf(wo_v[n, g0 * 256:g1 * 256, :])) for n in range(8)], axis=1)

        ng = NP // 2
        for g in range(ng):
            ja, jb = 2 * g, 2 * g + 1
            qa, ka, qb, kb = proj(ja, 0), proj(ja, 1), proj(jb, 0), proj(jb, 1)
            vs[ja], vs[jb] = proj(ja, 2), proj(jb, 2)
            for j, q, k in ((ja, qa, ka), (jb, qb, kb)):
                ps[j] = qk(q, k)
                if g > 0:
                    pv(j - 2)
        res = wo(0, 4)
        pv(NP - 2)
        pv(NP - 1)
        res = res + wo(4, ng - 1)
        res = res + wo(ng - 1, ng)
        outa_v[s // 2, u % 2, 8:32, :] = res[8:32].astype(BF)
        return res[0:8]

    def loop_body(it, mem):
        @pl.when(it == 1)
        def _():
            for cp in b_cps:
                cp.wait()

        gen = b_mid(it)
        opost = {}
        state = {'mid': False}

        def slot():
            if state['mid']:
                return None
            vals = next(gen, None)
            if vals is MID:
                state['mid'] = True
                return None
            return vals

        for u in range(UN):
            state['mid'] = False
            mem = seg_step(UN * it + u, u, mem, slot, opost)
        for _ in gen:
            pass
        return mem

    lax.fori_loop(0, NSEG // UN, loop_body, mem0_v[...].astype(F32))
    idx = (slice(None), slice(None), pl.ds(8, SEG - 8), pl.ds(0, DM))
    start_out(outa_v.at[idx], out_hbm.at[idx])

    def b_inv_all():
        nyq = b_nyq()
        zz = None
        for i in range(8):
            ul = []
            for k, c in enumerate(b_inv(i, ul)):
                if k % 10 == 0:
                    next(nyq, None)
                yield c
            if i > 0:
                yield from b_fin(i - 1, zz)
            else:
                yield MID
            zz = [_bdot(_bf(jnp.concatenate(ul[n], axis=0)), _bf(cst[C_MD + 8 + n])) for n in range(8)]
            if i < 7:
                yield [zz[3], zz[7]]
        yield MID
        yield MID
        yield from b_fin(7, zz)

    gen = b_inv_all()
    dot = paced_dot(gen, 450)
    for n in range(4):
        def done(r, *cs):
            for p, cc in enumerate(cs):
                idx = (slice(None), r, pl.ds(0, 8), pl.ds(128 * (n + 4 * p), 128))
                outa_v[idx] = cc.reshape(NSEG // 2, 8, 128).astype(BF)
                start_out(outa_v.at[idx], out_hbm.at[idx])

        heads = lambda k: jnp.concatenate([wo_v[n + 4 * k, 64 * h:64 * h + 64, :] for h in range(k, H, 2)], axis=0)
        right = lambda m: _bf(heads(m // 6) if m % 6 == 0 else ws_v[n, m - 1])
        _strassen(lambda m: _bf(os_v[m]), right, done, dot=dot)
    for _ in gen:
        pass
    for cp in out_cps:
        cp.wait()


def pallas_concat_heads__memory_aug_recurrent_mem_tr__spectral_gfnet__prompt_kernel(
    A_x, A_mem0, A_Wq, A_Wk, A_Wv, A_Wo, A_seg_len, B_x, B_w_r, B_w_i,
):
    assert A_x.shape == (1, S, DM) and A_Wq.shape == (DM, H, E) and A_mem0.shape == (1, M, DM)
    assert B_x.shape == (1, S, DM) and (not isinstance(A_seg_len, int) or A_seg_len == SEG)
    hbm = pl.BlockSpec(memory_space=pltpu.HBM)
    wr = lambda w: w.reshape(DM // 16, 16, H, E)
    out = pl.pallas_call(
        _kernel,
        out_shape=jax.ShapeDtypeStruct((NSEG // 2, 2, SEG, 2 * DM), BF),
        in_specs=[hbm] * 11,
        out_specs=hbm,
        scratch_shapes=[
            pltpu.VMEM((NSEG, SEG, DM), BF),
            pltpu.VMEM((NSEG, 8, DM), BF),
            pltpu.VMEM((7, NSEG * 2, DM // 2), U32),
            pltpu.VMEM((M, DM), BF),
            pltpu.VMEM((80, 80), F32),
            pltpu.VMEM((NP, 3, DM // 16, 16, E), U32),
            pltpu.VMEM((8, H * E // 2, 128), U32),
            pltpu.VMEM((NP, 3, NSEG // 2, 2, 8, E), U32),
            pltpu.VMEM((7, NSEG * 2, H * E // 2), U32),
            pltpu.VMEM((4, 5, H * E // 4, 128), U32),
            pltpu.VMEM((NSEG // 2, 2, SEG, DM), BF),
            pltpu.VMEM((NSEG // 2, 2, SEG, DM), BF),
            pltpu.VMEM((2, 16, 256, 128), U32),
            pltpu.VMEM((2, 1, S), BF),
            pltpu.VMEM((2, 2, 32 * WP, 128), U32),
            pltpu.VMEM((C_NUM, 64, 128), U32),
            pltpu.VMEM((32, 4, 128, 128), BF),
            pltpu.VMEM((32, 128, 512), F32),
            pltpu.VMEM((64, 128), F32),
            pltpu.VMEM((NSEG // 2, 2, SEG, DM), BF),
            pltpu.SemaphoreType.DMA((NP + 3,)),
            pltpu.SemaphoreType.DMA((2,)),
            pltpu.SemaphoreType.DMA((1,)),
        ],
        compiler_params=pltpu.CompilerParams(vmem_limit_bytes=118 * 1024 * 1024, disable_semaphore_checks=True),
    )(A_x.reshape(NSEG, SEG, DM), A_mem0.reshape(M, DM), wr(A_Wq), wr(A_Wk), wr(A_Wv),
      A_Wo.reshape(H * E, DM), B_x.reshape(NSEG // 2, 2, SEG, DM), B_w_r.T, B_w_i.T, _mask_fill(), _fft_consts())
    return out.reshape(1, S, 2 * DM)
```

```python
import functools
import math

import jax
import jax.numpy as jnp
import numpy as np
from jax import lax
import jax.experimental.pallas as pl
import jax.experimental.pallas.tpu as pltpu

BF, F32, U32, I32 = jnp.bfloat16, jnp.float32, jnp.uint32, jnp.int32

S, DM, H, E, M, SEG = 2048, 1024, 32, 128, 8, 32
NSEG = S // SEG
NP = H // 2
UN = 4
R2 = math.sqrt(0.5)
MID = 'mid'
PAD = 28
HEAD = (0, 1, 2, 3, 5, 8, 13, 19, 24)
LATER = {3: (0, 1), 4: (2,), 5: (3, 4, 5), 6: (6, 7)}


def _to_u32(m):
    u = np.ascontiguousarray(m, dtype=np.float32).view(np.uint32)
    h = ((u + 0x7FFF + ((u >> 16) & 1)) >> 16).astype(np.uint32)
    return h[..., 0::2, :] | (h[..., 1::2, :] << 16)


def _mask_fill():
    r = np.arange(80)
    pos = np.where(r < 64, np.where(r % 32 < M, r % 32, r % 32 + M), (r - 64) % 8 + M)
    kpos = np.concatenate([pos[0:32], pos[64:72]])
    vis = (pos[None, :] < M) | (pos[None, :] >= kpos[:, None])
    return np.where(vis, 0.0, -1e9).astype(np.float32)


RES = ((0, 12, 8, 4), (1, 15, 9, 7), (2, 14, 10, 6), (3, 13, 11, 5))
WP = 72
C_MD, C_MN, C_TW, C_MS, C_NUM = 0, 16, 22, 24, 88


@functools.lru_cache(maxsize=None)
def _fft_consts():
    md = np.zeros((16, 128, 128))
    for q in range(4):
        if q == 0:
            lay = [[(0, 0), (0, 1), (2, 0), (2, 1)], [(3, 1), (1, 0), (1, 1), (3, 0)]]
        else:
            lay = [[(0, 0), (1, 0), (0, 1), (1, 1)], [(2, 1), (3, 1), (2, 0), (3, 0)]]
        for h in range(2):
            ms_, ws_ = [], []
            for g, part in lay[h]:
                k = 16 * np.arange(32) + RES[q][g]
                th = 2 * np.pi * np.outer(np.arange(128 if q == 0 else 64), k) / DM
                c, s = np.cos(th), np.sin(th)
                if q == 0:
                    ms_.append(-s if part else c)
                else:
                    sg = (1.0 if RES[q][g] % 8 == q else -1.0) * (1.0 - 2.0 * h)
                    ms_.append(np.concatenate([-s, sg * c] if part else [c, sg * s]))
                ws_.append(np.where(k == 0, 1.0, 2.0) / DM)
            m = np.concatenate(ms_, axis=1)
            md[2 * q + h] = m
            md[8 + 2 * q + h] = (m * np.concatenate(ws_)[None, :]).T
    a, l = np.arange(64), np.arange(128)
    re = 16 * (a // 8) + a % 8
    im = re + 8
    ms = np.zeros((64, 128, 128))
    for dl in range(32):
        th = 2 * np.pi * np.outer(32 * a + dl, a) / S
        c, s = np.cos(th), np.sin(th)
        ms[2 * dl][:, re], ms[2 * dl][:, im] = np.concatenate([c, -s]), np.concatenate([s, c])
        ms[2 * dl + 1][:, re] = np.concatenate([c.T, s.T]) / S
        ms[2 * dl + 1][:, im] = np.concatenate([-s.T, c.T]) / S
    mn = np.zeros((6, 128, 128))
    th = 2 * np.pi * np.outer(np.arange(32), l) / 32
    mn[0, :32], mn[1, :32] = np.cos(th), -np.sin(th)
    mn[4, :, :32], mn[5, :, :32] = np.cos(th).T / DM, -np.sin(th).T / DM
    th = 2 * np.pi * np.outer(np.arange(16), a) / 16
    c, s = np.cos(th), np.sin(th)
    mn[2, :32] = np.block([[c, s], [-s, c]])
    mn[3, :, :32] = np.block([[c.T, -s.T], [s.T, c.T]]) / S
    th = 2 * np.pi * np.outer(a, l) / S
    tw = np.stack([np.cos(th), np.sin(th)]).astype(np.float32).view(np.uint32)
    return np.concatenate([_to_u32(md), _to_u32(mn), tw, _to_u32(ms)], axis=0)


def _bdot(a, b):
    return jnp.dot(a, b, preferred_element_type=F32)


def _bf(u):
    return pltpu.bitcast(u, BF)


def _cat(rows):
    return jnp.concatenate(rows, axis=0).astype(BF)


def _unpack2(u, p):
    if p == 0:
        return pltpu.bitcast(u << 16, F32)
    return pltpu.bitcast(u & jnp.uint32(0xFFFF0000), F32)


def _strassen_left(n, a):
    return (lambda: a(1, 0) + a(1, 1), lambda: a(1, 0) - a(0, 0), lambda: a(1, 1), lambda: a(0, 0) + a(1, 1),
            lambda: a(0, 0), lambda: a(0, 1) - a(1, 1), lambda: a(0, 0) + a(0, 1))[n]()


def _strassen_right(n, w):
    add = lambda u, v: (u.astype(F32) + v.astype(F32)).astype(BF)
    sub = lambda u, v: (u.astype(F32) - v.astype(F32)).astype(BF)
    return (lambda: w(0, 0), lambda: add(w(0, 0), w(0, 1)), lambda: sub(w(1, 0), w(0, 0)),
            lambda: add(w(0, 0), w(1, 1)), lambda: sub(w(0, 1), w(1, 1)), lambda: add(w(1, 0), w(1, 1)),
            lambda: w(1, 1))[n]()


def _strassen(left, right, done, ready=lambda k: None, dot=None):
    def mm(n):
        a, r, acc = left(n), right(n), None
        for k in range(0, r.shape[0], 512):
            d = (dot or _bdot)(a[:, k:k + 512], r[k:k + 512])
            acc = d if acc is None else acc + d
        return acc

    ready(0)
    m2 = mm(0)
    c22 = mm(1) - m2
    ready(1)
    m4 = mm(2)
    c21 = m2 + m4
    m1 = mm(3)
    c11, c22 = m1 + m4, c22 + m1
    m3 = mm(4)
    done(1, c21, c22 + m3)
    c11 = c11 + mm(5)
    ready(2)
    m5 = mm(6)
    done(0, c11 - m5, m3 + m5)


def _twiddle(z, k, n, sign):
    r, i = z
    if k == 0:
        return r, i
    if 4 * k == n:
        return (-i, r) if sign > 0 else (i, -r)
    c, s = math.cos(2 * math.pi * k / n), sign * math.sin(2 * math.pi * k / n)
    if 8 * k == n or 8 * k == 3 * n:
        if c * s > 0:
            return (r - i) * c, (r + i) * c
        return (r + i) * c, (i - r) * c
    return r * c - i * s, r * s + i * c


def _cfft(xs, sign):
    n = len(xs)
    if n == 1:
        return xs
    ev, od = _cfft(xs[0::2], sign), _cfft(xs[1::2], sign)
    out = [None] * n
    for k in range(n // 2):
        er, ei = ev[k]
        if 4 * k == n:
            orr, oi = od[k]
            lo, hi = (er - oi, ei + orr), (er + oi, ei - orr)
            out[k], out[k + n // 2] = (lo, hi) if sign > 0 else (hi, lo)
        else:
            tr, ti = _twiddle(od[k], k, n, sign)
            out[k], out[k + n // 2] = (er + tr, ei + ti), (er - tr, ei - ti)
    return out


def _rfft8(x):
    a0, a1, b0, b1 = x[0] + x[4], x[0] - x[4], x[2] + x[6], x[2] - x[6]
    c0, c1, d0, d1 = x[1] + x[5], x[1] - x[5], x[3] + x[7], x[3] - x[7]
    e, f = a0 + b0, c0 + d0
    g, h = (c1 - d1) * R2, (c1 + d1) * R2
    return [e + f, e - f, a1 + g, b1 + h, a0 - b0, c0 - d0, a1 - g, b1 - h]


def _irfft8(z):
    z0, z4, z1r, z1i, z2r, z2i, z3r, z3i = z
    e, f = z0 + z4, z0 - z4
    a1, g = z1r + z3r, (z1r - z3r) * R2
    b1, h = z1i + z3i, (z1i - z3i) * R2
    a0, b0, c0, d0 = e + z2r, e - z2r, f + z2i, f - z2i
    c1, d1 = g + h, h - g
    return [a0 + a1, c0 + c1, b0 + b1, d0 + d1, a0 - a1, c0 - c1, b0 - b1, d0 - d1]


def _kernel(x_hbm, mem0_hbm, wq_hbm, wk_hbm, wv_hbm, wo_hbm, bx_hbm, wr_hbm, wi_hbm, fill_hbm, cst_hbm,
            out_hbm,
            x_v, xpre_v, xs_v, mem0_v, fill_v, wqkv, wo_v, pre, os_v, ws_v, outa_v,
            bx_v, w_v, wn_v, wt, cst, zs, vv, tn, outb_v,
            sem_w, sem_in, sem_out):
    scale = E ** -0.5
    wus = [w.bitcast(U32) for w in (wq_hbm, wk_hbm, wv_hbm)]
    wo_u = wo_hbm.bitcast(U32)
    fus = [w.at[pl.ds(0, 512)].bitcast(U32) for w in (wr_hbm, wi_hbm)]

    def w_copy(j, t, sem):
        return pltpu.make_async_copy(wus[t].at[:, :, j, :], wqkv.at[j, t], sem)

    xpre_cp = pltpu.make_async_copy(x_hbm.at[:, pl.ds(0, 8), :], xpre_v, sem_w.at[17])
    head = [[divmod(f, 3) for f in range(HEAD[b], HEAD[b + 1])] for b in range(len(HEAD) - 1)]
    head_cps = [[w_copy(j, t, sem_w.at[b]) for j, t in grp] for b, grp in enumerate(head) if b > 0]
    first_cps = [pltpu.make_async_copy(wus[0].at[pl.ds(32 * k, 32), :, 0, :], wqkv.at[0, 0, pl.ds(32 * k, 32)],
                                       sem_w.at[18 * k]) for k in range(2)]
    head_cps.insert(0, first_cps)

    def b_rows(i, b):
        return b, i // 4, pl.ds(pl.multiple_of((i % 4) * 8, 8), 8)

    def fwd_cps(i):
        rows = b_rows(i, slice(None))
        sem = sem_w.at[8 + i]
        return ([w_copy(8 + i, t, sem) for t in range(3)]
                + [pltpu.make_async_copy(bx_hbm.at[rows], bx_v.at[rows], sem)]
                + [pltpu.make_async_copy(fus[t].at[:, pl.ds(pl.multiple_of(128 * (2 * i + h), 128), 128)],
                                         w_v.at[t, 2 * i + h], sem) for t in range(2) for h in range(2)])

    def part(src, dst, lo, hi, sem):
        return pltpu.make_async_copy(src.at[pl.ds(lo, hi - lo)], dst.at[pl.ds(lo, hi - lo)], sem)

    c0_cp = part(cst_hbm, cst, 0, C_MS, sem_w.at[16])
    a_cps = [pltpu.make_async_copy(wo_u.at[:, pl.ds(128 * n, 128)], wo_v.at[n], sem_in.at[0]) for n in range(8)]
    a_cps += [part(x_hbm, x_v, 0, UN, sem_in.at[0]), part(cst_hbm, cst, C_MS, C_MS + UN, sem_in.at[0]),
              pltpu.make_async_copy(mem0_hbm, mem0_v, sem_in.at[0]),
              pltpu.make_async_copy(fill_hbm, fill_v, sem_in.at[0])]
    b_cps = [part(x_hbm, x_v, UN, NSEG, sem_in.at[1]), part(cst_hbm, cst, C_MS + UN, C_NUM, sem_in.at[1])]
    b_cps += [pltpu.make_async_copy(w.at[pl.ds(512, 1)], wn_v.at[t], sem_in.at[1])
              for t, w in enumerate((wr_hbm, wi_hbm))]

    lane = lax.broadcasted_iota(I32, (8, 128), 1)
    alt = jnp.where(lane % 2 == 0, 1.0, -1.0).astype(F32)
    lo_half = lane < 64
    ev_grp = (lane // 32) % 2 == 0

    def half_coef(q):
        sg = -1.0 if q < 3 else 1.0
        tc, ts = math.cos(2 * math.pi * q / 16), -math.sin(2 * math.pi * q / 16)
        f = lambda lo, hi: jnp.where(lo_half, lo, hi).astype(F32)
        return f(1.0, ts), f(0.0, sg * tc), f(0.0, tc), f(sg, -sg * ts)

    pace = {'tok': None}

    def token(v):
        return (v if v.dtype == U32 else pltpu.bitcast(v, U32)) & cst[C_MN, 56:64, :]

    def gate(v):
        tok = pace['tok']
        if tok is None:
            return v
        return v | tok if v.dtype == U32 else pltpu.bitcast(pltpu.bitcast(v, U32) | tok, v.dtype)

    def gate2(z):
        return gate(z[0]), gate(z[1])

    def as_u32(rows):
        return pltpu.bitcast(_cat(rows), U32)

    def b_fwd(i):
        r0 = pl.multiple_of(i * 8, 8)
        hc = [None] + [half_coef(q) for q in range(1, 4)]
        tacc = jnp.zeros((8, 128), F32)
        zl = []

        def filt(k):
            e, t, ty = 2 * i + k // 4, (k // 2) % 2, k % 2
            u = jnp.concatenate([gate(w_v[t, e, pl.ds(m + ty + 64 * v, 8, stride=8), :])
                                 for m in (0, 6, 4, 2) for v in range(4)], axis=0)
            ut = pltpu.bitcast(pltpu.bitcast(u, F32).T, U32)
            for v in range(16):
                wt[t, ty, pl.ds(8 * (v % 4) * WP + 4 * e + v // 4, 8, stride=WP), :] = ut[8 * v:8 * v + 8]

        for b0 in range(0, 32, 2):
            rows = []
            for b in (b0, b0 + 1):
                xb = bx_v[(*b_rows(i, b), slice(None))].astype(F32)
                z = _rfft8([gate(xb[:, 128 * t:128 * t + 128]) for t in range(8)])
                tacc = jnp.where(lane == b, jnp.sum(z[0] * alt, axis=1, keepdims=True), tacc)
                for q in range(1, 4):
                    c1, c2, c3, c4 = hc[q]
                    zr, zi = z[2 * q], z[2 * q + 1]
                    pp = c1 * zr + c2 * zi
                    qq = pltpu.roll(c3 * zr + c4 * zi, 64, 1)
                    z[2 * q], z[2 * q + 1] = pp + qq, pp - qq
                rows.append(z)
            zl.append([as_u32([rows[0][n], rows[1][n]]) for n in range(8)])
            yield 200
            if b0 % 4 == 0:
                filt(b0 // 4)
                yield 40
        tn[pl.ds(r0, 8), :] = tacc

        def mm(n):
            return _bdot(_bf(jnp.concatenate([z[n] for z in zl], axis=0)), _bf(cst[C_MD + n]))

        yield MID
        oo = [mm(n) for n in range(4)]
        yield MID
        oo += [mm(n) for n in range(4, 8)]
        yield MID
        for q in range(4):
            sel, sh = (ev_grp, 96) if q == 0 else (lo_half, 64)
            ys = []
            for b0 in range(4):
                xs = []
                for b in range(b0, 32, 4):
                    e_, o_ = gate(oo[2 * q][8 * b:8 * b + 8]), oo[2 * q + 1][8 * b:8 * b + 8]
                    xs.append((jnp.where(sel, e_, o_), pltpu.roll(jnp.where(sel, o_, e_), sh, 1)))
                ys.append([_twiddle(y, b0 * k1, 32, -1) for k1, y in enumerate(_cfft(xs, -1))])
                yield 110
            for k1 in range(8):
                for k0, y in enumerate(_cfft([gate2(ys[b0][k1]) for b0 in range(4)], -1)):
                    zs[k1 + 8 * k0, q, pl.ds(pl.multiple_of(2 * r0, 16), 16), :] = _cat(y)
                yield 30

    def b_mid(it):
        def fwd(dl):
            return _bdot(_bf(cst[C_MS + 2 * dl]), jnp.concatenate([zs[dl, q] for q in range(4)], axis=1))

        def mult(dl, y, rows):
            yield from [None] * 4
            w0 = pl.multiple_of(dl * WP, 8)
            for r in range(8):
                wq = []
                for t in range(2):
                    ta, tb = wt[t, 0, pl.ds(w0 + 8 * r, 8), :], wt[t, 1, pl.ds(w0 + 8 * r, 8), :]
                    wq.append([_unpack2(ta, 0), _unpack2(jnp.where(ev_grp, ta, tb), 1),
                               _unpack2(tb, 0), _unpack2(jnp.where(ev_grp, tb, ta), 1)])
                cols = []
                for q in range(4):
                    yr = gate(y[8 * r:8 * r + 8, 128 * q:128 * q + 128])
                    yi = gate(y[64 + 8 * r:72 + 8 * r, 128 * q:128 * q + 128])
                    wr, wi = wq[0][q], wq[1][q]
                    cols.append(as_u32([yr * wr - yi * wi, yr * wi + yi * wr]))
                rows.append(jnp.concatenate(cols, axis=1))
                yield from [None] * 2

        def inv(dl, rows):
            vv[dl] = _bdot(_bf(cst[C_MS + 2 * dl + 1]), _bf(jnp.concatenate(rows, axis=0)))

        def rights():
            for n in range(4):
                for r in range(0, 64, 8):
                    blk = lambda k, p: _bf(gate(
                        wo_v[n + 4 * p, pl.ds(pl.multiple_of((2 * it + k) * 64 + r, 8), 8), :]))
                    vals = [pltpu.bitcast(_strassen_right(m, blk), U32) for m in range(1, 6)]
                    for m in range(5):
                        ws_v[n, m, pl.ds(pl.multiple_of(it * 64 + r, 8), 8), :] = vals[m]
                    yield vals

        yield from [None] * 2
        for h in range(2):
            rows = []
            y = fwd(2 * it + h)
            yield from mult(2 * it + h, y, rows)
            yield MID
            inv(2 * it + h, rows)
            if h == 0:
                yield from [None] * 4
                yield from rights()
                yield MID

    def b_nyq():
        c, s = pltpu.bitcast(cst[C_TW], F32), pltpu.bitcast(cst[C_TW + 1], F32)
        tb = tn[...].astype(BF)
        tr, ti = _bdot(tb, _bf(cst[C_MN])), _bdot(tb, _bf(cst[C_MN + 1]))
        yield MID
        y = _bdot(_bf(cst[C_MN + 2, 0:16, :]), _cat([tr * c + ti * s, ti * c - tr * s]))
        row = lax.broadcasted_iota(I32, (16, 128), 0)
        wn = []
        for t in range(2):
            wrow = wn_v[t].astype(F32)
            acc = jnp.zeros((16, 128), F32)
            for e in range(16):
                acc = jnp.where(row == e, wrow[:, 128 * e:128 * e + 128], acc)
            wn.append(acc)
        yr, yi = y[0:16], y[16:32]
        yield MID
        v = _bdot(_bf(cst[C_MN + 3, :, 0:32]), _cat([yr * wn[0] - yi * wn[1], yr * wn[1] + yi * wn[0]]))
        vr, vi = v[0:64], v[64:128]
        yield MID
        tn[...] = (_bdot((vr * c - vi * s).astype(BF), _bf(cst[C_MN + 4]))
                   + _bdot((vr * s + vi * c).astype(BF), _bf(cst[C_MN + 5])))

    def b_inv(i, ul):
        r0 = i * 8
        for q in range(4):
            sel, sh = (ev_grp, 32) if q == 0 else (lo_half, 64)
            ys = []
            for b0 in range(4):
                xs = [(gate(vv[dl, pl.ds(r0, 8), 128 * q:128 * q + 128]),
                       gate(vv[dl, pl.ds(64 + r0, 8), 128 * q:128 * q + 128])) for dl in range(b0, 32, 4)]
                ys.append([_twiddle(y, b0 * k1, 32, +1) for k1, y in enumerate(_cfft(xs, +1))])
                yield 110
            ie, io = [], []
            for k1 in range(8):
                es, os_ = [], []
                for ur, ui in _cfft([gate2(ys[b0][k1]) for b0 in range(4)], +1):
                    tmp = pltpu.roll(ui, sh, 1)
                    es.append(jnp.where(sel, ur, tmp))
                    os_.append(jnp.where(sel, tmp, ur))
                ie += [as_u32(es[0:2]), as_u32(es[2:4])]
                io += [as_u32(os_[0:2]), as_u32(os_[2:4])]
                yield 55, ie[-2:] + io[-2:]
            ul += [ie, io]

    def b_fin(i, zz):
        r0 = i * 8
        hc = [None] + [half_coef(q) for q in range(1, 4)]
        tb = tn[pl.ds(r0, 8), :]
        for g in range(32):
            b = g // 4 + 8 * (g % 4)
            z = [gate(zz[n][8 * g:8 * g + 8]) for n in range(8)]
            z[0] = z[0] + jnp.sum(jnp.where(lane == b, tb, 0.0), axis=1, keepdims=True) * alt
            for q in range(1, 4):
                c1, c2, c3, c4 = hc[q]
                pp = z[2 * q] + z[2 * q + 1]
                qq = pltpu.roll(z[2 * q] - z[2 * q + 1], 64, 1)
                z[2 * q], z[2 * q + 1] = c1 * pp + c3 * qq, c2 * pp + c4 * qq
            y = _irfft8(z)
            outb_v[(*b_rows(i, b), slice(None))] = jnp.concatenate(y, axis=1).astype(BF)
            yield 75, y
        rows = b_rows(i, slice(None))
        start_out(outb_v.at[rows], out_hbm.at[(*rows, pl.ds(DM, DM))])

    def tie(w, vals):
        if not vals:
            return w
        acc = None
        for v in vals:
            v = v if v.dtype == U32 else pltpu.bitcast(v, U32)
            acc = v if acc is None else acc | v
        return jnp.concatenate([w[0:8] | token(acc), w[8:]], axis=0)

    def paced_dot(gen, budget):
        st = {'debt': 0, 'k': 0}
        due = {}

        def emit(d, b):
            while st['debt'] < b:
                r = 8 * (32 * st['debt'] // b)
                pace['tok'] = token(d[r:r + 8])
                c = next(gen, MID)
                if c is MID:
                    st['debt'] = b
                elif isinstance(c, list):
                    st['debt'] = 0
                    for own in c:
                        emit(own, 300)
                    return
                else:
                    if isinstance(c, tuple):
                        due.setdefault(st['k'] + 2, []).extend(c[1])
                        c = c[0]
                    st['debt'] += c
            st['debt'] -= b

        def dot(a, w):
            vals = due.pop(st['k'], None)
            if vals:
                a = jnp.concatenate([_bf(tie(pltpu.bitcast(a[:, 0:128], U32), vals)), a[:, 128:]], axis=1)
            d = _bdot(a, w)
            st['k'] += 1
            emit(d, budget)
            return d

        return dot

    out_cps = []

    def start_out(src, dst):
        out_cps.append(pltpu.make_async_copy(src, dst, sem_out.at[0]))
        out_cps[-1].start()

    hb = DM // 32

    def retile(j, t, k):
        blk = pl.ds(k * hb, hb)
        a, b = wqkv[j, t, blk, pl.ds(0, 8, stride=2), :], wqkv[j, t, blk, pl.ds(1, 8, stride=2), :]
        lo, hi = (a & jnp.uint32(0xFFFF)) | (b << 16), (a >> 16) | (b & jnp.uint32(0xFFFF0000))
        wqkv[j, t, blk, 0:8, :] = lo
        wqkv[j, t, blk, 8:16, :] = hi
        return lo

    def strassen_lhs():
        for g in range(NSEG // 4):
            xa = [xpre_v[4 * g + k].astype(F32) for k in range(4)]
            a1, a2 = jnp.concatenate([xa[0], xa[2]], axis=0), jnp.concatenate([xa[1], xa[3]], axis=0)
            a11, a12, a21, a22 = a1[:, :DM // 2], a1[:, DM // 2:], a2[:, :DM // 2], a2[:, DM // 2:]
            for n in range(7):
                v = _strassen_left(n, lambda r, k: ((a11, a12), (a21, a22))[r][k])
                xs_v[n, 8 * g:8 * g + 8, :] = pltpu.bitcast(v.astype(BF), U32)

    def pre_step(j, t, dot=None, sync=None, first=False):
        fresh = {}

        def w(k, p):
            v = fresh.pop((k, p), None)
            if v is None:
                v = wqkv[j, t, k * hb:(k + 1) * hb, 8 * p:8 * p + 8, :]
            return _bf(v.reshape(DM // 4, E))

        def done(h, c1, c2):
            v = jnp.concatenate([c.reshape(NSEG // 2, 8, E) for c in (c1, c2)], axis=1)
            pre[j, t, :, h] = pltpu.bitcast(v.astype(BF), U32)

        def ready(k):
            if k < 2:
                if first:
                    first_cps[k].wait()
                fresh[k, 0] = retile(j, t, k)
            elif sync:
                sync()

        _strassen(lambda n: _bf(xs_v[n]), lambda n: _strassen_right(n, w), done, ready, dot)

    for cp in [xpre_cp] + [cp for grp in head_cps for cp in grp]:
        cp.start()
    vv[0:PAD] = jnp.zeros((PAD,) + vv.shape[1:], F32)
    xpre_cp.wait()
    strassen_lhs()

    def pre_fwd(steps, i, budget):
        gen = b_fwd(i)
        dot = paced_dot(gen, budget)
        for j, t in steps + [(8 + i, t) for t in range(3)]:
            pre_step(j, t, dot)
        for _ in gen:
            pass

    def sync(b):
        for i in LATER.get(b, ()):
            for cp in ([c0_cp] if i == 0 else []) + fwd_cps(i):
                cp.start()
        for cp in head_cps[b + 1] + ([c0_cp] + fwd_cps(0) if b + 2 == len(head) else []):
            cp.wait()

    for b, grp in enumerate(head[:-1]):
        for j, t in grp:
            pre_step(j, t, sync=functools.partial(sync, b) if (j, t) == grp[-1] else None, first=b == 0)
    pre_fwd(head[-1], 0, 130)
    for cp in a_cps + b_cps:
        cp.start()

    def pre_fwd_body(i, carry):
        for cp in fwd_cps(i):
            cp.wait()
        pre_fwd([], i, 340)
        return carry

    lax.fori_loop(1, 8, pre_fwd_body, 0)
    for cp in a_cps:
        cp.wait()

    def seg_step(s, u, mem, slot, opost):
        lhs = _cat([mem, x_v[s][8:32].astype(F32)])
        fill = fill_v[...]
        toks = []
        pace['tok'] = None

        def proj(j, t):
            w0, w1 = [wqkv[j, t, :, 8 * p:8 * p + 8, :].reshape(DM // 2, E) for p in range(2)]
            r0, r1 = _bdot(lhs, _bf(tie(w0, slot()))), _bdot(lhs, _bf(w1))
            toks.append(r0[0:8])
            if len(toks) >= 4:
                pace['tok'] = token(toks[-4])
            return _cat([r0, r1, _bf(pre[j, t, s // 2, u % 2]).astype(F32)])

        def qk(q, k):
            sc = lax.dot_general(k, q, (((1,), (1,)), ((), ())), preferred_element_type=F32)
            col = lax.broadcasted_iota(I32, (40, 80), 1)
            h0 = (col < 32) | ((col >= 64) & (col < 72))
            sc = jnp.where(h0, jnp.concatenate([sc[0:32], sc[64:72]], axis=0),
                           jnp.concatenate([sc[32:64], sc[72:80]], axis=0)) * scale
            sc = jnp.where(fill == 0.0, sc, fill)
            e = jnp.exp(sc - jnp.max(sc, axis=0, keepdims=True))
            p = e * (1.0 / jnp.sum(e, axis=0, keepdims=True))
            p0, p1 = jnp.where(h0, p, 0.0), jnp.where(h0, 0.0, p)
            return jnp.concatenate([p0[0:32], p1[0:32], p0[32:40], p1[32:40]], axis=0).T.astype(BF)

        ob, ps, vs = {}, {}, {}

        def pv(j):
            o = _bdot(ps[j], vs[j])
            opost[u, j] = (o[64:72], o[72:80])
            if u == UN - 1:
                vals = [as_u32([_strassen_left(n, lambda r, k: opost[2 * g + r, j][k]) for g in range(2)])
                        for n in range(7)]
                for n in range(7):
                    os_v[n, pl.ds(pl.multiple_of(2 * (s - u), 8), 8), 128 * j:128 * j + 128] = vals[n]
            ob[j] = [o[0:32], o[32:64]]

        def wo(g0, g1):
            og = jnp.concatenate([o for j in range(2 * g0, 2 * g1) for o in ob[j]], axis=1).astype(BF)
            return jnp.concatenate([_bdot(og, _bf(wo_v[n, g0 * 256:g1 * 256, :])) for n in range(8)], axis=1)

        ng = NP // 2
        for g in range(ng):
            ja, jb = 2 * g, 2 * g + 1
            qa, ka, qb, kb = proj(ja, 0), proj(ja, 1), proj(jb, 0), proj(jb, 1)
            vs[ja], vs[jb] = proj(ja, 2), proj(jb, 2)
            for j, q, k in ((ja, qa, ka), (jb, qb, kb)):
                ps[j] = qk(q, k)
                if g > 0:
                    pv(j - 2)
        res = wo(0, 2)
        pv(NP - 2)
        pv(NP - 1)
        res = res + wo(2, ng - 1)
        res = res + wo(ng - 1, ng)
        outa_v[s // 2, u % 2, 8:32, :] = res[8:32].astype(BF)
        return res[0:8]

    def loop_body(it, mem):
        @pl.when(it == 1)
        def _():
            for cp in b_cps:
                cp.wait()

        gen = b_mid(it)
        opost = {}
        state = {'mid': False}

        def slot():
            if state['mid']:
                return None
            vals = next(gen, None)
            if vals is MID:
                state['mid'] = True
                return None
            return vals

        for u in range(UN):
            state['mid'] = False
            mem = seg_step(UN * it + u, u, mem, slot, opost)
        for _ in gen:
            pass
        return mem

    lax.fori_loop(0, NSEG // UN, loop_body, mem0_v[...].astype(F32))
    idx = (slice(None), slice(None), pl.ds(8, SEG - 8), pl.ds(0, DM))
    start_out(outa_v.at[idx], out_hbm.at[idx])

    def b_inv_all():
        nyq = b_nyq()
        zz = None
        for i in range(8):
            ul = []
            for k, c in enumerate(b_inv(i, ul)):
                if k % 10 == 0:
                    next(nyq, None)
                yield c
            if i > 0:
                yield from b_fin(i - 1, zz)
            else:
                yield MID
            zz = [_bdot(_bf(jnp.concatenate(ul[n], axis=0)), _bf(cst[C_MD + 8 + n])) for n in range(8)]
            if i < 7:
                yield [zz[3], zz[7]]
        yield MID
        yield MID
        yield from b_fin(7, zz)

    gen = b_inv_all()
    dot = paced_dot(gen, 450)
    for n in range(4):
        def done(r, *cs):
            for p, cc in enumerate(cs):
                idx = (slice(None), r, pl.ds(0, 8), pl.ds(128 * (n + 4 * p), 128))
                outa_v[idx] = cc.reshape(NSEG // 2, 8, 128).astype(BF)
                start_out(outa_v.at[idx], out_hbm.at[idx])

        heads = lambda k: jnp.concatenate([wo_v[n + 4 * k, 64 * h:64 * h + 64, :] for h in range(k, H, 2)], axis=0)
        right = lambda m: _bf(heads(m // 6) if m % 6 == 0 else ws_v[n, m - 1])
        _strassen(lambda m: _bf(os_v[m]), right, done, dot=dot)
    for _ in gen:
        pass
    for cp in out_cps:
        cp.wait()


def pallas_concat_heads__memory_aug_recurrent_mem_tr__spectral_gfnet__prompt_kernel(
    A_x, A_mem0, A_Wq, A_Wk, A_Wv, A_Wo, A_seg_len, B_x, B_w_r, B_w_i,
):
    assert A_x.shape == (1, S, DM) and A_Wq.shape == (DM, H, E) and A_mem0.shape == (1, M, DM)
    assert B_x.shape == (1, S, DM) and (not isinstance(A_seg_len, int) or A_seg_len == SEG)
    hbm = pl.BlockSpec(memory_space=pltpu.HBM)
    wr = lambda w: w.reshape(DM // 16, 16, H, E)
    out = pl.pallas_call(
        _kernel,
        out_shape=jax.ShapeDtypeStruct((NSEG // 2, 2, SEG, 2 * DM), BF),
        in_specs=[hbm] * 11,
        out_specs=hbm,
        scratch_shapes=[
            pltpu.VMEM((NSEG, SEG, DM), BF),
            pltpu.VMEM((NSEG, 8, DM), BF),
            pltpu.VMEM((7, NSEG * 2, DM // 2), U32),
            pltpu.VMEM((M, DM), BF),
            pltpu.VMEM((40, 80), F32),
            pltpu.VMEM((NP, 3, DM // 16, 16, E), U32),
            pltpu.VMEM((8, H * E // 2, 128), U32),
            pltpu.VMEM((NP, 3, NSEG // 2, 2, 8, E), U32),
            pltpu.VMEM((7, NSEG * 2, H * E // 2), U32),
            pltpu.VMEM((4, 5, H * E // 4, 128), U32),
            pltpu.VMEM((NSEG // 2, 2, SEG, DM), BF),
            pltpu.VMEM((NSEG // 2, 2, SEG, DM), BF),
            pltpu.VMEM((2, 16, 256, 128), U32),
            pltpu.VMEM((2, 1, S), BF),
            pltpu.VMEM((2, 2, 32 * WP, 128), U32),
            pltpu.VMEM((C_NUM, 64, 128), U32),
            pltpu.VMEM((32, 4, 128, 128), BF),
            pltpu.VMEM((32, 128, 512), F32),
            pltpu.VMEM((64, 128), F32),
            pltpu.VMEM((NSEG // 2, 2, SEG, DM), BF),
            pltpu.SemaphoreType.DMA((NP + 3,)),
            pltpu.SemaphoreType.DMA((2,)),
            pltpu.SemaphoreType.DMA((1,)),
        ],
        compiler_params=pltpu.CompilerParams(vmem_limit_bytes=118 * 1024 * 1024, disable_semaphore_checks=True),
    )(A_x.reshape(NSEG, SEG, DM), A_mem0.reshape(M, DM), wr(A_Wq), wr(A_Wk), wr(A_Wv),
      A_Wo.reshape(H * E, DM), B_x.reshape(NSEG // 2, 2, SEG, DM), B_w_r.T, B_w_i.T, _mask_fill(), _fft_consts())
    return out.reshape(1, S, 2 * DM)
```

```python
import functools
import math

import jax
import jax.numpy as jnp
import numpy as np
from jax import lax
import jax.experimental.pallas as pl
import jax.experimental.pallas.tpu as pltpu

BF, F32, U32, I32 = jnp.bfloat16, jnp.float32, jnp.uint32, jnp.int32

S, DM, H, E, M, SEG = 2048, 1024, 32, 128, 8, 32
NSEG = S // SEG
NP = H // 2
UN = 4
R2 = math.sqrt(0.5)
MID = 'mid'
PAD = 28
HEAD = (0, 1, 2, 3, 5, 8, 13, 19, 24)
LATER = {3: (0, 1), 4: (2,), 5: (3, 4, 5), 6: (6, 7)}


def _to_u32(m):
    u = np.ascontiguousarray(m, dtype=np.float32).view(np.uint32)
    h = ((u + 0x7FFF + ((u >> 16) & 1)) >> 16).astype(np.uint32)
    return h[..., 0::2, :] | (h[..., 1::2, :] << 16)


def _mask_fill():
    r = np.arange(80)
    pos = np.where(r < 64, np.where(r % 32 < M, r % 32, r % 32 + M), (r - 64) % 8 + M)
    kpos = np.concatenate([pos[0:32], pos[64:72]])
    vis = (pos[None, :] < M) | (pos[None, :] >= kpos[:, None])
    return np.where(vis, 0.0, -1e9).astype(np.float32)


RES = ((0, 12, 8, 4), (1, 15, 9, 7), (2, 14, 10, 6), (3, 13, 11, 5))
WP = 72
C_MD, C_MN, C_TW, C_MS, C_NUM = 0, 16, 22, 24, 88


@functools.lru_cache(maxsize=None)
def _fft_consts():
    md = np.zeros((16, 128, 128))
    for q in range(4):
        if q == 0:
            lay = [[(0, 0), (0, 1), (2, 0), (2, 1)], [(3, 1), (1, 0), (1, 1), (3, 0)]]
        else:
            lay = [[(0, 0), (1, 0), (0, 1), (1, 1)], [(2, 1), (3, 1), (2, 0), (3, 0)]]
        for h in range(2):
            ms_, ws_ = [], []
            for g, part in lay[h]:
                k = 16 * np.arange(32) + RES[q][g]
                th = 2 * np.pi * np.outer(np.arange(128 if q == 0 else 64), k) / DM
                c, s = np.cos(th), np.sin(th)
                if q == 0:
                    ms_.append(-s if part else c)
                else:
                    sg = (1.0 if RES[q][g] % 8 == q else -1.0) * (1.0 - 2.0 * h)
                    ms_.append(np.concatenate([-s, sg * c] if part else [c, sg * s]))
                ws_.append(np.where(k == 0, 1.0, 2.0) / DM)
            m = np.concatenate(ms_, axis=1)
            md[2 * q + h] = m
            md[8 + 2 * q + h] = (m * np.concatenate(ws_)[None, :]).T
    a, l = np.arange(64), np.arange(128)
    re = 16 * (a // 8) + a % 8
    im = re + 8
    ms = np.zeros((64, 128, 128))
    for dl in range(32):
        th = 2 * np.pi * np.outer(32 * a + dl, a) / S
        c, s = np.cos(th), np.sin(th)
        ms[2 * dl][:, re], ms[2 * dl][:, im] = np.concatenate([c, -s]), np.concatenate([s, c])
        ms[2 * dl + 1][:, re] = np.concatenate([c.T, s.T]) / S
        ms[2 * dl + 1][:, im] = np.concatenate([-s.T, c.T]) / S
    mn = np.zeros((6, 128, 128))
    th = 2 * np.pi * np.outer(np.arange(32), l) / 32
    mn[0, :32], mn[1, :32] = np.cos(th), -np.sin(th)
    mn[4, :, :32], mn[5, :, :32] = np.cos(th).T / DM, -np.sin(th).T / DM
    th = 2 * np.pi * np.outer(np.arange(16), a) / 16
    c, s = np.cos(th), np.sin(th)
    mn[2, :32] = np.block([[c, s], [-s, c]])
    mn[3, :, :32] = np.block([[c.T, -s.T], [s.T, c.T]]) / S
    th = 2 * np.pi * np.outer(a, l) / S
    tw = np.stack([np.cos(th), np.sin(th)]).astype(np.float32).view(np.uint32)
    return np.concatenate([_to_u32(md), _to_u32(mn), tw, _to_u32(ms)], axis=0)


def _bdot(a, b):
    return jnp.dot(a, b, preferred_element_type=F32)


def _bf(u):
    return pltpu.bitcast(u, BF)


def _cat(rows):
    return jnp.concatenate(rows, axis=0).astype(BF)


def _unpack2(u, p):
    if p == 0:
        return pltpu.bitcast(u << 16, F32)
    return pltpu.bitcast(u & jnp.uint32(0xFFFF0000), F32)


def _strassen_left(n, a):
    return (lambda: a(1, 0) + a(1, 1), lambda: a(1, 0) - a(0, 0), lambda: a(1, 1), lambda: a(0, 0) + a(1, 1),
            lambda: a(0, 0), lambda: a(0, 1) - a(1, 1), lambda: a(0, 0) + a(0, 1))[n]()


def _strassen_right(n, w):
    add = lambda u, v: (u.astype(F32) + v.astype(F32)).astype(u.dtype)
    sub = lambda u, v: (u.astype(F32) - v.astype(F32)).astype(u.dtype)
    return (lambda: w(0, 0), lambda: add(w(0, 0), w(0, 1)), lambda: sub(w(1, 0), w(0, 0)),
            lambda: add(w(0, 0), w(1, 1)), lambda: sub(w(0, 1), w(1, 1)), lambda: add(w(1, 0), w(1, 1)),
            lambda: w(1, 1))[n]()


def _strassen(left, right, done, ready=lambda k: None, dot=None):
    def mm(n):
        a, r, acc = left(n), right(n), None
        for k in range(0, r.shape[0], 512):
            d = (dot or _bdot)(a[:, k:k + 512], r[k:k + 512])
            acc = d if acc is None else acc + d
        return acc

    ready(0)
    m2 = mm(0)
    c22 = mm(1) - m2
    ready(1)
    m4 = mm(2)
    c21 = m2 + m4
    m1 = mm(3)
    c11, c22 = m1 + m4, c22 + m1
    m3 = mm(4)
    done(1, c21, c22 + m3)
    c11 = c11 + mm(5)
    ready(2)
    m5 = mm(6)
    done(0, c11 - m5, m3 + m5)


def _twiddle(z, k, n, sign):
    r, i = z
    if k == 0:
        return r, i
    if 4 * k == n:
        return (-i, r) if sign > 0 else (i, -r)
    c, s = math.cos(2 * math.pi * k / n), sign * math.sin(2 * math.pi * k / n)
    if 8 * k == n or 8 * k == 3 * n:
        if c * s > 0:
            return (r - i) * c, (r + i) * c
        return (r + i) * c, (i - r) * c
    return r * c - i * s, r * s + i * c


def _cfft(xs, sign):
    n = len(xs)
    if n == 1:
        return xs
    ev, od = _cfft(xs[0::2], sign), _cfft(xs[1::2], sign)
    out = [None] * n
    for k in range(n // 2):
        er, ei = ev[k]
        if 4 * k == n:
            orr, oi = od[k]
            lo, hi = (er - oi, ei + orr), (er + oi, ei - orr)
            out[k], out[k + n // 2] = (lo, hi) if sign > 0 else (hi, lo)
        else:
            tr, ti = _twiddle(od[k], k, n, sign)
            out[k], out[k + n // 2] = (er + tr, ei + ti), (er - tr, ei - ti)
    return out


def _rfft8(x):
    a0, a1, b0, b1 = x[0] + x[4], x[0] - x[4], x[2] + x[6], x[2] - x[6]
    c0, c1, d0, d1 = x[1] + x[5], x[1] - x[5], x[3] + x[7], x[3] - x[7]
    e, f = a0 + b0, c0 + d0
    g, h = (c1 - d1) * R2, (c1 + d1) * R2
    return [e + f, e - f, a1 + g, b1 + h, a0 - b0, c0 - d0, a1 - g, b1 - h]


def _irfft8(z):
    z0, z4, z1r, z1i, z2r, z2i, z3r, z3i = z
    e, f = z0 + z4, z0 - z4
    a1, g = z1r + z3r, (z1r - z3r) * R2
    b1, h = z1i + z3i, (z1i - z3i) * R2
    a0, b0, c0, d0 = e + z2r, e - z2r, f + z2i, f - z2i
    c1, d1 = g + h, h - g
    return [a0 + a1, c0 + c1, b0 + b1, d0 + d1, a0 - a1, c0 - c1, b0 - b1, d0 - d1]


def _kernel(x_hbm, mem0_hbm, wq_hbm, wk_hbm, wv_hbm, wo_hbm, bx_hbm, wr_hbm, wi_hbm, fill_hbm, cst_hbm,
            out_hbm,
            x_v, xpre_v, xs_v, mem0_v, fill_v, wqkv, wo_v, pre, os_v, ws_v, outa_v,
            bx_v, w_v, wn_v, wt, cst, zs, vv, tn, outb_v,
            sem_w, sem_in, sem_out):
    scale = E ** -0.5
    wus = [w.bitcast(U32) for w in (wq_hbm, wk_hbm, wv_hbm)]
    wo_u = wo_hbm.bitcast(U32)
    fus = [w.at[pl.ds(0, 512)].bitcast(U32) for w in (wr_hbm, wi_hbm)]

    def w_copy(j, t, sem):
        return pltpu.make_async_copy(wus[t].at[:, :, j, :], wqkv.at[j, t], sem)

    xpre_cp = pltpu.make_async_copy(x_hbm.at[:, pl.ds(0, 8), :], xpre_v, sem_w.at[17])
    head = [[divmod(f, 3) for f in range(HEAD[b], HEAD[b + 1])] for b in range(len(HEAD) - 1)]
    head_cps = [[w_copy(j, t, sem_w.at[b]) for j, t in grp] for b, grp in enumerate(head) if b > 0]
    first_cps = [pltpu.make_async_copy(wus[0].at[pl.ds(32 * k, 32), :, 0, :], wqkv.at[0, 0, pl.ds(32 * k, 32)],
                                       sem_w.at[18 * k]) for k in range(2)]
    head_cps.insert(0, first_cps)

    def b_rows(i, b):
        return b, i // 4, pl.ds(pl.multiple_of((i % 4) * 8, 8), 8)

    def fwd_cps(i):
        rows = b_rows(i, slice(None))
        sem = sem_w.at[8 + i]
        return ([w_copy(8 + i, t, sem) for t in range(3)]
                + [pltpu.make_async_copy(bx_hbm.at[rows], bx_v.at[rows], sem)]
                + [pltpu.make_async_copy(fus[t].at[:, pl.ds(pl.multiple_of(128 * (2 * i + h), 128), 128)],
                                         w_v.at[t, 2 * i + h], sem) for t in range(2) for h in range(2)])

    def part(src, dst, lo, hi, sem):
        return pltpu.make_async_copy(src.at[pl.ds(lo, hi - lo)], dst.at[pl.ds(lo, hi - lo)], sem)

    c0_cp = part(cst_hbm, cst, 0, C_MS, sem_w.at[16])
    a_cps = [pltpu.make_async_copy(wo_u.at[:, pl.ds(128 * n, 128)], wo_v.at[n], sem_in.at[0]) for n in range(8)]
    a_cps += [part(x_hbm, x_v, 0, UN, sem_in.at[0]), part(cst_hbm, cst, C_MS, C_MS + UN, sem_in.at[0]),
              pltpu.make_async_copy(mem0_hbm, mem0_v, sem_in.at[0]),
              pltpu.make_async_copy(fill_hbm, fill_v, sem_in.at[0])]
    b_cps = [part(x_hbm, x_v, UN, NSEG, sem_in.at[1]), part(cst_hbm, cst, C_MS + UN, C_NUM, sem_in.at[1])]
    b_cps += [pltpu.make_async_copy(w.at[pl.ds(512, 1)], wn_v.at[t], sem_in.at[1])
              for t, w in enumerate((wr_hbm, wi_hbm))]

    lane = lax.broadcasted_iota(I32, (8, 128), 1)
    alt = jnp.where(lane % 2 == 0, 1.0, -1.0).astype(F32)
    lo_half = lane < 64
    ev_grp = (lane // 32) % 2 == 0

    def half_coef(q):
        sg = -1.0 if q < 3 else 1.0
        tc, ts = math.cos(2 * math.pi * q / 16), -math.sin(2 * math.pi * q / 16)
        f = lambda lo, hi: jnp.where(lo_half, lo, hi).astype(F32)
        return f(1.0, ts), f(0.0, sg * tc), f(0.0, tc), f(sg, -sg * ts)

    pace = {'tok': None}

    def token(v):
        return (v if v.dtype == U32 else pltpu.bitcast(v, U32)) & cst[C_MN, 56:64, :]

    def gate(v):
        tok = pace['tok']
        if tok is None:
            return v
        return v | tok if v.dtype == U32 else pltpu.bitcast(pltpu.bitcast(v, U32) | tok, v.dtype)

    def gate2(z):
        return gate(z[0]), gate(z[1])

    def as_u32(rows):
        return pltpu.bitcast(_cat(rows), U32)

    def b_fwd(i):
        r0 = pl.multiple_of(i * 8, 8)
        hc = [None] + [half_coef(q) for q in range(1, 4)]
        tacc = jnp.zeros((8, 128), F32)
        zl = []

        def filt(k):
            e, t, ty = 2 * i + k // 4, (k // 2) % 2, k % 2
            u = jnp.concatenate([gate(w_v[t, e, pl.ds(m + ty + 64 * v, 8, stride=8), :])
                                 for m in (0, 6, 4, 2) for v in range(4)], axis=0)
            ut = pltpu.bitcast(pltpu.bitcast(u, F32).T, U32)
            for v in range(16):
                wt[t, ty, pl.ds(8 * (v % 4) * WP + 4 * e + v // 4, 8, stride=WP), :] = ut[8 * v:8 * v + 8]

        for b0 in range(0, 32, 2):
            rows = []
            for b in (b0, b0 + 1):
                xb = bx_v[(*b_rows(i, b), slice(None))].astype(F32)
                z = _rfft8([gate(xb[:, 128 * t:128 * t + 128]) for t in range(8)])
                tacc = jnp.where(lane == b, jnp.sum(z[0] * alt, axis=1, keepdims=True), tacc)
                for q in range(1, 4):
                    c1, c2, c3, c4 = hc[q]
                    zr, zi = z[2 * q], z[2 * q + 1]
                    pp = c1 * zr + c2 * zi
                    qq = pltpu.roll(c3 * zr + c4 * zi, 64, 1)
                    z[2 * q], z[2 * q + 1] = pp + qq, pp - qq
                rows.append(z)
                if b == b0:
                    yield 80
            zl.append([as_u32([rows[0][n], rows[1][n]]) for n in range(8)])
            yield 120
            if b0 % 4 == 0:
                filt(b0 // 4)
                yield 40
        tn[pl.ds(r0, 8), :] = tacc

        def mm(n):
            return _bdot(_bf(jnp.concatenate([z[n] for z in zl], axis=0)), _bf(cst[C_MD + n]))

        yield MID
        oo = [mm(n) for n in range(4)]
        yield MID
        oo += [mm(n) for n in range(4, 8)]
        yield MID
        for q in range(4):
            sel, sh = (ev_grp, 96) if q == 0 else (lo_half, 64)
            ys = []
            for b0 in range(4):
                xs = []
                for b in range(b0, 32, 4):
                    e_, o_ = gate(oo[2 * q][8 * b:8 * b + 8]), oo[2 * q + 1][8 * b:8 * b + 8]
                    xs.append((jnp.where(sel, e_, o_), pltpu.roll(jnp.where(sel, o_, e_), sh, 1)))
                ys.append([_twiddle(y, b0 * k1, 32, -1) for k1, y in enumerate(_cfft(xs, -1))])
                yield 110
            for k1 in range(8):
                for k0, y in enumerate(_cfft([gate2(ys[b0][k1]) for b0 in range(4)], -1)):
                    zs[k1 + 8 * k0, q, pl.ds(pl.multiple_of(2 * r0, 16), 16), :] = _cat(y)
                yield 30

    def b_mid(it):
        def fwd(dl):
            return _bdot(_bf(cst[C_MS + 2 * dl]), jnp.concatenate([zs[dl, q] for q in range(4)], axis=1))

        def mult(dl, y, rows):
            yield from [None] * 4
            w0 = pl.multiple_of(dl * WP, 8)
            for r in range(8):
                wq = []
                for t in range(2):
                    ta, tb = wt[t, 0, pl.ds(w0 + 8 * r, 8), :], wt[t, 1, pl.ds(w0 + 8 * r, 8), :]
                    wq.append([_unpack2(ta, 0), _unpack2(jnp.where(ev_grp, ta, tb), 1),
                               _unpack2(tb, 0), _unpack2(jnp.where(ev_grp, tb, ta), 1)])
                cols = []
                for q in range(4):
                    yr = gate(y[8 * r:8 * r + 8, 128 * q:128 * q + 128])
                    yi = gate(y[64 + 8 * r:72 + 8 * r, 128 * q:128 * q + 128])
                    wr, wi = wq[0][q], wq[1][q]
                    cols.append(as_u32([yr * wr - yi * wi, yr * wi + yi * wr]))
                rows.append(jnp.concatenate(cols, axis=1))
                yield from [None] * 2

        def inv(dl, rows):
            vv[dl] = _bdot(_bf(cst[C_MS + 2 * dl + 1]), _bf(jnp.concatenate(rows, axis=0)))

        def rights():
            for n in range(4):
                for r in range(0, 64, 8):
                    blk = functools.lru_cache(None)(lambda k, p: _bf(gate(
                        wo_v[n + 4 * p, pl.ds(pl.multiple_of((2 * it + k) * 64 + r, 8), 8), :])).astype(F32))
                    vals = [_strassen_right(m, blk) for m in range(1, 6)]
                    for m in range(5):
                        ws_v[n, m, pl.ds(pl.multiple_of(2 * (it * 64 + r), 16), 16), :] = vals[m].astype(BF)
                    yield [v[8 * h:8 * h + 8] for v in vals for h in range(2)]

        yield from [None] * 2
        for h in range(2):
            rows = []
            y = fwd(2 * it + h)
            yield from mult(2 * it + h, y, rows)
            yield MID
            inv(2 * it + h, rows)
            if h == 0:
                yield from [None] * 4
                yield from rights()
                yield MID

    def b_nyq():
        c, s = pltpu.bitcast(cst[C_TW], F32), pltpu.bitcast(cst[C_TW + 1], F32)
        tb = tn[...].astype(BF)
        tr, ti = _bdot(tb, _bf(cst[C_MN])), _bdot(tb, _bf(cst[C_MN + 1]))
        yield MID
        y = _bdot(_bf(cst[C_MN + 2, 0:16, :]), _cat([tr * c + ti * s, ti * c - tr * s]))
        row = lax.broadcasted_iota(I32, (16, 128), 0)
        wn = []
        for t in range(2):
            wrow = wn_v[t].astype(F32)
            acc = jnp.zeros((16, 128), F32)
            for e in range(16):
                acc = jnp.where(row == e, wrow[:, 128 * e:128 * e + 128], acc)
            wn.append(acc)
        yr, yi = y[0:16], y[16:32]
        yield MID
        v = _bdot(_bf(cst[C_MN + 3, :, 0:32]), _cat([yr * wn[0] - yi * wn[1], yr * wn[1] + yi * wn[0]]))
        vr, vi = v[0:64], v[64:128]
        yield MID
        tn[...] = (_bdot((vr * c - vi * s).astype(BF), _bf(cst[C_MN + 4]))
                   + _bdot((vr * s + vi * c).astype(BF), _bf(cst[C_MN + 5])))

    def b_inv(i, ul):
        r0 = i * 8
        for q in range(4):
            sel, sh = (ev_grp, 32) if q == 0 else (lo_half, 64)
            ys = []
            for b0 in range(4):
                xs = [(gate(vv[dl, pl.ds(r0, 8), 128 * q:128 * q + 128]),
                       gate(vv[dl, pl.ds(64 + r0, 8), 128 * q:128 * q + 128])) for dl in range(b0, 32, 4)]
                ys.append([_twiddle(y, b0 * k1, 32, +1) for k1, y in enumerate(_cfft(xs, +1))])
                yield 110
            ie, io = [], []
            for k1 in range(8):
                es, os_ = [], []
                for ur, ui in _cfft([gate2(ys[b0][k1]) for b0 in range(4)], +1):
                    tmp = pltpu.roll(ui, sh, 1)
                    es.append(jnp.where(sel, ur, tmp))
                    os_.append(jnp.where(sel, tmp, ur))
                ie += [as_u32(es[0:2]), as_u32(es[2:4])]
                io += [as_u32(os_[0:2]), as_u32(os_[2:4])]
                yield 55, ie[-2:] + io[-2:]
            ul += [ie, io]

    def b_fin(i, zz):
        r0 = i * 8
        hc = [None] + [half_coef(q) for q in range(1, 4)]
        tb = tn[pl.ds(r0, 8), :]
        for g in range(32):
            b = g // 4 + 8 * (g % 4)
            z = [gate(zz[n][8 * g:8 * g + 8]) for n in range(8)]
            z[0] = z[0] + jnp.sum(jnp.where(lane == b, tb, 0.0), axis=1, keepdims=True) * alt
            for q in range(1, 4):
                c1, c2, c3, c4 = hc[q]
                pp = z[2 * q] + z[2 * q + 1]
                qq = pltpu.roll(z[2 * q] - z[2 * q + 1], 64, 1)
                z[2 * q], z[2 * q + 1] = c1 * pp + c3 * qq, c2 * pp + c4 * qq
            y = _irfft8(z)
            outb_v[(*b_rows(i, b), slice(None))] = jnp.concatenate(y, axis=1).astype(BF)
            yield 75, y
        rows = b_rows(i, slice(None))
        start_out(outb_v.at[rows], out_hbm.at[(*rows, pl.ds(DM, DM))])

    def tie(w, vals):
        if not vals:
            return w
        acc = None
        for v in vals:
            v = v if v.dtype == U32 else pltpu.bitcast(v, U32)
            acc = v if acc is None else acc | v
        return jnp.concatenate([w[0:8] | token(acc), w[8:]], axis=0)

    def paced_dot(gen, budget):
        st = {'debt': 0, 'k': 0}
        due = {}

        def emit(d, b):
            while st['debt'] < b:
                r = 8 * (32 * st['debt'] // b)
                pace['tok'] = token(d[r:r + 8])
                c = next(gen, MID)
                if c is MID:
                    st['debt'] = b
                elif isinstance(c, list):
                    st['debt'] = 0
                    for own in c:
                        emit(own, 300)
                    return
                else:
                    if isinstance(c, tuple):
                        due.setdefault(st['k'] + 2, []).extend(c[1])
                        c = c[0]
                    st['debt'] += c
            st['debt'] -= b

        def dot(a, w):
            vals = due.pop(st['k'], None)
            if vals:
                a = jnp.concatenate([_bf(tie(pltpu.bitcast(a[:, 0:128], U32), vals)), a[:, 128:]], axis=1)
            d = _bdot(a, w)
            st['k'] += 1
            emit(d, budget)
            return d

        return dot

    out_cps = []

    def start_out(src, dst):
        out_cps.append(pltpu.make_async_copy(src, dst, sem_out.at[0]))
        out_cps[-1].start()

    hb = DM // 32

    def retile(j, t, k):
        blk = pl.ds(k * hb, hb)
        a, b = wqkv[j, t, blk, pl.ds(0, 8, stride=2), :], wqkv[j, t, blk, pl.ds(1, 8, stride=2), :]
        lo, hi = (a & jnp.uint32(0xFFFF)) | (b << 16), (a >> 16) | (b & jnp.uint32(0xFFFF0000))
        wqkv[j, t, blk, 0:8, :] = lo
        wqkv[j, t, blk, 8:16, :] = hi
        return lo

    def strassen_lhs():
        for g in range(NSEG // 4):
            xa = [xpre_v[4 * g + k].astype(F32) for k in range(4)]
            a1, a2 = jnp.concatenate([xa[0], xa[2]], axis=0), jnp.concatenate([xa[1], xa[3]], axis=0)
            a11, a12, a21, a22 = a1[:, :DM // 2], a1[:, DM // 2:], a2[:, :DM // 2], a2[:, DM // 2:]
            for n in range(7):
                v = _strassen_left(n, lambda r, k: ((a11, a12), (a21, a22))[r][k])
                xs_v[n, 8 * g:8 * g + 8, :] = pltpu.bitcast(v.astype(BF), U32)

    def pre_step(j, t, dot=None, sync=None, first=False):
        fresh = {}

        def w(k, p):
            v = fresh.pop((k, p), None)
            if v is None:
                v = wqkv[j, t, k * hb:(k + 1) * hb, 8 * p:8 * p + 8, :]
            return _bf(v.reshape(DM // 4, E))

        def done(h, c1, c2):
            v = jnp.concatenate([c.reshape(NSEG // 2, 8, E) for c in (c1, c2)], axis=1)
            pre[j, t, :, h] = pltpu.bitcast(v.astype(BF), U32)

        def ready(k):
            if k < 2:
                if first:
                    first_cps[k].wait()
                fresh[k, 0] = retile(j, t, k)
            elif sync:
                sync()

        _strassen(lambda n: _bf(xs_v[n]), lambda n: _strassen_right(n, w), done, ready, dot)

    for cp in [xpre_cp] + [cp for grp in head_cps for cp in grp]:
        cp.start()
    vv[0:PAD] = jnp.zeros((PAD,) + vv.shape[1:], F32)
    xpre_cp.wait()
    strassen_lhs()

    def pre_fwd(steps, i, budget):
        gen = b_fwd(i)
        dot = paced_dot(gen, budget)
        for j, t in steps + [(8 + i, t) for t in range(3)]:
            pre_step(j, t, dot)
        for _ in gen:
            pass

    def sync(b):
        for i in LATER.get(b, ()):
            for cp in ([c0_cp] if i == 0 else []) + fwd_cps(i):
                cp.start()
        for cp in head_cps[b + 1] + ([c0_cp] + fwd_cps(0) if b + 2 == len(head) else []):
            cp.wait()

    for b, grp in enumerate(head[:-1]):
        for j, t in grp:
            pre_step(j, t, sync=functools.partial(sync, b) if (j, t) == grp[-1] else None, first=b == 0)
    pre_fwd(head[-1], 0, 130)
    for cp in a_cps + b_cps:
        cp.start()

    def pre_fwd_body(i, carry):
        for cp in fwd_cps(i):
            cp.wait()
        pre_fwd([], i, 340)
        return carry

    lax.fori_loop(1, 8, pre_fwd_body, 0)
    for cp in a_cps:
        cp.wait()

    def seg_step(s, u, mem, slot, opost):
        lhs = _cat([mem, x_v[s][8:32].astype(F32)])
        fill = fill_v[...]
        toks = []
        pace['tok'] = None

        def proj(j, t):
            w0, w1 = [wqkv[j, t, :, 8 * p:8 * p + 8, :].reshape(DM // 2, E) for p in range(2)]
            r0, r1 = _bdot(lhs, _bf(tie(w0, slot()))), _bdot(lhs, _bf(w1))
            toks.append(r0[0:8])
            if len(toks) >= 4:
                pace['tok'] = token(toks[-4])
            return _cat([r0, r1, _bf(pre[j, t, s // 2, u % 2]).astype(F32)])

        def qk(q, k):
            sc = lax.dot_general(k, q, (((1,), (1,)), ((), ())), preferred_element_type=F32)
            col = lax.broadcasted_iota(I32, (40, 80), 1)
            h0 = (col < 32) | ((col >= 64) & (col < 72))
            sc = jnp.where(h0, jnp.concatenate([sc[0:32], sc[64:72]], axis=0),
                           jnp.concatenate([sc[32:64], sc[72:80]], axis=0)) * scale
            sc = jnp.where(fill == 0.0, sc, fill)
            e = jnp.exp(sc - jnp.max(sc, axis=0, keepdims=True))
            p = e * (1.0 / jnp.sum(e, axis=0, keepdims=True))
            p0, p1 = jnp.where(h0, p, 0.0), jnp.where(h0, 0.0, p)
            return jnp.concatenate([p0[0:32], p1[0:32], p0[32:40], p1[32:40]], axis=0).T.astype(BF)

        ob, ps, vs = {}, {}, {}

        def pv(j):
            o = _bdot(ps[j], vs[j])
            opost[u, j] = (o[64:72], o[72:80])
            if u == UN - 1:
                vals = [as_u32([_strassen_left(n, lambda r, k: opost[2 * g + r, j][k]) for g in range(2)])
                        for n in range(7)]
                for n in range(7):
                    os_v[n, pl.ds(pl.multiple_of(2 * (s - u), 8), 8), 128 * j:128 * j + 128] = vals[n]
            ob[j] = [o[0:32], o[32:64]]

        def wo(g0, g1):
            og = jnp.concatenate([o for j in range(2 * g0, 2 * g1) for o in ob[j]], axis=1).astype(BF)
            return jnp.concatenate([_bdot(og, _bf(wo_v[n, g0 * 256:g1 * 256, :])) for n in range(8)], axis=1)

        ng = NP // 2
        for g in range(ng):
            ja, jb = 2 * g, 2 * g + 1
            qa, ka, qb, kb = proj(ja, 0), proj(ja, 1), proj(jb, 0), proj(jb, 1)
            vs[ja], vs[jb] = proj(ja, 2), proj(jb, 2)
            for j, q, k in ((ja, qa, ka), (jb, qb, kb)):
                ps[j] = qk(q, k)
                if g > 0:
                    pv(j - 2)
        res = wo(0, 2)
        pv(NP - 2)
        pv(NP - 1)
        res = res + wo(2, ng - 1)
        res = res + wo(ng - 1, ng)
        outa_v[s // 2, u % 2, 8:32, :] = res[8:32].astype(BF)
        return res[0:8]

    def loop_body(it, mem):
        @pl.when(it == 1)
        def _():
            for cp in b_cps:
                cp.wait()

        gen = b_mid(it)
        opost = {}
        state = {'mid': False}

        def slot():
            if state['mid']:
                return None
            vals = next(gen, None)
            if vals is MID:
                state['mid'] = True
                return None
            return vals

        for u in range(UN):
            state['mid'] = False
            mem = seg_step(UN * it + u, u, mem, slot, opost)
        for _ in gen:
            pass
        return mem

    lax.fori_loop(0, NSEG // UN, loop_body, mem0_v[...].astype(F32))
    idx = (slice(None), slice(None), pl.ds(8, SEG - 8), pl.ds(0, DM))
    start_out(outa_v.at[idx], out_hbm.at[idx])

    def b_inv_all():
        nyq = b_nyq()
        zz = None
        for i in range(8):
            ul = []
            for k, c in enumerate(b_inv(i, ul)):
                if k % 10 == 0:
                    next(nyq, None)
                yield c
            if i > 0:
                yield from b_fin(i - 1, zz)
            else:
                yield MID
            zz = [_bdot(_bf(jnp.concatenate(ul[n], axis=0)), _bf(cst[C_MD + 8 + n])) for n in range(8)]
            if i < 7:
                yield [zz[3], zz[7]]
        yield MID
        yield MID
        yield from b_fin(7, zz)

    gen = b_inv_all()
    dot = paced_dot(gen, 450)
    for n in range(4):
        def done(r, *cs):
            for p, cc in enumerate(cs):
                idx = (slice(None), r, pl.ds(0, 8), pl.ds(128 * (n + 4 * p), 128))
                outa_v[idx] = cc.reshape(NSEG // 2, 8, 128).astype(BF)
                start_out(outa_v.at[idx], out_hbm.at[idx])

        heads = lambda k: jnp.concatenate([wo_v[n + 4 * k, 64 * h:64 * h + 64, :] for h in range(k, H, 2)], axis=0)
        right = lambda m: _bf(heads(m // 6)) if m % 6 == 0 else ws_v[n, m - 1]
        _strassen(lambda m: _bf(os_v[m]), right, done, dot=dot)
    for _ in gen:
        pass
    for cp in out_cps:
        cp.wait()


def pallas_concat_heads__memory_aug_recurrent_mem_tr__spectral_gfnet__prompt_kernel(
    A_x, A_mem0, A_Wq, A_Wk, A_Wv, A_Wo, A_seg_len, B_x, B_w_r, B_w_i,
):
    assert A_x.shape == (1, S, DM) and A_Wq.shape == (DM, H, E) and A_mem0.shape == (1, M, DM)
    assert B_x.shape == (1, S, DM) and (not isinstance(A_seg_len, int) or A_seg_len == SEG)
    hbm = pl.BlockSpec(memory_space=pltpu.HBM)
    wr = lambda w: w.reshape(DM // 16, 16, H, E)
    out = pl.pallas_call(
        _kernel,
        out_shape=jax.ShapeDtypeStruct((NSEG // 2, 2, SEG, 2 * DM), BF),
        in_specs=[hbm] * 11,
        out_specs=hbm,
        scratch_shapes=[
            pltpu.VMEM((NSEG, SEG, DM), BF),
            pltpu.VMEM((NSEG, 8, DM), BF),
            pltpu.VMEM((7, NSEG * 2, DM // 2), U32),
            pltpu.VMEM((M, DM), BF),
            pltpu.VMEM((40, 80), F32),
            pltpu.VMEM((NP, 3, DM // 16, 16, E), U32),
            pltpu.VMEM((8, H * E // 2, 128), U32),
            pltpu.VMEM((NP, 3, NSEG // 2, 2, 8, E), U32),
            pltpu.VMEM((7, NSEG * 2, H * E // 2), U32),
            pltpu.VMEM((4, 5, H * E // 2, 128), BF),
            pltpu.VMEM((NSEG // 2, 2, SEG, DM), BF),
            pltpu.VMEM((NSEG // 2, 2, SEG, DM), BF),
            pltpu.VMEM((2, 16, 256, 128), U32),
            pltpu.VMEM((2, 1, S), BF),
            pltpu.VMEM((2, 2, 32 * WP, 128), U32),
            pltpu.VMEM((C_NUM, 64, 128), U32),
            pltpu.VMEM((32, 4, 128, 128), BF),
            pltpu.VMEM((32, 128, 512), F32),
            pltpu.VMEM((64, 128), F32),
            pltpu.VMEM((NSEG // 2, 2, SEG, DM), BF),
            pltpu.SemaphoreType.DMA((NP + 3,)),
            pltpu.SemaphoreType.DMA((2,)),
            pltpu.SemaphoreType.DMA((1,)),
        ],
        compiler_params=pltpu.CompilerParams(vmem_limit_bytes=118 * 1024 * 1024, disable_semaphore_checks=True),
    )(A_x.reshape(NSEG, SEG, DM), A_mem0.reshape(M, DM), wr(A_Wq), wr(A_Wk), wr(A_Wv),
      A_Wo.reshape(H * E, DM), B_x.reshape(NSEG // 2, 2, SEG, DM), B_w_r.T, B_w_i.T, _mask_fill(), _fft_consts())
    return out.reshape(1, S, 2 * DM)
```
